```python
import jax
import jax.numpy as jnp

def _softmax(x, axis=-1):
    return jax.nn.softmax(x, axis=axis)
def _gelu(x):
    return jax.nn.gelu(x, approximate=True)
def _silu(x):
    return jax.nn.silu(x)
def _sigmoid(x):
    return jax.nn.sigmoid(x)
def _layernorm(x, axis=-1, eps=1e-5):
    m = jnp.mean(x, axis=axis, keepdims=True)
    v = jnp.var(x, axis=axis, keepdims=True)
    return (x - m) / jnp.sqrt(v + eps)
def _scatter_add(tgt, idx, src, axis=0):
    return tgt.at[idx].add(src)
def _segment_sum(src, seg, n):
    return jax.ops.segment_sum(src, seg, n)
class _Rng:
    def __init__(self, key):
        self._k = key
    def _next(self):
        self._k, sub = jax.random.split(self._k)
        return sub
    def normal(self, shape):
        return jax.random.normal(self._next(), shape, dtype=jnp.bfloat16)
    def randint(self, lo, hi, shape):
        return jax.random.randint(self._next(), shape, lo, hi, dtype=jnp.int32)
    def uniform(self, shape, lo=0.0, hi=1.0):
        return jax.random.uniform(self._next(), shape, jnp.bfloat16, lo, hi)
    def permutation(self, n):
        return jax.random.permutation(self._next(), n)


kernel_name = 'interleave_layers__sliding_block_cached__mixer_s_mlp__decode'

def setup_inputs():
    _rng = _Rng(jax.random.key(int.from_bytes(__import__("os").urandom(4), "little")))
    _w = (lambda a: (lambda t: t.astype(jnp.bfloat16) if jnp.issubdtype(t.dtype, jnp.floating) else t)(jnp.asarray(a)))
    def _A_setup():
        B, Sq, D = 1, 1, 640
        Hq, Hkv, Sk, Dh = 32, 32, 32768, 192
        assert Hq % Hkv == 0, (Hq, Hkv)
        return {
            "x": _w((lambda *s: _rng.normal(s) * 0.05)(B, Sq, D)),
            "k_cache": _w((lambda *s: _rng.normal(s) * 0.05)(B, Hkv, Sk, Dh)),
            "v_cache": _w((lambda *s: _rng.normal(s) * 0.05)(B, Hkv, Sk, Dh)),
            "wq": _w((lambda *s: _rng.normal(s) * 0.05)(D, Hq * Dh) * (D ** -0.5)),
            "wo": _w((lambda *s: _rng.normal(s) * 0.05)(Hq * Dh, D) * ((Hq * Dh) ** -0.5)),
        }
    _A_in = _A_setup()

    def _B_setup():
        B, S, D, F = 1, 1, 640, 1536
        return {
            "x":  _w((lambda *s: _rng.normal(s) * 0.05)(B, S, D)),
            "w1": _w((lambda *s: _rng.normal(s) * 0.05)(D, D) * (D ** -0.5)),
            "w2": _w((lambda *s: _rng.normal(s) * 0.05)(D, D) * (D ** -0.5)),
            "w3": _w((lambda *s: _rng.normal(s) * 0.05)(D, F) * (D ** -0.5)),
            "w4": _w((lambda *s: _rng.normal(s) * 0.05)(F, D) * (F ** -0.5)),
        }
    _B_in = _B_setup()

    return {
        "A_x": _A_in["x"],
        "A_k_cache": _A_in["k_cache"],
        "A_v_cache": _A_in["v_cache"],
        "A_wq": _A_in["wq"],
        "A_wo": _A_in["wo"],
        "B_x": _B_in["x"],
        "B_w1": _B_in["w1"],
        "B_w2": _B_in["w2"],
        "B_w3": _B_in["w3"],
        "B_w4": _B_in["w4"],
    }

def reference(A_x, A_k_cache, A_v_cache, A_wq, A_wo, B_x, B_w1, B_w2, B_w3, B_w4):
    def _A_ref(x, k_cache, v_cache, wq, wo):
        B, Sq, D = x.shape
        Hq, Dh = 32, 192
        Hkv, Sk = k_cache.shape[1], k_cache.shape[2]
        W = min(4096, max(256, Sk // 4))
        rep = Hq // Hkv
        q = (lambda x, *d: x.transpose(*d))((x @ wq).reshape(B, Sq, Hq, Dh), 0, 2, 1, 3)
        k = jnp.repeat(k_cache[:, :, Sk - W:, :], rep, axis=1)
        v = jnp.repeat(v_cache[:, :, Sk - W:, :], rep, axis=1)
        scores = jnp.einsum("bhqd,bhkd->bhqk", q, k) * (Dh ** -0.5)
        p = _softmax(scores, axis=-1)
        o = jnp.einsum("bhqk,bhkd->bhqd", p, v)
        return (lambda x, *d: x.transpose(*d))(o, 0, 2, 1, 3).reshape(B, Sq, Hq * Dh) @ wo

    def _B_ref(x, w1, w2, w3, w4):
        B, S, D = x.shape
        h = _gelu(_layernorm(x, axis=-1) @ w1)
        c = D // 4
        g0 = jnp.pad(h[:, :, 0*c:1*c], ((0, 0), (1, 0), (0, 0)))[:, :S, :]
        g1 = jnp.pad(h[:, :, 1*c:2*c], ((0, 0), (0, 1), (0, 0)))[:, 1:, :]
        g2 = jnp.pad(h[:, :, 2*c:3*c], ((0, 0), (2, 0), (0, 0)))[:, :S, :]
        g3 = jnp.pad(h[:, :, 3*c:   ], ((0, 0), (0, 2), (0, 0)))[:, 2:, :]
        hs = jnp.concatenate([g0, g1, g2, g3], axis=-1) @ w2
        x1 = x + hs
        h2 = _gelu(_layernorm(x1, axis=-1) @ w3) @ w4
        return x1 + h2

    x = A_x
    x = x + _A_ref(_layernorm(x, axis=-1), A_k_cache, A_v_cache, A_wq, A_wo)
    x = x + _B_ref(_layernorm(x, axis=-1), B_w1, B_w2, B_w3, B_w4)
    x = x + _A_ref(_layernorm(x, axis=-1), A_k_cache, A_v_cache, A_wq, A_wo)
    x = x + _B_ref(_layernorm(x, axis=-1), B_w1, B_w2, B_w3, B_w4)
    return x
```

```python
import functools

import jax
import jax.numpy as jnp
from jax import lax
import jax.experimental.pallas as pl
import jax.experimental.pallas.tpu as pltpu

D = 640
H = 32
DH = 192
F = 1536
EPS = 1e-5
NP = H // 2
GP = 2 * DH // 8
HI = 0xFFFF0000

f32 = jnp.float32
bf16 = jnp.bfloat16
u32 = jnp.uint32


def _ln(x):
    m = jnp.mean(x, axis=-1, keepdims=True)
    c = x - m
    v = jnp.mean(c * c, axis=-1, keepdims=True)
    return c * lax.rsqrt(v + EPS)


def _wtile(wu, rows, nt):
    blk = wu[rows, nt]
    return pltpu.bitcast(blk.reshape(blk.shape[0] * 8, 128), bf16)


def _kernel(x_hbm, k_hbm, v_hbm, wq_hbm, wo_hbm, w3_hbm, w4_hbm, o_ref,
            kbuf, vbuf, wq, wo, w3, w4, xbuf, qc, pbuf, abuf, sems, *, t0, wt):
    ku = kbuf.bitcast(u32)
    vu = vbuf.bitcast(u32)
    wqu = wq.bitcast(u32)
    wou = wo.bitcast(u32)
    w3u = w3.bitcast(u32)
    w4u = w4.bitcast(u32)

    W4A = 80

    def w_copies(src, dst, sem0, rows=None):
        out = []
        for e in range(2):
            if rows is None:
                s, d = src.at[:, e], dst.at[:, :, pl.ds(8 * e, 8), :]
            else:
                s, d = src.at[rows, e], dst.at[rows, :, pl.ds(8 * e, 8), :]
            out.append(pltpu.make_async_copy(s, d, sems.at[sem0 + e]))
        return out

    x_cp = pltpu.make_async_copy(x_hbm, xbuf, sems.at[0])
    wq_cp = w_copies(wq_hbm, wq, 1)
    wo_cp = w_copies(wo_hbm, wo, 3)
    w3_cp = w_copies(w3_hbm, w3, 5)
    w4a_cp = w_copies(w4_hbm, w4, 7, pl.ds(0, W4A))
    w4b_cp = w_copies(w4_hbm, w4, 9, pl.ds(W4A, F // 16 - W4A))
    S0 = 11

    def k_cp(i):
        return pltpu.make_async_copy(
            k_hbm.at[pl.ds(i * GP, GP), pl.ds(t0 * 8, wt * 8), :],
            kbuf.at[pl.ds(i * GP, GP)], sems.at[S0 + i])

    def v_cp(i):
        return pltpu.make_async_copy(
            v_hbm.at[pl.ds(i * GP, GP), pl.ds(t0 * 8, wt * 8), :],
            vbuf.at[pl.ds(i * GP, GP)], sems.at[S0 + NP + i])

    for c in wq_cp:
        c.start()
    x_cp.start()
    k_cp(0).start()
    for c in wo_cp:
        c.start()
    for i in range(1, NP):
        k_cp(i).start()
        v_cp(i - 1).start()
    v_cp(NP - 1).start()
    for c in w3_cp + w4a_cp + w4b_cp:
        c.start()

    lane = lax.broadcasted_iota(jnp.int32, (8, 128), 1)
    sub = lax.broadcasted_iota(jnp.int32, (8, 128), 0)
    kmask = jnp.where(
        ((lane & 63) >> 4) == sub,
        jnp.where((lane & 8) == 0, jnp.uint32(0xFFFF), jnp.uint32(HI)),
        jnp.uint32(0))
    lane_lo64 = lane < 64
    lane_b3 = (lane & 8) == 0
    sub_b0 = (sub & 1) == 1
    sub_b1 = (sub & 2) == 2
    scale = DH ** -0.5

    def s1_q(yb, i):
        w = jnp.concatenate(
            [_wtile(wqu, slice(None), 3 * i + n) for n in range(3)], axis=1)
        q = jnp.dot(yb, w, preferred_element_type=f32)
        qb = pltpu.bitcast(q.astype(bf16).astype(f32), u32)
        q0, q1, q2 = qb[:, 0:128], qb[:, 128:256], qb[:, 256:384]
        q1a = jnp.where(lane_lo64, q1, pltpu.roll(q1, 32, 1))
        q1b = jnp.where(lane_lo64, pltpu.roll(q1, 64, 1), pltpu.roll(q1, 96, 1))
        for n, qq in enumerate((q0, q1a, q1b, q2)):
            c = (qq >> 16) | pltpu.roll(qq, 8, 1)
            c = jnp.where(sub_b0, pltpu.roll(c, 16, 1), c)
            qc[i, n] = jnp.where(sub_b1, pltpu.roll(c, 32, 1), c)

    def s2_scores(i, slot):
        g0 = i * GP
        plan = (
            [(0, a, a, a + 8) for a in range(8)] + [(1, a, 16 + a, 20 + a) for a in range(4)],
            [(2, a, 24 + a, 28 + a) for a in range(4)] + [(3, a, 32 + a, 40 + a) for a in range(8)],
        )
        for hh in range(2):
            s = None
            for (n, a, ga, gb) in plan[hh]:
                c = qc[i, n]
                if a:
                    c = pltpu.roll(c, 128 - 8 * a, 1)
                lhs = pltpu.bitcast(c & kmask, bf16)
                w = jnp.concatenate(
                    [jnp.concatenate(
                        [ku[g0 + g, 32 * t:32 * t + 32, :] for t in range(4)], axis=1)
                     for g in (ga, gb)], axis=0)
                r = jnp.dot(lhs, pltpu.bitcast(w, bf16),
                            preferred_element_type=f32)[0:8]
                s = r if s is None else s + r
            m = jnp.max(jnp.max(s, axis=1, keepdims=True), axis=0, keepdims=True)
            p = jnp.exp((s - m) * scale)
            l = jnp.sum(jnp.sum(p, axis=1, keepdims=True), axis=0, keepdims=True)
            p = p * (1.0 / l)
            for t in range(4):
                pt = p[:, 128 * t:128 * t + 128]
                for k in range(4):
                    pbuf[slot, hh, pl.ds(32 * t + k, 8, stride=4), :] = pt

    def s3_pv(i, slot):
        g0 = i * GP
        for hh in range(2):
            pv = [pbuf[slot, hh, 8 * j:8 * j + 8, :] for j in range(16)]
            for gg in range(GP // 2):
                g = hh * (GP // 2) + gg
                lo = [None, None]
                hi = [None, None]
                for j in range(16):
                    w = vu[g0 + g, 8 * j:8 * j + 8, :]
                    a = pltpu.bitcast(w << 16, f32) * pv[j]
                    b = pltpu.bitcast(w & jnp.uint32(HI), f32) * pv[j]
                    k = j % 2
                    lo[k] = a if lo[k] is None else lo[k] + a
                    hi[k] = b if hi[k] is None else hi[k] + b
                beta, g8, e = g // 16, (g % 16) // 2, g % 2
                abuf[slot, beta, e, pl.ds(16 * g8, 8, stride=2), :] = lo[0] + lo[1]
                abuf[slot, beta, e, pl.ds(16 * g8 + 1, 8, stride=2), :] = hi[0] + hi[1]

    def s4_out(i, slot):
        fs = []
        for beta in range(3):
            z = [jnp.sum(abuf[slot, beta, e].T.reshape(16, 8, 128), axis=0) for e in range(2)]
            fold = jnp.where(lane_b3,
                             z[0] + pltpu.roll(z[0], 120, 1),
                             z[1] + pltpu.roll(z[1], 8, 1))
            fs.append(jnp.sum(fold, axis=0, keepdims=True))
        o = jnp.broadcast_to(jnp.concatenate(fs, axis=1), (8, 384)).astype(bf16)
        rows = pl.ds(i * (GP // 2), GP // 2)
        w = jnp.concatenate([_wtile(wou, rows, n) for n in range(5)], axis=1)
        return jnp.dot(o, w, preferred_element_type=f32)

    def layer(it, x):
        first = it == 0
        yb = _ln(x).astype(bf16)

        @pl.when(first)
        def _():
            for c in wq_cp:
                c.wait()
            k_cp(0).wait()
            for c in wo_cp:
                c.wait()

        s1_q(yb, 0)
        s1_q(yb, 1)
        s2_scores(0, 0)

        def body(i, acc):
            @pl.when(first)
            def _():
                @pl.when(i + 1 < NP)
                def _():
                    k_cp(i + 1).wait()
                v_cp(i).wait()

            slot = i % 2
            prev = s4_out(jnp.maximum(i - 1, 0), 1 - slot)
            s3_pv(i, slot)
            s2_scores(jnp.minimum(i + 1, NP - 1), 1 - slot)
            s1_q(yb, jnp.minimum(i + 2, NP - 1))
            return acc + jnp.where(i > 0, prev, 0.0)

        acc = lax.fori_loop(0, NP, body, jnp.zeros((8, D), f32))
        x = x + acc + s4_out(NP - 1, (NP - 1) % 2)

        y = _ln(x)
        z = _ln(y).astype(bf16)

        @pl.when(first)
        def _():
            for c in w3_cp:
                c.wait()

        w = jnp.concatenate([_wtile(w3u, slice(None), n) for n in range(F // 128)], axis=1)
        h = jax.nn.gelu(jnp.dot(z, w, preferred_element_type=f32), approximate=True).astype(bf16)

        @pl.when(first)
        def _():
            for c in w4a_cp:
                c.wait()

        w = jnp.concatenate([_wtile(w4u, slice(0, W4A), n) for n in range(5)], axis=1)
        x = x + y + jnp.dot(h[:, :W4A * 16], w, preferred_element_type=f32)

        @pl.when(first)
        def _():
            for c in w4b_cp:
                c.wait()

        w = jnp.concatenate([_wtile(w4u, slice(W4A, F // 16), n) for n in range(5)], axis=1)
        return x + jnp.dot(h[:, W4A * 16:], w, preferred_element_type=f32)

    x_cp.wait()
    x = jnp.broadcast_to(xbuf[...].astype(f32), (8, D))
    x = lax.fori_loop(0, 2, layer, x)
    o_ref[...] = x[0:1].astype(o_ref.dtype)


def _cache_view(c):
    s = c.shape[2]
    c = jnp.transpose(c, (0, 1, 3, 2)).reshape(H * DH // 8, 8, s // 128, 128)
    return jnp.transpose(c, (0, 2, 1, 3)).reshape(H * DH // 8, s // 128 * 8, 128)


def _weight_view(w):
    k, n = w.shape
    return jnp.transpose(w.reshape(k // 16, 2, 8, n // 128, 128), (0, 1, 3, 2, 4))


@jax.jit
def pallas_interleave_layers__sliding_block_cached__mixer_s_mlp__decode_kernel(
    A_x: jax.Array,
    A_k_cache: jax.Array,
    A_v_cache: jax.Array,
    A_wq: jax.Array,
    A_wo: jax.Array,
    B_x: jax.Array,
    B_w1: jax.Array,
    B_w2: jax.Array,
    B_w3: jax.Array,
    B_w4: jax.Array,
):
    sk = A_k_cache.shape[2]
    win = min(4096, max(256, sk // 4))
    assert win == 4096 and sk % 128 == 0
    assert A_x.shape == (1, 1, D) and A_k_cache.shape == (1, H, sk, DH)
    wt = win // 128
    t0 = sk // 128 - wt
    ng = H * DH // 8
    hbm = pl.BlockSpec(memory_space=pl.ANY)
    out = pl.pallas_call(
        functools.partial(_kernel, t0=t0, wt=wt),
        out_shape=jax.ShapeDtypeStruct((1, D), A_x.dtype),
        in_specs=[hbm] * 7,
        out_specs=pl.BlockSpec(memory_space=pltpu.VMEM),
        scratch_shapes=[
            pltpu.VMEM((ng, wt * 8, 128), bf16),
            pltpu.VMEM((ng, wt * 8, 128), bf16),
            pltpu.VMEM((D // 16, H * DH // 128, 16, 128), bf16),
            pltpu.VMEM((H * DH // 16, D // 128, 16, 128), bf16),
            pltpu.VMEM((D // 16, F // 128, 16, 128), bf16),
            pltpu.VMEM((F // 16, D // 128, 16, 128), bf16),
            pltpu.VMEM((1, D), bf16),
            pltpu.VMEM((NP, 4, 8, 128), u32),
            pltpu.VMEM((2, 2, 128, 128), f32),
            pltpu.VMEM((2, 3, 2, 128, 128), f32),
            pltpu.SemaphoreType.DMA((11 + 2 * NP,)),
        ],
        compiler_params=pltpu.CompilerParams(vmem_limit_bytes=124 * 1024 * 1024),
    )(A_x.reshape(1, D), _cache_view(A_k_cache), _cache_view(A_v_cache),
      _weight_view(A_wq), _weight_view(A_wo), _weight_view(B_w3), _weight_view(B_w4))
    return out.reshape(1, 1, D)
```

```python
import functools

import jax
import jax.numpy as jnp
from jax import lax
import jax.experimental.pallas as pl
import jax.experimental.pallas.tpu as pltpu

D = 640
H = 32
DH = 192
F = 1536
EPS = 1e-5
NP = H // 2
GP = 2 * DH // 8
HI = 0xFFFF0000
LOG2E = 1.4426950408889634

f32 = jnp.float32
bf16 = jnp.bfloat16
u32 = jnp.uint32

L_Y = 0
L_O = 5
L_DUMMY = 8
SEG = 25.5
NREV = 7


def _ln(x):
    m = jnp.mean(x, axis=-1, keepdims=True)
    c = x - m
    v = jnp.mean(c * c, axis=-1, keepdims=True)
    return c * lax.rsqrt(v + EPS)


def _wtile(wu, rows, nt):
    blk = wu[rows, nt]
    return pltpu.bitcast(blk.reshape(blk.shape[0] * 8, 128), bf16)


def _pack_rows(x):
    return pltpu.bitcast(jnp.concatenate([x, x], axis=0).astype(bf16), u32)


def _slot(G, t):
    j = 4 * (t >> 3) + ((((t >> 1) & 3) + G + 2 * (t & 1) + (t >> 3)) & 3)
    return 2 * G + (t & 1), 8 * j


def _kernel(x_hbm, k_hbm, v_hbm, wq_hbm, wo_hbm, w3_hbm, w4_hbm, o_ref,
            kbuf, vbuf, wq, wo, w3, w4, xbuf, lref, qref, sbuf, abuf, zs, sems, *pT,
            t0, wt):
    ku = kbuf.bitcast(u32)
    vu = vbuf.bitcast(u32)
    wqu = wq.bitcast(u32)
    wou = wo.bitcast(u32)
    w3u = w3.bitcast(u32)
    w4u = w4.bitcast(u32)

    W4A = 80

    def w_copies(src, dst, sem0, rows=None):
        out = []
        for e in range(2):
            if rows is None:
                s, d = src.at[:, e], dst.at[:, :, pl.ds(8 * e, 8), :]
            else:
                s, d = src.at[rows, e], dst.at[rows, :, pl.ds(8 * e, 8), :]
            out.append(pltpu.make_async_copy(s, d, sems.at[sem0 + e]))
        return out

    x_cp = pltpu.make_async_copy(x_hbm, xbuf, sems.at[0])
    wq_cp = w_copies(wq_hbm, wq, 1)
    wo_cp = w_copies(wo_hbm, wo, 3)
    w3_cp = w_copies(w3_hbm, w3, 5)
    w4a_cp = w_copies(w4_hbm, w4, 7, pl.ds(0, W4A))
    w4b_cp = w_copies(w4_hbm, w4, 9, pl.ds(W4A, F // 16 - W4A))
    S0 = 11

    def k_cp(i):
        return pltpu.make_async_copy(
            k_hbm.at[pl.ds(i * GP, GP), pl.ds(t0 * 8, wt * 8), :],
            kbuf.at[pl.ds(i * GP, GP)], sems.at[S0 + i])

    def v_cp(i):
        return pltpu.make_async_copy(
            v_hbm.at[pl.ds(i * GP, GP), pl.ds(t0 * 8, wt * 8), :],
            vbuf.at[pl.ds(i * GP, GP)], sems.at[S0 + NP + i])

    k_cp(0).start()
    x_cp.start()
    for c in wq_cp + wo_cp:
        c.start()
    for i in range(1, NP):
        k_cp(i).start()
        v_cp(i - 1).start()
    v_cp(NP - 1).start()
    for c in w3_cp + w4a_cp + w4b_cp:
        c.start()

    zs[0] = 0

    lane = lax.broadcasted_iota(jnp.int32, (8, 128), 1)
    sub = lax.broadcasted_iota(jnp.int32, (8, 128), 0)
    lane_lo = lane < 64
    sub_lo = sub < 4
    cexp = DH ** -0.5 * LOG2E

    def tile(ref, g0, G, t):
        g, r = _slot(G, t)
        return ref[g0 + g, r:r + 8, :]

    def retile(ref, i):
        def body(c, carry):
            g0 = i * GP + 8 * c
            for G in range(4):
                for J in range(4):
                    xs = [[ref[g0 + 2 * G + e, 32 * J + 8 * jj:32 * J + 8 * jj + 8, :]
                           for jj in range(4)] for e in range(2)]
                    for jj in range(4):
                        x0, x1 = xs[0][jj], xs[1][jj]
                        ys = (jnp.where(sub_lo, x0, pltpu.roll(x1, 4, 0)),
                              jnp.where(sub_lo, pltpu.roll(x0, 4, 0), x1))
                        for e in range(2):
                            g, r = _slot(G, 8 * J + 2 * jj + e)
                            ref[g0 + g, r:r + 8, :] = ys[e]
            return carry
        lax.fori_loop(0, GP // 8, body, 0)

    def lhs_at(ref, n):
        return pltpu.bitcast(ref[8 * n:8 * n + 8, :], bf16)

    def q_dots(i, st):
        def step(k):
            def run():
                w = jnp.concatenate(
                    [_wtile(wqu, slice(8 * k, 8 * k + 8), 3 * i + n) for n in range(3)], axis=1)
                r = jnp.dot(lhs_at(lref, L_Y + k), w, preferred_element_type=f32)[0:8]
                st["q"] = r if k == 0 else st["q"] + r
                if k == 4:
                    qb = pltpu.bitcast(st["q"].astype(bf16).astype(f32), u32)
                    q0, q1, q2 = qb[:, 0:128], qb[:, 128:256], qb[:, 256:384]
                    q1r = pltpu.roll(q1, 64, 1)
                    ua = jnp.where(lane_lo, q1 >> 16, q1r)
                    ub = jnp.where(lane_lo, q1r >> 16, q1)
                    zero = jnp.zeros((8, 128), u32)
                    for hh, (qf, u) in enumerate(((q0, ua), (q2, ub))):
                        halves = (qf >> 16, qf)
                        for rho in range(8):
                            qref[8 * (12 * hh + rho):8 * (12 * hh + rho) + 8, :] = jnp.where(
                                sub == rho // 2, halves[rho % 2], zero)
                        for n in range(4):
                            qref[8 * (12 * hh + 8 + n):8 * (12 * hh + 8 + n) + 8, :] = jnp.where(
                                sub == n, u, zero)
                return r[:, 256:384]
            return 3, run
        return [step(k) for k in range(5)]

    def o_dots(i, st):
        def step(b):
            def run():
                rows = pl.ds(i * (GP // 2) + 8 * b, 8)
                w = jnp.concatenate([_wtile(wou, rows, n) for n in range(5)], axis=1)
                r = jnp.dot(lhs_at(lref, L_O + b), w, preferred_element_type=f32)[0:8]
                st["acc"] = st["acc"] + r
                return r[:, 512:640]
            return 5, run
        return [step(b) for b in range(3)]

    def softmax_store(s, hh):
        m = jnp.maximum(jnp.maximum(s[:, 0:128], s[:, 128:256]),
                        jnp.maximum(s[:, 256:384], s[:, 384:512]))
        m = jnp.max(jnp.max(m, axis=1, keepdims=True), axis=0, keepdims=True)
        p = jnp.exp2((s - m) * cexp)
        l = (p[:, 0:128] + p[:, 128:256]) + (p[:, 256:384] + p[:, 384:512])
        l = jnp.sum(jnp.sum(l, axis=1, keepdims=True), axis=0, keepdims=True)
        p = p * (1.0 / l)
        for T in range(4):
            for k in range(8):
                pT[4 * hh + T][pl.ds(k, 8, stride=8), :] = p[:, 128 * T:128 * T + 128]

    def k_dots(i, st):
        g0 = i * GP

        def step(hh, r):
            def run():
                gf, gh = ((0, 8), (16, 12))[hh]
                if r < 8:
                    cols = [[tile(ku, g0, gf + G, 8 * T + r) for G in range(8)] for T in range(4)]
                else:
                    cols = [[tile(ku, g0, gh + G % 4, 8 * T + 2 * (r - 8) + G // 4)
                             for G in range(8)] for T in range(4)]
                w = jnp.concatenate([jnp.concatenate(c, axis=0) for c in cols], axis=1)
                res = jnp.dot(lhs_at(qref, 12 * hh + r), pltpu.bitcast(w, bf16),
                              preferred_element_type=f32)[0:8]
                st["s"] = res if r == 0 else st["s"] + res
                if r == 11:
                    if hh == 0:
                        st["sA"] = st["s"]
                    else:
                        sbuf[...] = st["s"]
                return res[:, 384:512]
            return 4, run
        return [step(hh, r) for hh in range(2) for r in range(12)]

    def reduce_o():
        outs = []
        for b in range(3):
            z = jnp.sum(abuf[b].T.reshape(16, 8, 128), axis=0)
            outs.append(jnp.broadcast_to(jnp.sum(z, axis=0, keepdims=True), (8, 128)))
        return outs

    def store_o(outs):
        for b in range(3):
            lref[8 * (L_O + b):8 * (L_O + b) + 8, :] = _pack_rows(outs[b])

    def body(i, acc, first):
        @pl.when(first)
        def _():
            @pl.when(i + 1 < NP)
            def _():
                k_cp(i + 1).wait()
                retile(ku, i + 1)
            v_cp(i).wait()
            retile(vu, i)

        g0 = i * GP
        z = zs[0]
        nxt = jnp.minimum(i + 1, NP - 1)
        st = {"acc": acc}
        softmax_store(sbuf[...], 1)
        o_prev = reduce_o()
        dots = q_dots(nxt, st) + o_dots(jnp.maximum(i - 2, 0), st) + k_dots(nxt, st)
        issue, tiles = [], 0
        for n, _ in dots:
            tiles += n
            issue.append(8 * tiles)
        clock = []

        def emit(upto):
            while len(clock) < upto:
                clock.append(dots[len(clock)][1]())
                if len(clock) == 8:
                    store_o(o_prev)

        seg = 0
        prev = None
        for hh in range(2):
            for gp in range(6):
                a4 = [None] * 4
                for T in range(4):
                    pref = pT[4 * hh + T]
                    if seg < NREV:
                        emit(sum(1 for c in issue if c < SEG * (seg + 1) + 12))
                        if seg >= 4:
                            pref[pl.ds(pl.multiple_of(z + 64, 8), 8), :] = prev
                    else:
                        emit(len(dots))
                        n = sum(1 for c in issue if c + 140 <= SEG * seg)
                        pref[pl.ds(pl.multiple_of(z + 64, 8), 8), :] = clock[max(n, 1) - 1]
                    for rho in range(8):
                        pv = pref[8 * rho:8 * rho + 8, :]
                        for e in range(2):
                            w = tile(vu, g0, 12 * hh + 2 * gp + e, 8 * T + rho)
                            a = pltpu.bitcast(w << 16, f32) * pv
                            b = pltpu.bitcast(w & jnp.uint32(HI), f32) * pv
                            a4[2 * e] = a if a4[2 * e] is None else a4[2 * e] + a
                            a4[2 * e + 1] = b if a4[2 * e + 1] is None else a4[2 * e + 1] + b
                    if T == 0:
                        prev = a4[0]
                    if seg < NREV:
                        for k in range(4):
                            lref[pl.ds(pl.multiple_of(z + 8 * (L_DUMMY + k), 8), 8), :] = (
                                pltpu.bitcast(a4[k], u32))
                    seg += 1
                for e in range(2):
                    G = 12 * hh + 2 * gp + e
                    abuf[G // 8, pl.ds(16 * (G % 8), 8, stride=2), :] = a4[2 * e]
                    abuf[G // 8, pl.ds(16 * (G % 8) + 1, 8, stride=2), :] = a4[2 * e + 1]
            if hh == 0:
                softmax_store(st["sA"], 0)
        return st["acc"]

    def layer(it, x):
        first = it == 0
        y = _ln(x)
        yp = _pack_rows(y)
        for k in range(5):
            lref[8 * (L_Y + k):8 * (L_Y + k) + 8, :] = yp[:, 128 * k:128 * k + 128]
        lref[8 * L_O:8 * L_O + 24, :] = jnp.zeros((24, 128), u32)
        abuf[...] = jnp.zeros(abuf.shape, f32)

        @pl.when(first)
        def _():
            k_cp(0).wait()
            retile(ku, 0)
            for c in wq_cp + wo_cp:
                c.wait()

        st = {}
        for _, run in q_dots(0, st) + k_dots(0, st):
            run()
        softmax_store(st["sA"], 0)

        acc = lax.fori_loop(0, NP, functools.partial(body, first=first), x)

        st = {"acc": acc}
        o_prev = reduce_o()
        for _, run in o_dots(NP - 2, st):
            run()
        store_o(o_prev)
        for _, run in o_dots(NP - 1, st):
            run()
        x = st["acc"]

        y = _ln(x)
        zz = _ln(y).astype(bf16)

        @pl.when(first)
        def _():
            for c in w3_cp:
                c.wait()

        w = jnp.concatenate([_wtile(w3u, slice(None), n) for n in range(F // 128)], axis=1)
        h = jax.nn.gelu(jnp.dot(zz, w, preferred_element_type=f32), approximate=True).astype(bf16)

        @pl.when(first)
        def _():
            for c in w4a_cp:
                c.wait()

        w = jnp.concatenate([_wtile(w4u, slice(0, W4A), n) for n in range(5)], axis=1)
        x = x + y + jnp.dot(h[:, :W4A * 16], w, preferred_element_type=f32)

        @pl.when(first)
        def _():
            for c in w4b_cp:
                c.wait()

        w = jnp.concatenate([_wtile(w4u, slice(W4A, F // 16), n) for n in range(5)], axis=1)
        return x + jnp.dot(h[:, W4A * 16:], w, preferred_element_type=f32)

    x_cp.wait()
    x = jnp.broadcast_to(xbuf[...].astype(f32), (8, D))
    x = lax.fori_loop(0, 2, layer, x)
    o_ref[...] = x[0:1].astype(o_ref.dtype)


def _cache_view(c):
    s = c.shape[2]
    c = jnp.transpose(c, (0, 1, 3, 2)).reshape(H * DH // 8, 8, s // 128, 128)
    return jnp.transpose(c, (0, 2, 1, 3)).reshape(H * DH // 8, s // 128 * 8, 128)


def _weight_view(w):
    k, n = w.shape
    return jnp.transpose(w.reshape(k // 16, 2, 8, n // 128, 128), (0, 1, 3, 2, 4))


@jax.jit
def pallas_interleave_layers__sliding_block_cached__mixer_s_mlp__decode_kernel(
    A_x: jax.Array,
    A_k_cache: jax.Array,
    A_v_cache: jax.Array,
    A_wq: jax.Array,
    A_wo: jax.Array,
    B_x: jax.Array,
    B_w1: jax.Array,
    B_w2: jax.Array,
    B_w3: jax.Array,
    B_w4: jax.Array,
):
    sk = A_k_cache.shape[2]
    win = min(4096, max(256, sk // 4))
    assert win == 4096 and sk % 128 == 0
    assert A_x.shape == (1, 1, D) and A_k_cache.shape == (1, H, sk, DH)
    wt = win // 128
    t0 = sk // 128 - wt
    ng = H * DH // 8
    hbm = pl.BlockSpec(memory_space=pl.ANY)
    out = pl.pallas_call(
        functools.partial(_kernel, t0=t0, wt=wt),
        out_shape=jax.ShapeDtypeStruct((1, D), A_x.dtype),
        in_specs=[hbm] * 7,
        out_specs=pl.BlockSpec(memory_space=pltpu.VMEM),
        scratch_shapes=[
            pltpu.VMEM((ng, wt * 8, 128), bf16),
            pltpu.VMEM((ng, wt * 8, 128), bf16),
            pltpu.VMEM((D // 16, H * DH // 128, 16, 128), bf16),
            pltpu.VMEM((H * DH // 16, D // 128, 16, 128), bf16),
            pltpu.VMEM((D // 16, F // 128, 16, 128), bf16),
            pltpu.VMEM((F // 16, D // 128, 16, 128), bf16),
            pltpu.VMEM((1, D), bf16),
            pltpu.VMEM((96, 128), u32),
            pltpu.VMEM((192, 128), u32),
            pltpu.VMEM((8, 512), f32),
            pltpu.VMEM((3, 128, 128), f32),
            pltpu.SMEM((1,), jnp.int32),
            pltpu.SemaphoreType.DMA((11 + 2 * NP,)),
        ] + [pltpu.VMEM((72, 128), f32)] * 8,
        compiler_params=pltpu.CompilerParams(vmem_limit_bytes=124 * 1024 * 1024),
    )(A_x.reshape(1, D), _cache_view(A_k_cache), _cache_view(A_v_cache),
      _weight_view(A_wq), _weight_view(A_wo), _weight_view(B_w3), _weight_view(B_w4))
    return out.reshape(1, 1, D)
```

```python
import functools

import jax
import jax.numpy as jnp
from jax import lax
import jax.experimental.pallas as pl
import jax.experimental.pallas.tpu as pltpu

D = 640
H = 32
DH = 192
F = 1536
EPS = 1e-5
NP = H // 2
GP = 2 * DH // 8
HI = 0xFFFF0000
CEXP = DH ** -0.5 * 1.4426950408889634

f32 = jnp.float32
bf16 = jnp.bfloat16
u32 = jnp.uint32

L_Y = 0
L_O = 5
L_DUMMY = 8
S_MAXB, S_LB, S_INVA = 4, 5, 6
SEG = 25.5
LAT = 140
W4_CHUNKS = (64, 24, 8)


def _mean(x):
    return jnp.mean(x, axis=-1, keepdims=True)


def _ln(x):
    c = x - _mean(x)
    return c * lax.rsqrt(_mean(c * c) + EPS)


def _wtile(wu, rows, nt):
    blk = wu[rows, nt]
    return pltpu.bitcast(blk.reshape(blk.shape[0] * 8, 128), bf16)


def _wcols(wu, rows, nts):
    return jnp.concatenate([_wtile(wu, rows, n) for n in nts], axis=1)


def _rows16(a, b):
    return jnp.concatenate([a, b], axis=0).astype(bf16)


def _slot(G, t):
    j = 4 * (t >> 3) + ((((t >> 1) & 3) + G + 2 * (t & 1) + (t >> 3)) & 3)
    return 2 * G + (t & 1), 8 * j


def _vr(n):
    return slice(8 * n, 8 * n + 8)


def _kernel(x_hbm, k_hbm, v_hbm, wq_hbm, wo_hbm, w3_hbm, w4_hbm, o_ref,
            kbuf, vbuf, wq, wo, w3, w4, xbuf, lref, qa, qb, scl, sbuf, abuf, zs, sems,
            *pT, t0, wt):
    ku = kbuf.bitcast(u32)
    vu = vbuf.bitcast(u32)
    wqu = wq.bitcast(u32)
    wou = wo.bitcast(u32)
    w3u = w3.bitcast(u32)
    w4u = w4.bitcast(u32)

    def w_copies(src, dst, sem0, rows=slice(None)):
        return [pltpu.make_async_copy(src.at[rows, e], dst.at[rows, :, pl.ds(8 * e, 8), :],
                                      sems.at[sem0 + e]) for e in range(2)]

    x_cp = pltpu.make_async_copy(x_hbm, xbuf, sems.at[0])
    wq_cp = w_copies(wq_hbm, wq, 1)
    wo_cp = w_copies(wo_hbm, wo, 3)
    w3_cp = w_copies(w3_hbm, w3, 5)
    w4_rows, r0 = [], 0
    for n in W4_CHUNKS:
        w4_rows.append((r0, r0 + n))
        r0 += n
    w4_cp = [w_copies(w4_hbm, w4, 7 + 2 * c, pl.ds(a, b - a)) for c, (a, b) in enumerate(w4_rows)]
    S0 = 7 + 2 * len(W4_CHUNKS)

    def k_cp(i):
        return pltpu.make_async_copy(
            k_hbm.at[pl.ds(i * GP, GP), pl.ds(t0 * 8, wt * 8), :],
            kbuf.at[pl.ds(i * GP, GP)], sems.at[S0 + i])

    def v_cp(i):
        return pltpu.make_async_copy(
            v_hbm.at[pl.ds(i * GP, GP), pl.ds(t0 * 8, wt * 8), :],
            vbuf.at[pl.ds(i * GP, GP)], sems.at[S0 + NP + i])

    k_cp(0).start()
    x_cp.start()
    for c in wq_cp + wo_cp:
        c.start()
    v_cp(0).start()
    for i in range(1, NP):
        k_cp(i).start()
        v_cp(i).start()
    for c in w3_cp + sum(w4_cp, []):
        c.start()

    zs[0] = 0

    lane = lax.broadcasted_iota(jnp.int32, (8, 128), 1)
    sub = lax.broadcasted_iota(jnp.int32, (8, 128), 0)
    lane_lo = lane < 64
    sub_lo = sub < 4

    def tile(ref, g0, G, t):
        g, r = _slot(G, t)
        return ref[g0 + g, r:r + 8, :]

    def retile(ref, i):
        def body(c, carry):
            g0 = i * GP + 8 * c
            for G in range(4):
                for J in range(4):
                    xs = [[ref[g0 + 2 * G + e, _vr(4 * J + jj), :] for jj in range(4)]
                          for e in range(2)]
                    for jj in range(4):
                        x0, x1 = xs[0][jj], xs[1][jj]
                        ys = (jnp.where(sub_lo, x0, pltpu.roll(x1, 4, 0)),
                              jnp.where(sub_lo, pltpu.roll(x0, 4, 0), x1))
                        for e in range(2):
                            g, r = _slot(G, 8 * J + 2 * jj + e)
                            ref[g0 + g, r:r + 8, :] = ys[e]
            return carry
        lax.fori_loop(0, GP // 8, body, 0)

    def lhs_at(ref, n):
        return pltpu.bitcast(ref[_vr(n), :], bf16)

    cur = [None]

    def tick(ref, n, val):
        if val.dtype != ref.dtype:
            val = pltpu.bitcast(val, ref.dtype)
        ref[pl.ds(pl.multiple_of(cur[0] + 8 * n, 8), 8), :] = val

    def q_dots(i, st, qref, lhs=None, mean=None):
        def step(k):
            def run():
                w = _wcols(wqu, _vr(k), [3 * i + n for n in range(3)])
                if lhs is None:
                    r = jnp.dot(lhs_at(lref, L_Y + k), w, preferred_element_type=f32)[0:8]
                else:
                    r = jnp.dot(lhs[:, 128 * k:128 * k + 128], w, preferred_element_type=f32)
                st["q"] = r if k == 0 else st["q"] + r
                if k == 4:
                    q = st["q"] if lhs is None else st["q"][0:8] - mean * st["q"][8:16]
                    qq = pltpu.bitcast(q.astype(bf16).astype(f32), u32)
                    q0, q1, q2 = qq[:, 0:128], qq[:, 128:256], qq[:, 256:384]
                    for n, v in enumerate((q0 >> 16, q0, q2 >> 16, q2, q1, pltpu.roll(q1, 64, 1))):
                        qref[_vr(n), :] = v
                return r[0:8, 256:384]
            return 3, lref, L_DUMMY, run
        return [step(k) for k in range(5)]

    def o_dots(i, st):
        def step(b):
            def run():
                w = _wcols(wou, pl.ds(i * (GP // 2) + 8 * b, 8), range(5))
                r = jnp.dot(lhs_at(lref, L_O + b), w, preferred_element_type=f32)[0:8]
                st["acc"] = st["acc"] + r
                return r[:, 512:640]
            return 5, lref, L_DUMMY, run
        return [step(b) for b in range(3)]

    def k_dots(i, hh, st, qref, order=tuple(range(12))):
        g0 = i * GP
        gf, gh = ((0, 8), (16, 12))[hh]

        def step(r):
            def run():
                if r < 8:
                    cols = [[tile(ku, g0, gf + G, 8 * T + r) for G in range(8)] for T in range(4)]
                    base, row = qref[_vr(2 * hh + r % 2), :], r // 2
                else:
                    cols = [[tile(ku, g0, gh + G % 4, 8 * T + 2 * (r - 8) + G // 4)
                             for G in range(8)] for T in range(4)]
                    if r == 8:
                        st["u"] = jnp.where(lane_lo, qref[_vr(4 + hh), :] >> 16,
                                            qref[_vr(5 - hh), :])
                    base, row = st["u"], r - 8
                lhs = jnp.where(sub == row, base, jnp.zeros((8, 128), u32))
                w = jnp.concatenate([jnp.concatenate(c, axis=0) for c in cols], axis=1)
                res = jnp.dot(pltpu.bitcast(lhs, bf16), pltpu.bitcast(w, bf16),
                              preferred_element_type=f32)[0:8]
                st["s", hh] = res if r == order[0] else st["s", hh] + res
                return res[:, 384:512]
            return 4, qref, 6, run
        return [step(r) for r in order]

    def col(s, T):
        return s[:, 128 * T:128 * T + 128]

    def row_max(s):
        m = jnp.maximum(jnp.maximum(col(s, 0), col(s, 1)), jnp.maximum(col(s, 2), col(s, 3)))
        return jnp.max(jnp.max(m, axis=1, keepdims=True), axis=0, keepdims=True)

    def prob(s, m):
        return jnp.exp2((s - m) * scl[_vr(0), :])

    def put_p(hh, T, p, ks=range(8)):
        for k in ks:
            pT[4 * hh + T][pl.ds(k, 8, stride=8), :] = p

    def part_sum(p):
        return (p[0] + p[1]) + (p[2] + p[3])

    def inv_sum(l):
        l = jnp.sum(jnp.sum(l, axis=1, keepdims=True), axis=0, keepdims=True)
        return jnp.broadcast_to(1.0 / l, (8, 128))

    def softmax(s, hh):
        m = row_max(s)
        p = [prob(col(s, T), m) for T in range(4)]
        for T in range(4):
            put_p(hh, T, p[T])
        return p, part_sum(p)

    def stash_b(i, s):
        for T in range(4):
            sbuf[i, _vr(T), :] = col(s, T)
        m = jnp.broadcast_to(row_max(s), (8, 128))
        sbuf[i, _vr(S_MAXB), :] = m
        return m

    def reduce_o(aref, a0, inva, invb):
        out = []
        for b, inv in enumerate((inva, jnp.where(lane_lo, inva, invb), invb)):
            z = jnp.sum(pltpu.bitcast(aref[a0 + b], f32).T.reshape(16, 8, 128), axis=0)
            o = jnp.sum(z, axis=0, keepdims=True) * inv
            out.append(pltpu.bitcast(_rows16(o, o), u32))
        return out

    def put_o(o):
        for b in range(3):
            lref[_vr(L_O + b), :] = o[b]

    def run_block(i, aref, a0, dots, issue, tv0, hooks):
        g0 = i * GP
        clock = []

        def emit(upto):
            while len(clock) < upto:
                n = len(clock)
                for h in hooks.get(("dot", n), ()):
                    h()
                clock.append(dots[n][3]())

        seg = 0
        prev = None
        for hh in range(2):
            for gp in range(6):
                a4 = [None] * 4
                for T in range(4):
                    pref = pT[4 * hh + T]
                    start = tv0 + SEG * seg
                    emit(sum(1 for c in issue if c < start + SEG + 12))
                    done = sum(1 for c in issue if c + LAT <= start)
                    if done:
                        tick(pref, 8, clock[done - 1])
                    elif gp:
                        tick(pref, 8, prev)
                    for h in hooks.get(("seg", seg), ()):
                        h(clock[done - 1] if done else prev)
                    for rho in range(8):
                        pv = pref[_vr(rho), :]
                        for e in range(2):
                            w = tile(vu, g0, 12 * hh + 2 * gp + e, 8 * T + rho)
                            a = pltpu.bitcast(w << 16, f32) * pv
                            b = pltpu.bitcast(w & jnp.uint32(HI), f32) * pv
                            a4[2 * e] = a if a4[2 * e] is None else a4[2 * e] + a
                            a4[2 * e + 1] = b if a4[2 * e + 1] is None else a4[2 * e + 1] + b
                    if T == 0:
                        prev = a4[0]
                    if not done and len(clock) < len(dots):
                        _, ref, slot, _ = dots[len(clock)]
                        for k in range(4):
                            tick(ref, slot + k, a4[k])
                    seg += 1
                for e in range(2):
                    G = 12 * hh + 2 * gp + e
                    for k in range(2):
                        aref[a0 + G // 8, pl.ds(16 * (G % 8) + k, 8, stride=2), :] = (
                            pltpu.bitcast(a4[2 * e + k], u32))
        emit(len(dots))

    def times(dots, t=0):
        out = []
        for d in dots:
            t += 8 * d[0]
            out.append(t)
        return out

    def run_all(dots):
        for d in dots:
            d[3]()

    def set_input(c, scale):
        cp = pltpu.bitcast(_rows16(c, c), u32)
        for k in range(5):
            lref[_vr(L_Y + k), :] = cp[:, 128 * k:128 * k + 128]
        scl[_vr(0), :] = jnp.broadcast_to(scale, (8, 128))

    x_cp.wait()
    x = jnp.broadcast_to(xbuf[...].astype(f32), (8, D))
    set_input(_ln(x), jnp.full((8, 1), CEXP, f32))
    for c in wq_cp + wo_cp:
        c.wait()

    def body1(i, acc):
        st = {"acc": acc}
        k_cp(i).wait()
        retile(ku, i)
        run_all(q_dots(i, st, qa))
        inv = []
        for hh in range(2):
            run_all(k_dots(i, hh, st, qa))
            inv.append(inv_sum(softmax(st["s", hh], hh)[1]))
        v_cp(i).wait()
        retile(vu, i)
        cur[0] = zs[0]
        run_block(i, abuf, 0, [], [], 0, {})
        put_o(reduce_o(abuf, 0, inv[0], inv[1]))
        run_all(o_dots(i, st))
        return st["acc"]

    x = lax.fori_loop(0, NP, body1, x)

    y = _ln(x)
    zz = _ln(y).astype(bf16)
    for c in w3_cp:
        c.wait()
    h = jnp.dot(zz, _wcols(w3u, slice(None), range(F // 128)), preferred_element_type=f32)
    h = jax.nn.gelu(h, approximate=True).astype(bf16)
    x = x + y
    for cps, (a, b) in zip(w4_cp, w4_rows):
        for c in cps:
            c.wait()
        x = x + jnp.dot(h[:, 16 * a:16 * b], _wcols(w4u, slice(a, b), range(5)),
                        preferred_element_type=f32)

    ones = jnp.ones((8, D), f32)
    xl = _rows16(x, ones)
    xb = xl[0:8].astype(f32)
    mean = _mean(xb)
    c = xb - mean
    set_input(c, lax.rsqrt(_mean(c * c) + EPS) * CEXP)
    lref[8 * L_O:8 * L_O + 24, :] = jnp.zeros((24, 128), u32)

    def tail_hooks(i, st, hooks, seg0):
        def first(_):
            m = row_max(st["s", 0])
            st["pa"] = [prob(col(st["s", 0], T), m) for T in range(4)]
            sbuf[i, _vr(S_INVA), :] = inv_sum(part_sum(st["pa"]))

        def put(T, half):
            def run(clk):
                tick(pT[T], 8, clk)
                put_p(0, T, st["pa"][T], range(4 * half, 4 * half + 4))
            return run
        hooks.setdefault(("seg", seg0), []).append(first)
        for n in range(8):
            hooks.setdefault(("seg", seg0 + n), []).append(put(n // 2, n % 2))

    def head_b_hooks(i, seg0):
        pb = []

        def put_b(T):
            def run(clk):
                tick(scl, 1, clk)
                pb.append(prob(sbuf[i, _vr(T), :], sbuf[i, _vr(S_MAXB), :]))
                put_p(1, T, pb[T])
                if T == 3:
                    sbuf[i, _vr(S_LB), :] = part_sum(pb)
            return run
        return {("seg", seg0 + 3 * T): [put_b(T)] for T in range(4)}

    def reduce_pair(i):
        return reduce_o(ku, i * GP, sbuf[i, _vr(S_INVA), :], inv_sum(sbuf[i, _vr(S_LB), :]))

    st = {}
    zero = cur[0] = zs[0]
    late = tuple(range(8, 12)) + tuple(range(8))
    d0 = q_dots(0, st, qb, xl, mean) + q_dots(1, st, qa, xl, mean)
    d1 = k_dots(0, 0, st, qb) + k_dots(0, 1, st, qb, late) + k_dots(1, 0, st, qa, late) \
        + k_dots(1, 1, st, qa) + q_dots(2, st, qa)
    issue = times(d0 + d1)

    def sm_a0():
        m = row_max(st["s", 0])
        p = [prob(col(st["s", 0], T), m) for T in range(4)]
        tick(qb, 6, part_sum(p))
        for T in range(4):
            put_p(0, T, p[T])
        sbuf[0, _vr(S_INVA), :] = inv_sum(part_sum(p))

    def sm_b0():
        tick(qa, 6, stash_b(0, st["s", 1]))

    hooks = head_b_hooks(0, 15)
    hooks.update({("dot", 31): [sm_a0], ("dot", 43): [sm_b0]})
    tail_hooks(1, st, hooks, 36)
    run_block(0, ku, 0, d0 + d1, issue, 240 + 384 + LAT + 170, hooks)
    stash_b(1, st["s", 1])

    def body2(j, acc, last=False):
        cur[0] = zs[0]
        st = {"acc": acc}
        o = reduce_pair(j)
        dots = o_dots(jnp.maximum(j - 1, 0), st)
        hooks = head_b_hooks(j + 1, 9)
        if last:
            run_all(dots)
            dots = []
        else:
            dots = k_dots(j + 2, 0, st, qa) + k_dots(j + 2, 1, st, qa) \
                + q_dots(jnp.minimum(j + 3, NP - 1), st, qa) + dots
            tail_hooks(j + 2, st, hooks, 39)
            hooks["dot", 24] = [lambda: stash_b(j + 2, st["s", 1])]
        run_block(j + 1, ku, (j + 1) * GP, dots, times(dots), 0, hooks)
        put_o(o)
        return st["acc"]

    x = lax.fori_loop(0, NP - 2, body2, x)
    x = lax.fori_loop(NP - 2, NP - 1 + zero, functools.partial(body2, last=True), x)

    st = {"acc": x}
    o = reduce_pair(NP - 1)
    run_all(o_dots(NP - 2, st))
    put_o(o)
    run_all(o_dots(NP - 1, st))
    x = st["acc"]

    xl = _rows16(x, ones)
    xb = xl[0:8].astype(f32)
    mean = _mean(xb)
    c = xb - mean
    r1 = lax.rsqrt(_mean(c * c) + EPS)
    y = c * r1
    my = _mean(y)
    r2 = lax.rsqrt(_mean(y * y) - my * my + EPS)
    h = jnp.dot(xl, _wcols(w3u, slice(None), range(F // 128)), preferred_element_type=f32)
    h = h[0:8] * (r1 * r2) - h[8:16] * ((mean * r1 + my) * r2)
    h = jax.nn.gelu(h, approximate=True).astype(bf16)
    x = x + y + jnp.dot(h, _wcols(w4u, slice(None), range(5)), preferred_element_type=f32)
    o_ref[...] = x[0:1].astype(o_ref.dtype)


def _cache_view(c):
    s = c.shape[2]
    c = jnp.transpose(c, (0, 1, 3, 2)).reshape(H * DH // 8, 8, s // 128, 128)
    return jnp.transpose(c, (0, 2, 1, 3)).reshape(H * DH // 8, s // 128 * 8, 128)


def _weight_view(w):
    k, n = w.shape
    return jnp.transpose(w.reshape(k // 16, 2, 8, n // 128, 128), (0, 1, 3, 2, 4))


@jax.jit
def pallas_interleave_layers__sliding_block_cached__mixer_s_mlp__decode_kernel(
    A_x: jax.Array,
    A_k_cache: jax.Array,
    A_v_cache: jax.Array,
    A_wq: jax.Array,
    A_wo: jax.Array,
    B_x: jax.Array,
    B_w1: jax.Array,
    B_w2: jax.Array,
    B_w3: jax.Array,
    B_w4: jax.Array,
):
    sk = A_k_cache.shape[2]
    win = min(4096, max(256, sk // 4))
    assert win == 4096 and sk % 128 == 0
    assert A_x.shape == (1, 1, D) and A_k_cache.shape == (1, H, sk, DH)
    wt = win // 128
    t0 = sk // 128 - wt
    ng = H * DH // 8
    hbm = pl.BlockSpec(memory_space=pl.ANY)
    out = pl.pallas_call(
        functools.partial(_kernel, t0=t0, wt=wt),
        out_shape=jax.ShapeDtypeStruct((1, D), A_x.dtype),
        in_specs=[hbm] * 7,
        out_specs=pl.BlockSpec(memory_space=pltpu.VMEM),
        scratch_shapes=[
            pltpu.VMEM((ng, wt * 8, 128), bf16),
            pltpu.VMEM((ng, wt * 8, 128), bf16),
            pltpu.VMEM((D // 16, H * DH // 128, 16, 128), bf16),
            pltpu.VMEM((H * DH // 16, D // 128, 16, 128), bf16),
            pltpu.VMEM((D // 16, F // 128, 16, 128), bf16),
            pltpu.VMEM((F // 16, D // 128, 16, 128), bf16),
            pltpu.VMEM((1, D), bf16),
            pltpu.VMEM((96, 128), u32),
            pltpu.VMEM((80, 128), u32),
            pltpu.VMEM((80, 128), u32),
            pltpu.VMEM((16, 128), f32),
            pltpu.VMEM((NP, 56, 128), f32),
            pltpu.VMEM((3, 128, 128), u32),
            pltpu.SMEM((1,), jnp.int32),
            pltpu.SemaphoreType.DMA((7 + 2 * len(W4_CHUNKS) + 2 * NP,)),
        ] + [pltpu.VMEM((72, 128), f32)] * 8,
        compiler_params=pltpu.CompilerParams(vmem_limit_bytes=124 * 1024 * 1024),
    )(A_x.reshape(1, D), _cache_view(A_k_cache), _cache_view(A_v_cache),
      _weight_view(A_wq), _weight_view(A_wo), _weight_view(B_w3), _weight_view(B_w4))
    return out.reshape(1, 1, D)
```

```python
import functools

import jax
import jax.numpy as jnp
from jax import lax
import jax.experimental.pallas as pl
import jax.experimental.pallas.tpu as pltpu

D = 640
H = 32
DH = 192
F = 1536
EPS = 1e-5
NP = H // 2
GP = 2 * DH // 8
HI = 0xFFFF0000
CEXP = DH ** -0.5 * 1.4426950408889634

f32 = jnp.float32
bf16 = jnp.bfloat16
u32 = jnp.uint32

L_Y = 0
L_O = 5
L_DUMMY = 8
S_MAXB, S_LB, S_INVA = 4, 5, 6
SEG = 25.5
LAT = 140
W4_CHUNKS = (1024, 384, 128)


def _mean(x):
    return jnp.mean(x, axis=-1, keepdims=True)


def _ln(x):
    c = x - _mean(x)
    return c * lax.rsqrt(_mean(c * c) + EPS)


def _wtile(wu, rows, nt):
    blk = wu[rows, nt]
    return pltpu.bitcast(blk.reshape(blk.shape[0] * 8, 128), bf16)


def _wcols(wu, rows, nts):
    return jnp.concatenate([_wtile(wu, rows, n) for n in nts], axis=1)


def _rows16(a, b):
    return jnp.concatenate([a, b], axis=0).astype(bf16)


def _slot(G, t):
    j = 4 * (t >> 3) + ((((t >> 1) & 3) + G + 2 * (t & 1) + (t >> 3)) & 3)
    return 2 * G + (t & 1), 8 * j


def _vr(n):
    return slice(8 * n, 8 * n + 8)


def _kernel(*refs, t0, wt):
    pl.run_scoped(functools.partial(_body, refs, t0, wt),
                  pltpu.SemaphoreType.DMA((4 + len(W4_CHUNKS) + 2 * NP,)))


def _body(refs, t0, wt, sems):
    (x_hbm, k_hbm, v_hbm, wq_hbm, wo_hbm, w3_hbm, w4_hbm, o_ref,
     kbuf, vbuf, wq, wo, w3, w4, xbuf, lref, qa, qb, scl, sbuf, abuf, zs) = refs[:22]
    pT = refs[22:]
    ku = kbuf.bitcast(u32)
    vu = vbuf.bitcast(u32)
    wqu = wq.bitcast(u32)
    wou = wo.bitcast(u32)

    x_cp = pltpu.make_async_copy(x_hbm, xbuf, sems.at[0])
    wq_cp = pltpu.make_async_copy(wq_hbm, wq, sems.at[1])
    wo_cp = pltpu.make_async_copy(wo_hbm, wo, sems.at[2])
    w3_cp = pltpu.make_async_copy(w3_hbm, w3, sems.at[3])
    w4_rows, r0 = [], 0
    for n in W4_CHUNKS:
        w4_rows.append((r0, r0 + n))
        r0 += n
    w4_cp = [pltpu.make_async_copy(w4_hbm.at[a:b], w4.at[a:b], sems.at[4 + c])
             for c, (a, b) in enumerate(w4_rows)]
    S0 = 4 + len(W4_CHUNKS)

    def k_cp(i):
        return pltpu.make_async_copy(
            k_hbm.at[pl.ds(i * GP, GP), pl.ds(t0 * 8, wt * 8), :],
            kbuf.at[pl.ds(i * GP, GP)], sems.at[S0 + i])

    def v_cp(i):
        return pltpu.make_async_copy(
            v_hbm.at[pl.ds(i * GP, GP), pl.ds(t0 * 8, wt * 8), :],
            vbuf.at[pl.ds(i * GP, GP)], sems.at[S0 + NP + i])

    for c in (wq_cp, x_cp, wo_cp):
        c.start()
    for i in range(NP):
        k_cp(i).start()
        v_cp(i).start()
    for c in [w3_cp] + w4_cp:
        c.start()

    zs[0] = 0

    lane = lax.broadcasted_iota(jnp.int32, (8, 128), 1)
    sub = lax.broadcasted_iota(jnp.int32, (8, 128), 0)
    lane_lo = lane < 64
    sub_lo = sub < 4

    def tile(ref, g0, G, t):
        g, r = _slot(G, t)
        return ref[g0 + g, r:r + 8, :]

    def retile(ref, i):
        def body(c, carry):
            g0 = i * GP + 8 * c
            for G in range(4):
                for J in range(4):
                    xs = [[ref[g0 + 2 * G + e, _vr(4 * J + jj), :] for jj in range(4)]
                          for e in range(2)]
                    for jj in range(4):
                        x0, x1 = xs[0][jj], xs[1][jj]
                        ys = (jnp.where(sub_lo, x0, pltpu.roll(x1, 4, 0)),
                              jnp.where(sub_lo, pltpu.roll(x0, 4, 0), x1))
                        for e in range(2):
                            g, r = _slot(G, 8 * J + 2 * jj + e)
                            ref[g0 + g, r:r + 8, :] = ys[e]
            return carry
        lax.fori_loop(0, GP // 8, body, 0)

    def retile_w(wu, unroll):
        nt = wu.shape[1]

        def body(c, carry):
            for u in range(unroll):
                G = c * unroll + u
                xs = [wu[G, n] for n in range(nt)]
                for n in range(nt):
                    lo, hi = xs[n // 2], xs[(nt + n) // 2]
                    if n % 2:
                        lo = pltpu.roll(lo, 4, 0)
                    if (nt + n) % 2 == 0:
                        hi = pltpu.roll(hi, 4, 0)
                    wu[G, n] = jnp.where(sub_lo, lo, hi)
            return carry
        lax.fori_loop(0, wu.shape[0] // unroll, body, 0)

    def lhs_at(ref, n):
        return pltpu.bitcast(ref[_vr(n), :], bf16)

    cur = [None]

    def tick(ref, n, val):
        if val.dtype != ref.dtype:
            val = pltpu.bitcast(val, ref.dtype)
        ref[pl.ds(pl.multiple_of(cur[0] + 8 * n, 8), 8), :] = val

    def q_dots(i, st, qref, lhs=None, mean=None):
        def step(k):
            def run():
                w = _wcols(wqu, _vr(k), [3 * i + n for n in range(3)])
                if lhs is None:
                    r = jnp.dot(lhs_at(lref, L_Y + k), w, preferred_element_type=f32)[0:8]
                else:
                    r = jnp.dot(lhs[:, 128 * k:128 * k + 128], w, preferred_element_type=f32)
                st["q"] = r if k == 0 else st["q"] + r
                if k == 4:
                    q = st["q"] if lhs is None else st["q"][0:8] - mean * st["q"][8:16]
                    qq = pltpu.bitcast(q.astype(bf16).astype(f32), u32)
                    q0, q1, q2 = qq[:, 0:128], qq[:, 128:256], qq[:, 256:384]
                    for n, v in enumerate((q0 >> 16, q0, q2 >> 16, q2, q1, pltpu.roll(q1, 64, 1))):
                        qref[_vr(n), :] = v
                return r[0:8, 256:384]
            return 3, lref, L_DUMMY, run
        return [step(k) for k in range(5)]

    def o_dots(i, st):
        def step(b):
            def run():
                w = _wcols(wou, pl.ds(i * (GP // 2) + 8 * b, 8), range(5))
                r = jnp.dot(lhs_at(lref, L_O + b), w, preferred_element_type=f32)[0:8]
                st["acc"] = st["acc"] + r
                return r[:, 512:640]
            return 5, lref, L_DUMMY, run
        return [step(b) for b in range(3)]

    def k_dots(i, hh, st, qref, order=tuple(range(12))):
        g0 = i * GP
        gf, gh = ((0, 8), (16, 12))[hh]

        def step(r):
            def run():
                if r < 8:
                    cols = [[tile(ku, g0, gf + G, 8 * T + r) for G in range(8)] for T in range(4)]
                    base, row = qref[_vr(2 * hh + r % 2), :], r // 2
                else:
                    cols = [[tile(ku, g0, gh + G % 4, 8 * T + 2 * (r - 8) + G // 4)
                             for G in range(8)] for T in range(4)]
                    if r == 8:
                        st["u"] = jnp.where(lane_lo, qref[_vr(4 + hh), :] >> 16,
                                            qref[_vr(5 - hh), :])
                    base, row = st["u"], r - 8
                lhs = jnp.where(sub == row, base, jnp.zeros((8, 128), u32))
                w = jnp.concatenate([jnp.concatenate(c, axis=0) for c in cols], axis=1)
                res = jnp.dot(pltpu.bitcast(lhs, bf16), pltpu.bitcast(w, bf16),
                              preferred_element_type=f32)[0:8]
                st["s", hh] = res if r == order[0] else st["s", hh] + res
                return res[:, 384:512]
            return 4, qref, 6, run
        return [step(r) for r in order]

    def col(s, T):
        return s[:, 128 * T:128 * T + 128]

    def row_max(s):
        m = jnp.maximum(jnp.maximum(col(s, 0), col(s, 1)), jnp.maximum(col(s, 2), col(s, 3)))
        return jnp.max(jnp.max(m, axis=1, keepdims=True), axis=0, keepdims=True)

    def prob(s, m):
        return jnp.exp2((s - m) * scl[_vr(0), :])

    def put_p(hh, T, p, ks=range(8)):
        for k in ks:
            pT[4 * hh + T][pl.ds(k, 8, stride=8), :] = p

    def part_sum(p):
        return (p[0] + p[1]) + (p[2] + p[3])

    def inv_sum(l):
        l = jnp.sum(jnp.sum(l, axis=1, keepdims=True), axis=0, keepdims=True)
        return jnp.broadcast_to(1.0 / l, (8, 128))

    def softmax(s, hh):
        m = row_max(s)
        p = [prob(col(s, T), m) for T in range(4)]
        for T in range(4):
            put_p(hh, T, p[T])
        return p, part_sum(p)

    def stash_b(i, s):
        for T in range(4):
            sbuf[i, _vr(T), :] = col(s, T)
        m = jnp.broadcast_to(row_max(s), (8, 128))
        sbuf[i, _vr(S_MAXB), :] = m
        return m

    def reduce_o(aref, a0, inva, invb):
        out = []
        for b, inv in enumerate((inva, jnp.where(lane_lo, inva, invb), invb)):
            z = jnp.sum(pltpu.bitcast(aref[a0 + b], f32).T.reshape(16, 8, 128), axis=0)
            o = jnp.sum(z, axis=0, keepdims=True) * inv
            out.append(pltpu.bitcast(_rows16(o, o), u32))
        return out

    def put_o(o):
        for b in range(3):
            lref[_vr(L_O + b), :] = o[b]

    def run_block(i, aref, a0, dots, issue, tv0, hooks):
        g0 = i * GP
        clock = []

        def emit(upto):
            while len(clock) < upto:
                n = len(clock)
                for h in hooks.get(("dot", n), ()):
                    h()
                clock.append(dots[n][3]())

        seg = 0
        prev = None
        for hh in range(2):
            for gp in range(6):
                a4 = [None] * 4
                for T in range(4):
                    pref = pT[4 * hh + T]
                    start = tv0 + SEG * seg
                    emit(sum(1 for c in issue if c < start + SEG + 12))
                    done = sum(1 for c in issue if c + LAT <= start)
                    if done:
                        tick(pref, 8, clock[done - 1])
                    elif gp:
                        tick(pref, 8, prev)
                    for h in hooks.get(("seg", seg), ()):
                        h(clock[done - 1] if done else prev)
                    for rho in range(8):
                        pv = pref[_vr(rho), :]
                        for e in range(2):
                            w = tile(vu, g0, 12 * hh + 2 * gp + e, 8 * T + rho)
                            a = pltpu.bitcast(w << 16, f32) * pv
                            b = pltpu.bitcast(w & jnp.uint32(HI), f32) * pv
                            a4[2 * e] = a if a4[2 * e] is None else a4[2 * e] + a
                            a4[2 * e + 1] = b if a4[2 * e + 1] is None else a4[2 * e + 1] + b
                    if T == 0:
                        prev = a4[0]
                    if not done and len(clock) < len(dots):
                        _, ref, slot, _ = dots[len(clock)]
                        for k in range(4):
                            tick(ref, slot + k, a4[k])
                    seg += 1
                for e in range(2):
                    G = 12 * hh + 2 * gp + e
                    for k in range(2):
                        aref[a0 + G // 8, pl.ds(16 * (G % 8) + k, 8, stride=2), :] = (
                            pltpu.bitcast(a4[2 * e + k], u32))
        emit(len(dots))

    def times(dots, t=0):
        out = []
        for d in dots:
            t += 8 * d[0]
            out.append(t)
        return out

    def run_all(dots):
        for d in dots:
            d[3]()

    def set_input(c, scale):
        cp = pltpu.bitcast(_rows16(c, c), u32)
        for k in range(5):
            lref[_vr(L_Y + k), :] = cp[:, 128 * k:128 * k + 128]
        scl[_vr(0), :] = jnp.broadcast_to(scale, (8, 128))

    x_cp.wait()
    x = jnp.broadcast_to(xbuf[...].astype(f32), (8, D))
    set_input(_ln(x), jnp.full((8, 1), CEXP, f32))
    wq_cp.wait()
    retile_w(wqu, 1)
    wo_cp.wait()
    retile_w(wou, 8)

    def body1(i, acc):
        st = {"acc": acc}
        k_cp(i).wait()
        retile(ku, i)
        run_all(q_dots(i, st, qa))
        inv = []
        for hh in range(2):
            run_all(k_dots(i, hh, st, qa))
            inv.append(inv_sum(softmax(st["s", hh], hh)[1]))
        v_cp(i).wait()
        retile(vu, i)
        cur[0] = zs[0]
        run_block(i, abuf, 0, [], [], 0, {})
        put_o(reduce_o(abuf, 0, inv[0], inv[1]))
        run_all(o_dots(i, st))
        return st["acc"]

    x = lax.fori_loop(0, NP, body1, x)

    y = _ln(x)
    zz = _ln(y).astype(bf16)
    w3_cp.wait()
    h = jnp.dot(zz, w3[...], preferred_element_type=f32)
    h = jax.nn.gelu(h, approximate=True).astype(bf16)
    x = x + y
    for cp, (a, b) in zip(w4_cp, w4_rows):
        cp.wait()
        x = x + jnp.dot(h[:, a:b], w4[a:b, :], preferred_element_type=f32)

    ones = jnp.ones((8, D), f32)
    xl = _rows16(x, ones)
    xb = xl[0:8].astype(f32)
    mean = _mean(xb)
    c = xb - mean
    set_input(c, lax.rsqrt(_mean(c * c) + EPS) * CEXP)
    lref[8 * L_O:8 * L_O + 24, :] = jnp.zeros((24, 128), u32)

    def tail_hooks(i, st, hooks, seg0):
        def first(_):
            m = row_max(st["s", 0])
            st["pa"] = [prob(col(st["s", 0], T), m) for T in range(4)]
            sbuf[i, _vr(S_INVA), :] = inv_sum(part_sum(st["pa"]))

        def put(T, half):
            def run(clk):
                tick(pT[T], 8, clk)
                put_p(0, T, st["pa"][T], range(4 * half, 4 * half + 4))
            return run
        hooks.setdefault(("seg", seg0), []).append(first)
        for n in range(8):
            hooks.setdefault(("seg", seg0 + n), []).append(put(n // 2, n % 2))

    def head_b_hooks(i, seg0):
        pb = []

        def put_b(T):
            def run(clk):
                tick(scl, 1, clk)
                pb.append(prob(sbuf[i, _vr(T), :], sbuf[i, _vr(S_MAXB), :]))
                put_p(1, T, pb[T])
                if T == 3:
                    sbuf[i, _vr(S_LB), :] = part_sum(pb)
            return run
        return {("seg", seg0 + 3 * T): [put_b(T)] for T in range(4)}

    def reduce_pair(i):
        return reduce_o(ku, i * GP, sbuf[i, _vr(S_INVA), :], inv_sum(sbuf[i, _vr(S_LB), :]))

    st = {}
    zero = cur[0] = zs[0]
    late = tuple(range(8, 12)) + tuple(range(8))
    d0 = q_dots(0, st, qb, xl, mean) + q_dots(1, st, qa, xl, mean)
    d1 = k_dots(0, 0, st, qb) + k_dots(0, 1, st, qb, late) + k_dots(1, 0, st, qa, late) \
        + k_dots(1, 1, st, qa) + q_dots(2, st, qa)
    issue = times(d0 + d1)

    def sm_a0():
        m = row_max(st["s", 0])
        p = [prob(col(st["s", 0], T), m) for T in range(4)]
        tick(qb, 6, part_sum(p))
        for T in range(4):
            put_p(0, T, p[T])
        sbuf[0, _vr(S_INVA), :] = inv_sum(part_sum(p))

    def sm_b0():
        tick(qa, 6, stash_b(0, st["s", 1]))

    hooks = head_b_hooks(0, 15)
    hooks.update({("dot", 31): [sm_a0], ("dot", 43): [sm_b0]})
    tail_hooks(1, st, hooks, 36)
    run_block(0, ku, 0, d0 + d1, issue, 240 + 384 + LAT + 170, hooks)
    stash_b(1, st["s", 1])

    def body2(j, acc, last=False):
        cur[0] = zs[0]
        st = {"acc": acc}
        o = reduce_pair(j)
        dots = o_dots(jnp.maximum(j - 1, 0), st)
        hooks = head_b_hooks(j + 1, 9)
        if last:
            run_all(dots)
            dots = []
        else:
            dots = k_dots(j + 2, 0, st, qa) + k_dots(j + 2, 1, st, qa) \
                + q_dots(jnp.minimum(j + 3, NP - 1), st, qa) + dots
            tail_hooks(j + 2, st, hooks, 39)
            hooks["dot", 24] = [lambda: stash_b(j + 2, st["s", 1])]
        run_block(j + 1, ku, (j + 1) * GP, dots, times(dots), 0, hooks)
        put_o(o)
        return st["acc"]

    x = lax.fori_loop(0, NP - 2, body2, x)
    x = lax.fori_loop(NP - 2, NP - 1 + zero, functools.partial(body2, last=True), x)

    st = {"acc": x}
    o = reduce_pair(NP - 1)
    run_all(o_dots(NP - 2, st))
    put_o(o)
    run_all(o_dots(NP - 1, st))
    x = st["acc"]

    xl = _rows16(x, ones)
    xb = xl[0:8].astype(f32)
    mean = _mean(xb)
    c = xb - mean
    r1 = lax.rsqrt(_mean(c * c) + EPS)
    y = c * r1
    my = _mean(y)
    r2 = lax.rsqrt(_mean(y * y) - my * my + EPS)
    h = jnp.dot(xl, w3[...], preferred_element_type=f32)
    h = h[0:8] * (r1 * r2) - h[8:16] * ((mean * r1 + my) * r2)
    h = jax.nn.gelu(h, approximate=True).astype(bf16)
    x = x + y + jnp.dot(h, w4[...], preferred_element_type=f32)
    o_ref[...] = x[0:1].astype(o_ref.dtype)


def _cache_view(c):
    s = c.shape[2]
    c = jnp.transpose(c, (0, 1, 3, 2)).reshape(H * DH // 8, 8, s // 128, 128)
    return jnp.transpose(c, (0, 2, 1, 3)).reshape(H * DH // 8, s // 128 * 8, 128)


def _weight_view(w):
    k, n = w.shape
    w = jnp.transpose(w.reshape(k // 16, 2, 8, n // 128, 128), (0, 1, 3, 2, 4))
    return w.reshape(k // 16, n // 128, 16, 128)


@jax.jit
def pallas_interleave_layers__sliding_block_cached__mixer_s_mlp__decode_kernel(
    A_x: jax.Array,
    A_k_cache: jax.Array,
    A_v_cache: jax.Array,
    A_wq: jax.Array,
    A_wo: jax.Array,
    B_x: jax.Array,
    B_w1: jax.Array,
    B_w2: jax.Array,
    B_w3: jax.Array,
    B_w4: jax.Array,
):
    sk = A_k_cache.shape[2]
    win = min(4096, max(256, sk // 4))
    assert win == 4096 and sk % 128 == 0
    assert A_x.shape == (1, 1, D) and A_k_cache.shape == (1, H, sk, DH)
    wt = win // 128
    t0 = sk // 128 - wt
    ng = H * DH // 8
    hbm = pl.BlockSpec(memory_space=pl.ANY)
    out = pl.pallas_call(
        functools.partial(_kernel, t0=t0, wt=wt),
        out_shape=jax.ShapeDtypeStruct((1, D), A_x.dtype),
        in_specs=[hbm] * 7,
        out_specs=pl.BlockSpec(memory_space=pltpu.VMEM),
        scratch_shapes=[
            pltpu.VMEM((ng, wt * 8, 128), bf16),
            pltpu.VMEM((ng, wt * 8, 128), bf16),
            pltpu.VMEM((D // 16, H * DH // 128, 16, 128), bf16),
            pltpu.VMEM((H * DH // 16, D // 128, 16, 128), bf16),
            pltpu.VMEM((D, F), bf16),
            pltpu.VMEM((F, D), bf16),
            pltpu.VMEM((1, D), bf16),
            pltpu.VMEM((96, 128), u32),
            pltpu.VMEM((80, 128), u32),
            pltpu.VMEM((80, 128), u32),
            pltpu.VMEM((16, 128), f32),
            pltpu.VMEM((NP, 56, 128), f32),
            pltpu.VMEM((3, 128, 128), u32),
            pltpu.SMEM((1,), jnp.int32),
        ] + [pltpu.VMEM((72, 128), f32)] * 8,
        compiler_params=pltpu.CompilerParams(vmem_limit_bytes=124 * 1024 * 1024),
    )(A_x.reshape(1, D), _cache_view(A_k_cache), _cache_view(A_v_cache),
      _weight_view(A_wq), _weight_view(A_wo), B_w3, B_w4)
    return out.reshape(1, 1, D)
```

```python
import functools

import jax
import jax.numpy as jnp
from jax import lax
import jax.experimental.pallas as pl
import jax.experimental.pallas.tpu as pltpu

D = 640
H = 32
DH = 192
F = 1536
EPS = 1e-5
NP = H // 2
GP = 2 * DH // 8
HI = 0xFFFF0000
CEXP = DH ** -0.5 * 1.4426950408889634

f32 = jnp.float32
bf16 = jnp.bfloat16
u32 = jnp.uint32

L_Y = 0
L_DUMMY = 5
S_MAXB, S_LB, S_INVA = 4, 5, 6
SEG = 23.0
LAT = 145
B_SEG0 = 9
A_SEG0 = 39
W4_CHUNKS = (1024, 384, 128)


def _mean(x):
    return jnp.mean(x, axis=-1, keepdims=True)


def _ln(x):
    c = x - _mean(x)
    return c * lax.rsqrt(_mean(c * c) + EPS)


def _wtile(wu, rows, nt):
    blk = wu[rows, nt]
    return pltpu.bitcast(blk.reshape(blk.shape[0] * 8, 128), bf16)


def _wcols(wu, rows, nts):
    return jnp.concatenate([_wtile(wu, rows, n) for n in nts], axis=1)


def _rows16(a, b):
    return jnp.concatenate([a, b], axis=0).astype(bf16)


def _slot(G, t):
    j = 4 * (t >> 3) + ((((t >> 1) & 3) + G + 2 * (t & 1) + (t >> 3)) & 3)
    return 2 * G + (t & 1), 8 * j


def _xslot(G, t):
    return G // 2, 8 * (4 * (t >> 3) + ((((t >> 1) & 3) + G + (t >> 3)) & 3))


def _vr(n):
    return slice(8 * n, 8 * n + 8)


def _kernel(*refs, t0, wt):
    pl.run_scoped(functools.partial(_body, refs, t0, wt),
                  pltpu.SemaphoreType.DMA((4 + len(W4_CHUNKS) + 2 * NP,)))


def _body(refs, t0, wt, sems):
    (x_hbm, k_hbm, v_hbm, wq_hbm, wo_hbm, w3_hbm, w4_hbm, o_ref,
     kbuf, vbuf, vx, wq, wo, w3, w4, xbuf, lref, obuf, qa, qb, scl, zs) = refs[:22]
    pT = refs[22:]
    ku = kbuf.bitcast(u32)
    vu = vbuf.bitcast(u32)
    wqu = wq.bitcast(u32)
    wou = wo.bitcast(u32)

    x_cp = pltpu.make_async_copy(x_hbm, xbuf, sems.at[0])
    wq_cp = pltpu.make_async_copy(wq_hbm, wq, sems.at[1])
    wo_cp = pltpu.make_async_copy(wo_hbm, wo, sems.at[2])
    w3_cp = pltpu.make_async_copy(w3_hbm, w3, sems.at[3])
    w4_rows, r0 = [], 0
    for n in W4_CHUNKS:
        w4_rows.append((r0, r0 + n))
        r0 += n
    w4_cp = [pltpu.make_async_copy(w4_hbm.at[a:b], w4.at[a:b], sems.at[4 + c])
             for c, (a, b) in enumerate(w4_rows)]
    S0 = 4 + len(W4_CHUNKS)

    def k_cp(i):
        return pltpu.make_async_copy(
            k_hbm.at[pl.ds(i * GP, GP), pl.ds(t0 * 8, wt * 8), :],
            kbuf.at[pl.ds(i * GP, GP)], sems.at[S0 + i])

    def v_cp(i):
        return pltpu.make_async_copy(
            v_hbm.at[pl.ds(i * GP, GP), pl.ds(t0 * 8, wt * 8), :],
            vbuf.at[pl.ds(i * GP, GP)], sems.at[S0 + NP + i])

    for c in (wq_cp, x_cp, wo_cp):
        c.start()
    for i in range(NP):
        k_cp(i).start()
        v_cp(i).start()
    for c in [w3_cp] + w4_cp:
        c.start()

    zs[0] = 0

    lane = lax.broadcasted_iota(jnp.int32, (8, 128), 1)
    sub = lax.broadcasted_iota(jnp.int32, (8, 128), 0)
    lane_lo = lane < 64
    sub_lo = sub < 4

    def tile(ref, g0, G, t):
        g, r = _slot(G, t)
        return ref[g0 + g, r:r + 8, :]

    def retile(ref, i, expand):
        def body(c, carry):
            g0 = i * GP + 8 * c
            for G in range(4):
                for J in range(4):
                    xs = [[ref[g0 + 2 * G + e, _vr(4 * J + jj), :] for jj in range(4)]
                          for e in range(2)]
                    for jj in range(4):
                        x0, x1 = xs[0][jj], xs[1][jj]
                        ys = (jnp.where(sub_lo, x0, pltpu.roll(x1, 4, 0)),
                              jnp.where(sub_lo, pltpu.roll(x0, 4, 0), x1))
                        for e in range(2):
                            t = 8 * J + 2 * jj + e
                            g, r = _slot(G, t)
                            if expand and G % 2 and e:
                                ref[g0 + g, r:r + 8, :] = ys[e] << 16
                                g, r = _xslot(G, t)
                                vx[i * (GP // 4) + 2 * c + g, r:r + 8, :] = ys[e] & jnp.uint32(HI)
                            else:
                                ref[g0 + g, r:r + 8, :] = ys[e]
            return carry
        lax.fori_loop(0, GP // 8, body, 0)

    def retile_w(wu, unroll):
        nt = wu.shape[1]

        def body(c, carry):
            for u in range(unroll):
                G = c * unroll + u
                xs = [wu[G, n] for n in range(nt)]
                for n in range(nt):
                    lo, hi = xs[n // 2], xs[(nt + n) // 2]
                    if n % 2:
                        lo = pltpu.roll(lo, 4, 0)
                    if (nt + n) % 2 == 0:
                        hi = pltpu.roll(hi, 4, 0)
                    wu[G, n] = jnp.where(sub_lo, lo, hi)
            return carry
        lax.fori_loop(0, wu.shape[0] // unroll, body, 0)

    def lhs_at(ref, n):
        return pltpu.bitcast(ref[_vr(n), :], bf16)

    cur = [None]

    def tick(ref, n, val):
        if val.dtype != ref.dtype:
            val = pltpu.bitcast(val, ref.dtype)
        ref[pl.ds(pl.multiple_of(cur[0] + 8 * n, 8), 8), :] = val

    def q_dots(i, st, qref, lhs=None, mean=None):
        def step(k):
            def run():
                w = _wcols(wqu, _vr(k), [3 * i + n for n in range(3)])
                if lhs is None:
                    r = jnp.dot(lhs_at(lref, L_Y + k), w, preferred_element_type=f32)[0:8]
                else:
                    r = jnp.dot(lhs[:, 128 * k:128 * k + 128], w, preferred_element_type=f32)
                st["q"] = r if k == 0 else st["q"] + r
                if k == 4:
                    q = st["q"] if lhs is None else st["q"][0:8] - mean * st["q"][8:16]
                    qq = pltpu.bitcast(q.astype(bf16).astype(f32), u32)
                    q0, q1, q2 = qq[:, 0:128], qq[:, 128:256], qq[:, 256:384]
                    for n, v in enumerate((q0 >> 16, q0, q2 >> 16, q2, q1, pltpu.roll(q1, 64, 1))):
                        qref[_vr(n), :] = v
                return r[0:8, 256:384]
            return 3, lref, L_DUMMY, run
        return [step(k) for k in range(5)]

    def o_dots(slot, i, st, chunks=range(3)):
        def step(b):
            def run():
                w = _wcols(wou, pl.ds(i * (GP // 2) + 8 * b, 8), range(5))
                lhs = obuf[pl.ds(pl.multiple_of(24 * slot + 8 * b, 8), 8), :]
                r = jnp.dot(pltpu.bitcast(lhs, bf16), w, preferred_element_type=f32)[0:8]
                st["acc"] = st["acc"] + r
                return r[:, 512:640]
            return 5, obuf, 3 * (NP + 1), run
        return [step(b) for b in chunks]

    def k_dots(i, hh, st, qref, order=tuple(range(12))):
        g0 = i * GP
        gf, gh = ((0, 8), (16, 12))[hh]

        def step(r):
            def run():
                if r < 8:
                    cols = [[tile(ku, g0, gf + G, 8 * T + r) for G in range(8)] for T in range(4)]
                    base, row = qref[_vr(2 * hh + r % 2), :], r // 2
                else:
                    cols = [[tile(ku, g0, gh + G % 4, 8 * T + 2 * (r - 8) + G // 4)
                             for G in range(8)] for T in range(4)]
                    if r == 8:
                        st["u"] = jnp.where(lane_lo, qref[_vr(4 + hh), :] >> 16,
                                            qref[_vr(5 - hh), :])
                    base, row = st["u"], r - 8
                lhs = jnp.where(sub == row, base, jnp.zeros((8, 128), u32))
                w = jnp.concatenate([jnp.concatenate(c, axis=0) for c in cols], axis=1)
                res = jnp.dot(pltpu.bitcast(lhs, bf16), pltpu.bitcast(w, bf16),
                              preferred_element_type=f32)[0:8]
                st["s", hh] = res if r == order[0] else st["s", hh] + res
                return res[:, 384:512]
            return 4, qref, 6, run
        return [step(r) for r in order]

    def col(s, T):
        return s[:, 128 * T:128 * T + 128]

    def row_max(s):
        m = jnp.maximum(jnp.maximum(col(s, 0), col(s, 1)), jnp.maximum(col(s, 2), col(s, 3)))
        return jnp.max(jnp.max(m, axis=1, keepdims=True), axis=0, keepdims=True)

    def prob(s, m):
        return jnp.exp2((s - m) * scl[_vr(0), :])

    def put_p(hh, T, p, ks=range(8)):
        for k in ks:
            pT[4 * hh + T][pl.ds(k, 8, stride=8), :] = p

    def part_sum(p):
        return (p[0] + p[1]) + (p[2] + p[3])

    def inv_sum(l):
        l = jnp.sum(jnp.sum(l, axis=1, keepdims=True), axis=0, keepdims=True)
        return jnp.broadcast_to(1.0 / l, (8, 128))

    def softmax(s, hh):
        m = row_max(s)
        p = [prob(col(s, T), m) for T in range(4)]
        for T in range(4):
            put_p(hh, T, p[T])
        return p, part_sum(p)

    def get_state(i, n):
        return pltpu.bitcast(ku[i * GP + 3, _vr(n), :], f32)

    def set_state(i, n, v):
        ku[i * GP + 3, _vr(n), :] = pltpu.bitcast(v, u32)

    def stash_b(i, s):
        for T in range(4):
            set_state(i, T, col(s, T))
        m = jnp.broadcast_to(row_max(s), (8, 128))
        set_state(i, S_MAXB, m)
        return m

    def reduce_o(blocks, inva, invb):
        out = []
        for b, inv in enumerate((inva, jnp.where(lane_lo, inva, invb), invb)):
            z = jnp.sum(pltpu.bitcast(blocks[b], f32).T.reshape(16, 8, 128), axis=0)
            o = jnp.sum(z, axis=0, keepdims=True) * inv
            out.append(pltpu.bitcast(_rows16(o, o), u32))
        return out

    def put_o(slot, o):
        for b in range(3):
            obuf[pl.ds(pl.multiple_of(24 * slot + 8 * b, 8), 8), :] = o[b]

    def mac(acc, n, c, G, t, pv):
        w = tile(vu, 8 * c, G, t)
        if G % 2 and t % 2:
            g, r = _xslot(G, t)
            halves = (w, vx[2 * c + g, r:r + 8, :])
        else:
            halves = (w << 16, w & jnp.uint32(HI))
        for k in range(2):
            a = pltpu.bitcast(halves[k], f32) * pv
            acc[n + k] = a if acc[n + k] is None else acc[n + k] + a

    def run_block(i, put_a, dots, issue, tv0, hooks):
        clock = []

        def emit(upto):
            while len(clock) < upto:
                n = len(clock)
                for h in hooks.get(("dot", n), ()):
                    h()
                clock.append(dots[n][3]())

        seg = 0
        prev = None
        for hh in range(2):
            for gp in range(6):
                a4 = [None] * 4
                for T in range(4):
                    pref = pT[4 * hh + T]
                    start = tv0 + SEG * seg
                    emit(max(sum(1 for c in issue if c < start + SEG + 12),
                             hooks.get(("need", seg), 0)))
                    done = sum(1 for c in issue if c + LAT <= start)
                    if done:
                        tick(pref, 8, clock[done - 1])
                    elif gp:
                        tick(pref, 8, prev)
                    for h in hooks.get(("seg", seg), ()):
                        h(clock[done - 1] if done else prev)
                    for rho in range(8):
                        pv = pref[_vr(rho), :]
                        for e in range(2):
                            mac(a4, 2 * e, i * 6, 12 * hh + 2 * gp + e, 8 * T + rho, pv)
                    if T == 0:
                        prev = a4[0]
                    if not done and len(clock) < len(dots):
                        _, ref, slot, _ = dots[len(clock)]
                        for k in range(4):
                            tick(ref, slot + k, a4[k])
                    seg += 1
                for e in range(2):
                    G = 12 * hh + 2 * gp + e
                    for k in range(2):
                        put_a(G // 8, 16 * (G % 8) + k, pltpu.bitcast(a4[2 * e + k], u32))
        emit(len(dots))

    def times(dots, t=0, rate=8):
        out = []
        for d in dots:
            t += rate * d[0]
            out.append(t)
        return out

    def run_all(dots):
        for d in dots:
            d[3]()

    def set_input(c, scale):
        cp = pltpu.bitcast(_rows16(c, c), u32)
        for k in range(5):
            lref[_vr(L_Y + k), :] = cp[:, 128 * k:128 * k + 128]
        scl[_vr(0), :] = jnp.broadcast_to(scale, (8, 128))

    x_cp.wait()
    x = jnp.broadcast_to(xbuf[...].astype(f32), (8, D))
    set_input(_ln(x), jnp.full((8, 1), CEXP, f32))
    wq_cp.wait()
    retile_w(wqu, 1)
    wo_cp.wait()
    retile_w(wou, 8)

    def body1(i, acc):
        st = {"acc": acc}
        k_cp(i).wait()
        retile(ku, i, False)
        run_all(q_dots(i, st, qa))
        inv = []
        for hh in range(2):
            run_all(k_dots(i, hh, st, qa))
            inv.append(inv_sum(softmax(st["s", hh], hh)[1]))
        v_cp(i).wait()
        retile(vu, i, True)
        for hh in range(2):
            def pv_step(c, carry, hh=hh):
                acc8 = [None] * 8
                for t in range(32):
                    pv = pT[4 * hh + t // 8][_vr(t % 8), :]
                    for G in range(4):
                        mac(acc8, 2 * G, i * 6 + c, G, t, pv)
                for n in range(8):
                    obuf[pl.ds(64 * c + 16 * (n // 2) + n % 2, 8, stride=2), :] = (
                        pltpu.bitcast(acc8[n], u32))
                return carry
            lax.fori_loop(3 * hh, 3 * hh + 3, pv_step, 0)
        put_o(NP, reduce_o([obuf[128 * b:128 * b + 128, :] for b in range(3)], inv[0], inv[1]))
        run_all(o_dots(NP, i, st))
        return st["acc"]

    x = lax.fori_loop(0, NP, body1, x)

    y = _ln(x)
    zz = _ln(y).astype(bf16)
    w3_cp.wait()
    h = jnp.dot(zz, w3[...], preferred_element_type=f32)
    h = jax.nn.gelu(h, approximate=True).astype(bf16)
    x = x + y
    for cp, (a, b) in zip(w4_cp, w4_rows):
        cp.wait()
        x = x + jnp.dot(h[:, a:b], w4[a:b, :], preferred_element_type=f32)

    ones = jnp.ones((8, D), f32)
    xl = _rows16(x, ones)
    xb = xl[0:8].astype(f32)
    mean = _mean(xb)
    c = xb - mean
    set_input(c, lax.rsqrt(_mean(c * c) + EPS) * CEXP)
    obuf[0:24, :] = jnp.zeros((24, 128), u32)

    def tail_hooks(i, st, hooks, seg0):
        def first(_):
            m = row_max(st["s", 0])
            st["pa"] = [prob(col(st["s", 0], T), m) for T in range(4)]
            set_state(i, S_INVA, inv_sum(part_sum(st["pa"])))

        def put(T, half):
            def run(clk):
                tick(pT[T], 8, clk)
                put_p(0, T, st["pa"][T], range(4 * half, 4 * half + 4))
            return run
        hooks.setdefault(("seg", seg0), []).append(first)
        for n in range(8):
            hooks.setdefault(("seg", seg0 + n), []).append(put(n // 2, n % 2))

    def head_b_hooks(i, seg0):
        pb = []

        def put_b(T):
            def run(clk):
                tick(scl, 1, clk)
                pb.append(prob(get_state(i, T), get_state(i, S_MAXB)))
                put_p(1, T, pb[T])
                if T == 3:
                    set_state(i, S_LB, part_sum(pb))
            return run
        return {("seg", seg0 + 3 * T): [put_b(T)] for T in range(4)}

    def reduce_pair(i):
        return reduce_o([ku[i * GP + b] for b in range(3)],
                        get_state(i, S_INVA), inv_sum(get_state(i, S_LB)))

    def put_k(i):
        def put_a(b, r, v):
            ku[i * GP + b, pl.ds(r, 8, stride=2), :] = v
        return put_a

    st = {}
    zero = cur[0] = zs[0]
    late = tuple(range(8, 12)) + tuple(range(8))
    d0 = q_dots(0, st, qb, xl, mean) + q_dots(1, st, qa, xl, mean)
    d1 = k_dots(0, 0, st, qb) + k_dots(0, 1, st, qb, late) + k_dots(1, 0, st, qa, late) \
        + k_dots(1, 1, st, qa) + q_dots(2, st, qa)
    issue = times(d0 + d1)

    def sm_a0():
        m = row_max(st["s", 0])
        p = [prob(col(st["s", 0], T), m) for T in range(4)]
        tick(qb, 6, part_sum(p))
        for T in range(4):
            put_p(0, T, p[T])
        set_state(0, S_INVA, inv_sum(part_sum(p)))

    def sm_b0():
        tick(qa, 6, stash_b(0, st["s", 1]))

    hooks = head_b_hooks(0, 15)
    hooks.update({("dot", 31): [sm_a0], ("dot", 43): [sm_b0],
                  ("need", 0): 32, ("need", 15): 44, ("need", 36): 46})
    tail_hooks(1, st, hooks, 36)
    run_block(0, put_k(0), d0 + d1, issue, 240 + 384 + LAT + 170, hooks)
    stash_b(1, st["s", 1])

    def body2(j, acc, last=False):
        cur[0] = zs[0]
        st = {"acc": acc}
        o = reduce_pair(j)
        hooks = head_b_hooks(j + 1, B_SEG0)
        if last:
            dots = o_dots(NP - 2, NP - 3, st)
            for n in range(NP - 3):
                dots += o_dots(n + 1, n, st, [2])
            issue = times(dots, rate=11.5)
        else:
            dots = k_dots(j + 2, 0, st, qa) + k_dots(j + 2, 1, st, qa) \
                + q_dots(jnp.minimum(j + 3, NP - 1), st, qa) \
                + o_dots(j, jnp.maximum(j - 1, 0), st, [0, 1])
            issue = times(dots)
            tail_hooks(j + 2, st, hooks, A_SEG0)
            hooks["need", A_SEG0] = 12
            hooks["dot", 24] = [lambda: stash_b(j + 2, st["s", 1])]
        run_block(j + 1, put_k(j + 1), dots, issue, 0, hooks)
        put_o(j + 1, o)
        return st["acc"]

    x = lax.fori_loop(0, NP - 2, body2, x)
    x = lax.fori_loop(NP - 2, NP - 1 + zero, functools.partial(body2, last=True), x)

    st = {"acc": x}
    o = reduce_pair(NP - 1)
    run_all(o_dots(NP - 1, NP - 2, st))
    put_o(NP, o)
    run_all(o_dots(NP, NP - 1, st))
    x = st["acc"]

    xl = _rows16(x, ones)
    xb = xl[0:8].astype(f32)
    mean = _mean(xb)
    c = xb - mean
    r1 = lax.rsqrt(_mean(c * c) + EPS)
    y = c * r1
    my = _mean(y)
    r2 = lax.rsqrt(_mean(y * y) - my * my + EPS)
    h = jnp.dot(xl, w3[...], preferred_element_type=f32)
    h = h[0:8] * (r1 * r2) - h[8:16] * ((mean * r1 + my) * r2)
    h = jax.nn.gelu(h, approximate=True).astype(bf16)
    x = x + y + jnp.dot(h, w4[...], preferred_element_type=f32)
    o_ref[...] = x[0:1].astype(o_ref.dtype)


def _cache_view(c):
    s = c.shape[2]
    c = jnp.transpose(c, (0, 1, 3, 2)).reshape(H * DH // 8, 8, s // 128, 128)
    return jnp.transpose(c, (0, 2, 1, 3)).reshape(H * DH // 8, s // 128 * 8, 128)


def _weight_view(w):
    k, n = w.shape
    w = jnp.transpose(w.reshape(k // 16, 2, 8, n // 128, 128), (0, 1, 3, 2, 4))
    return w.reshape(k // 16, n // 128, 16, 128)


@jax.jit
def pallas_interleave_layers__sliding_block_cached__mixer_s_mlp__decode_kernel(
    A_x: jax.Array,
    A_k_cache: jax.Array,
    A_v_cache: jax.Array,
    A_wq: jax.Array,
    A_wo: jax.Array,
    B_x: jax.Array,
    B_w1: jax.Array,
    B_w2: jax.Array,
    B_w3: jax.Array,
    B_w4: jax.Array,
):
    sk = A_k_cache.shape[2]
    win = min(4096, max(256, sk // 4))
    assert win == 4096 and sk % 128 == 0
    assert A_x.shape == (1, 1, D) and A_k_cache.shape == (1, H, sk, DH)
    wt = win // 128
    t0 = sk // 128 - wt
    ng = H * DH // 8
    hbm = pl.BlockSpec(memory_space=pl.ANY)
    out = pl.pallas_call(
        functools.partial(_kernel, t0=t0, wt=wt),
        out_shape=jax.ShapeDtypeStruct((1, D), A_x.dtype),
        in_specs=[hbm] * 7,
        out_specs=pl.BlockSpec(memory_space=pltpu.VMEM),
        scratch_shapes=[
            pltpu.VMEM((ng, wt * 8, 128), bf16),
            pltpu.VMEM((ng, wt * 8, 128), bf16),
            pltpu.VMEM((ng // 4, 128, 128), u32),
            pltpu.VMEM((D // 16, H * DH // 128, 16, 128), bf16),
            pltpu.VMEM((H * DH // 16, D // 128, 16, 128), bf16),
            pltpu.VMEM((D, F), bf16),
            pltpu.VMEM((F, D), bf16),
            pltpu.VMEM((1, D), bf16),
            pltpu.VMEM((72, 128), u32),
            pltpu.VMEM((24 * (NP + 1) + 32, 128), u32),
            pltpu.VMEM((80, 128), u32),
            pltpu.VMEM((80, 128), u32),
            pltpu.VMEM((16, 128), f32),
            pltpu.SMEM((1,), jnp.int32),
        ] + [pltpu.VMEM((72, 128), f32)] * 8,
        compiler_params=pltpu.CompilerParams(vmem_limit_bytes=128 * 1024 * 1024),
    )(A_x.reshape(1, D), _cache_view(A_k_cache), _cache_view(A_v_cache),
      _weight_view(A_wq), _weight_view(A_wo), B_w3, B_w4)
    return out.reshape(1, 1, D)
```

```python
import functools

import jax
import jax.numpy as jnp
from jax import lax
import jax.experimental.pallas as pl
import jax.experimental.pallas.tpu as pltpu

D = 640
H = 32
DH = 192
F = 1536
EPS = 1e-5
NP = H // 2
GP = 2 * DH // 8
HI = 0xFFFF0000
CEXP = DH ** -0.5 * 1.4426950408889634

f32 = jnp.float32
bf16 = jnp.bfloat16
u32 = jnp.uint32

L_Y = 0
L_DUMMY = 5
S_MAXB, S_LB, S_INVA = 4, 5, 6
SEG = 24.5
SEG0 = 22.5
SEGL = 23.0
LAT = 145
B_SEG0 = 9
LAG = 20
MIX = (0, 1, 8, 2, 3, 9, 4, 5, 10, 6, 7, 11)
MINLAG = 20
LAT2 = 170
TIEG = 2
A_SEG0 = 39
W4_CHUNKS = (1024, 384, 128)


def _mean(x):
    return jnp.mean(x, axis=-1, keepdims=True)


def _ln(x):
    c = x - _mean(x)
    return c * lax.rsqrt(_mean(c * c) + EPS)


def _wtile(wu, rows, nt):
    blk = wu[rows, nt]
    return pltpu.bitcast(blk.reshape(blk.shape[0] * 8, 128), bf16)


def _wcols(wu, rows, nts):
    return jnp.concatenate([_wtile(wu, rows, n) for n in nts], axis=1)


def _rows16(a, b):
    return jnp.concatenate([a, b], axis=0).astype(bf16)


def _slot(G, t):
    j = 4 * (t >> 3) + ((((t >> 1) & 3) + G + 2 * (t & 1) + (t >> 3)) & 3)
    return 2 * G + (t & 1), 8 * j


def _xslot(G, t):
    return G // 2, 8 * (4 * (t >> 3) + ((((t >> 1) & 3) + G + (t >> 3)) & 3))


def _vr(n):
    return slice(8 * n, 8 * n + 8)


def _kernel(*refs, t0, wt):
    pl.run_scoped(functools.partial(_body, refs, t0, wt),
                  pltpu.SemaphoreType.DMA((4 + len(W4_CHUNKS) + 2 * NP,)))


def _body(refs, t0, wt, sems):
    (x_hbm, k_hbm, v_hbm, wq_hbm, wo_hbm, w3_hbm, w4_hbm, o_ref,
     kbuf, vbuf, vx, wq, wo, w3, w4, xbuf, lref, obuf, qa, qb, scl, zs) = refs[:22]
    pT = refs[22:]
    ku = kbuf.bitcast(u32)
    vu = vbuf.bitcast(u32)
    wqu = wq.bitcast(u32)
    wou = wo.bitcast(u32)

    x_cp = pltpu.make_async_copy(x_hbm, xbuf, sems.at[0])
    wq_cp = pltpu.make_async_copy(wq_hbm, wq, sems.at[1])
    wo_cp = pltpu.make_async_copy(wo_hbm, wo, sems.at[2])
    w3_cp = pltpu.make_async_copy(w3_hbm, w3, sems.at[3])
    w4_rows, r0 = [], 0
    for n in W4_CHUNKS:
        w4_rows.append((r0, r0 + n))
        r0 += n
    w4_cp = [pltpu.make_async_copy(w4_hbm.at[a:b], w4.at[a:b], sems.at[4 + c])
             for c, (a, b) in enumerate(w4_rows)]
    S0 = 4 + len(W4_CHUNKS)

    def k_cp(i):
        return pltpu.make_async_copy(
            k_hbm.at[pl.ds(i * GP, GP), pl.ds(t0 * 8, wt * 8), :],
            kbuf.at[pl.ds(i * GP, GP)], sems.at[S0 + i])

    def v_cp(i):
        return pltpu.make_async_copy(
            v_hbm.at[pl.ds(i * GP, GP), pl.ds(t0 * 8, wt * 8), :],
            vbuf.at[pl.ds(i * GP, GP)], sems.at[S0 + NP + i])

    for c in (wq_cp, x_cp, wo_cp):
        c.start()
    for i in range(NP):
        k_cp(i).start()
        v_cp(i).start()
    for c in [w3_cp] + w4_cp:
        c.start()

    zs[0] = 0

    lane = lax.broadcasted_iota(jnp.int32, (8, 128), 1)
    sub = lax.broadcasted_iota(jnp.int32, (8, 128), 0)
    lane_lo = lane < 64
    sub_lo = sub < 4

    def tile(ref, g0, G, t):
        g, r = _slot(G, t)
        return ref[g0 + g, r:r + 8, :]

    def retile(ref, i, expand):
        def body(c, carry):
            g0 = i * GP + 8 * c
            for G in range(4):
                for J in range(4):
                    xs = [[ref[g0 + 2 * G + e, _vr(4 * J + jj), :] for jj in range(4)]
                          for e in range(2)]
                    for jj in range(4):
                        x0, x1 = xs[0][jj], xs[1][jj]
                        ys = (jnp.where(sub_lo, x0, pltpu.roll(x1, 4, 0)),
                              jnp.where(sub_lo, pltpu.roll(x0, 4, 0), x1))
                        for e in range(2):
                            t = 8 * J + 2 * jj + e
                            g, r = _slot(G, t)
                            if expand and G % 2 and e:
                                ref[g0 + g, r:r + 8, :] = ys[e] << 16
                                g, r = _xslot(G, t)
                                vx[i * (GP // 4) + 2 * c + g, r:r + 8, :] = ys[e] & jnp.uint32(HI)
                            else:
                                ref[g0 + g, r:r + 8, :] = ys[e]
            return carry
        lax.fori_loop(0, GP // 8, body, 0)

    def retile_w(wu, unroll):
        nt = wu.shape[1]

        def body(c, carry):
            for u in range(unroll):
                G = c * unroll + u
                xs = [wu[G, n] for n in range(nt)]
                for n in range(nt):
                    lo, hi = xs[n // 2], xs[(nt + n) // 2]
                    if n % 2:
                        lo = pltpu.roll(lo, 4, 0)
                    if (nt + n) % 2 == 0:
                        hi = pltpu.roll(hi, 4, 0)
                    wu[G, n] = jnp.where(sub_lo, lo, hi)
            return carry
        lax.fori_loop(0, wu.shape[0] // unroll, body, 0)

    def lhs_at(ref, n):
        return pltpu.bitcast(ref[_vr(n), :], bf16)

    cur = [None]

    def tick(ref, n, val):
        if val.dtype != ref.dtype:
            val = pltpu.bitcast(val, ref.dtype)
        ref[pl.ds(pl.multiple_of(cur[0] + 8 * n, 8), 8), :] = val

    def q_dots(i, st, qref, lhs=None, mean=None):
        def step(k):
            def run():
                w = _wcols(wqu, _vr(k), [3 * i + n for n in range(3)])
                if lhs is None:
                    r = jnp.dot(lhs_at(lref, L_Y + k), w, preferred_element_type=f32)[0:8]
                else:
                    r = jnp.dot(lhs[:, 128 * k:128 * k + 128], w, preferred_element_type=f32)
                st["q"] = r if k == 0 else st["q"] + r
                if k == 4:
                    q = st["q"] if lhs is None else st["q"][0:8] - mean * st["q"][8:16]
                    qq = pltpu.bitcast(q.astype(bf16).astype(f32), u32)
                    q0, q1, q2 = qq[:, 0:128], qq[:, 128:256], qq[:, 256:384]
                    for n, v in enumerate((q0 >> 16, q0, q2 >> 16, q2, q1, pltpu.roll(q1, 64, 1))):
                        qref[_vr(n), :] = v
                return r[0:8, 256:384]
            return 3, lref, L_DUMMY, run
        return [step(k) for k in range(5)]

    def o_dots(slot, i, st, chunks=range(3)):
        def step(b):
            def run():
                w = _wcols(wou, pl.ds(i * (GP // 2) + 8 * b, 8), range(5))
                lhs = obuf[pl.ds(pl.multiple_of(24 * slot + 8 * b, 8), 8), :]
                r = jnp.dot(pltpu.bitcast(lhs, bf16), w, preferred_element_type=f32)[0:8]
                st["acc"] = st["acc"] + r
                return r[:, 512:640]
            return 5, obuf, 3 * (NP + 1), run
        return [step(b) for b in chunks]

    def k_dots(i, hh, st, qref, order=tuple(range(12))):
        g0 = i * GP
        gf, gh = ((0, 8), (16, 12))[hh]

        def step(r):
            def run():
                if r < 8:
                    cols = [[tile(ku, g0, gf + G, 8 * T + r) for G in range(8)] for T in range(4)]
                    base, row = qref[_vr(2 * hh + r % 2), :], r // 2
                else:
                    cols = [[tile(ku, g0, gh + G % 4, 8 * T + 2 * (r - 8) + G // 4)
                             for G in range(8)] for T in range(4)]
                    if r == 8:
                        st["u"] = jnp.where(lane_lo, qref[_vr(4 + hh), :] >> 16,
                                            qref[_vr(5 - hh), :])
                    base, row = st["u"], r - 8
                lhs = jnp.where(sub == row, base, jnp.zeros((8, 128), u32))
                w = jnp.concatenate([jnp.concatenate(c, axis=0) for c in cols], axis=1)
                res = jnp.dot(pltpu.bitcast(lhs, bf16), pltpu.bitcast(w, bf16),
                              preferred_element_type=f32)[0:8]
                st["s", hh] = res if r == order[0] else st["s", hh] + res
                return res[:, 384:512]
            return 4, (qref if r < 8 else None), 6, run
        return [step(r) for r in order]

    def col(s, T):
        return s[:, 128 * T:128 * T + 128]

    def row_max(s):
        m = jnp.maximum(jnp.maximum(col(s, 0), col(s, 1)), jnp.maximum(col(s, 2), col(s, 3)))
        return jnp.max(jnp.max(m, axis=1, keepdims=True), axis=0, keepdims=True)

    def prob(s, m):
        return jnp.exp2((s - m) * scl[_vr(0), :])

    def put_p(hh, T, p, ks=range(8)):
        for k in ks:
            pT[4 * hh + T][pl.ds(k, 8, stride=8), :] = p

    def part_sum(p):
        return (p[0] + p[1]) + (p[2] + p[3])

    def inv_sum(l):
        l = jnp.sum(jnp.sum(l, axis=1, keepdims=True), axis=0, keepdims=True)
        return jnp.broadcast_to(1.0 / l, (8, 128))

    def softmax(s, hh):
        m = row_max(s)
        p = [prob(col(s, T), m) for T in range(4)]
        for T in range(4):
            put_p(hh, T, p[T])
        return p, part_sum(p)

    def get_state(i, n):
        return pltpu.bitcast(ku[i * GP + 3, _vr(n), :], f32)

    def set_state(i, n, v):
        ku[i * GP + 3, _vr(n), :] = pltpu.bitcast(v, u32)

    def stash_b(i, s):
        for T in range(4):
            set_state(i, T, col(s, T))
        m = jnp.broadcast_to(row_max(s), (8, 128))
        set_state(i, S_MAXB, m)
        return m

    def reduce_o(blocks, inva, invb):
        out = []
        for b, inv in enumerate((inva, jnp.where(lane_lo, inva, invb), invb)):
            z = jnp.sum(pltpu.bitcast(blocks[b], f32).T.reshape(16, 8, 128), axis=0)
            o = jnp.sum(z, axis=0, keepdims=True) * inv
            out.append(pltpu.bitcast(_rows16(o, o), u32))
        return out

    def put_o(slot, o):
        for b in range(3):
            obuf[pl.ds(pl.multiple_of(24 * slot + 8 * b, 8), 8), :] = o[b]

    def mac(acc, n, c, G, t, pv):
        w = tile(vu, 8 * c, G, t)
        if G % 2 and t % 2:
            g, r = _xslot(G, t)
            halves = (w, vx[2 * c + g, r:r + 8, :])
        else:
            halves = (w << 16, w & jnp.uint32(HI))
        for k in range(2):
            a = pltpu.bitcast(halves[k], f32) * pv
            acc[n + k] = a if acc[n + k] is None else acc[n + k] + a

    def run_block(i, put_a, dots, issue, tv0, hooks, SEG, rev=True):
        clock = []

        def emit(upto):
            while len(clock) < upto:
                n = len(clock)
                for h in hooks.get(("dot", n), ()):
                    h()
                clock.append(dots[n][3]())

        tie = {}
        for seg in range(TIEG - 1, 48 if rev else 0, TIEG):
            end = tv0 + SEG * (seg + 1)
            ok = [n for n, c in enumerate(issue) if dots[n][1] is not None and c >= end + MINLAG]
            good = [n for n in ok if issue[n] >= end + LAG]
            if ok:
                tie[seg] = good[0] if good else ok[-1]
        zero = jnp.zeros((8, 128), f32)
        seg = 0
        for hh in range(2):
            for gp in range(6):
                a4 = [None] * 4
                for T in range(4):
                    pref = pT[4 * hh + T]
                    start = tv0 + SEG * seg
                    grp = seg - seg % TIEG + TIEG - 1
                    emit(max(tie.get(grp, len(dots)) if rev else sum(1 for c in issue if c < start + SEG + 12), hooks.get(("need", seg), 0)))
                    done = max(1, sum(1 for c in issue if c + (LAT2 if rev else LAT) <= start))
                    if grp not in tie:
                        tick(pref, 8, clock[done - 1])
                    elif gp:
                        tick(pref, 8, zero)
                    for h in hooks.get(("seg", seg), ()):
                        h(clock[done - 1])
                    for rho in range(8):
                        pv = pref[_vr(rho), :]
                        for e in range(2):
                            mac(a4, 2 * e, i * 6, 12 * hh + 2 * gp + e, 8 * T + rho, pv)
                    if seg in tie:
                        _, ref, slot, _ = dots[tie[seg]]
                        for k in range(4):
                            tick(ref, slot + k, a4[k])
                    seg += 1
                for e in range(2):
                    G = 12 * hh + 2 * gp + e
                    for k in range(2):
                        put_a(G // 8, 16 * (G % 8) + k, pltpu.bitcast(a4[2 * e + k], u32))
        emit(len(dots))

    def times(dots, t=0, rate=8):
        out = []
        for d in dots:
            t += rate * d[0]
            out.append(t)
        return out

    def run_all(dots):
        for d in dots:
            d[3]()

    def set_input(c, scale):
        cp = pltpu.bitcast(_rows16(c, c), u32)
        for k in range(5):
            lref[_vr(L_Y + k), :] = cp[:, 128 * k:128 * k + 128]
        scl[_vr(0), :] = jnp.broadcast_to(scale, (8, 128))

    x_cp.wait()
    x = jnp.broadcast_to(xbuf[...].astype(f32), (8, D))
    set_input(_ln(x), jnp.full((8, 1), CEXP, f32))
    wq_cp.wait()
    retile_w(wqu, 1)
    wo_cp.wait()
    retile_w(wou, 8)

    def body1(i, acc):
        st = {"acc": acc}
        k_cp(i).wait()
        retile(ku, i, False)
        run_all(q_dots(i, st, qa))
        inv = []
        for hh in range(2):
            run_all(k_dots(i, hh, st, qa))
            inv.append(inv_sum(softmax(st["s", hh], hh)[1]))
        v_cp(i).wait()
        retile(vu, i, True)
        for hh in range(2):
            def pv_step(c, carry, hh=hh):
                acc8 = [None] * 8
                for t in range(32):
                    pv = pT[4 * hh + t // 8][_vr(t % 8), :]
                    for G in range(4):
                        mac(acc8, 2 * G, i * 6 + c, G, t, pv)
                for n in range(8):
                    obuf[pl.ds(64 * c + 16 * (n // 2) + n % 2, 8, stride=2), :] = (
                        pltpu.bitcast(acc8[n], u32))
                return carry
            lax.fori_loop(3 * hh, 3 * hh + 3, pv_step, 0)
        put_o(NP, reduce_o([obuf[128 * b:128 * b + 128, :] for b in range(3)], inv[0], inv[1]))
        run_all(o_dots(NP, i, st))
        return st["acc"]

    x = lax.fori_loop(0, NP, body1, x)

    y = _ln(x)
    zz = _ln(y).astype(bf16)
    w3_cp.wait()
    h = jnp.dot(zz, w3[...], preferred_element_type=f32)
    h = jax.nn.gelu(h, approximate=True).astype(bf16)
    x = x + y
    for cp, (a, b) in zip(w4_cp, w4_rows):
        cp.wait()
        x = x + jnp.dot(h[:, a:b], w4[a:b, :], preferred_element_type=f32)

    ones = jnp.ones((8, D), f32)
    xl = _rows16(x, ones)
    xb = xl[0:8].astype(f32)
    mean = _mean(xb)
    c = xb - mean
    set_input(c, lax.rsqrt(_mean(c * c) + EPS) * CEXP)
    obuf[0:24, :] = jnp.zeros((24, 128), u32)

    def tail_hooks(i, st, hooks, seg0):
        def first(_):
            m = row_max(st["s", 0])
            st["pa"] = [prob(col(st["s", 0], T), m) for T in range(4)]
            set_state(i, S_INVA, inv_sum(part_sum(st["pa"])))

        def put(T, half):
            def run(clk):
                tick(pT[T], 8, clk)
                put_p(0, T, st["pa"][T], range(4 * half, 4 * half + 4))
            return run
        hooks.setdefault(("seg", seg0), []).append(first)
        for n in range(8):
            hooks.setdefault(("seg", seg0 + n), []).append(put(n // 2, n % 2))

    def head_b_hooks(i, seg0):
        pb = []

        def put_b(T):
            def run(clk):
                tick(scl, 1, clk)
                pb.append(prob(get_state(i, T), get_state(i, S_MAXB)))
                put_p(1, T, pb[T])
                if T == 3:
                    set_state(i, S_LB, part_sum(pb))
            return run
        return {("seg", seg0 + 3 * T): [put_b(T)] for T in range(4)}

    def reduce_pair(i):
        return reduce_o([ku[i * GP + b] for b in range(3)],
                        get_state(i, S_INVA), inv_sum(get_state(i, S_LB)))

    def put_k(i):
        def put_a(b, r, v):
            ku[i * GP + b, pl.ds(r, 8, stride=2), :] = v
        return put_a

    st = {}
    zero = cur[0] = zs[0]
    late = tuple(range(8, 12)) + tuple(range(8))
    d0 = q_dots(0, st, qb, xl, mean) + q_dots(1, st, qa, xl, mean)
    d1 = k_dots(0, 0, st, qb) + k_dots(0, 1, st, qb, late) + k_dots(1, 0, st, qa, late) \
        + k_dots(1, 1, st, qa) + q_dots(2, st, qa)
    issue = times(d0 + d1)

    def sm_a0():
        m = row_max(st["s", 0])
        p = [prob(col(st["s", 0], T), m) for T in range(4)]
        tick(qb, 6, part_sum(p))
        for T in range(4):
            put_p(0, T, p[T])
        set_state(0, S_INVA, inv_sum(part_sum(p)))

    def sm_b0():
        tick(qa, 6, stash_b(0, st["s", 1]))

    hooks = head_b_hooks(0, 15)
    hooks.update({("dot", 31): [sm_a0], ("dot", 43): [sm_b0],
                  ("need", 0): 32, ("need", 15): 44, ("need", 36): 46})
    tail_hooks(1, st, hooks, 36)
    run_block(0, put_k(0), d0 + d1, issue, 240 + 384 + LAT + 170, hooks, SEG0, False)
    stash_b(1, st["s", 1])

    def body2(j, acc, last=False):
        cur[0] = zs[0]
        st = {"acc": acc}
        o = reduce_pair(j)
        hooks = head_b_hooks(j + 1, B_SEG0)
        if last:
            dots = o_dots(NP - 2, NP - 3, st)
            for n in range(NP - 3):
                dots += o_dots(n + 1, n, st, [2])
            issue = times(dots, rate=11.5)
        else:
            dots = k_dots(j + 2, 0, st, qa, MIX) + k_dots(j + 2, 1, st, qa, MIX) \
                + q_dots(jnp.minimum(j + 3, NP - 1), st, qa) \
                + o_dots(j, jnp.maximum(j - 1, 0), st, [0, 1])
            issue = times(dots)
            tail_hooks(j + 2, st, hooks, A_SEG0)
            hooks["need", A_SEG0] = 12
            hooks["dot", 24] = [lambda: stash_b(j + 2, st["s", 1])]
        run_block(j + 1, put_k(j + 1), dots, issue, 0, hooks, SEGL if last else SEG)
        put_o(j + 1, o)
        return st["acc"]

    x = lax.fori_loop(0, NP - 2, body2, x)
    x = lax.fori_loop(NP - 2, NP - 1 + zero, functools.partial(body2, last=True), x)

    st = {"acc": x}
    o = reduce_pair(NP - 1)
    run_all(o_dots(NP - 1, NP - 2, st))
    put_o(NP, o)
    run_all(o_dots(NP, NP - 1, st))
    x = st["acc"]

    xl = _rows16(x, ones)
    xb = xl[0:8].astype(f32)
    mean = _mean(xb)
    c = xb - mean
    r1 = lax.rsqrt(_mean(c * c) + EPS)
    y = c * r1
    my = _mean(y)
    r2 = lax.rsqrt(_mean(y * y) - my * my + EPS)
    h = jnp.dot(xl, w3[...], preferred_element_type=f32)
    h = h[0:8] * (r1 * r2) - h[8:16] * ((mean * r1 + my) * r2)
    h = jax.nn.gelu(h, approximate=True).astype(bf16)
    x = x + y + jnp.dot(h, w4[...], preferred_element_type=f32)
    o_ref[...] = x[0:1].astype(o_ref.dtype)


def _cache_view(c):
    s = c.shape[2]
    c = jnp.transpose(c, (0, 1, 3, 2)).reshape(H * DH // 8, 8, s // 128, 128)
    return jnp.transpose(c, (0, 2, 1, 3)).reshape(H * DH // 8, s // 128 * 8, 128)


def _weight_view(w):
    k, n = w.shape
    w = jnp.transpose(w.reshape(k // 16, 2, 8, n // 128, 128), (0, 1, 3, 2, 4))
    return w.reshape(k // 16, n // 128, 16, 128)


@jax.jit
def pallas_interleave_layers__sliding_block_cached__mixer_s_mlp__decode_kernel(
    A_x: jax.Array,
    A_k_cache: jax.Array,
    A_v_cache: jax.Array,
    A_wq: jax.Array,
    A_wo: jax.Array,
    B_x: jax.Array,
    B_w1: jax.Array,
    B_w2: jax.Array,
    B_w3: jax.Array,
    B_w4: jax.Array,
):
    sk = A_k_cache.shape[2]
    win = min(4096, max(256, sk // 4))
    assert win == 4096 and sk % 128 == 0
    assert A_x.shape == (1, 1, D) and A_k_cache.shape == (1, H, sk, DH)
    wt = win // 128
    t0 = sk // 128 - wt
    ng = H * DH // 8
    hbm = pl.BlockSpec(memory_space=pl.ANY)
    out = pl.pallas_call(
        functools.partial(_kernel, t0=t0, wt=wt),
        out_shape=jax.ShapeDtypeStruct((1, D), A_x.dtype),
        in_specs=[hbm] * 7,
        out_specs=pl.BlockSpec(memory_space=pltpu.VMEM),
        scratch_shapes=[
            pltpu.VMEM((ng, wt * 8, 128), bf16),
            pltpu.VMEM((ng, wt * 8, 128), bf16),
            pltpu.VMEM((ng // 4, 128, 128), u32),
            pltpu.VMEM((D // 16, H * DH // 128, 16, 128), bf16),
            pltpu.VMEM((H * DH // 16, D // 128, 16, 128), bf16),
            pltpu.VMEM((D, F), bf16),
            pltpu.VMEM((F, D), bf16),
            pltpu.VMEM((1, D), bf16),
            pltpu.VMEM((72, 128), u32),
            pltpu.VMEM((24 * (NP + 1) + 32, 128), u32),
            pltpu.VMEM((80, 128), u32),
            pltpu.VMEM((80, 128), u32),
            pltpu.VMEM((16, 128), f32),
            pltpu.SMEM((1,), jnp.int32),
        ] + [pltpu.VMEM((72, 128), f32)] * 8,
        compiler_params=pltpu.CompilerParams(vmem_limit_bytes=128 * 1024 * 1024),
    )(A_x.reshape(1, D), _cache_view(A_k_cache), _cache_view(A_v_cache),
      _weight_view(A_wq), _weight_view(A_wo), B_w3, B_w4)
    return out.reshape(1, 1, D)
```

```python
import functools

import jax
import jax.numpy as jnp
from jax import lax
import jax.experimental.pallas as pl
import jax.experimental.pallas.tpu as pltpu

D = 640
H = 32
DH = 192
F = 1536
EPS = 1e-5
NP = H // 2
GP = 2 * DH // 8
HI = 0xFFFF0000
CEXP = DH ** -0.5 * 1.4426950408889634

f32 = jnp.float32
bf16 = jnp.bfloat16
u32 = jnp.uint32

L_Y = 0
L_DUMMY = 5
S_MAXB, S_LB, S_INVA, S_X, S_PA = 4, 5, 6, 7, 9
XROWS = ((2,), ())
XROWS_LAST = ((2, 6), (2, 6))
GX = (0, 16)
CPO = 25.5 / 88
CPO0 = 22.5 / 88
CPOL = 23.0 / 88
RATEL = 8.5
LAT = 145
B_SEG0 = 9
LAG = 20
MIX = (0, 1, 8, 2, 3, 9, 4, 5, 10, 6, 7, 11)
LAT2 = 145
MIXA = (0, 1, 2, 3, 4, 8, 5, 9, 6, 10, 7, 11)
TIEG = 2
A_SEG0 = 39
W4_CHUNKS = (1024, 384, 128)


def _mean(x):
    return jnp.mean(x, axis=-1, keepdims=True)


def _ln(x):
    c = x - _mean(x)
    return c * lax.rsqrt(_mean(c * c) + EPS)


def _wtile(wu, rows, nt):
    blk = wu[rows, nt]
    return pltpu.bitcast(blk.reshape(blk.shape[0] * 8, 128), bf16)


def _wcols(wu, rows, nts):
    return jnp.concatenate([_wtile(wu, rows, n) for n in nts], axis=1)


def _rows16(a, b):
    return jnp.concatenate([a, b], axis=0).astype(bf16)


def _slot(G, t):
    j = 4 * (t >> 3) + ((((t >> 1) & 3) + G + 2 * (t & 1) + (t >> 3)) & 3)
    return 2 * G + (t & 1), 8 * j


def _xslot(G, t):
    return G // 2, 8 * (4 * (t >> 3) + ((((t >> 1) & 3) + G + (t >> 3)) & 3))


def _vr(n):
    return slice(8 * n, 8 * n + 8)


def _kernel(*refs, t0, wt):
    pl.run_scoped(functools.partial(_body, refs, t0, wt),
                  pltpu.SemaphoreType.DMA((4 + len(W4_CHUNKS) + 2 * NP,)))


def _body(refs, t0, wt, sems):
    (x_hbm, k_hbm, v_hbm, wq_hbm, wo_hbm, w3_hbm, w4_hbm, o_ref,
     kbuf, vbuf, vx, wq, wo, w3, w4, xbuf, lref, obuf, qa, qb, scl, zs) = refs[:22]
    pT = refs[22:]
    ku = kbuf.bitcast(u32)
    vu = vbuf.bitcast(u32)
    wqu = wq.bitcast(u32)
    wou = wo.bitcast(u32)

    x_cp = pltpu.make_async_copy(x_hbm, xbuf, sems.at[0])
    wq_cp = pltpu.make_async_copy(wq_hbm, wq, sems.at[1])
    wo_cp = pltpu.make_async_copy(wo_hbm, wo, sems.at[2])
    w3_cp = pltpu.make_async_copy(w3_hbm, w3, sems.at[3])
    w4_rows, r0 = [], 0
    for n in W4_CHUNKS:
        w4_rows.append((r0, r0 + n))
        r0 += n
    w4_cp = [pltpu.make_async_copy(w4_hbm.at[a:b], w4.at[a:b], sems.at[4 + c])
             for c, (a, b) in enumerate(w4_rows)]
    S0 = 4 + len(W4_CHUNKS)

    def k_cp(i):
        return pltpu.make_async_copy(
            k_hbm.at[pl.ds(i * GP, GP), pl.ds(t0 * 8, wt * 8), :],
            kbuf.at[pl.ds(i * GP, GP)], sems.at[S0 + i])

    def v_cp(i):
        return pltpu.make_async_copy(
            v_hbm.at[pl.ds(i * GP, GP), pl.ds(t0 * 8, wt * 8), :],
            vbuf.at[pl.ds(i * GP, GP)], sems.at[S0 + NP + i])

    for c in (wq_cp, x_cp, wo_cp):
        c.start()
    for i in range(NP):
        k_cp(i).start()
        v_cp(i).start()
    for c in [w3_cp] + w4_cp:
        c.start()

    zs[0] = 0

    lane = lax.broadcasted_iota(jnp.int32, (8, 128), 1)
    sub = lax.broadcasted_iota(jnp.int32, (8, 128), 0)
    lane_lo = lane < 64
    sub_lo = sub < 4

    def tile(ref, g0, G, t):
        g, r = _slot(G, t)
        return ref[g0 + g, r:r + 8, :]

    def retile(ref, i, expand):
        def body(c, carry):
            g0 = i * GP + 8 * c
            for G in range(4):
                for J in range(4):
                    xs = [[ref[g0 + 2 * G + e, _vr(4 * J + jj), :] for jj in range(4)]
                          for e in range(2)]
                    for jj in range(4):
                        x0, x1 = xs[0][jj], xs[1][jj]
                        ys = (jnp.where(sub_lo, x0, pltpu.roll(x1, 4, 0)),
                              jnp.where(sub_lo, pltpu.roll(x0, 4, 0), x1))
                        for e in range(2):
                            t = 8 * J + 2 * jj + e
                            g, r = _slot(G, t)
                            if expand and G % 2 and e:
                                ref[g0 + g, r:r + 8, :] = ys[e] << 16
                                g, r = _xslot(G, t)
                                vx[i * (GP // 4) + 2 * c + g, r:r + 8, :] = ys[e] & jnp.uint32(HI)
                            else:
                                ref[g0 + g, r:r + 8, :] = ys[e]
            return carry
        lax.fori_loop(0, GP // 8, body, 0)

    def retile_w(wu, unroll):
        nt = wu.shape[1]

        def body(c, carry):
            for u in range(unroll):
                G = c * unroll + u
                xs = [wu[G, n] for n in range(nt)]
                for n in range(nt):
                    lo, hi = xs[n // 2], xs[(nt + n) // 2]
                    if n % 2:
                        lo = pltpu.roll(lo, 4, 0)
                    if (nt + n) % 2 == 0:
                        hi = pltpu.roll(hi, 4, 0)
                    wu[G, n] = jnp.where(sub_lo, lo, hi)
            return carry
        lax.fori_loop(0, wu.shape[0] // unroll, body, 0)

    def lhs_at(ref, n):
        return pltpu.bitcast(ref[_vr(n), :], bf16)

    cur = [None]

    def tick(ref, n, val):
        if val.dtype != ref.dtype:
            val = pltpu.bitcast(val, ref.dtype)
        ref[pl.ds(pl.multiple_of(cur[0] + 8 * n, 8), 8), :] = val

    def q_dots(i, st, qref, lhs=None, mean=None):
        def step(k):
            def run():
                w = _wcols(wqu, _vr(k), [3 * i + n for n in range(3)])
                if lhs is None:
                    r = jnp.dot(lhs_at(lref, L_Y + k), w, preferred_element_type=f32)[0:8]
                else:
                    r = jnp.dot(lhs[:, 128 * k:128 * k + 128], w, preferred_element_type=f32)
                st["q"] = r if k == 0 else st["q"] + r
                if k == 4:
                    q = st["q"] if lhs is None else st["q"][0:8] - mean * st["q"][8:16]
                    qq = pltpu.bitcast(q.astype(bf16).astype(f32), u32)
                    q0, q1, q2 = qq[:, 0:128], qq[:, 128:256], qq[:, 256:384]
                    for n, v in enumerate((q0 >> 16, q0, q2 >> 16, q2, q1)):
                        qref[_vr(n), :] = v
                return r[0:8, 256:384]
            return 3, lref, L_DUMMY, run
        return [step(k) for k in range(5)]

    def o_dots(slot, i, st, chunks=range(3)):
        def step(b):
            def run():
                w = _wcols(wou, pl.ds(i * (GP // 2) + 8 * b, 8), range(5))
                lhs = obuf[pl.ds(pl.multiple_of(24 * slot + 8 * b, 8), 8), :]
                r = jnp.dot(pltpu.bitcast(lhs, bf16), w, preferred_element_type=f32)[0:8]
                st["acc"] = st["acc"] + r
                return r[:, 512:640]
            return 5, obuf, 3 * (NP + 1), run
        return [step(b) for b in chunks]

    def mid_q(st, qref):
        q1 = qref[_vr(4), :]
        q1r = pltpu.roll(q1, 64, 1)
        st["u", 0] = jnp.where(lane_lo, q1 >> 16, q1r)
        st["u", 1] = jnp.where(lane_lo, q1r >> 16, q1)

    def k_dots(i, hh, st, qref, order=tuple(range(12))):
        g0 = i * GP
        gf, gh = ((0, 8), (16, 12))[hh]

        def step(r):
            def run():
                if r < 8:
                    cols = [[tile(ku, g0, gf + G, 8 * T + r) for G in range(8)] for T in range(4)]
                    base, row = qref[_vr(2 * hh + r % 2), :], r // 2
                else:
                    cols = [[tile(ku, g0, gh + G % 4, 8 * T + 2 * (r - 8) + G // 4)
                             for G in range(8)] for T in range(4)]
                    if r == 8 and hh == 0 and "pre" not in st:
                        mid_q(st, qref)
                    base, row = st["u", hh], r - 8
                lhs = jnp.where(sub == row, base, jnp.zeros((8, 128), u32))
                w = jnp.concatenate([jnp.concatenate(c, axis=0) for c in cols], axis=1)
                res = jnp.dot(pltpu.bitcast(lhs, bf16), pltpu.bitcast(w, bf16),
                              preferred_element_type=f32)[0:8]
                st["s", hh] = res if r == order[0] else st["s", hh] + res
                return res[:, 384:512]
            return 4, (qref if r < 8 else None), 6, run
        return [step(r) for r in order]

    def col(s, T):
        return s[:, 128 * T:128 * T + 128]

    def row_max(s):
        m = jnp.maximum(jnp.maximum(col(s, 0), col(s, 1)), jnp.maximum(col(s, 2), col(s, 3)))
        return jnp.max(jnp.max(m, axis=1, keepdims=True), axis=0, keepdims=True)

    def prob(s, m):
        return jnp.exp2((s - m) * scl[_vr(0), :])

    def put_p(hh, T, p, ks=range(8)):
        for k in ks:
            pT[4 * hh + T][pl.ds(k, 8, stride=8), :] = p

    def part_sum(p):
        return (p[0] + p[1]) + (p[2] + p[3])

    def inv_sum(l):
        l = jnp.sum(jnp.sum(l, axis=1, keepdims=True), axis=0, keepdims=True)
        return jnp.broadcast_to(1.0 / l, (8, 128))

    def softmax(s, hh):
        m = row_max(s)
        p = [prob(col(s, T), m) for T in range(4)]
        for T in range(4):
            put_p(hh, T, p[T])
        return p, part_sum(p)

    def get_state(i, n):
        return pltpu.bitcast(ku[i * GP + 3, _vr(n), :], f32)

    def set_state(i, n, v):
        ku[i * GP + 3, _vr(n), :] = pltpu.bitcast(v, u32)

    def stash_b(i, s):
        for T in range(4):
            set_state(i, T, col(s, T))
        m = jnp.broadcast_to(row_max(s), (8, 128))
        set_state(i, S_MAXB, m)
        return m

    def pack_p(p):
        return pltpu.bitcast(_rows16(p, p), u32)

    def x_dots(i, hh, rows, get_lhs):
        st = {}

        def step(n, rho):
            def run():
                res = []
                for T in range(4):
                    w = jnp.concatenate(
                        [tile(vu, i * GP, GX[hh] + G, 8 * T + rho) for G in range(8)], axis=0)
                    res.append(jnp.dot(pltpu.bitcast(get_lhs(T), bf16), pltpu.bitcast(w, bf16),
                                       preferred_element_type=f32)[0:8])
                st["x"] = jnp.where(sub == rho, part_sum(res), st["x"] if n else 0.0)
                if n == len(rows) - 1:
                    set_state(i, S_X + hh, st["x"])
                return res[3]
            return 4, None, 0, run
        return [step(n, rho) for n, rho in enumerate(rows)]

    def transpose_x(i, xrows):
        for hh in range(2):
            for t in [8 * T + rho for T in range(4) for rho in xrows[hh]]:
                w = jnp.concatenate([tile(vu, i * GP, GX[hh] + G, t) for G in range(8)], axis=0)
                w = pltpu.bitcast(pltpu.bitcast(w, bf16).astype(f32).T.astype(bf16), u32)
                for G in range(8):
                    g, r = _slot(GX[hh] + G, t)
                    vu[i * GP + g, r:r + 8, :] = w[_vr(G), :]

    def reduce_o(blocks, inva, invb, extra=(None, None, None)):
        out = []
        for b, inv in enumerate((inva, jnp.where(lane_lo, inva, invb), invb)):
            z = jnp.sum(pltpu.bitcast(blocks[b], f32).T.reshape(16, 8, 128), axis=0)
            if extra[b] is not None:
                z = z + extra[b]
            o = jnp.sum(z, axis=0, keepdims=True) * inv
            out.append(pltpu.bitcast(_rows16(o, o), u32))
        return out

    def put_o(slot, o):
        for b in range(3):
            obuf[pl.ds(pl.multiple_of(24 * slot + 8 * b, 8), 8), :] = o[b]

    def mac(acc, n, c, G, t, pv):
        w = tile(vu, 8 * c, G, t)
        if G % 2 and t % 2:
            g, r = _xslot(G, t)
            halves = (w, vx[2 * c + g, r:r + 8, :])
        else:
            halves = (w << 16, w & jnp.uint32(HI))
        for k in range(2):
            a = pltpu.bitcast(halves[k], f32) * pv
            acc[n + k] = a if acc[n + k] is None else acc[n + k] + a

    def run_block(i, xrows, dots, issue, tv0, hooks, cpo, rev=True):
        clock = []

        def emit(upto):
            while len(clock) < upto:
                n = len(clock)
                for h in hooks.get(("dot", n), ()):
                    h()
                clock.append(dots[n][3]())

        def seg_rows(hh, gp):
            on_mxu = GX[hh] <= 12 * hh + 2 * gp < GX[hh] + 8
            return [rho for rho in range(8) if not (on_mxu and rho in xrows[hh])]

        at = [tv0]
        for seg in range(48):
            at.append(at[-1] + cpo * sum(10 if rho % 2 else 12
                                         for rho in seg_rows(seg // 24, seg % 24 // 4)))
        tie = {}
        for seg in range(TIEG - 1, 48 if rev else 0, TIEG):
            ok = [n for n, c in enumerate(issue)
                  if dots[n][1] is not None and c >= at[seg + 1] + LAG]
            if ok:
                tie[seg] = ok[0]
        zero = jnp.zeros((8, 128), f32)
        seg = 0
        for hh in range(2):
            for gp in range(6):
                a4 = [None] * 4
                for T in range(4):
                    pref = pT[4 * hh + T]
                    grp = seg - seg % TIEG + TIEG - 1
                    upto = (tie.get(grp, len(dots)) if rev
                            else sum(1 for c in issue if c < at[seg + 1] + 12))
                    upto = min([upto] + [k[1] for k, v in hooks.items()
                                         if k[0] == "after" and v >= seg])
                    emit(max(upto, hooks.get(("need", seg), 0)))
                    done = sum(1 for c in issue if c + (LAT2 if rev else LAT) <= at[seg])
                    done = min(max(1, done), len(clock))
                    if grp not in tie:
                        tick(pref, 8, clock[done - 1])
                    elif gp:
                        tick(pref, 8, zero)
                    for h in hooks.get(("seg", seg), ()):
                        h(clock[done - 1])
                    for rho in seg_rows(hh, gp):
                        pv = pref[_vr(rho), :]
                        for e in range(2):
                            mac(a4, 2 * e, i * 6, 12 * hh + 2 * gp + e, 8 * T + rho, pv)
                    if seg in tie:
                        _, ref, slot, _ = dots[tie[seg]]
                        for k in range(4):
                            tick(ref, slot + k, a4[k])
                    seg += 1
                for n in range(4):
                    G = 12 * hh + 2 * gp + n // 2
                    ku[i * GP + G // 8, pl.ds(16 * (G % 8) + n % 2, 8, stride=2), :] = (
                        pltpu.bitcast(a4[n], u32))
        emit(len(dots))

    def times(dots, t=0, rate=8):
        out = []
        for d in dots:
            t += rate * d[0]
            out.append(t)
        return out

    def run_all(dots):
        for d in dots:
            d[3]()

    def set_input(c, scale):
        cp = pltpu.bitcast(_rows16(c, c), u32)
        for k in range(5):
            lref[_vr(L_Y + k), :] = cp[:, 128 * k:128 * k + 128]
        scl[_vr(0), :] = jnp.broadcast_to(scale, (8, 128))

    x_cp.wait()
    x = jnp.broadcast_to(xbuf[...].astype(f32), (8, D))
    set_input(_ln(x), jnp.full((8, 1), CEXP, f32))
    wq_cp.wait()
    retile_w(wqu, 1)
    wo_cp.wait()
    retile_w(wou, 8)

    def body1(i, acc):
        st = {"acc": acc}
        k_cp(i).wait()
        retile(ku, i, False)
        run_all(q_dots(i, st, qa))
        inv = []
        for hh in range(2):
            run_all(k_dots(i, hh, st, qa))
            inv.append(inv_sum(softmax(st["s", hh], hh)[1]))

        @pl.when(i > 1)
        def _():
            transpose_x(i - 1, XROWS)

        v_cp(i).wait()
        retile(vu, i, True)
        for hh in range(2):
            def pv_step(c, carry, hh=hh):
                acc8 = [None] * 8
                for t in range(32):
                    pv = pT[4 * hh + t // 8][_vr(t % 8), :]
                    for G in range(4):
                        mac(acc8, 2 * G, i * 6 + c, G, t, pv)
                for n in range(8):
                    obuf[pl.ds(64 * c + 16 * (n // 2) + n % 2, 8, stride=2), :] = (
                        pltpu.bitcast(acc8[n], u32))
                return carry
            lax.fori_loop(3 * hh, 3 * hh + 3, pv_step, 0)
        put_o(NP, reduce_o([obuf[128 * b:128 * b + 128, :] for b in range(3)], inv[0], inv[1]))
        run_all(o_dots(NP, i, st))
        return st["acc"]

    x = lax.fori_loop(0, NP, body1, x)

    y = _ln(x)
    zz = _ln(y).astype(bf16)
    w3_cp.wait()
    h = jnp.dot(zz, w3[...], preferred_element_type=f32)
    h = jax.nn.gelu(h, approximate=True).astype(bf16)
    x = x + y
    transpose_x(NP - 1, XROWS_LAST)
    for cp, (a, b) in zip(w4_cp, w4_rows):
        cp.wait()
        x = x + jnp.dot(h[:, a:b], w4[a:b, :], preferred_element_type=f32)

    ones = jnp.ones((8, D), f32)
    xl = _rows16(x, ones)
    xb = xl[0:8].astype(f32)
    mean = _mean(xb)
    c = xb - mean
    set_input(c, lax.rsqrt(_mean(c * c) + EPS) * CEXP)
    obuf[0:24, :] = jnp.zeros((24, 128), u32)

    def tail_hooks(i, st, hooks, seg0):
        def first(_):
            m = row_max(st["s", 0])
            st["pa"] = [prob(col(st["s", 0], T), m) for T in range(4)]
            set_state(i, S_INVA, inv_sum(part_sum(st["pa"])))
            for T in range(4):
                ku[i * GP + 3, _vr(S_PA + T), :] = pack_p(st["pa"][T])

        def put(T, half):
            def run(clk):
                tick(pT[T], 8, clk)
                put_p(0, T, st["pa"][T], range(4 * half, 4 * half + 4))
            return run
        hooks.setdefault(("seg", seg0), []).append(first)
        for n in range(8):
            hooks.setdefault(("seg", seg0 + n), []).append(put(n // 2, n % 2))

    def head_b_hooks(i, seg0, pb):
        def put_b(T):
            def run(clk):
                tick(scl, 1, clk)
                pb.append(prob(get_state(i, T), get_state(i, S_MAXB)))
                put_p(1, T, pb[T])
                if T == 3:
                    set_state(i, S_LB, part_sum(pb))
            return run
        return {("seg", seg0 + 3 * T): [put_b(T)] for T in range(4)}

    def reduce_pair(i, xrows):
        xa, xb = (get_state(i, S_X + hh) if xrows[hh] else None for hh in range(2))
        return reduce_o([ku[i * GP + b] for b in range(3)],
                        get_state(i, S_INVA), inv_sum(get_state(i, S_LB)), (xa, None, xb))

    st = {}
    zero = cur[0] = zs[0]
    late = tuple(range(8, 12)) + tuple(range(8))
    d0 = q_dots(0, st, qb, xl, mean) + q_dots(1, st, qa, xl, mean)
    d1 = k_dots(0, 0, st, qb) + k_dots(0, 1, st, qb, late) + k_dots(1, 0, st, qa, late) \
        + k_dots(1, 1, st, qa) + q_dots(2, st, qa)
    issue = times(d0 + d1)

    def sm_a0():
        m = row_max(st["s", 0])
        p = [prob(col(st["s", 0], T), m) for T in range(4)]
        tick(qb, 6, part_sum(p))
        for T in range(4):
            put_p(0, T, p[T])
        set_state(0, S_INVA, inv_sum(part_sum(p)))

    def sm_b0():
        tick(qa, 6, stash_b(0, st["s", 1]))

    hooks = head_b_hooks(0, 15, [])
    hooks.update({("dot", 31): [sm_a0], ("dot", 43): [sm_b0],
                  ("need", 0): 32, ("need", 15): 44, ("need", 36): 46})
    tail_hooks(1, st, hooks, 36)
    run_block(0, ((), ()), d0 + d1, issue, 240 + 384 + LAT + 170, hooks, CPO0, False)
    set_state(0, S_X, jnp.zeros((8, 128), f32))
    stash_b(1, st["s", 1])

    def body2(j, acc, last=False):
        cur[0] = zs[0]
        st = {"acc": acc, "pre": True}
        if not last:
            mid_q(st, qa)
        o = reduce_pair(j, XROWS)
        pb = []
        hooks = head_b_hooks(j + 1, B_SEG0, pb)
        xrows = XROWS_LAST if last else XROWS
        xa = x_dots(j + 1, 0, xrows[0], lambda T: ku[(j + 1) * GP + 3, _vr(S_PA + T), :])
        if last:
            dots = o_dots(NP - 2, NP - 3, st)
            for n in range(NP - 3):
                dots += o_dots(n + 1, n, st, [2])
            hooks["after", len(dots)] = B_SEG0 + 9
            dots += x_dots(j + 1, 1, xrows[1], lambda T: pack_p(pb[T])) + xa
            issue = times(dots, rate=RATEL)
        else:
            dots = k_dots(j + 2, 0, st, qa, MIXA) + k_dots(j + 2, 1, st, qa, MIX) \
                + q_dots(jnp.minimum(j + 3, NP - 1), st, qa) \
                + o_dots(j, jnp.maximum(j - 1, 0), st, [0, 1]) + xa
            issue = times(dots)
            tail_hooks(j + 2, st, hooks, A_SEG0)
            hooks["need", A_SEG0] = 12
            hooks["dot", 24] = [lambda: stash_b(j + 2, st["s", 1])]
        run_block(j + 1, xrows, dots, issue, 0, hooks, CPOL if last else CPO)
        put_o(j + 1, o)
        return st["acc"]

    x = lax.fori_loop(0, NP - 2, body2, x)
    x = lax.fori_loop(NP - 2, NP - 1 + zero, functools.partial(body2, last=True), x)

    st = {"acc": x}
    o = reduce_pair(NP - 1, XROWS_LAST)
    run_all(o_dots(NP - 1, NP - 2, st))
    put_o(NP, o)
    run_all(o_dots(NP, NP - 1, st))
    x = st["acc"]

    xl = _rows16(x, ones)
    xb = xl[0:8].astype(f32)
    mean = _mean(xb)
    c = xb - mean
    r1 = lax.rsqrt(_mean(c * c) + EPS)
    y = c * r1
    my = _mean(y)
    r2 = lax.rsqrt(_mean(y * y) - my * my + EPS)
    h = jnp.dot(xl, w3[...], preferred_element_type=f32)
    h = h[0:8] * (r1 * r2) - h[8:16] * ((mean * r1 + my) * r2)
    h = jax.nn.gelu(h, approximate=True).astype(bf16)
    x = x + y + jnp.dot(h, w4[...], preferred_element_type=f32)
    o_ref[...] = x[0:1].astype(o_ref.dtype)


def _cache_view(c):
    s = c.shape[2]
    c = jnp.transpose(c, (0, 1, 3, 2)).reshape(H * DH // 8, 8, s // 128, 128)
    return jnp.transpose(c, (0, 2, 1, 3)).reshape(H * DH // 8, s // 128 * 8, 128)


def _weight_view(w):
    k, n = w.shape
    w = jnp.transpose(w.reshape(k // 16, 2, 8, n // 128, 128), (0, 1, 3, 2, 4))
    return w.reshape(k // 16, n // 128, 16, 128)


@jax.jit
def pallas_interleave_layers__sliding_block_cached__mixer_s_mlp__decode_kernel(
    A_x: jax.Array,
    A_k_cache: jax.Array,
    A_v_cache: jax.Array,
    A_wq: jax.Array,
    A_wo: jax.Array,
    B_x: jax.Array,
    B_w1: jax.Array,
    B_w2: jax.Array,
    B_w3: jax.Array,
    B_w4: jax.Array,
):
    sk = A_k_cache.shape[2]
    win = min(4096, max(256, sk // 4))
    assert win == 4096 and sk % 128 == 0
    assert A_x.shape == (1, 1, D) and A_k_cache.shape == (1, H, sk, DH)
    wt = win // 128
    t0 = sk // 128 - wt
    ng = H * DH // 8
    hbm = pl.BlockSpec(memory_space=pl.ANY)
    out = pl.pallas_call(
        functools.partial(_kernel, t0=t0, wt=wt),
        out_shape=jax.ShapeDtypeStruct((1, D), A_x.dtype),
        in_specs=[hbm] * 7,
        out_specs=pl.BlockSpec(memory_space=pltpu.VMEM),
        scratch_shapes=[
            pltpu.VMEM((ng, wt * 8, 128), bf16),
            pltpu.VMEM((ng, wt * 8, 128), bf16),
            pltpu.VMEM((ng // 4, 128, 128), u32),
            pltpu.VMEM((D // 16, H * DH // 128, 16, 128), bf16),
            pltpu.VMEM((H * DH // 16, D // 128, 16, 128), bf16),
            pltpu.VMEM((D, F), bf16),
            pltpu.VMEM((F, D), bf16),
            pltpu.VMEM((1, D), bf16),
            pltpu.VMEM((72, 128), u32),
            pltpu.VMEM((24 * (NP + 1) + 32, 128), u32),
            pltpu.VMEM((80, 128), u32),
            pltpu.VMEM((80, 128), u32),
            pltpu.VMEM((16, 128), f32),
            pltpu.SMEM((1,), jnp.int32),
        ] + [pltpu.VMEM((72, 128), f32)] * 8,
        compiler_params=pltpu.CompilerParams(vmem_limit_bytes=128 * 1024 * 1024),
    )(A_x.reshape(1, D), _cache_view(A_k_cache), _cache_view(A_v_cache),
      _weight_view(A_wq), _weight_view(A_wo), B_w3, B_w4)
    return out.reshape(1, 1, D)
```

```python
import functools

import jax
import jax.numpy as jnp
from jax import lax
import jax.experimental.pallas as pl
import jax.experimental.pallas.tpu as pltpu

D = 640
H = 32
DH = 192
F = 1536
EPS = 1e-5
NP = H // 2
GP = 2 * DH // 8
HI = 0xFFFF0000
CEXP = DH ** -0.5 * 1.4426950408889634

f32 = jnp.float32
bf16 = jnp.bfloat16
u32 = jnp.uint32

L_Y = 0
L_DUMMY = 5
S_MAXB, S_LB, S_INVA, S_X, S_PA = 4, 5, 6, 7, 9
XROWS = ((2,), ())
XROWS_LAST = ((0, 2, 4, 6), (2, 6))
GX = (0, 16)
CPO = 25.5 / 88
CPO0 = 22.5 / 88
CPOL = 23.0 / 88
RATEL = 8
LAT = 145
B_SEG0 = 9
B_SEGL = 9
NLATE = 0
LAG = 20
MIX = (0, 1, 8, 2, 3, 9, 4, 5, 10, 6, 7, 11)
LAT2 = 145
MIXA = (0, 1, 2, 3, 4, 8, 5, 9, 6, 10, 7, 11)
TIEG = 2
DA0 = 32
DB0 = 43
TV0 = 939
B0_SEG = 15
A1_SEG = 36
A_SEG0 = 39
W4_CHUNKS = (1024, 384, 128)


def _mean(x):
    return jnp.mean(x, axis=-1, keepdims=True)


def _ln(x):
    c = x - _mean(x)
    return c * lax.rsqrt(_mean(c * c) + EPS)


def _wtile(wu, rows, nt):
    blk = wu[rows, nt]
    return pltpu.bitcast(blk.reshape(blk.shape[0] * 8, 128), bf16)


def _wcols(wu, rows, nts):
    return jnp.concatenate([_wtile(wu, rows, n) for n in nts], axis=1)


def _rows16(a, b):
    return jnp.concatenate([a, b], axis=0).astype(bf16)


def _slot(G, t):
    j = 4 * (t >> 3) + ((((t >> 1) & 3) + G + 2 * (t & 1) + (t >> 3)) & 3)
    return 2 * G + (t & 1), 8 * j


def _xslot(G, t):
    return G // 2, 8 * (4 * (t >> 3) + ((((t >> 1) & 3) + G + (t >> 3)) & 3))


def _vr(n):
    return slice(8 * n, 8 * n + 8)


def _kernel(*refs, t0, wt):
    pl.run_scoped(functools.partial(_body, refs, t0, wt),
                  pltpu.SemaphoreType.DMA((4 + len(W4_CHUNKS) + 2 * NP,)))


def _body(refs, t0, wt, sems):
    (x_hbm, k_hbm, v_hbm, wq_hbm, wo_hbm, w3_hbm, w4_hbm, o_ref,
     kbuf, vbuf, vx, wq, wo, w3, w4, xbuf, lref, obuf, qa, qb, scl, zs) = refs[:22]
    pT = refs[22:]
    ku = kbuf.bitcast(u32)
    vu = vbuf.bitcast(u32)
    wqu = wq.bitcast(u32)
    wou = wo.bitcast(u32)

    x_cp = pltpu.make_async_copy(x_hbm, xbuf, sems.at[0])
    wq_cp = pltpu.make_async_copy(wq_hbm, wq, sems.at[1])
    wo_cp = pltpu.make_async_copy(wo_hbm, wo, sems.at[2])
    w3_cp = pltpu.make_async_copy(w3_hbm, w3, sems.at[3])
    w4_rows, r0 = [], 0
    for n in W4_CHUNKS:
        w4_rows.append((r0, r0 + n))
        r0 += n
    w4_cp = [pltpu.make_async_copy(w4_hbm.at[a:b], w4.at[a:b], sems.at[4 + c])
             for c, (a, b) in enumerate(w4_rows)]
    S0 = 4 + len(W4_CHUNKS)

    def k_cp(i):
        return pltpu.make_async_copy(
            k_hbm.at[pl.ds(i * GP, GP), pl.ds(t0 * 8, wt * 8), :],
            kbuf.at[pl.ds(i * GP, GP)], sems.at[S0 + i])

    def v_cp(i):
        return pltpu.make_async_copy(
            v_hbm.at[pl.ds(i * GP, GP), pl.ds(t0 * 8, wt * 8), :],
            vbuf.at[pl.ds(i * GP, GP)], sems.at[S0 + NP + i])

    for c in (wq_cp, x_cp, wo_cp):
        c.start()
    for i in range(NP):
        k_cp(i).start()
        v_cp(i).start()
    for c in [w3_cp] + w4_cp:
        c.start()

    zs[0] = 0

    lane = lax.broadcasted_iota(jnp.int32, (8, 128), 1)
    sub = lax.broadcasted_iota(jnp.int32, (8, 128), 0)
    lane_lo = lane < 64
    sub_lo = sub < 4

    def tile(ref, g0, G, t):
        g, r = _slot(G, t)
        return ref[g0 + g, r:r + 8, :]

    def retile(ref, i, expand):
        def body(c, carry):
            g0 = i * GP + 8 * c
            for G in range(4):
                for J in range(4):
                    xs = [[ref[g0 + 2 * G + e, _vr(4 * J + jj), :] for jj in range(4)]
                          for e in range(2)]
                    for jj in range(4):
                        x0, x1 = xs[0][jj], xs[1][jj]
                        ys = (jnp.where(sub_lo, x0, pltpu.roll(x1, 4, 0)),
                              jnp.where(sub_lo, pltpu.roll(x0, 4, 0), x1))
                        for e in range(2):
                            t = 8 * J + 2 * jj + e
                            g, r = _slot(G, t)
                            if expand and G % 2 and e:
                                ref[g0 + g, r:r + 8, :] = ys[e] << 16
                                g, r = _xslot(G, t)
                                vx[i * (GP // 4) + 2 * c + g, r:r + 8, :] = ys[e] & jnp.uint32(HI)
                            else:
                                ref[g0 + g, r:r + 8, :] = ys[e]
            return carry
        lax.fori_loop(0, GP // 8, body, 0)

    def retile_w(wu, unroll):
        nt = wu.shape[1]

        def body(c, carry):
            for u in range(unroll):
                G = c * unroll + u
                xs = [wu[G, n] for n in range(nt)]
                for n in range(nt):
                    lo, hi = xs[n // 2], xs[(nt + n) // 2]
                    if n % 2:
                        lo = pltpu.roll(lo, 4, 0)
                    if (nt + n) % 2 == 0:
                        hi = pltpu.roll(hi, 4, 0)
                    wu[G, n] = jnp.where(sub_lo, lo, hi)
            return carry
        lax.fori_loop(0, wu.shape[0] // unroll, body, 0)

    def lhs_at(ref, n):
        return pltpu.bitcast(ref[_vr(n), :], bf16)

    cur = [None]

    def tick(ref, n, val):
        if val.dtype != ref.dtype:
            val = pltpu.bitcast(val, ref.dtype)
        ref[pl.ds(pl.multiple_of(cur[0] + 8 * n, 8), 8), :] = val

    def q_dots(i, st, qref, lhs=None, mean=None):
        def step(k):
            def run():
                w = _wcols(wqu, _vr(k), [3 * i + n for n in range(3)])
                if lhs is None:
                    r = jnp.dot(lhs_at(lref, L_Y + k), w, preferred_element_type=f32)[0:8]
                else:
                    r = jnp.dot(lhs[:, 128 * k:128 * k + 128], w, preferred_element_type=f32)
                st["q"] = r if k == 0 else st["q"] + r
                if k == 4:
                    q = st["q"] if lhs is None else st["q"][0:8] - mean * st["q"][8:16]
                    qq = pltpu.bitcast(q.astype(bf16).astype(f32), u32)
                    q0, q1, q2 = qq[:, 0:128], qq[:, 128:256], qq[:, 256:384]
                    for n, v in enumerate((q0 >> 16, q0, q2 >> 16, q2, q1)):
                        qref[_vr(n), :] = v
                return r[0:8, 256:384]
            return 3, lref, L_DUMMY, run
        return [step(k) for k in range(5)]

    def o_dots(slot, i, st, chunks=range(3)):
        def step(b):
            def run():
                w = _wcols(wou, pl.ds(i * (GP // 2) + 8 * b, 8), range(5))
                lhs = obuf[pl.ds(pl.multiple_of(24 * slot + 8 * b, 8), 8), :]
                r = jnp.dot(pltpu.bitcast(lhs, bf16), w, preferred_element_type=f32)[0:8]
                st["acc"] = st["acc"] + r
                return r[:, 512:640]
            return 5, obuf, 3 * (NP + 1), run
        return [step(b) for b in chunks]

    def mid_q(st, qref):
        q1 = qref[_vr(4), :]
        q1r = pltpu.roll(q1, 64, 1)
        st["u", 0] = jnp.where(lane_lo, q1 >> 16, q1r)
        st["u", 1] = jnp.where(lane_lo, q1r >> 16, q1)

    def k_dots(i, hh, st, qref, order=tuple(range(12))):
        g0 = i * GP
        gf, gh = ((0, 8), (16, 12))[hh]

        def step(r):
            def run():
                if r < 8:
                    cols = [[tile(ku, g0, gf + G, 8 * T + r) for G in range(8)] for T in range(4)]
                    base, row = qref[_vr(2 * hh + r % 2), :], r // 2
                else:
                    cols = [[tile(ku, g0, gh + G % 4, 8 * T + 2 * (r - 8) + G // 4)
                             for G in range(8)] for T in range(4)]
                    if r == 8 and hh == 0 and "pre" not in st:
                        mid_q(st, qref)
                    base, row = st["u", hh], r - 8
                lhs = jnp.where(sub == row, base, jnp.zeros((8, 128), u32))
                w = jnp.concatenate([jnp.concatenate(c, axis=0) for c in cols], axis=1)
                res = jnp.dot(pltpu.bitcast(lhs, bf16), pltpu.bitcast(w, bf16),
                              preferred_element_type=f32)[0:8]
                st["s", hh] = res if r == order[0] else st["s", hh] + res
                return res[:, 384:512]
            return 4, (qref if r < 8 else None), 6, run
        return [step(r) for r in order]

    def col(s, T):
        return s[:, 128 * T:128 * T + 128]

    def row_max(s):
        m = jnp.maximum(jnp.maximum(col(s, 0), col(s, 1)), jnp.maximum(col(s, 2), col(s, 3)))
        return jnp.max(jnp.max(m, axis=1, keepdims=True), axis=0, keepdims=True)

    def prob(s, m):
        return jnp.exp2((s - m) * scl[_vr(0), :])

    def put_p(hh, T, p, ks=range(8)):
        for k in ks:
            pT[4 * hh + T][pl.ds(k, 8, stride=8), :] = p

    def part_sum(p):
        return (p[0] + p[1]) + (p[2] + p[3])

    def inv_sum(l):
        l = jnp.sum(jnp.sum(l, axis=1, keepdims=True), axis=0, keepdims=True)
        return jnp.broadcast_to(1.0 / l, (8, 128))

    def softmax(s, hh):
        m = row_max(s)
        p = [prob(col(s, T), m) for T in range(4)]
        for T in range(4):
            put_p(hh, T, p[T])
        return p, part_sum(p)

    def get_state(i, n):
        return pltpu.bitcast(ku[i * GP + 3, _vr(n), :], f32)

    def set_state(i, n, v):
        ku[i * GP + 3, _vr(n), :] = pltpu.bitcast(v, u32)

    def stash_b(i, s):
        for T in range(4):
            set_state(i, T, col(s, T))
        m = jnp.broadcast_to(row_max(s), (8, 128))
        set_state(i, S_MAXB, m)
        return m

    def pack_p(p):
        return pltpu.bitcast(_rows16(p, p), u32)

    def x_dots(i, hh, rows, get_lhs):
        st = {}

        def step(n, rho):
            def run():
                res = []
                for T in range(4):
                    w = jnp.concatenate(
                        [tile(vu, i * GP, GX[hh] + G, 8 * T + rho) for G in range(8)], axis=0)
                    res.append(jnp.dot(pltpu.bitcast(get_lhs(T), bf16), pltpu.bitcast(w, bf16),
                                       preferred_element_type=f32)[0:8])
                st["x"] = jnp.where(sub == rho, part_sum(res), st["x"] if n else 0.0)
                if n == len(rows) - 1:
                    set_state(i, S_X + hh, st["x"])
                return res[3]
            return 4, None, 0, run
        return [step(n, rho) for n, rho in enumerate(rows)]

    def transpose_x(i, xrows):
        for hh in range(2):
            for t in [8 * T + rho for T in range(4) for rho in xrows[hh]]:
                w = jnp.concatenate([tile(vu, i * GP, GX[hh] + G, t) for G in range(8)], axis=0)
                w = pltpu.bitcast(pltpu.bitcast(w, bf16).astype(f32).T.astype(bf16), u32)
                for G in range(8):
                    g, r = _slot(GX[hh] + G, t)
                    vu[i * GP + g, r:r + 8, :] = w[_vr(G), :]

    def reduce_o(blocks, inva, invb, extra=(None, None, None)):
        out = []
        for b, inv in enumerate((inva, jnp.where(lane_lo, inva, invb), invb)):
            z = jnp.sum(pltpu.bitcast(blocks[b], f32).T.reshape(16, 8, 128), axis=0)
            if extra[b] is not None:
                z = z + extra[b]
            o = jnp.sum(z, axis=0, keepdims=True) * inv
            out.append(pltpu.bitcast(_rows16(o, o), u32))
        return out

    def put_o(slot, o):
        for b in range(3):
            obuf[pl.ds(pl.multiple_of(24 * slot + 8 * b, 8), 8), :] = o[b]

    def mac(acc, n, c, G, t, pv):
        w = tile(vu, 8 * c, G, t)
        if G % 2 and t % 2:
            g, r = _xslot(G, t)
            halves = (w, vx[2 * c + g, r:r + 8, :])
        else:
            halves = (w << 16, w & jnp.uint32(HI))
        for k in range(2):
            a = pltpu.bitcast(halves[k], f32) * pv
            acc[n + k] = a if acc[n + k] is None else acc[n + k] + a

    def run_block(i, xrows, dots, issue, tv0, hooks, cpo, rev=True):
        clock = []

        def emit(upto):
            while len(clock) < upto:
                n = len(clock)
                for h in hooks.get(("dot", n), ()):
                    h()
                clock.append(dots[n][3]())

        def seg_rows(hh, gp):
            on_mxu = GX[hh] <= 12 * hh + 2 * gp < GX[hh] + 8
            return [rho for rho in range(8) if not (on_mxu and rho in xrows[hh])]

        at = [tv0]
        for seg in range(48):
            at.append(at[-1] + cpo * sum(10 if rho % 2 else 12
                                         for rho in seg_rows(seg // 24, seg % 24 // 4)))
        tie = {}
        for seg in range(TIEG - 1, 48 if rev else 0, TIEG):
            ok = [n for n, c in enumerate(issue)
                  if dots[n][1] is not None and c >= at[seg + 1] + LAG]
            if ok:
                tie[seg] = ok[0]
        zero = jnp.zeros((8, 128), f32)
        seg = 0
        for hh in range(2):
            for gp in range(6):
                a4 = [None] * 4
                for T in range(4):
                    pref = pT[4 * hh + T]
                    grp = seg - seg % TIEG + TIEG - 1
                    upto = (tie.get(grp, len(dots)) if rev
                            else sum(1 for c in issue if c < at[seg + 1] + 12))
                    upto = min([upto] + [k[1] for k, v in hooks.items()
                                         if k[0] == "after" and v >= seg])
                    emit(max(upto, hooks.get(("need", seg), 0)))
                    done = sum(1 for c in issue if c + (LAT2 if rev else LAT) <= at[seg])
                    done = min(max(1, done), len(clock))
                    if grp not in tie:
                        tick(pref, 8, clock[done - 1])
                    elif gp:
                        tick(pref, 8, zero)
                    for h in hooks.get(("seg", seg), ()):
                        h(clock[done - 1])
                    for rho in seg_rows(hh, gp):
                        pv = pref[_vr(rho), :]
                        for e in range(2):
                            mac(a4, 2 * e, i * 6, 12 * hh + 2 * gp + e, 8 * T + rho, pv)
                    if seg in tie:
                        _, ref, slot, _ = dots[tie[seg]]
                        for k in range(4):
                            tick(ref, slot + k, a4[k])
                    seg += 1
                for n in range(4):
                    G = 12 * hh + 2 * gp + n // 2
                    ku[i * GP + G // 8, pl.ds(16 * (G % 8) + n % 2, 8, stride=2), :] = (
                        pltpu.bitcast(a4[n], u32))
        emit(len(dots))

    def times(dots, t=0, rate=8):
        out = []
        for d in dots:
            t += rate * d[0]
            out.append(t)
        return out

    def run_all(dots):
        for d in dots:
            d[3]()

    def set_input(c, scale):
        cp = pltpu.bitcast(_rows16(c, c), u32)
        for k in range(5):
            lref[_vr(L_Y + k), :] = cp[:, 128 * k:128 * k + 128]
        scl[_vr(0), :] = jnp.broadcast_to(scale, (8, 128))

    x_cp.wait()
    x = jnp.broadcast_to(xbuf[...].astype(f32), (8, D))
    set_input(_ln(x), jnp.full((8, 1), CEXP, f32))
    wq_cp.wait()
    retile_w(wqu, 1)
    wo_cp.wait()
    retile_w(wou, 8)

    def body1(i, acc):
        st = {"acc": acc}
        k_cp(i).wait()
        retile(ku, i, False)
        run_all(q_dots(i, st, qa))
        inv = []
        for hh in range(2):
            run_all(k_dots(i, hh, st, qa))
            inv.append(inv_sum(softmax(st["s", hh], hh)[1]))

        @pl.when(i > 1)
        def _():
            transpose_x(i - 1, XROWS)

        v_cp(i).wait()
        retile(vu, i, True)
        for hh in range(2):
            def pv_step(c, carry, hh=hh):
                acc8 = [None] * 8
                for t in range(32):
                    pv = pT[4 * hh + t // 8][_vr(t % 8), :]
                    for G in range(4):
                        mac(acc8, 2 * G, i * 6 + c, G, t, pv)
                for n in range(8):
                    obuf[pl.ds(64 * c + 16 * (n // 2) + n % 2, 8, stride=2), :] = (
                        pltpu.bitcast(acc8[n], u32))
                return carry
            lax.fori_loop(3 * hh, 3 * hh + 3, pv_step, 0)
        put_o(NP, reduce_o([obuf[128 * b:128 * b + 128, :] for b in range(3)], inv[0], inv[1]))
        run_all(o_dots(NP, i, st))
        return st["acc"]

    x = lax.fori_loop(0, NP, body1, x)

    y = _ln(x)
    zz = _ln(y).astype(bf16)
    w3_cp.wait()
    h = jnp.dot(zz, w3[...], preferred_element_type=f32)
    h = jax.nn.gelu(h, approximate=True).astype(bf16)
    x = x + y
    transpose_x(NP - 1, XROWS_LAST)
    for cp, (a, b) in zip(w4_cp, w4_rows):
        cp.wait()
        x = x + jnp.dot(h[:, a:b], w4[a:b, :], preferred_element_type=f32)

    ones = jnp.ones((8, D), f32)
    xl = _rows16(x, ones)
    xb = xl[0:8].astype(f32)
    mean = _mean(xb)
    c = xb - mean
    set_input(c, lax.rsqrt(_mean(c * c) + EPS) * CEXP)
    obuf[0:24, :] = jnp.zeros((24, 128), u32)

    def tail_hooks(i, st, hooks, seg0):
        def first(_):
            m = row_max(st["s", 0])
            st["pa"] = [prob(col(st["s", 0], T), m) for T in range(4)]
            set_state(i, S_INVA, inv_sum(part_sum(st["pa"])))
            for T in range(4):
                ku[i * GP + 3, _vr(S_PA + T), :] = pack_p(st["pa"][T])

        def put(T, half):
            def run(clk):
                tick(pT[T], 8, clk)
                put_p(0, T, st["pa"][T], range(4 * half, 4 * half + 4))
            return run
        hooks.setdefault(("seg", seg0), []).append(first)
        for n in range(8):
            hooks.setdefault(("seg", seg0 + n), []).append(put(n // 2, n % 2))

    def head_b_hooks(i, seg0, pb, final=False):
        def put_b(T):
            def run(clk):
                tick(scl, 1, clk)
                pb.append(prob(get_state(i, T), get_state(i, S_MAXB)))
                put_p(1, T, pb[T])
                if T == 3:
                    set_state(i, S_LB, inv_sum(part_sum(pb)) if final else part_sum(pb))
            return run
        return {("seg", seg0 + 3 * T): [put_b(T)] for T in range(4)}

    def reduce_pair(i, xrows, final=False):
        xa, xb = (get_state(i, S_X + hh) if xrows[hh] else None for hh in range(2))
        invb = get_state(i, S_LB) if final else inv_sum(get_state(i, S_LB))
        return reduce_o([ku[i * GP + b] for b in range(3)],
                        get_state(i, S_INVA), invb, (xa, None, xb))

    st = {}
    zero = cur[0] = zs[0]
    late = tuple(range(8, 12)) + tuple(range(8))
    d0 = q_dots(0, st, qb, xl, mean) + q_dots(1, st, qa, xl, mean)
    d1 = k_dots(0, 0, st, qb) + k_dots(0, 1, st, qb, late) + k_dots(1, 0, st, qa, late) \
        + k_dots(1, 1, st, qa) + q_dots(2, st, qa)
    issue = times(d0 + d1)

    def sm_a0():
        m = row_max(st["s", 0])
        p = [prob(col(st["s", 0], T), m) for T in range(4)]
        tick(qb, 6, part_sum(p))
        put_p(0, 0, p[0])
        st["p0"] = p
        set_state(0, S_INVA, inv_sum(part_sum(p)))

    def put_a0(T):
        def run(clk):
            tick(pT[T], 8, clk)
            put_p(0, T, st["p0"][T])
        return run

    def sm_b0():
        tick(qa, 6, stash_b(0, st["s", 1]))

    hooks = head_b_hooks(0, B0_SEG, [])
    hooks.update({("dot", DA0): [sm_a0], ("dot", DB0): [sm_b0],
                  ("need", 0): DA0 + 1, ("need", B0_SEG): DB0 + 1, ("need", A1_SEG): 46})
    hooks.update({("seg", T): [put_a0(T + 1)] for T in range(3)})
    tail_hooks(1, st, hooks, A1_SEG)
    run_block(0, ((), ()), d0 + d1, issue, TV0, hooks, CPO0, False)
    set_state(0, S_X, jnp.zeros((8, 128), f32))
    stash_b(1, st["s", 1])

    def body2(j, acc, last=False):
        cur[0] = zs[0]
        st = {"acc": acc, "pre": True}
        if not last:
            mid_q(st, qa)
        o = reduce_pair(j, XROWS)
        pb = []
        hooks = head_b_hooks(j + 1, B_SEGL if last else B_SEG0, pb, last)
        xrows = XROWS_LAST if last else XROWS
        xa = x_dots(j + 1, 0, xrows[0], lambda T: ku[(j + 1) * GP + 3, _vr(S_PA + T), :])
        if last:
            dots = o_dots(NP - 2, NP - 3, st)
            for n in range(NP - 3):
                dots += o_dots(n + 1, n, st, [2])
            dots = dots[:len(dots) - NLATE]
            hooks["after", len(dots)] = B_SEGL + 9
            dots += x_dots(j + 1, 1, xrows[1], lambda T: pack_p(pb[T]))
            issue = times(dots, rate=RATEL)
        else:
            dots = k_dots(j + 2, 0, st, qa, MIXA) + k_dots(j + 2, 1, st, qa, MIX) \
                + q_dots(jnp.minimum(j + 3, NP - 1), st, qa) \
                + o_dots(j, jnp.maximum(j - 1, 0), st, [0, 1]) + xa
            issue = times(dots)
            tail_hooks(j + 2, st, hooks, A_SEG0)
            hooks["need", A_SEG0] = 12
            hooks["dot", 24] = [lambda: stash_b(j + 2, st["s", 1])]
        run_block(j + 1, xrows, dots, issue, 0, hooks, CPOL if last else CPO)
        put_o(j + 1, o)
        return st["acc"]

    x = lax.fori_loop(0, NP - 2, body2, x)
    x = lax.fori_loop(NP - 2, NP - 1 + zero, functools.partial(body2, last=True), x)

    st = {"acc": x}
    run_all(x_dots(NP - 1, 0, XROWS_LAST[0], lambda T: ku[(NP - 1) * GP + 3, _vr(S_PA + T), :]))
    o = reduce_pair(NP - 1, XROWS_LAST, True)
    run_all(o_dots(NP - 1, NP - 2, st))
    for n in range(NP - 3 - NLATE, NP - 3):
        run_all(o_dots(n + 1, n, st, [2]))
    put_o(NP, o)
    run_all(o_dots(NP, NP - 1, st))
    x = st["acc"]

    xl = _rows16(x, ones)
    d = xl[0:8].astype(f32) - mean
    md = _mean(d)
    r1 = lax.rsqrt(jnp.maximum(_mean(d * d) - md * md, 0.0) + EPS)
    mean = mean + md
    y = (d - md) * r1
    my = _mean(y)
    r2 = lax.rsqrt(jnp.maximum(_mean(y * y) - my * my, 0.0) + EPS)
    h = jnp.dot(xl, w3[...], preferred_element_type=f32)
    h = h[0:8] * (r1 * r2) - h[8:16] * ((mean * r1 + my) * r2)
    h = jax.nn.gelu(h, approximate=True).astype(bf16)
    x = x + y
    for k in range(0, F, 128):
        x = x + jnp.dot(h[:, k:k + 128], w4[k:k + 128, :], preferred_element_type=f32)
    o_ref[...] = x[0:1].astype(o_ref.dtype)


def _cache_view(c):
    s = c.shape[2]
    c = jnp.transpose(c, (0, 1, 3, 2)).reshape(H * DH // 8, 8, s // 128, 128)
    return jnp.transpose(c, (0, 2, 1, 3)).reshape(H * DH // 8, s // 128 * 8, 128)


def _weight_view(w):
    k, n = w.shape
    w = jnp.transpose(w.reshape(k // 16, 2, 8, n // 128, 128), (0, 1, 3, 2, 4))
    return w.reshape(k // 16, n // 128, 16, 128)


@jax.jit
def pallas_interleave_layers__sliding_block_cached__mixer_s_mlp__decode_kernel(
    A_x: jax.Array,
    A_k_cache: jax.Array,
    A_v_cache: jax.Array,
    A_wq: jax.Array,
    A_wo: jax.Array,
    B_x: jax.Array,
    B_w1: jax.Array,
    B_w2: jax.Array,
    B_w3: jax.Array,
    B_w4: jax.Array,
):
    sk = A_k_cache.shape[2]
    win = min(4096, max(256, sk // 4))
    assert win == 4096 and sk % 128 == 0
    assert A_x.shape == (1, 1, D) and A_k_cache.shape == (1, H, sk, DH)
    wt = win // 128
    t0 = sk // 128 - wt
    ng = H * DH // 8
    hbm = pl.BlockSpec(memory_space=pl.ANY)
    out = pl.pallas_call(
        functools.partial(_kernel, t0=t0, wt=wt),
        out_shape=jax.ShapeDtypeStruct((1, D), A_x.dtype),
        in_specs=[hbm] * 7,
        out_specs=pl.BlockSpec(memory_space=pltpu.VMEM),
        scratch_shapes=[
            pltpu.VMEM((ng, wt * 8, 128), bf16),
            pltpu.VMEM((ng, wt * 8, 128), bf16),
            pltpu.VMEM((ng // 4, 128, 128), u32),
            pltpu.VMEM((D // 16, H * DH // 128, 16, 128), bf16),
            pltpu.VMEM((H * DH // 16, D // 128, 16, 128), bf16),
            pltpu.VMEM((D, F), bf16),
            pltpu.VMEM((F, D), bf16),
            pltpu.VMEM((1, D), bf16),
            pltpu.VMEM((72, 128), u32),
            pltpu.VMEM((24 * (NP + 1) + 32, 128), u32),
            pltpu.VMEM((80, 128), u32),
            pltpu.VMEM((80, 128), u32),
            pltpu.VMEM((16, 128), f32),
            pltpu.SMEM((1,), jnp.int32),
        ] + [pltpu.VMEM((72, 128), f32)] * 8,
        compiler_params=pltpu.CompilerParams(vmem_limit_bytes=128 * 1024 * 1024),
    )(A_x.reshape(1, D), _cache_view(A_k_cache), _cache_view(A_v_cache),
      _weight_view(A_wq), _weight_view(A_wo), B_w3, B_w4)
    return out.reshape(1, 1, D)
```

```python
import functools

import jax
import jax.numpy as jnp
from jax import lax
import jax.experimental.pallas as pl
import jax.experimental.pallas.tpu as pltpu

D = 640
H = 32
DH = 192
F = 1536
EPS = 1e-5
NP = H // 2
GP = 2 * DH // 8
HI = 0xFFFF0000
CEXP = DH ** -0.5 * 1.4426950408889634

f32 = jnp.float32
bf16 = jnp.bfloat16
u32 = jnp.uint32

L_Y = 0
L_DUMMY = 5
S_MAXB, S_LB, S_INVA, S_X, S_PA = 4, 5, 6, 7, 9
XROWS = ((2,), ())
XROWS_LAST = ((0, 2, 4, 6), (2, 6))
GX = (0, 16)
CPO = 25.5 / 88
CPO0 = 22.5 / 88
CPOL = 23.0 / 88
RATEL = 8
LAT = 145
B_SEG0 = 9
B_SEGL = 9
NLATE = 0
LAG = 20
MIX = (0, 1, 8, 2, 3, 9, 4, 5, 10, 6, 7, 11)
LAT2 = 145
MIXA = (0, 1, 2, 3, 4, 8, 5, 9, 6, 10, 7, 11)
TIEG = 2
DA0 = 32
DB0 = 43
TV0 = 939
B0_SEG = 15
A1_SEG = 36
A_SEG0 = 39
W4_CHUNKS = (1024, 384, 128)


def _mean(x):
    return jnp.mean(x, axis=-1, keepdims=True)


def _ln(x):
    c = x - _mean(x)
    return c * lax.rsqrt(_mean(c * c) + EPS)


def _wtile(wu, rows, nt):
    blk = wu[rows, nt]
    return pltpu.bitcast(blk.reshape(blk.shape[0] * 8, 128), bf16)


def _wcols(wu, rows, nts):
    return jnp.concatenate([_wtile(wu, rows, n) for n in nts], axis=1)


def _rows16(a, b):
    return jnp.concatenate([a, b], axis=0).astype(bf16)


def _slot(G, t):
    j = 4 * (t >> 3) + ((((t >> 1) & 3) + G + 2 * (t & 1) + (t >> 3)) & 3)
    return 2 * G + (t & 1), 8 * j


def _xslot(G, t):
    return G // 2, 8 * (4 * (t >> 3) + ((((t >> 1) & 3) + G + (t >> 3)) & 3))


def _vr(n):
    return slice(8 * n, 8 * n + 8)


def _kernel(*refs, t0, wt):
    pl.run_scoped(functools.partial(_body, refs, t0, wt),
                  pltpu.SemaphoreType.DMA((4 + len(W4_CHUNKS) + 2 * NP,)))


def _body(refs, t0, wt, sems):
    (x_hbm, k_hbm, v_hbm, wq_hbm, wo_hbm, w3_hbm, w4_hbm, o_ref,
     kbuf, vbuf, vx, wq, wo, w3, w4, xbuf, lref, obuf, qa, qb, scl, zs) = refs[:22]
    pT = refs[22:]
    ku = kbuf.bitcast(u32)
    vu = vbuf.bitcast(u32)
    wqu = wq.bitcast(u32)
    wou = wo.bitcast(u32)

    x_cp = pltpu.make_async_copy(x_hbm, xbuf, sems.at[0])
    wq_cp = pltpu.make_async_copy(wq_hbm, wq, sems.at[1])
    wo_cp = pltpu.make_async_copy(wo_hbm, wo, sems.at[2])
    w3_cp = pltpu.make_async_copy(w3_hbm, w3, sems.at[3])
    w4_rows, r0 = [], 0
    for n in W4_CHUNKS:
        w4_rows.append((r0, r0 + n))
        r0 += n
    w4_cp = [pltpu.make_async_copy(w4_hbm.at[a:b], w4.at[a:b], sems.at[4 + c])
             for c, (a, b) in enumerate(w4_rows)]
    S0 = 4 + len(W4_CHUNKS)

    def k_cp(i):
        return pltpu.make_async_copy(
            k_hbm.at[pl.ds(i * GP, GP), pl.ds(t0 * 8, wt * 8), :],
            kbuf.at[pl.ds(i * GP, GP)], sems.at[S0 + i])

    def v_cp(i):
        return pltpu.make_async_copy(
            v_hbm.at[pl.ds(i * GP, GP), pl.ds(t0 * 8, wt * 8), :],
            vbuf.at[pl.ds(i * GP, GP)], sems.at[S0 + NP + i])

    for c in (wq_cp, x_cp, wo_cp):
        c.start()
    for i in range(NP):
        k_cp(i).start()
        v_cp(i).start()
    for c in [w3_cp] + w4_cp:
        c.start()

    zs[0] = 0

    lane = lax.broadcasted_iota(jnp.int32, (8, 128), 1)
    sub = lax.broadcasted_iota(jnp.int32, (8, 128), 0)
    lane_lo = lane < 64
    sub_lo = sub < 4

    def tile(ref, g0, G, t):
        g, r = _slot(G, t)
        return ref[g0 + g, r:r + 8, :]

    def retile(ref, i, expand):
        def body(c, carry):
            g0 = i * GP + 8 * c
            for G in range(4):
                for J in range(4):
                    xs = [[ref[g0 + 2 * G + e, _vr(4 * J + jj), :] for jj in range(4)]
                          for e in range(2)]
                    for jj in range(4):
                        x0, x1 = xs[0][jj], xs[1][jj]
                        ys = (jnp.where(sub_lo, x0, pltpu.roll(x1, 4, 0)),
                              jnp.where(sub_lo, pltpu.roll(x0, 4, 0), x1))
                        for e in range(2):
                            t = 8 * J + 2 * jj + e
                            g, r = _slot(G, t)
                            if expand and G % 2 and e:
                                ref[g0 + g, r:r + 8, :] = ys[e] << 16
                                g, r = _xslot(G, t)
                                vx[i * (GP // 4) + 2 * c + g, r:r + 8, :] = ys[e] & jnp.uint32(HI)
                            else:
                                ref[g0 + g, r:r + 8, :] = ys[e]
            return carry
        lax.fori_loop(0, GP // 8, body, 0)

    def retile_w(wu, unroll):
        nt = wu.shape[1]

        def body(c, carry):
            for u in range(unroll):
                G = c * unroll + u
                xs = [wu[G, n] for n in range(nt)]
                for n in range(nt):
                    lo, hi = xs[n // 2], xs[(nt + n) // 2]
                    if n % 2:
                        lo = pltpu.roll(lo, 4, 0)
                    if (nt + n) % 2 == 0:
                        hi = pltpu.roll(hi, 4, 0)
                    wu[G, n] = jnp.where(sub_lo, lo, hi)
            return carry
        lax.fori_loop(0, wu.shape[0] // unroll, body, 0)

    def lhs_at(ref, n):
        return pltpu.bitcast(ref[_vr(n), :], bf16)

    cur = [None]

    def new_block():
        cur[0] = -8 * jnp.clip(zs[0], 0, 1)

    def tick(ref, n, val):
        if val.dtype != ref.dtype:
            val = pltpu.bitcast(val, ref.dtype)
        ref[pl.ds(pl.multiple_of(cur[0] + 8 * n, 8), 8), :] = val

    def q_dots(i, st, qref, lhs=None, mean=None):
        def step(k):
            def run():
                w = _wcols(wqu, _vr(k), [3 * i + n for n in range(3)])
                if lhs is None:
                    r = jnp.dot(lhs_at(lref, L_Y + k), w, preferred_element_type=f32)[0:8]
                else:
                    r = jnp.dot(lhs[:, 128 * k:128 * k + 128], w, preferred_element_type=f32)
                st["q"] = r if k == 0 else st["q"] + r
                if k == 4:
                    q = st["q"] if lhs is None else st["q"][0:8] - mean * st["q"][8:16]
                    qq = pltpu.bitcast(q.astype(bf16).astype(f32), u32)
                    q0, q1, q2 = qq[:, 0:128], qq[:, 128:256], qq[:, 256:384]
                    for n, v in enumerate((q0 >> 16, q0, q2 >> 16, q2, q1)):
                        qref[_vr(n), :] = v
                return r[0:8, 256:384]
            return 3, lref, L_DUMMY, run
        return [step(k) for k in range(5)]

    def o_dots(slot, i, st, chunks=range(3)):
        def step(b):
            def run():
                w = _wcols(wou, pl.ds(i * (GP // 2) + 8 * b, 8), range(5))
                lhs = obuf[pl.ds(pl.multiple_of(24 * slot + 8 * b, 8), 8), :]
                r = jnp.dot(pltpu.bitcast(lhs, bf16), w, preferred_element_type=f32)[0:8]
                st["acc"] = st["acc"] + r
                return r[:, 512:640]
            return 5, obuf, 3 * (NP + 1), run
        return [step(b) for b in chunks]

    def mid_q(st, qref):
        q1 = qref[_vr(4), :]
        q1r = pltpu.roll(q1, 64, 1)
        st["u", 0] = jnp.where(lane_lo, q1 >> 16, q1r)
        st["u", 1] = jnp.where(lane_lo, q1r >> 16, q1)

    def k_dots(i, hh, st, qref, order=tuple(range(12))):
        g0 = i * GP
        gf, gh = ((0, 8), (16, 12))[hh]

        def step(r):
            def run():
                if r < 8:
                    cols = [[tile(ku, g0, gf + G, 8 * T + r) for G in range(8)] for T in range(4)]
                    base, row = qref[_vr(2 * hh + r % 2), :], r // 2
                else:
                    cols = [[tile(ku, g0, gh + G % 4, 8 * T + 2 * (r - 8) + G // 4)
                             for G in range(8)] for T in range(4)]
                    if r == 8 and hh == 0 and "pre" not in st:
                        mid_q(st, qref)
                    base, row = st["u", hh], r - 8
                lhs = jnp.where(sub == row, base, jnp.zeros((8, 128), u32))
                w = jnp.concatenate([jnp.concatenate(c, axis=0) for c in cols], axis=1)
                res = jnp.dot(pltpu.bitcast(lhs, bf16), pltpu.bitcast(w, bf16),
                              preferred_element_type=f32)[0:8]
                st["s", hh] = res if r == order[0] else st["s", hh] + res
                return res[:, 384:512]
            return 4, (qref if r < 8 else None), 6, run
        return [step(r) for r in order]

    def col(s, T):
        return s[:, 128 * T:128 * T + 128]

    def row_max(s):
        m = jnp.maximum(jnp.maximum(col(s, 0), col(s, 1)), jnp.maximum(col(s, 2), col(s, 3)))
        return jnp.max(jnp.max(m, axis=1, keepdims=True), axis=0, keepdims=True)

    def prob(s, m):
        return jnp.exp2((s - m) * scl[_vr(0), :])

    def put_p(hh, T, p, ks=range(8)):
        for k in ks:
            pT[4 * hh + T][pl.ds(k, 8, stride=8), :] = p

    def part_sum(p):
        return (p[0] + p[1]) + (p[2] + p[3])

    def inv_sum(l):
        l = jnp.sum(jnp.sum(l, axis=1, keepdims=True), axis=0, keepdims=True)
        return jnp.broadcast_to(1.0 / l, (8, 128))

    def softmax(s, hh):
        m = row_max(s)
        p = [prob(col(s, T), m) for T in range(4)]
        for T in range(4):
            put_p(hh, T, p[T])
        return p, part_sum(p)

    def get_state(i, n):
        return pltpu.bitcast(ku[i * GP + 3, _vr(n), :], f32)

    def set_state(i, n, v):
        ku[i * GP + 3, _vr(n), :] = pltpu.bitcast(v, u32)

    def stash_b(i, s):
        for T in range(4):
            set_state(i, T, col(s, T))
        m = jnp.broadcast_to(row_max(s), (8, 128))
        set_state(i, S_MAXB, m)
        return m

    def pack_p(p):
        return pltpu.bitcast(_rows16(p, p), u32)

    def x_dots(i, hh, rows, get_lhs):
        st = {}

        def step(n, rho):
            def run():
                res = []
                for T in range(4):
                    w = jnp.concatenate(
                        [tile(vu, i * GP, GX[hh] + G, 8 * T + rho) for G in range(8)], axis=0)
                    res.append(jnp.dot(pltpu.bitcast(get_lhs(T), bf16), pltpu.bitcast(w, bf16),
                                       preferred_element_type=f32)[0:8])
                st["x"] = jnp.where(sub == rho, part_sum(res), st["x"] if n else 0.0)
                if n == len(rows) - 1:
                    set_state(i, S_X + hh, st["x"])
                return res[3]
            return 4, None, 0, run
        return [step(n, rho) for n, rho in enumerate(rows)]

    def transpose_x(i, xrows):
        for hh in range(2):
            for t in [8 * T + rho for T in range(4) for rho in xrows[hh]]:
                w = jnp.concatenate([tile(vu, i * GP, GX[hh] + G, t) for G in range(8)], axis=0)
                w = pltpu.bitcast(pltpu.bitcast(w, bf16).astype(f32).T.astype(bf16), u32)
                for G in range(8):
                    g, r = _slot(GX[hh] + G, t)
                    vu[i * GP + g, r:r + 8, :] = w[_vr(G), :]

    def reduce_o(blocks, inva, invb, extra=(None, None, None)):
        out = []
        for b, inv in enumerate((inva, jnp.where(lane_lo, inva, invb), invb)):
            z = jnp.sum(pltpu.bitcast(blocks[b], f32).T.reshape(16, 8, 128), axis=0)
            if extra[b] is not None:
                z = z + extra[b]
            o = jnp.sum(z, axis=0, keepdims=True) * inv
            out.append(pltpu.bitcast(_rows16(o, o), u32))
        return out

    def put_o(slot, o):
        for b in range(3):
            obuf[pl.ds(pl.multiple_of(24 * slot + 8 * b, 8), 8), :] = o[b]

    def mac(acc, n, c, G, t, pv):
        w = tile(vu, 8 * c, G, t)
        if G % 2 and t % 2:
            g, r = _xslot(G, t)
            halves = (w, vx[2 * c + g, r:r + 8, :])
        else:
            halves = (w << 16, w & jnp.uint32(HI))
        for k in range(2):
            a = pltpu.bitcast(halves[k], f32) * pv
            acc[n + k] = a if acc[n + k] is None else acc[n + k] + a

    def run_block(i, xrows, dots, issue, tv0, hooks, cpo, rev=True):
        clock = []

        def emit(upto):
            while len(clock) < upto:
                n = len(clock)
                for h in hooks.get(("dot", n), ()):
                    h()
                clock.append(dots[n][3]())

        def seg_rows(hh, gp):
            on_mxu = GX[hh] <= 12 * hh + 2 * gp < GX[hh] + 8
            return [rho for rho in range(8) if not (on_mxu and rho in xrows[hh])]

        at = [tv0]
        for seg in range(48):
            at.append(at[-1] + cpo * sum(10 if rho % 2 else 12
                                         for rho in seg_rows(seg // 24, seg % 24 // 4)))
        tie = {}
        for seg in range(TIEG - 1, 48 if rev else 0, TIEG):
            ok = [n for n, c in enumerate(issue)
                  if dots[n][1] is not None and c >= at[seg + 1] + LAG]
            if ok:
                tie[seg] = ok[0]
        zero = jnp.zeros((8, 128), f32)
        seg = 0
        for hh in range(2):
            for gp in range(6):
                a4 = [None] * 4
                for T in range(4):
                    pref = pT[4 * hh + T]
                    grp = seg - seg % TIEG + TIEG - 1
                    upto = (tie.get(grp, len(dots)) if rev
                            else sum(1 for c in issue if c < at[seg + 1] + 12))
                    upto = min([upto] + [k[1] for k, v in hooks.items()
                                         if k[0] == "after" and v >= seg])
                    emit(max(upto, hooks.get(("need", seg), 0)))
                    done = sum(1 for c in issue if c + (LAT2 if rev else LAT) <= at[seg])
                    done = min(max(1, done), len(clock))
                    if grp not in tie:
                        tick(pref, 8, clock[done - 1])
                    elif gp:
                        tick(pref, 8, zero)
                    for h in hooks.get(("seg", seg), ()):
                        h(clock[done - 1])
                    for rho in seg_rows(hh, gp):
                        pv = pref[_vr(rho), :]
                        for e in range(2):
                            mac(a4, 2 * e, i * 6, 12 * hh + 2 * gp + e, 8 * T + rho, pv)
                    if seg in tie:
                        _, ref, slot, _ = dots[tie[seg]]
                        for k in range(4):
                            tick(ref, slot + k, a4[k])
                    seg += 1
                for n in range(4):
                    G = 12 * hh + 2 * gp + n // 2
                    ku[i * GP + G // 8, pl.ds(16 * (G % 8) + n % 2, 8, stride=2), :] = (
                        pltpu.bitcast(a4[n], u32))
        emit(len(dots))

    def times(dots, t=0, rate=8):
        out = []
        for d in dots:
            t += rate * d[0]
            out.append(t)
        return out

    def run_all(dots):
        for d in dots:
            d[3]()

    def set_input(c, scale):
        cp = pltpu.bitcast(_rows16(c, c), u32)
        for k in range(5):
            lref[_vr(L_Y + k), :] = cp[:, 128 * k:128 * k + 128]
        scl[_vr(0), :] = jnp.broadcast_to(scale, (8, 128))

    x_cp.wait()
    x = jnp.broadcast_to(xbuf[...].astype(f32), (8, D))
    set_input(_ln(x), jnp.full((8, 1), CEXP, f32))
    wq_cp.wait()
    retile_w(wqu, 1)
    wo_cp.wait()
    retile_w(wou, 8)

    def body1(i, acc):
        st = {"acc": acc}
        k_cp(i).wait()
        retile(ku, i, False)
        run_all(q_dots(i, st, qa))
        inv = []
        for hh in range(2):
            run_all(k_dots(i, hh, st, qa))
            inv.append(inv_sum(softmax(st["s", hh], hh)[1]))

        @pl.when(i > 1)
        def _():
            transpose_x(i - 1, XROWS)

        v_cp(i).wait()
        retile(vu, i, True)
        for hh in range(2):
            def pv_step(c, carry, hh=hh):
                acc8 = [None] * 8
                for t in range(32):
                    pv = pT[4 * hh + t // 8][_vr(t % 8), :]
                    for G in range(4):
                        mac(acc8, 2 * G, i * 6 + c, G, t, pv)
                for n in range(8):
                    obuf[pl.ds(64 * c + 16 * (n // 2) + n % 2, 8, stride=2), :] = (
                        pltpu.bitcast(acc8[n], u32))
                return carry
            lax.fori_loop(3 * hh, 3 * hh + 3, pv_step, 0)
        put_o(NP, reduce_o([obuf[128 * b:128 * b + 128, :] for b in range(3)], inv[0], inv[1]))
        run_all(o_dots(NP, i, st))
        return st["acc"]

    x = lax.fori_loop(0, NP, body1, x)

    y = _ln(x)
    zz = _ln(y).astype(bf16)
    w3_cp.wait()
    h = jnp.dot(zz, w3[...], preferred_element_type=f32)
    h = jax.nn.gelu(h, approximate=True).astype(bf16)
    x = x + y
    transpose_x(NP - 1, XROWS_LAST)
    for cp, (a, b) in zip(w4_cp, w4_rows):
        cp.wait()
        x = x + jnp.dot(h[:, a:b], w4[a:b, :], preferred_element_type=f32)

    ones = jnp.ones((8, D), f32)
    xl = _rows16(x, ones)
    xb = xl[0:8].astype(f32)
    mean = _mean(xb)
    c = xb - mean
    set_input(c, lax.rsqrt(_mean(c * c) + EPS) * CEXP)
    obuf[0:24, :] = jnp.zeros((24, 128), u32)

    def tail_hooks(i, st, hooks, seg0):
        def first(_):
            m = row_max(st["s", 0])
            st["pa"] = [prob(col(st["s", 0], T), m) for T in range(4)]
            set_state(i, S_INVA, inv_sum(part_sum(st["pa"])))
            for T in range(4):
                ku[i * GP + 3, _vr(S_PA + T), :] = pack_p(st["pa"][T])

        def put(T, half):
            def run(clk):
                tick(pT[T], 8, clk)
                put_p(0, T, st["pa"][T], range(4 * half, 4 * half + 4))
            return run
        hooks.setdefault(("seg", seg0), []).append(first)
        for n in range(8):
            hooks.setdefault(("seg", seg0 + n), []).append(put(n // 2, n % 2))

    def head_b_hooks(i, seg0, pb, final=False):
        def put_b(T):
            def run(clk):
                tick(scl, 1, clk)
                pb.append(prob(get_state(i, T), get_state(i, S_MAXB)))
                put_p(1, T, pb[T])
                if T == 3:
                    set_state(i, S_LB, inv_sum(part_sum(pb)) if final else part_sum(pb))
            return run
        return {("seg", seg0 + 3 * T): [put_b(T)] for T in range(4)}

    def reduce_pair(i, xrows, final=False):
        xa, xb = (get_state(i, S_X + hh) if xrows[hh] else None for hh in range(2))
        invb = get_state(i, S_LB) if final else inv_sum(get_state(i, S_LB))
        return reduce_o([ku[i * GP + b] for b in range(3)],
                        get_state(i, S_INVA), invb, (xa, None, xb))

    st = {}
    new_block()
    late = tuple(range(8, 12)) + tuple(range(8))
    d0 = q_dots(0, st, qb, xl, mean) + q_dots(1, st, qa, xl, mean)
    d1 = k_dots(0, 0, st, qb) + k_dots(0, 1, st, qb, late) + k_dots(1, 0, st, qa, late) \
        + k_dots(1, 1, st, qa) + q_dots(2, st, qa)
    issue = times(d0 + d1)

    def sm_a0():
        m = row_max(st["s", 0])
        p = [prob(col(st["s", 0], T), m) for T in range(4)]
        tick(qb, 6, part_sum(p))
        put_p(0, 0, p[0])
        st["p0"] = p
        set_state(0, S_INVA, inv_sum(part_sum(p)))

    def put_a0(T):
        def run(clk):
            tick(pT[T], 8, clk)
            put_p(0, T, st["p0"][T])
        return run

    def sm_b0():
        tick(qa, 6, stash_b(0, st["s", 1]))

    hooks = head_b_hooks(0, B0_SEG, [])
    hooks.update({("dot", DA0): [sm_a0], ("dot", DB0): [sm_b0],
                  ("need", 0): DA0 + 1, ("need", B0_SEG): DB0 + 1, ("need", A1_SEG): 46})
    hooks.update({("seg", T): [put_a0(T + 1)] for T in range(3)})
    tail_hooks(1, st, hooks, A1_SEG)
    run_block(0, ((), ()), d0 + d1, issue, TV0, hooks, CPO0, False)
    set_state(0, S_X, jnp.zeros((8, 128), f32))
    stash_b(1, st["s", 1])

    def body2(j, acc, last=False):
        new_block()
        st = {"acc": acc, "pre": True}
        if not last:
            mid_q(st, qa)
        o = reduce_pair(j, XROWS)
        pb = []
        hooks = head_b_hooks(j + 1, B_SEGL if last else B_SEG0, pb, last)
        xrows = XROWS_LAST if last else XROWS
        xa = x_dots(j + 1, 0, xrows[0], lambda T: ku[(j + 1) * GP + 3, _vr(S_PA + T), :])
        if last:
            dots = o_dots(NP - 2, NP - 3, st)
            for n in range(NP - 3):
                dots += o_dots(n + 1, n, st, [2])
            dots = dots[:len(dots) - NLATE]
            hooks["after", len(dots)] = B_SEGL + 9
            dots += x_dots(j + 1, 1, xrows[1], lambda T: pack_p(pb[T]))
            issue = times(dots, rate=RATEL)
        else:
            dots = k_dots(j + 2, 0, st, qa, MIXA) + k_dots(j + 2, 1, st, qa, MIX) \
                + q_dots(jnp.minimum(j + 3, NP - 1), st, qa) \
                + o_dots(j, jnp.maximum(j - 1, 0), st, [0, 1]) + xa
            issue = times(dots)
            tail_hooks(j + 2, st, hooks, A_SEG0)
            hooks["need", A_SEG0] = 12
            hooks["dot", 24] = [lambda: stash_b(j + 2, st["s", 1])]
        run_block(j + 1, xrows, dots, issue, 0, hooks, CPOL if last else CPO)
        put_o(j + 1, o)
        return st["acc"]

    x = lax.fori_loop(0, NP - 2, body2, x)
    x = lax.cond(zs[0] == 0, lambda v: body2(NP - 2, v, True), lambda v: v, x)

    st = {"acc": x}
    run_all(x_dots(NP - 1, 0, XROWS_LAST[0], lambda T: ku[(NP - 1) * GP + 3, _vr(S_PA + T), :]))
    o = reduce_pair(NP - 1, XROWS_LAST, True)
    run_all(o_dots(NP - 1, NP - 2, st))
    for n in range(NP - 3 - NLATE, NP - 3):
        run_all(o_dots(n + 1, n, st, [2]))
    put_o(NP, o)
    run_all(o_dots(NP, NP - 1, st))
    x = st["acc"]

    xl = _rows16(x, ones)
    d = xl[0:8].astype(f32) - mean
    md = _mean(d)
    r1 = lax.rsqrt(jnp.maximum(_mean(d * d) - md * md, 0.0) + EPS)
    mean = mean + md
    y = (d - md) * r1
    my = _mean(y)
    r2 = lax.rsqrt(jnp.maximum(_mean(y * y) - my * my, 0.0) + EPS)
    h = jnp.dot(xl, w3[...], preferred_element_type=f32)
    h = h[0:8] * (r1 * r2) - h[8:16] * ((mean * r1 + my) * r2)
    h = jax.nn.gelu(h, approximate=True).astype(bf16)
    x = x + y
    for k in range(0, F, 128):
        x = x + jnp.dot(h[:, k:k + 128], w4[k:k + 128, :], preferred_element_type=f32)
    o_ref[...] = x[0:1].astype(o_ref.dtype)


def _cache_view(c):
    s = c.shape[2]
    c = jnp.transpose(c, (0, 1, 3, 2)).reshape(H * DH // 8, 8, s // 128, 128)
    return jnp.transpose(c, (0, 2, 1, 3)).reshape(H * DH // 8, s // 128 * 8, 128)


def _weight_view(w):
    k, n = w.shape
    w = jnp.transpose(w.reshape(k // 16, 2, 8, n // 128, 128), (0, 1, 3, 2, 4))
    return w.reshape(k // 16, n // 128, 16, 128)


@jax.jit
def pallas_interleave_layers__sliding_block_cached__mixer_s_mlp__decode_kernel(
    A_x: jax.Array,
    A_k_cache: jax.Array,
    A_v_cache: jax.Array,
    A_wq: jax.Array,
    A_wo: jax.Array,
    B_x: jax.Array,
    B_w1: jax.Array,
    B_w2: jax.Array,
    B_w3: jax.Array,
    B_w4: jax.Array,
):
    sk = A_k_cache.shape[2]
    win = min(4096, max(256, sk // 4))
    assert win == 4096 and sk % 128 == 0
    assert A_x.shape == (1, 1, D) and A_k_cache.shape == (1, H, sk, DH)
    wt = win // 128
    t0 = sk // 128 - wt
    ng = H * DH // 8
    hbm = pl.BlockSpec(memory_space=pl.ANY)
    out = pl.pallas_call(
        functools.partial(_kernel, t0=t0, wt=wt),
        out_shape=jax.ShapeDtypeStruct((1, D), A_x.dtype),
        in_specs=[hbm] * 7,
        out_specs=pl.BlockSpec(memory_space=pltpu.VMEM),
        scratch_shapes=[
            pltpu.VMEM((ng, wt * 8, 128), bf16),
            pltpu.VMEM((ng, wt * 8, 128), bf16),
            pltpu.VMEM((ng // 4, 128, 128), u32),
            pltpu.VMEM((D // 16, H * DH // 128, 16, 128), bf16),
            pltpu.VMEM((H * DH // 16, D // 128, 16, 128), bf16),
            pltpu.VMEM((D, F), bf16),
            pltpu.VMEM((F, D), bf16),
            pltpu.VMEM((1, D), bf16),
            pltpu.VMEM((72, 128), u32),
            pltpu.VMEM((24 * (NP + 1) + 32, 128), u32),
            pltpu.VMEM((80, 128), u32),
            pltpu.VMEM((80, 128), u32),
            pltpu.VMEM((16, 128), f32),
            pltpu.SMEM((1,), jnp.int32),
        ] + [pltpu.VMEM((72, 128), f32)] * 8,
        compiler_params=pltpu.CompilerParams(vmem_limit_bytes=128 * 1024 * 1024),
    )(A_x.reshape(1, D), _cache_view(A_k_cache), _cache_view(A_v_cache),
      _weight_view(A_wq), _weight_view(A_wo), B_w3, B_w4)
    return out.reshape(1, 1, D)
```

```python
import functools

import jax
import jax.numpy as jnp
from jax import lax
import jax.experimental.pallas as pl
import jax.experimental.pallas.tpu as pltpu

D = 640
H = 32
DH = 192
F = 1536
EPS = 1e-5
NP = H // 2
GP = 2 * DH // 8
HI = 0xFFFF0000
CEXP = DH ** -0.5 * 1.4426950408889634

f32 = jnp.float32
bf16 = jnp.bfloat16
u32 = jnp.uint32

L_Y = 0
L_DUMMY = 5
S_MAXB, S_LB, S_INVA, S_X, S_PA = 4, 5, 6, 7, 9
XROWS = ((10, 18, 26), ())
XROWS_LAST = (tuple(range(0, 32, 2)), tuple(range(2, 32, 4)))
GX = (0, 16)
CPO = 24.73 / 88
CPO0 = 22.8 / 88
CPOL = 24.2 / 88
RATEL = 8
LAT = 138
B_SEG0 = 9
B_SEGL = 9
NLATE = 0
LAG = -25
MIX = (0, 1, 8, 2, 3, 9, 4, 5, 10, 6, 7, 11)
LAT2 = 155
MIXA = (0, 1, 2, 3, 4, 8, 5, 9, 6, 10, 7, 11)
TIEG = 2
TIEH = True
LAGL = 0
DA0 = 32
DB0 = 43
TV0 = 960
B0_SEG = 13
A1_SEG = 34
A_SEG0 = 40
W4_CHUNKS = (1024, 384, 128)


def _mean(x):
    return jnp.mean(x, axis=-1, keepdims=True)


def _ln(x):
    c = x - _mean(x)
    return c * lax.rsqrt(_mean(c * c) + EPS)


def _wtile(wu, rows, nt):
    blk = wu[rows, nt]
    return pltpu.bitcast(blk.reshape(blk.shape[0] * 8, 128), bf16)


def _wcols(wu, rows, nts):
    return jnp.concatenate([_wtile(wu, rows, n) for n in nts], axis=1)


def _rows16(a, b):
    return jnp.concatenate([a, b], axis=0).astype(bf16)


def _slot(G, t):
    j = 4 * (t >> 3) + ((((t >> 1) & 3) + G + 2 * (t & 1) + (t >> 3)) & 3)
    return 2 * G + (t & 1), 8 * j


def _xslot(G, t):
    return G // 2, 8 * (4 * (t >> 3) + ((((t >> 1) & 3) + G + (t >> 3)) & 3))


def _vr(n):
    return slice(8 * n, 8 * n + 8)


def _kernel(*refs, t0, wt):
    pl.run_scoped(functools.partial(_body, refs, t0, wt),
                  pltpu.SemaphoreType.DMA((4 + len(W4_CHUNKS) + 2 * NP,)))


def _body(refs, t0, wt, sems):
    (x_hbm, k_hbm, v_hbm, wq_hbm, wo_hbm, w3_hbm, w4_hbm, o_ref,
     kbuf, vbuf, vx, wq, wo, w3, w4, xbuf, lref, obuf, qa, qb, scl, zs) = refs[:22]
    pT = refs[22:]
    ku = kbuf.bitcast(u32)
    vu = vbuf.bitcast(u32)
    wqu = wq.bitcast(u32)
    wou = wo.bitcast(u32)

    x_cp = pltpu.make_async_copy(x_hbm, xbuf, sems.at[0])
    wq_cp = pltpu.make_async_copy(wq_hbm, wq, sems.at[1])
    wo_cp = pltpu.make_async_copy(wo_hbm, wo, sems.at[2])
    w3_cp = pltpu.make_async_copy(w3_hbm, w3, sems.at[3])
    w4_rows, r0 = [], 0
    for n in W4_CHUNKS:
        w4_rows.append((r0, r0 + n))
        r0 += n
    w4_cp = [pltpu.make_async_copy(w4_hbm.at[a:b], w4.at[a:b], sems.at[4 + c])
             for c, (a, b) in enumerate(w4_rows)]
    S0 = 4 + len(W4_CHUNKS)

    def k_cp(i):
        return pltpu.make_async_copy(
            k_hbm.at[pl.ds(i * GP, GP), pl.ds(t0 * 8, wt * 8), :],
            kbuf.at[pl.ds(i * GP, GP)], sems.at[S0 + i])

    def v_cp(i):
        return pltpu.make_async_copy(
            v_hbm.at[pl.ds(i * GP, GP), pl.ds(t0 * 8, wt * 8), :],
            vbuf.at[pl.ds(i * GP, GP)], sems.at[S0 + NP + i])

    for c in (wq_cp, x_cp, wo_cp):
        c.start()
    for i in range(NP):
        k_cp(i).start()
        v_cp(i).start()
    for c in [w3_cp] + w4_cp:
        c.start()

    zs[0] = 0
    qa[_vr(5), :] = jnp.zeros((8, 128), u32)

    lane = lax.broadcasted_iota(jnp.int32, (8, 128), 1)
    sub = lax.broadcasted_iota(jnp.int32, (8, 128), 0)
    lane_lo = lane < 64
    sub_lo = sub < 4

    def tile(ref, g0, G, t):
        g, r = _slot(G, t)
        return ref[g0 + g, r:r + 8, :]

    def retile(ref, i, expand):
        def body(c, carry):
            g0 = i * GP + 8 * c
            for G in range(4):
                for J in range(4):
                    xs = [[ref[g0 + 2 * G + e, _vr(4 * J + jj), :] for jj in range(4)]
                          for e in range(2)]
                    for jj in range(4):
                        x0, x1 = xs[0][jj], xs[1][jj]
                        ys = (jnp.where(sub_lo, x0, pltpu.roll(x1, 4, 0)),
                              jnp.where(sub_lo, pltpu.roll(x0, 4, 0), x1))
                        for e in range(2):
                            t = 8 * J + 2 * jj + e
                            g, r = _slot(G, t)
                            if expand and G % 2 and e:
                                ref[g0 + g, r:r + 8, :] = ys[e] << 16
                                g, r = _xslot(G, t)
                                vx[i * (GP // 4) + 2 * c + g, r:r + 8, :] = ys[e] & jnp.uint32(HI)
                            else:
                                ref[g0 + g, r:r + 8, :] = ys[e]
            return carry
        lax.fori_loop(0, GP // 8, body, 0)

    def retile_w(wu, unroll):
        nt = wu.shape[1]

        def body(c, carry):
            for u in range(unroll):
                G = c * unroll + u
                xs = [wu[G, n] for n in range(nt)]
                for n in range(nt):
                    lo, hi = xs[n // 2], xs[(nt + n) // 2]
                    if n % 2:
                        lo = pltpu.roll(lo, 4, 0)
                    if (nt + n) % 2 == 0:
                        hi = pltpu.roll(hi, 4, 0)
                    wu[G, n] = jnp.where(sub_lo, lo, hi)
            return carry
        lax.fori_loop(0, wu.shape[0] // unroll, body, 0)

    def lhs_at(ref, n):
        return pltpu.bitcast(ref[_vr(n), :], bf16)

    cur = [None]

    def new_block():
        cur[0] = -8 * jnp.clip(zs[0], 0, 1)

    def tick(ref, n, val):
        if val.dtype != ref.dtype:
            val = pltpu.bitcast(val, ref.dtype)
        ref[pl.ds(pl.multiple_of(cur[0] + 8 * n, 8), 8), :] = val

    def q_dots(i, st, qref, lhs=None, mean=None):
        def step(k):
            def run(tied=False):
                w = _wcols(wqu, _vr(k), [3 * i + n for n in range(3)])
                if lhs is None:
                    r = jnp.dot(lhs_at(lref, L_Y + k), w, preferred_element_type=f32)[0:8]
                else:
                    r = jnp.dot(lhs[:, 128 * k:128 * k + 128], w, preferred_element_type=f32)
                st["q"] = r if k == 0 else st["q"] + r
                if k == 4:
                    q = st["q"] if lhs is None else st["q"][0:8] - mean * st["q"][8:16]
                    qq = pltpu.bitcast(q.astype(bf16).astype(f32), u32)
                    q0, q1, q2 = qq[:, 0:128], qq[:, 128:256], qq[:, 256:384]
                    for n, v in enumerate((q0 >> 16, q0, q2 >> 16, q2, q1)):
                        qref[_vr(n), :] = v
                return r[0:8, 256:384]
            return 3, lref, L_DUMMY, run
        return [step(k) for k in range(5)]

    def o_dots(slot, i, st, chunks=range(3)):
        def step(b):
            def run(tied=False):
                w = _wcols(wou, pl.ds(i * (GP // 2) + 8 * b, 8), range(5))
                lhs = obuf[pl.ds(pl.multiple_of(24 * slot + 8 * b, 8), 8), :]
                r = jnp.dot(pltpu.bitcast(lhs, bf16), w, preferred_element_type=f32)[0:8]
                st["acc"] = st["acc"] + r
                return r[:, 512:640]
            return 5, obuf, 3 * (NP + 1), run
        return [step(b) for b in chunks]

    def mid_q(st, qref):
        q1 = qref[_vr(4), :]
        q1r = pltpu.roll(q1, 64, 1)
        st["u", 0] = jnp.where(lane_lo, q1 >> 16, q1r)
        st["u", 1] = jnp.where(lane_lo, q1r >> 16, q1)

    def k_dots(i, hh, st, qref, order=tuple(range(12))):
        g0 = i * GP
        gf, gh = ((0, 8), (16, 12))[hh]

        def step(r):
            def run(tied=False):
                if r < 8:
                    cols = [[tile(ku, g0, gf + G, 8 * T + r) for G in range(8)] for T in range(4)]
                    base, row = qref[_vr(2 * hh + r % 2), :], r // 2
                else:
                    cols = [[tile(ku, g0, gh + G % 4, 8 * T + 2 * (r - 8) + G // 4)
                             for G in range(8)] for T in range(4)]
                    if r == 8 and hh == 0 and "pre" not in st:
                        mid_q(st, qref)
                    base, row = st["u", hh], r - 8
                    if tied:
                        base = base | qref[_vr(5), :]
                lhs = jnp.where(sub == row, base, jnp.zeros((8, 128), u32))
                w = jnp.concatenate([jnp.concatenate(c, axis=0) for c in cols], axis=1)
                res = jnp.dot(pltpu.bitcast(lhs, bf16), pltpu.bitcast(w, bf16),
                              preferred_element_type=f32)[0:8]
                st["s", hh] = res if r == order[0] else st["s", hh] + res
                return res[:, 384:512]
            return 4, (qref if r < 8 or TIEH else None), 6, run
        return [step(r) for r in order]

    def col(s, T):
        return s[:, 128 * T:128 * T + 128]

    def row_max(s):
        m = jnp.maximum(jnp.maximum(col(s, 0), col(s, 1)), jnp.maximum(col(s, 2), col(s, 3)))
        return jnp.max(jnp.max(m, axis=1, keepdims=True), axis=0, keepdims=True)

    def prob(s, m):
        return jnp.exp2((s - m) * scl[_vr(0), :])

    def put_p(hh, T, p, ks=range(8)):
        for k in ks:
            pT[4 * hh + T][pl.ds(k, 8, stride=8), :] = p

    def part_sum(p):
        return (p[0] + p[1]) + (p[2] + p[3])

    def inv_sum(l):
        l = jnp.sum(jnp.sum(l, axis=1, keepdims=True), axis=0, keepdims=True)
        return jnp.broadcast_to(1.0 / l, (8, 128))

    def softmax(s, hh):
        m = row_max(s)
        p = [prob(col(s, T), m) for T in range(4)]
        for T in range(4):
            put_p(hh, T, p[T])
        return p, part_sum(p)

    def get_state(i, n):
        return pltpu.bitcast(ku[i * GP + 3, _vr(n), :], f32)

    def set_state(i, n, v):
        ku[i * GP + 3, _vr(n), :] = pltpu.bitcast(v, u32)

    def stash_b(i, s):
        for T in range(4):
            set_state(i, T, col(s, T))
        m = jnp.broadcast_to(row_max(s), (8, 128))
        set_state(i, S_MAXB, m)
        return m

    def pack_p(p):
        return pltpu.bitcast(_rows16(p, p), u32)

    def x_dots(i, hh, ts, get_lhs):
        st = {}
        rows = sorted({t % 8 for t in ts})

        def step(n, rho):
            def run(tied=False):
                res = []
                for T in [t // 8 for t in ts if t % 8 == rho]:
                    w = jnp.concatenate(
                        [tile(vu, i * GP, GX[hh] + G, 8 * T + rho) for G in range(8)], axis=0)
                    res.append(jnp.dot(pltpu.bitcast(get_lhs(T), bf16), pltpu.bitcast(w, bf16),
                                       preferred_element_type=f32)[0:8])
                st["x"] = jnp.where(sub == rho, sum(res[1:], res[0]), st["x"] if n else 0.0)
                if n == len(rows) - 1:
                    set_state(i, S_X + hh, st["x"])
                return res[-1]
            return sum(1 for t in ts if t % 8 == rho), None, 0, run
        return [step(n, rho) for n, rho in enumerate(rows)]

    def transpose_x(i, xrows):
        for hh in range(2):
            for t in xrows[hh]:
                w = jnp.concatenate([tile(vu, i * GP, GX[hh] + G, t) for G in range(8)], axis=0)
                w = pltpu.bitcast(pltpu.bitcast(w, bf16).astype(f32).T.astype(bf16), u32)
                for G in range(8):
                    g, r = _slot(GX[hh] + G, t)
                    vu[i * GP + g, r:r + 8, :] = w[_vr(G), :]

    def reduce_o(blocks, inva, invb, extra=(None, None, None)):
        out = []
        for b, inv in enumerate((inva, jnp.where(lane_lo, inva, invb), invb)):
            z = jnp.sum(pltpu.bitcast(blocks[b], f32).T.reshape(16, 8, 128), axis=0)
            if extra[b] is not None:
                z = z + extra[b]
            o = jnp.sum(z, axis=0, keepdims=True) * inv
            out.append(pltpu.bitcast(_rows16(o, o), u32))
        return out

    def put_o(slot, o):
        for b in range(3):
            obuf[pl.ds(pl.multiple_of(24 * slot + 8 * b, 8), 8), :] = o[b]

    def mac(acc, n, c, G, t, pv):
        w = tile(vu, 8 * c, G, t)
        if G % 2 and t % 2:
            g, r = _xslot(G, t)
            halves = (w, vx[2 * c + g, r:r + 8, :])
        else:
            halves = (w << 16, w & jnp.uint32(HI))
        for k in range(2):
            a = pltpu.bitcast(halves[k], f32) * pv
            acc[n + k] = a if acc[n + k] is None else acc[n + k] + a

    def run_block(i, xrows, dots, issue, tv0, hooks, cpo, rev=True, lag=0):
        clock = []
        tie = {}

        def emit(upto):
            while len(clock) < upto:
                n = len(clock)
                for h in hooks.get(("dot", n), ()):
                    h()
                clock.append(dots[n][3](n in tie.values()))

        def seg_rows(hh, gp, T):
            on_mxu = GX[hh] <= 12 * hh + 2 * gp < GX[hh] + 8
            return [rho for rho in range(8) if not (on_mxu and 8 * T + rho in xrows[hh])]

        at = [tv0]
        for seg in range(48):
            at.append(at[-1] + cpo * sum(10 if rho % 2 else 12
                                         for rho in seg_rows(seg // 24, seg % 24 // 4, seg % 4)))
        for seg in range(TIEG - 1, 48 if rev else 0, TIEG):
            ok = [n for n, c in enumerate(issue)
                  if dots[n][1] is not None and c >= at[seg + 1] + lag]
            if ok:
                tie[seg] = ok[0]
        zero = jnp.zeros((8, 128), f32)
        used = {}
        seg = 0
        for hh in range(2):
            for gp in range(6):
                a4 = [None] * 4
                for T in range(4):
                    pref = pT[4 * hh + T]
                    grp = seg - seg % TIEG + TIEG - 1
                    upto = (tie.get(grp, len(dots)) if rev
                            else sum(1 for c in issue if c < at[seg + 1] + 12))
                    upto = min([upto] + [k[1] for k, v in hooks.items()
                                         if k[0] == "after" and v >= seg])
                    emit(max(upto, hooks.get(("need", seg), 0)))
                    done = sum(1 for c in issue if c + (LAT2 if rev else LAT) <= at[seg])
                    done = min(max(1, done), len(clock))
                    if grp not in tie:
                        tick(pref, 8, clock[done - 1])
                    elif gp:
                        tick(pref, 8, zero)
                    for h in hooks.get(("seg", seg), ()):
                        h(clock[done - 1])
                    for rho in seg_rows(hh, gp, T):
                        pv = pref[_vr(rho), :]
                        for e in range(2):
                            mac(a4, 2 * e, i * 6, 12 * hh + 2 * gp + e, 8 * T + rho, pv)
                    if seg in tie and (T == 3 or tie.get(seg + TIEG) != tie[seg]):
                        _, ref, slot, _ = dots[tie[seg]]
                        used[tie[seg]] = used.get(tie[seg], -1) + 1
                        for k in range(4):
                            tick(ref, slot + 4 * used[tie[seg]] + k, a4[k])
                    seg += 1
                for n in range(4):
                    G = 12 * hh + 2 * gp + n // 2
                    ku[i * GP + G // 8, pl.ds(16 * (G % 8) + n % 2, 8, stride=2), :] = (
                        pltpu.bitcast(a4[n], u32))
        emit(len(dots))

    def times(dots, t=0, rate=8):
        out = []
        for d in dots:
            t += rate * d[0]
            out.append(t)
        return out

    def run_all(dots):
        for d in dots:
            d[3]()

    def set_input(c, scale):
        cp = pltpu.bitcast(_rows16(c, c), u32)
        for k in range(5):
            lref[_vr(L_Y + k), :] = cp[:, 128 * k:128 * k + 128]
        scl[_vr(0), :] = jnp.broadcast_to(scale, (8, 128))

    x_cp.wait()
    x = jnp.broadcast_to(xbuf[...].astype(f32), (8, D))
    set_input(_ln(x), jnp.full((8, 1), CEXP, f32))
    wq_cp.wait()
    retile_w(wqu, 1)
    wo_cp.wait()
    retile_w(wou, 8)

    def body1(i, acc):
        st = {"acc": acc}
        k_cp(i).wait()
        retile(ku, i, False)
        run_all(q_dots(i, st, qa))
        inv = []
        for hh in range(2):
            run_all(k_dots(i, hh, st, qa))
            inv.append(inv_sum(softmax(st["s", hh], hh)[1]))

        @pl.when(i > 1)
        def _():
            transpose_x(i - 1, XROWS)

        v_cp(i).wait()
        retile(vu, i, True)
        for hh in range(2):
            def pv_step(c, carry, hh=hh):
                acc8 = [None] * 8
                for t in range(32):
                    pv = pT[4 * hh + t // 8][_vr(t % 8), :]
                    for G in range(4):
                        mac(acc8, 2 * G, i * 6 + c, G, t, pv)
                for n in range(8):
                    obuf[pl.ds(64 * c + 16 * (n // 2) + n % 2, 8, stride=2), :] = (
                        pltpu.bitcast(acc8[n], u32))
                return carry
            lax.fori_loop(3 * hh, 3 * hh + 3, pv_step, 0)
        put_o(NP, reduce_o([obuf[128 * b:128 * b + 128, :] for b in range(3)], inv[0], inv[1]))
        run_all(o_dots(NP, i, st))
        return st["acc"]

    x = lax.fori_loop(0, NP, body1, x)

    y = _ln(x)
    zz = _ln(y).astype(bf16)
    w3_cp.wait()
    h = jnp.dot(zz, w3[...], preferred_element_type=f32)
    h = jax.nn.gelu(h, approximate=True).astype(bf16)
    x = x + y
    transpose_x(NP - 1, XROWS_LAST)
    for cp, (a, b) in zip(w4_cp, w4_rows):
        cp.wait()
        x = x + jnp.dot(h[:, a:b], w4[a:b, :], preferred_element_type=f32)

    ones = jnp.ones((8, D), f32)
    xl = _rows16(x, ones)
    xb = xl[0:8].astype(f32)
    mean = _mean(xb)
    c = xb - mean
    set_input(c, lax.rsqrt(_mean(c * c) + EPS) * CEXP)
    obuf[0:24, :] = jnp.zeros((24, 128), u32)

    def tail_hooks(i, st, hooks, seg0):
        def first(_):
            m = row_max(st["s", 0])
            st["pa"] = [prob(col(st["s", 0], T), m) for T in range(4)]
            set_state(i, S_INVA, inv_sum(part_sum(st["pa"])))
            for T in range(4):
                ku[i * GP + 3, _vr(S_PA + T), :] = pack_p(st["pa"][T])

        def put(T, half):
            def run(clk):
                tick(pT[T], 8, clk)
                put_p(0, T, st["pa"][T], range(4 * half, 4 * half + 4))
            return run
        hooks.setdefault(("seg", seg0), []).append(first)
        for n in range(8):
            hooks.setdefault(("seg", seg0 + n), []).append(put(n // 2, n % 2))

    def head_b_hooks(i, seg0, pb, final=False):
        def put_b(T):
            def run(clk):
                tick(scl, 1, clk)
                pb.append(prob(get_state(i, T), get_state(i, S_MAXB)))
                put_p(1, T, pb[T])
                if T == 3:
                    set_state(i, S_LB, inv_sum(part_sum(pb)) if final else part_sum(pb))
            return run
        return {("seg", seg0 + 3 * T): [put_b(T)] for T in range(4)}

    def reduce_pair(i, xrows, final=False):
        xa, xb = (get_state(i, S_X + hh) if xrows[hh] else None for hh in range(2))
        invb = get_state(i, S_LB) if final else inv_sum(get_state(i, S_LB))
        return reduce_o([ku[i * GP + b] for b in range(3)],
                        get_state(i, S_INVA), invb, (xa, None, xb))

    st = {}
    new_block()
    late = tuple(range(8, 12)) + tuple(range(8))
    d0 = q_dots(0, st, qb, xl, mean) + q_dots(1, st, qa, xl, mean)
    d1 = k_dots(0, 0, st, qb) + k_dots(0, 1, st, qb, late) + k_dots(1, 0, st, qa, late) \
        + k_dots(1, 1, st, qa) + q_dots(2, st, qa)
    issue = times(d0 + d1)

    def sm_a0():
        m = row_max(st["s", 0])
        p = [prob(col(st["s", 0], T), m) for T in range(4)]
        tick(qb, 6, part_sum(p))
        put_p(0, 0, p[0])
        st["p0"] = p
        set_state(0, S_INVA, inv_sum(part_sum(p)))

    def put_a0(T):
        def run(clk):
            tick(pT[T], 8, clk)
            put_p(0, T, st["p0"][T])
        return run

    def sm_b0():
        tick(qa, 6, stash_b(0, st["s", 1]))

    hooks = head_b_hooks(0, B0_SEG, [])
    hooks.update({("dot", DA0): [sm_a0], ("dot", DB0): [sm_b0],
                  ("need", 0): DA0 + 1, ("need", B0_SEG): DB0 + 1, ("need", A1_SEG): 46})
    hooks.update({("seg", T): [put_a0(T + 1)] for T in range(3)})
    tail_hooks(1, st, hooks, A1_SEG)
    run_block(0, ((), ()), d0 + d1, issue, TV0, hooks, CPO0, False)
    set_state(0, S_X, jnp.zeros((8, 128), f32))
    stash_b(1, st["s", 1])

    def body2(j, acc, last=False):
        new_block()
        st = {"acc": acc, "pre": True}
        if not last:
            mid_q(st, qa)
        o = reduce_pair(j, XROWS)
        pb = []
        hooks = head_b_hooks(j + 1, B_SEGL if last else B_SEG0, pb, last)
        xrows = XROWS_LAST if last else XROWS
        xa = x_dots(j + 1, 0, xrows[0], lambda T: ku[(j + 1) * GP + 3, _vr(S_PA + T), :])
        if last:
            dots = o_dots(NP - 2, NP - 3, st)
            for n in range(NP - 3):
                dots += o_dots(n + 1, n, st, [2])
            dots = dots[:len(dots) - NLATE]
            hooks["after", len(dots)] = B_SEGL + 9
            dots += x_dots(j + 1, 1, xrows[1], lambda T: pack_p(pb[T]))
            issue = times(dots, rate=RATEL)
        else:
            dots = k_dots(j + 2, 0, st, qa, MIXA) + k_dots(j + 2, 1, st, qa, MIX) \
                + q_dots(jnp.minimum(j + 3, NP - 1), st, qa) \
                + o_dots(j, jnp.maximum(j - 1, 0), st, [0, 1]) + xa
            issue = times(dots)
            tail_hooks(j + 2, st, hooks, A_SEG0)
            hooks["need", A_SEG0] = 12
            hooks["dot", 24] = [lambda: stash_b(j + 2, st["s", 1])]
        run_block(j + 1, xrows, dots, issue, 0, hooks, CPOL if last else CPO, True, LAGL if last else LAG)
        put_o(j + 1, o)
        return st["acc"]

    x = lax.fori_loop(0, NP - 2, body2, x)
    x = lax.cond(zs[0] == 0, lambda v: body2(NP - 2, v, True), lambda v: v, x)

    st = {"acc": x}
    run_all(x_dots(NP - 1, 0, XROWS_LAST[0], lambda T: ku[(NP - 1) * GP + 3, _vr(S_PA + T), :]))
    o = reduce_pair(NP - 1, XROWS_LAST, True)
    run_all(o_dots(NP - 1, NP - 2, st))
    for n in range(NP - 3 - NLATE, NP - 3):
        run_all(o_dots(n + 1, n, st, [2]))
    put_o(NP, o)
    run_all(o_dots(NP, NP - 1, st))
    x = st["acc"]

    xl = _rows16(x, ones)
    d = xl[0:8].astype(f32) - mean
    md = _mean(d)
    r1 = lax.rsqrt(jnp.maximum(_mean(d * d) - md * md, 0.0) + EPS)
    mean = mean + md
    y = (d - md) * r1
    my = _mean(y)
    r2 = lax.rsqrt(jnp.maximum(_mean(y * y) - my * my, 0.0) + EPS)
    h = jnp.dot(xl, w3[...], preferred_element_type=f32)
    h = h[0:8] * (r1 * r2) - h[8:16] * ((mean * r1 + my) * r2)
    h = jax.nn.gelu(h, approximate=True).astype(bf16)
    x = x + y
    for k in range(0, F, 128):
        x = x + jnp.dot(h[:, k:k + 128], w4[k:k + 128, :], preferred_element_type=f32)
    o_ref[...] = x[0:1].astype(o_ref.dtype)


def _cache_view(c):
    s = c.shape[2]
    c = jnp.transpose(c, (0, 1, 3, 2)).reshape(H * DH // 8, 8, s // 128, 128)
    return jnp.transpose(c, (0, 2, 1, 3)).reshape(H * DH // 8, s // 128 * 8, 128)


def _weight_view(w):
    k, n = w.shape
    w = jnp.transpose(w.reshape(k // 16, 2, 8, n // 128, 128), (0, 1, 3, 2, 4))
    return w.reshape(k // 16, n // 128, 16, 128)


@jax.jit
def pallas_interleave_layers__sliding_block_cached__mixer_s_mlp__decode_kernel(
    A_x: jax.Array,
    A_k_cache: jax.Array,
    A_v_cache: jax.Array,
    A_wq: jax.Array,
    A_wo: jax.Array,
    B_x: jax.Array,
    B_w1: jax.Array,
    B_w2: jax.Array,
    B_w3: jax.Array,
    B_w4: jax.Array,
):
    sk = A_k_cache.shape[2]
    win = min(4096, max(256, sk // 4))
    assert win == 4096 and sk % 128 == 0
    assert A_x.shape == (1, 1, D) and A_k_cache.shape == (1, H, sk, DH)
    wt = win // 128
    t0 = sk // 128 - wt
    ng = H * DH // 8
    hbm = pl.BlockSpec(memory_space=pl.ANY)
    out = pl.pallas_call(
        functools.partial(_kernel, t0=t0, wt=wt),
        out_shape=jax.ShapeDtypeStruct((1, D), A_x.dtype),
        in_specs=[hbm] * 7,
        out_specs=pl.BlockSpec(memory_space=pltpu.VMEM),
        scratch_shapes=[
            pltpu.VMEM((ng, wt * 8, 128), bf16),
            pltpu.VMEM((ng, wt * 8, 128), bf16),
            pltpu.VMEM((ng // 4, 128, 128), u32),
            pltpu.VMEM((D // 16, H * DH // 128, 16, 128), bf16),
            pltpu.VMEM((H * DH // 16, D // 128, 16, 128), bf16),
            pltpu.VMEM((D, F), bf16),
            pltpu.VMEM((F, D), bf16),
            pltpu.VMEM((1, D), bf16),
            pltpu.VMEM((136, 128), u32),
            pltpu.VMEM((24 * (NP + 1) + 96, 128), u32),
            pltpu.VMEM((144, 128), u32),
            pltpu.VMEM((144, 128), u32),
            pltpu.VMEM((16, 128), f32),
            pltpu.SMEM((1,), jnp.int32),
        ] + [pltpu.VMEM((72, 128), f32)] * 8,
        compiler_params=pltpu.CompilerParams(vmem_limit_bytes=128 * 1024 * 1024),
    )(A_x.reshape(1, D), _cache_view(A_k_cache), _cache_view(A_v_cache),
      _weight_view(A_wq), _weight_view(A_wo), B_w3, B_w4)
    return out.reshape(1, 1, D)
```

```python
import functools

import jax
import jax.numpy as jnp
from jax import lax
import jax.experimental.pallas as pl
import jax.experimental.pallas.tpu as pltpu

D = 640
H = 32
DH = 192
F = 1536
EPS = 1e-5
NP = H // 2
GP = 2 * DH // 8
HI = 0xFFFF0000
CEXP = DH ** -0.5 * 1.4426950408889634

f32 = jnp.float32
bf16 = jnp.bfloat16
u32 = jnp.uint32

L_Y = 0
L_DUMMY = 5
S_MAXB, S_LB, S_INVA, S_X, S_PA = 4, 5, 6, 7, 9
XROWS = ((10, 18, 26), ())
XROWS_LAST = (tuple(range(0, 32, 2)), tuple(range(2, 32, 4)))
GX = (0, 16)
CPO = 24.73 / 88
CPO0 = 22.8 / 88
CPOL = 24.2 / 88
RATEL = 8
LAT = 138
B_SEG0 = 9
B_SEGL = 9
NLATE = 0
LAG = -25
MIX = (0, 1, 8, 2, 3, 9, 4, 5, 10, 6, 7, 11)
LAT2 = 155
MIXA = (0, 1, 2, 3, 4, 8, 5, 9, 6, 10, 7, 11)
TIEG = 2
FREE = ()
TIEX = True
TIEH = True
LAGL = 0
DA0 = 32
DB0 = 43
TV0 = 960
B0_SEG = 13
A1_SEG = 34
A_SEG0 = 40
W4_CHUNKS = (1024, 384, 128)


def _mean(x):
    return jnp.mean(x, axis=-1, keepdims=True)


def _ln(x):
    c = x - _mean(x)
    return c * lax.rsqrt(_mean(c * c) + EPS)


def _wtile(wu, rows, nt):
    blk = wu[rows, nt]
    return pltpu.bitcast(blk.reshape(blk.shape[0] * 8, 128), bf16)


def _wcols(wu, rows, nts):
    return jnp.concatenate([_wtile(wu, rows, n) for n in nts], axis=1)


def _rows16(a, b):
    return jnp.concatenate([a, b], axis=0).astype(bf16)


def _slot(G, t):
    j = 4 * (t >> 3) + ((((t >> 1) & 3) + G + 2 * (t & 1) + (t >> 3)) & 3)
    return 2 * G + (t & 1), 8 * j


def _xslot(G, t):
    return G // 2, 8 * (4 * (t >> 3) + ((((t >> 1) & 3) + G + (t >> 3)) & 3))


def _vr(n):
    return slice(8 * n, 8 * n + 8)


def _kernel(*refs, t0, wt):
    pl.run_scoped(functools.partial(_body, refs, t0, wt),
                  pltpu.SemaphoreType.DMA((4 + len(W4_CHUNKS) + 2 * NP,)))


def _body(refs, t0, wt, sems):
    (x_hbm, k_hbm, v_hbm, wq_hbm, wo_hbm, w3_hbm, w4_hbm, o_ref,
     kbuf, vbuf, vxbuf, wqu, wo, w3, w4, xbuf, lref, obuf, qa, qb, scl, abuf, zs) = refs[:23]
    pT = refs[23:]
    ku = kbuf.bitcast(u32)
    vu = vbuf.bitcast(u32)
    vx = vxbuf.bitcast(u32)
    wou = wo.bitcast(u32)

    x_cp = pltpu.make_async_copy(x_hbm, xbuf, sems.at[0])
    wq_cp = pltpu.make_async_copy(wq_hbm, vxbuf.at[0:D * 3 // 16], sems.at[1])
    wo_cp = pltpu.make_async_copy(wo_hbm, wo, sems.at[2])
    w3_cp = pltpu.make_async_copy(w3_hbm, w3, sems.at[3])
    w4_rows, r0 = [], 0
    for n in W4_CHUNKS:
        w4_rows.append((r0, r0 + n))
        r0 += n
    w4_cp = [pltpu.make_async_copy(w4_hbm.at[a:b], w4.at[a:b], sems.at[4 + c])
             for c, (a, b) in enumerate(w4_rows)]
    S0 = 4 + len(W4_CHUNKS)

    def k_cp(i):
        return pltpu.make_async_copy(
            k_hbm.at[pl.ds(i * GP, GP), pl.ds(t0 * 8, wt * 8), :],
            kbuf.at[pl.ds(i * GP, GP)], sems.at[S0 + i])

    def v_cp(i):
        return pltpu.make_async_copy(
            v_hbm.at[pl.ds(i * GP, GP), pl.ds(t0 * 8, wt * 8), :],
            vbuf.at[pl.ds(i * GP, GP)], sems.at[S0 + NP + i])

    for c in (wq_cp, x_cp, wo_cp):
        c.start()
    for i in range(NP):
        k_cp(i).start()
        v_cp(i).start()
    for c in [w3_cp] + w4_cp:
        c.start()

    zs[0] = 0
    qa[_vr(5), :] = jnp.zeros((8, 128), u32)

    lane = lax.broadcasted_iota(jnp.int32, (8, 128), 1)
    sub = lax.broadcasted_iota(jnp.int32, (8, 128), 0)
    lane_lo = lane < 64
    sub_lo = sub < 4

    def tile(ref, g0, G, t):
        g, r = _slot(G, t)
        return ref[g0 + g, r:r + 8, :]

    def retile(ref, i, expand):
        def body(c, carry):
            g0 = i * GP + 8 * c
            for G in range(4):
                for J in range(4):
                    xs = [[ref[g0 + 2 * G + e, _vr(4 * J + jj), :] for jj in range(4)]
                          for e in range(2)]
                    for jj in range(4):
                        x0, x1 = xs[0][jj], xs[1][jj]
                        ys = (jnp.where(sub_lo, x0, pltpu.roll(x1, 4, 0)),
                              jnp.where(sub_lo, pltpu.roll(x0, 4, 0), x1))
                        for e in range(2):
                            t = 8 * J + 2 * jj + e
                            g, r = _slot(G, t)
                            if expand and G % 2 and e:
                                ref[g0 + g, r:r + 8, :] = ys[e] << 16
                                g, r = _xslot(G, t)
                                vx[i * (GP // 4) + 2 * c + g, r:r + 8, :] = ys[e] & jnp.uint32(HI)
                            else:
                                ref[g0 + g, r:r + 8, :] = ys[e]
            return carry
        lax.fori_loop(0, GP // 8, body, 0)

    def merge_halves(get, nt, n):
        lo, hi = get(n // 2), get((nt + n) // 2)
        if n % 2:
            lo = pltpu.roll(lo, 4, 0)
        if (nt + n) % 2 == 0:
            hi = pltpu.roll(hi, 4, 0)
        return jnp.where(sub_lo, lo, hi)

    def retile_wq(G, carry):
        for n in range(3 * NP):
            wqu[n // 3 * (D // 16) + G, n % 3] = merge_halves(
                lambda v: vx[3 * G + v // 16, _vr(v % 16), :], 3 * NP, n)
        return carry

    def retile_wo(c, carry):
        for G in range(8):
            xs = [wou[8 * c + G, n] for n in range(5)]
            for n in range(5):
                wou[8 * c + G, n] = merge_halves(lambda v: xs[v], 5, n)
        return carry

    def lhs_at(ref, n):
        return pltpu.bitcast(ref[_vr(n), :], bf16)

    cur = [None]

    def new_block():
        cur[0] = -8 * jnp.clip(zs[0], 0, 1)

    def tick(ref, n, val):
        if val.dtype != ref.dtype:
            val = pltpu.bitcast(val, ref.dtype)
        ref[pl.ds(pl.multiple_of(cur[0] + 8 * n, 8), 8), :] = val

    def q_dots(i, st, qref, lhs=None, mean=None):
        def step(k):
            def run(tied=False):
                w = _wcols(wqu, pl.ds(i * (D // 16) + 8 * k, 8), range(3))
                if lhs is None:
                    r = jnp.dot(lhs_at(lref, L_Y + k), w, preferred_element_type=f32)[0:8]
                else:
                    r = jnp.dot(lhs[:, 128 * k:128 * k + 128], w, preferred_element_type=f32)
                st["q"] = r if k == 0 else st["q"] + r
                if k == 4:
                    q = st["q"] if lhs is None else st["q"][0:8] - mean * st["q"][8:16]
                    qq = pltpu.bitcast(q.astype(bf16).astype(f32), u32)
                    q0, q1, q2 = qq[:, 0:128], qq[:, 128:256], qq[:, 256:384]
                    for n, v in enumerate((q0 >> 16, q0, q2 >> 16, q2, q1)):
                        qref[_vr(n), :] = v
                return r[0:8, 256:384]
            return 3, lref, L_DUMMY, run
        return [step(k) for k in range(5)]

    def o_dots(slot, i, st, chunks=range(3)):
        def step(b):
            def run(tied=False):
                w = _wcols(wou, pl.ds(i * (GP // 2) + 8 * b, 8), range(5))
                lhs = obuf[pl.ds(pl.multiple_of(24 * slot + 8 * b, 8), 8), :]
                r = jnp.dot(pltpu.bitcast(lhs, bf16), w, preferred_element_type=f32)[0:8]
                st["acc"] = st["acc"] + r if "acc" in st else r
                return r[:, 512:640]
            return 5, obuf, 3 * (NP + 1), run
        return [step(b) for b in chunks]

    def mid_q(st, qref):
        q1 = qref[_vr(4), :]
        q1r = pltpu.roll(q1, 64, 1)
        st["u", 0] = jnp.where(lane_lo, q1 >> 16, q1r)
        st["u", 1] = jnp.where(lane_lo, q1r >> 16, q1)

    def k_dots(i, hh, st, qref, order=tuple(range(12))):
        g0 = i * GP
        gf, gh = ((0, 8), (16, 12))[hh]

        def step(r):
            def run(tied=False):
                if r < 8:
                    cols = [[tile(ku, g0, gf + G, 8 * T + r) for G in range(8)] for T in range(4)]
                    base, row = qref[_vr(2 * hh + r % 2), :], r // 2
                else:
                    cols = [[tile(ku, g0, gh + G % 4, 8 * T + 2 * (r - 8) + G // 4)
                             for G in range(8)] for T in range(4)]
                    if r == 8 and hh == 0 and "pre" not in st:
                        mid_q(st, qref)
                    base, row = st["u", hh], r - 8
                    if tied:
                        base = base | qref[_vr(5), :]
                lhs = jnp.where(sub == row, base, jnp.zeros((8, 128), u32))
                w = jnp.concatenate([jnp.concatenate(c, axis=0) for c in cols], axis=1)
                res = jnp.dot(pltpu.bitcast(lhs, bf16), pltpu.bitcast(w, bf16),
                              preferred_element_type=f32)[0:8]
                st["s", hh] = res if r == order[0] else st["s", hh] + res
                return res[:, 384:512]
            return 4, (qref if r < 8 or TIEH else None), 6, run
        return [step(r) for r in order]

    def col(s, T):
        return s[:, 128 * T:128 * T + 128]

    def row_max(s):
        m = jnp.maximum(jnp.maximum(col(s, 0), col(s, 1)), jnp.maximum(col(s, 2), col(s, 3)))
        return jnp.max(jnp.max(m, axis=1, keepdims=True), axis=0, keepdims=True)

    def prob(s, m):
        return jnp.exp2((s - m) * scl[_vr(0), :])

    def put_p(hh, T, p, ks=range(8)):
        for k in ks:
            pT[4 * hh + T][pl.ds(k, 8, stride=8), :] = p

    def part_sum(p):
        return (p[0] + p[1]) + (p[2] + p[3])

    def inv_sum(l):
        l = jnp.sum(jnp.sum(l, axis=1, keepdims=True), axis=0, keepdims=True)
        r = pl.reciprocal(l, approx=True)
        return jnp.broadcast_to(r * (2.0 - l * r), (8, 128))

    def softmax(s, hh):
        m = row_max(s)
        p = [prob(col(s, T), m) for T in range(4)]
        for T in range(4):
            put_p(hh, T, p[T])
        return p, part_sum(p)

    def get_state(i, n):
        return pltpu.bitcast(ku[i * GP + 3, _vr(n), :], f32)

    def set_state(i, n, v):
        ku[i * GP + 3, _vr(n), :] = pltpu.bitcast(v, u32)

    def stash_b(i, s):
        for T in range(4):
            set_state(i, T, col(s, T))
        m = jnp.broadcast_to(row_max(s), (8, 128))
        set_state(i, S_MAXB, m)
        return m

    def pack8(v):
        return pltpu.bitcast(v.astype(bf16), u32)

    def x_dots(i, hh, ts, get_lhs):
        st = {}
        rows = sorted({t % 8 for t in ts})

        def step(n, rho):
            def run(tied=False):
                res = []
                for T in [t // 8 for t in ts if t % 8 == rho]:
                    w = jnp.concatenate(
                        [tile(vu, i * GP, GX[hh] + G, 8 * T + rho) for G in range(8)], axis=0)
                    lhs = get_lhs(T) | obuf[_vr(0), :] if tied else get_lhs(T)
                    res.append(jnp.dot(pltpu.bitcast(lhs, bf16), pltpu.bitcast(w, bf16),
                                       preferred_element_type=f32)[0:8])
                st["x"] = jnp.where(sub == rho, sum(res[1:], res[0]), st["x"] if n else 0.0)
                if n == len(rows) - 1:
                    set_state(i, S_X + hh, st["x"])
                return res[-1]
            return sum(1 for t in ts if t % 8 == rho), (obuf if TIEX else None), 3 * (NP + 1), run
        return [step(n, rho) for n, rho in enumerate(rows)]

    def transpose_x(i, xrows):
        for hh in range(2):
            for t in xrows[hh]:
                w = jnp.concatenate([tile(vu, i * GP, GX[hh] + G, t) for G in range(8)], axis=0)
                w = pltpu.bitcast(pltpu.bitcast(w, bf16).astype(f32).T.astype(bf16), u32)
                for G in range(8):
                    g, r = _slot(GX[hh] + G, t)
                    vu[i * GP + g, r:r + 8, :] = w[_vr(G), :]

    def reduce_o(blocks, inva, invb, extra=(None, None, None)):
        out = []
        for b, inv in enumerate((inva, jnp.where(lane_lo, inva, invb), invb)):
            z = jnp.sum(pltpu.bitcast(blocks[b], f32).T.reshape(16, 8, 128), axis=0)
            if extra[b] is not None:
                z = z + extra[b]
            out.append(pack8(z * inv))
        return out

    def put_o(slot, o):
        for b in range(3):
            obuf[pl.ds(pl.multiple_of(24 * slot + 8 * b, 8), 4), :] = o[b]

    def mac(acc, n, c, G, t, pv):
        w = tile(vu, 8 * c, G, t)
        if G % 2 and t % 2:
            g, r = _xslot(G, t)
            halves = (w, vx[2 * c + g, r:r + 8, :])
        else:
            halves = (w << 16, w & jnp.uint32(HI))
        for k in range(2):
            a = pltpu.bitcast(halves[k], f32) * pv
            acc[n + k] = a if acc[n + k] is None else acc[n + k] + a

    def run_block(i, xrows, dots, issue, tv0, hooks, cpo, rev=True, lag=0):
        clock = []
        tie = {}

        def emit(upto):
            while len(clock) < upto:
                n = len(clock)
                for h in hooks.get(("dot", n), ()):
                    h()
                clock.append(dots[n][3](n in tie.values()))

        def seg_rows(hh, gp, T):
            on_mxu = GX[hh] <= 12 * hh + 2 * gp < GX[hh] + 8
            return [rho for rho in range(8) if not (on_mxu and 8 * T + rho in xrows[hh])]

        at = [tv0]
        for seg in range(48):
            at.append(at[-1] + cpo * sum(10 if rho % 2 else 12
                                         for rho in seg_rows(seg // 24, seg % 24 // 4, seg % 4)))
        for seg in range(TIEG - 1, 48 if rev else 0, TIEG):
            ok = [n for n, c in enumerate(issue)
                  if dots[n][1] is not None and c >= at[seg + 1] + lag]
            if ok:
                tie[seg] = ok[0]
        zero = jnp.zeros((8, 128), f32)
        used = {}
        seg = 0
        for hh in range(2):
            for gp in range(6):
                a4 = [None] * 4
                for T in range(4):
                    pref = pT[4 * hh + T]
                    grp = seg - seg % TIEG + TIEG - 1
                    upto = (tie.get(grp, len(dots)) if rev
                            else sum(1 for c in issue if c < at[seg + 1] + 12))
                    upto = min([upto] + [k[1] for k, v in hooks.items()
                                         if k[0] == "after" and v >= seg])
                    emit(max(upto, hooks.get(("need", seg), 0)))
                    done = sum(1 for c in issue if c + (LAT2 if rev else LAT) <= at[seg])
                    done = min(max(1, done), len(clock))
                    if grp not in tie and not (rev and seg in FREE):
                        tick(pref, 8, clock[done - 1])
                    elif gp:
                        tick(pref, 8, zero)
                    for h in hooks.get(("seg", seg), ()):
                        h(clock[done - 1])
                    for rho in seg_rows(hh, gp, T):
                        pv = pref[_vr(rho), :]
                        for e in range(2):
                            mac(a4, 2 * e, i * 6, 12 * hh + 2 * gp + e, 8 * T + rho, pv)
                    if seg in tie and (T == 3 or tie.get(seg + TIEG) != tie[seg]):
                        _, ref, slot, _ = dots[tie[seg]]
                        used[tie[seg]] = used.get(tie[seg], -1) + 1
                        for k in range(4):
                            tick(ref, slot + 4 * used[tie[seg]] + k, a4[k])
                    seg += 1
                for n in range(4):
                    G = 12 * hh + 2 * gp + n // 2
                    ku[i * GP + G // 8, pl.ds(16 * (G % 8) + n % 2, 8, stride=2), :] = (
                        pltpu.bitcast(a4[n], u32))
        emit(len(dots))

    def times(dots, t=0, rate=8):
        out = []
        for d in dots:
            t += rate * d[0]
            out.append(t)
        return out

    def run_all(dots):
        for d in dots:
            d[3]()

    def set_input(c, scale):
        cp = pltpu.bitcast(_rows16(c, c), u32)
        for k in range(5):
            lref[_vr(L_Y + k), :] = cp[:, 128 * k:128 * k + 128]
        scl[_vr(0), :] = jnp.broadcast_to(scale, (8, 128))

    x_cp.wait()
    x = jnp.broadcast_to(xbuf[...].astype(f32), (8, D))
    set_input(_ln(x), jnp.full((8, 1), CEXP, f32))
    wq_cp.wait()
    lax.fori_loop(0, D // 16, retile_wq, 0)
    wo_cp.wait()
    lax.fori_loop(0, H * DH // 128, retile_wo, 0)

    def row_sum(a):
        return jnp.broadcast_to(jnp.sum(a, axis=0, keepdims=True), a.shape)

    obuf[24 * NP:24 * NP + 24, :] = jnp.zeros((24, 128), u32)

    def body1(i, acc):
        st = {"acc": acc}
        k_cp(i).wait()
        retile(ku, i, False)
        run_all(q_dots(i, st, qa))
        inv = []
        for hh in range(2):
            run_all(k_dots(i, hh, st, qa))
            inv.append(inv_sum(softmax(st["s", hh], hh)[1]))

        @pl.when(i > 1)
        def _():
            transpose_x(i - 1, XROWS)

        v_cp(i).wait()
        retile(vu, i, True)
        for hh in range(2):
            def pv_step(c, carry, hh=hh):
                acc8 = [None] * 8
                for t in range(32):
                    pv = pT[4 * hh + t // 8][_vr(t % 8), :]
                    for G in range(4):
                        mac(acc8, 2 * G, i * 6 + c, G, t, pv)
                for n in range(8):
                    obuf[pl.ds(64 * c + 16 * (n // 2) + n % 2, 8, stride=2), :] = (
                        pltpu.bitcast(acc8[n], u32))
                return carry
            lax.fori_loop(3 * hh, 3 * hh + 3, pv_step, 0)
        put_o(NP, reduce_o([obuf[128 * b:128 * b + 128, :] for b in range(3)], inv[0], inv[1]))
        run_all(o_dots(NP, i, st))
        return st["acc"]

    x = x + row_sum(lax.fori_loop(0, NP, body1, jnp.zeros((8, D), f32)))

    y = _ln(x)
    zz = _ln(y).astype(bf16)
    w3_cp.wait()
    h = jnp.dot(zz, w3[...], preferred_element_type=f32)
    h = jax.nn.gelu(h, approximate=True).astype(bf16)
    x = x + y
    transpose_x(NP - 1, XROWS_LAST)
    for cp, (a, b) in zip(w4_cp, w4_rows):
        cp.wait()
        x = x + jnp.dot(h[:, a:b], w4[a:b, :], preferred_element_type=f32)

    ones = jnp.ones((8, D), f32)
    xl = _rows16(x, ones)
    xb = xl[0:8].astype(f32)
    mean = _mean(xb)
    c = xb - mean
    set_input(c, lax.rsqrt(_mean(c * c) + EPS) * CEXP)
    obuf[0:24, :] = jnp.zeros((24, 128), u32)
    abuf[...] = jnp.where(lax.broadcasted_iota(jnp.int32, (8, D), 0) == 0, x, 0.0)

    def tail_hooks(i, st, hooks, seg0):
        def first(_):
            m = row_max(st["s", 0])
            st["pa"] = [prob(col(st["s", 0], T), m) for T in range(4)]
            set_state(i, S_INVA, inv_sum(part_sum(st["pa"])))
            for T in range(4):
                ku[i * GP + 3, 8 * (S_PA + T):8 * (S_PA + T) + 4, :] = pack8(st["pa"][T])

        def put(T, half):
            def run(clk):
                tick(pT[T], 8, clk)
                put_p(0, T, st["pa"][T], range(4 * half, 4 * half + 4))
            return run
        hooks.setdefault(("seg", seg0), []).append(first)
        for n in range(8):
            hooks.setdefault(("seg", seg0 + n), []).append(put(n // 2, n % 2))

    def head_b_hooks(i, seg0, pb, final=False):
        def put_b(T):
            def run(clk):
                tick(scl, 1, clk)
                pb.append(prob(get_state(i, T), get_state(i, S_MAXB)))
                put_p(1, T, pb[T])
                if T == 3:
                    set_state(i, S_LB, inv_sum(part_sum(pb)) if final else part_sum(pb))
            return run
        return {("seg", seg0 + 3 * T): [put_b(T)] for T in range(4)}

    def reduce_pair(i, xrows, final=False):
        xa, xb = (get_state(i, S_X + hh) if xrows[hh] else None for hh in range(2))
        invb = get_state(i, S_LB) if final else inv_sum(get_state(i, S_LB))
        return reduce_o([ku[i * GP + b] for b in range(3)],
                        get_state(i, S_INVA), invb, (xa, None, xb))

    st = {}
    new_block()
    late = tuple(range(8, 12)) + tuple(range(8))
    d0 = q_dots(0, st, qb, xl, mean) + q_dots(1, st, qa, xl, mean)
    d1 = k_dots(0, 0, st, qb) + k_dots(0, 1, st, qb, late) + k_dots(1, 0, st, qa, late) \
        + k_dots(1, 1, st, qa) + q_dots(2, st, qa)
    issue = times(d0 + d1)

    def sm_a0():
        m = row_max(st["s", 0])
        p = [prob(col(st["s", 0], T), m) for T in range(4)]
        tick(qb, 6, part_sum(p))
        put_p(0, 0, p[0])
        st["p0"] = p
        set_state(0, S_INVA, inv_sum(part_sum(p)))

    def put_a0(T):
        def run(clk):
            tick(pT[T], 8, clk)
            put_p(0, T, st["p0"][T])
        return run

    def sm_b0():
        tick(qa, 6, stash_b(0, st["s", 1]))

    hooks = head_b_hooks(0, B0_SEG, [])
    hooks.update({("dot", DA0): [sm_a0], ("dot", DB0): [sm_b0],
                  ("need", 0): DA0 + 1, ("need", B0_SEG): DB0 + 1, ("need", A1_SEG): 46})
    hooks.update({("seg", T): [put_a0(T + 1)] for T in range(3)})
    tail_hooks(1, st, hooks, A1_SEG)
    run_block(0, ((), ()), d0 + d1, issue, TV0, hooks, CPO0, False)
    set_state(0, S_X, jnp.zeros((8, 128), f32))
    stash_b(1, st["s", 1])

    def body2(j, carry, last=False):
        new_block()
        st = {"pre": True}
        if not last:
            mid_q(st, qa)
        o = reduce_pair(j, XROWS)
        pb = []
        hooks = head_b_hooks(j + 1, B_SEGL if last else B_SEG0, pb, last)
        xrows = XROWS_LAST if last else XROWS
        xa = x_dots(j + 1, 0, xrows[0], lambda T: ku[(j + 1) * GP + 3, _vr(S_PA + T), :])
        if last:
            dots = o_dots(NP - 2, NP - 3, st)
            for n in range(NP - 3):
                dots += o_dots(n + 1, n, st, [2])
            dots = dots[:len(dots) - NLATE]
            hooks["after", len(dots)] = B_SEGL + 9
            dots += x_dots(j + 1, 1, xrows[1], lambda T: pltpu.bitcast(_rows16(pb[T], pb[T]), u32))
            issue = times(dots, rate=RATEL)
        else:
            dots = k_dots(j + 2, 0, st, qa, MIXA) + k_dots(j + 2, 1, st, qa, MIX) \
                + q_dots(jnp.minimum(j + 3, NP - 1), st, qa) \
                + o_dots(j, jnp.maximum(j - 1, 0), st, [0, 1]) + xa
            issue = times(dots)
            tail_hooks(j + 2, st, hooks, A_SEG0)
            hooks["need", A_SEG0] = 12
            hooks["dot", 24] = [lambda: stash_b(j + 2, st["s", 1])]
        run_block(j + 1, xrows, dots, issue, 0, hooks, CPOL if last else CPO, True, LAGL if last else LAG)
        put_o(j + 1, o)
        abuf[...] += st["acc"]
        return carry

    lax.fori_loop(0, NP - 2, body2, 0)

    @pl.when(zs[0] == 0)
    def _():
        body2(NP - 2, 0, True)

    st = {"acc": abuf[...]}
    run_all(x_dots(NP - 1, 0, XROWS_LAST[0], lambda T: ku[(NP - 1) * GP + 3, _vr(S_PA + T), :]))
    o = reduce_pair(NP - 1, XROWS_LAST, True)
    run_all(o_dots(NP - 1, NP - 2, st))
    for n in range(NP - 3 - NLATE, NP - 3):
        run_all(o_dots(n + 1, n, st, [2]))
    put_o(NP, o)
    run_all(o_dots(NP, NP - 1, st))
    x = row_sum(st["acc"])

    xl = _rows16(x, ones)
    d = xl[0:8].astype(f32) - mean
    md = _mean(d)
    r1 = lax.rsqrt(jnp.maximum(_mean(d * d) - md * md, 0.0) + EPS)
    mean = mean + md
    y = (d - md) * r1
    my = _mean(y)
    r2 = lax.rsqrt(jnp.maximum(_mean(y * y) - my * my, 0.0) + EPS)
    h = jnp.dot(xl, w3[...], preferred_element_type=f32)
    h = h[0:8] * (r1 * r2) - h[8:16] * ((mean * r1 + my) * r2)
    h = jax.nn.gelu(h, approximate=True).astype(bf16)
    x = x + y
    for k in range(0, F, 128):
        x = x + jnp.dot(h[:, k:k + 128], w4[k:k + 128, :], preferred_element_type=f32)
    o_ref[...] = x[0:1].astype(o_ref.dtype)


def _cache_view(c):
    s = c.shape[2]
    c = jnp.transpose(c, (0, 1, 3, 2)).reshape(H * DH // 8, 8, s // 128, 128)
    return jnp.transpose(c, (0, 2, 1, 3)).reshape(H * DH // 8, s // 128 * 8, 128)


def _weight_view(w):
    k, n = w.shape
    w = jnp.transpose(w.reshape(k // 16, 2, 8, n // 128, 128), (0, 1, 3, 2, 4))
    return w.reshape(k // 16, n // 128, 16, 128)


@jax.jit
def pallas_interleave_layers__sliding_block_cached__mixer_s_mlp__decode_kernel(
    A_x: jax.Array,
    A_k_cache: jax.Array,
    A_v_cache: jax.Array,
    A_wq: jax.Array,
    A_wo: jax.Array,
    B_x: jax.Array,
    B_w1: jax.Array,
    B_w2: jax.Array,
    B_w3: jax.Array,
    B_w4: jax.Array,
):
    sk = A_k_cache.shape[2]
    win = min(4096, max(256, sk // 4))
    assert win == 4096 and sk % 128 == 0
    assert A_x.shape == (1, 1, D) and A_k_cache.shape == (1, H, sk, DH)
    wt = win // 128
    t0 = sk // 128 - wt
    ng = H * DH // 8
    hbm = pl.BlockSpec(memory_space=pl.ANY)
    out = pl.pallas_call(
        functools.partial(_kernel, t0=t0, wt=wt),
        out_shape=jax.ShapeDtypeStruct((1, D), A_x.dtype),
        in_specs=[hbm] * 7,
        out_specs=pl.BlockSpec(memory_space=pltpu.VMEM),
        scratch_shapes=[
            pltpu.VMEM((ng, wt * 8, 128), bf16),
            pltpu.VMEM((ng, wt * 8, 128), bf16),
            pltpu.VMEM((ng // 4, 256, 128), bf16),
            pltpu.VMEM((NP * D // 16, 3, 8, 128), u32),
            pltpu.VMEM((H * DH // 16, D // 128, 16, 128), bf16),
            pltpu.VMEM((D, F), bf16),
            pltpu.VMEM((F, D), bf16),
            pltpu.VMEM((1, D), bf16),
            pltpu.VMEM((136, 128), u32),
            pltpu.VMEM((24 * (NP + 1) + 96, 128), u32),
            pltpu.VMEM((144, 128), u32),
            pltpu.VMEM((144, 128), u32),
            pltpu.VMEM((16, 128), f32),
            pltpu.VMEM((8, D), f32),
            pltpu.SMEM((1,), jnp.int32),
        ] + [pltpu.VMEM((72, 128), f32)] * 8,
        compiler_params=pltpu.CompilerParams(vmem_limit_bytes=128 * 1024 * 1024),
    )(A_x.reshape(1, D), _cache_view(A_k_cache), _cache_view(A_v_cache),
      _weight_view(A_wq).reshape(D * 3 // 16, 256, 128), _weight_view(A_wo), B_w3, B_w4)
    return out.reshape(1, 1, D)
```

```python
import functools

import jax
import jax.numpy as jnp
from jax import lax
import jax.experimental.pallas as pl
import jax.experimental.pallas.tpu as pltpu

D = 640
H = 32
DH = 192
F = 1536
EPS = 1e-5
NP = H // 2
GP = 2 * DH // 8
HI = 0xFFFF0000
CEXP = DH ** -0.5 * 1.4426950408889634

f32 = jnp.float32
bf16 = jnp.bfloat16
u32 = jnp.uint32

L_Y = 0
L_DUMMY = 5
S_MAXB, S_LB, S_INVA, S_X, S_PA = 4, 5, 6, 7, 9
XROWS = ((10, 18, 26), ())
XROWS_LAST = (tuple(range(0, 32, 2)), tuple(range(2, 32, 4)))
GX = (0, 16)
PLAN_FIRST = (
    {},
    (27, 27, 28, 29, 30, 29, 31, 32, 31, 33, 34, 34, 35, 36, 37, 37, 38, 39, 40, 40, 41, 42,
    42, 43, 44, 44, 45, 46, 47, 47, 48, 49, 50, 50, 51, 52, 52, 53, 54, 55, 55, 56, 57, 58,
    59, 59, 60, 61))
PLAN_BODY = (
    {1: 0, 3: 1, 4: 4, 7: 4, 9: 6, 11: 7, 13: 8, 15: 10, 17: 11, 19: 12, 21: 14, 23: 16, 26:
    17, 27: 18, 28: 21, 31: 22, 33: 25, 35: 25, 37: 28, 39: 29, 40: 31},
    (0, 0, 0, 0, 0, 0, 0, 0, 0, 0, 0, 0, 2, 3, 4, 4, 6, 6, 6, 8, 6, 9, 9, 10, 11, 12, 12,
    13, 14, 15, 16, 16, 17, 18, 19, 23, 22, 22, 22, 23, 22, 23, 25, 26, 28, 28, 29, 29))
PLAN_LAST = (
    {1: 0, 3: 0, 5: 1, 6: 1, 7: 2, 9: 2, 11: 2, 13: 3, 15: 4, 17: 4, 19: 6, 23: 9, 25: 10,
    27: 11, 29: 13, 31: 13, 33: 14, 35: 15, 37: 16},
    (0, 0, 0, 0, 0, 0, 0, 0, 0, 0, 0, 0, 0, 0, 0, 0, 1, 1, 1, 2, 1, 1, 2, 2, 3, 4, 5, 6, 6,
    7, 7, 8, 9, 9, 10, 11, 11, 11, 11, 12, 12, 13, 13, 15, 14, 14, 14, 15))
MIX = (0, 1, 8, 2, 3, 9, 4, 5, 10, 6, 7, 11)
MIXA = (0, 1, 2, 3, 4, 8, 5, 9, 6, 10, 7, 11)
B_SEGS = (9, 12, 15, 18)
B_SEGL = 7
A_SEG0 = 40
DA0 = 31
DB0 = 45
B0_SEG = 13
A1_SEG = 34
W4_CHUNKS = (1024, 384, 128)


def _mean(x):
    return jnp.mean(x, axis=-1, keepdims=True)


def _ln(x):
    c = x - _mean(x)
    return c * lax.rsqrt(_mean(c * c) + EPS)


def _wtile(wu, rows, nt):
    blk = wu[rows, nt]
    return pltpu.bitcast(blk.reshape(blk.shape[0] * 8, 128), bf16)


def _wcols(wu, rows, nts):
    return jnp.concatenate([_wtile(wu, rows, n) for n in nts], axis=1)


def _rows16(a, b):
    return jnp.concatenate([a, b], axis=0).astype(bf16)


def _slot(G, t):
    j = 4 * (t >> 3) + ((((t >> 1) & 3) + G + 2 * (t & 1) + (t >> 3)) & 3)
    return 2 * G + (t & 1), 8 * j


def _xslot(G, t):
    return G // 2, 8 * (4 * (t >> 3) + ((((t >> 1) & 3) + G + (t >> 3)) & 3))


def _vr(n):
    return slice(8 * n, 8 * n + 8)


def _kernel(*refs, t0, wt):
    pl.run_scoped(functools.partial(_body, refs, t0, wt),
                  pltpu.SemaphoreType.DMA((4 + len(W4_CHUNKS) + 2 * NP,)))


def _body(refs, t0, wt, sems):
    (x_hbm, k_hbm, v_hbm, wq_hbm, wo_hbm, w3_hbm, w4_hbm, o_ref,
     kbuf, vbuf, vxbuf, wqu, wo, w3, w4, xbuf, lref, obuf, qa, qb, scl, abuf, zs) = refs[:23]
    pT = refs[23:]
    ku = kbuf.bitcast(u32)
    vu = vbuf.bitcast(u32)
    vx = vxbuf.bitcast(u32)
    wou = wo.bitcast(u32)

    x_cp = pltpu.make_async_copy(x_hbm, xbuf, sems.at[0])
    wq_cp = pltpu.make_async_copy(wq_hbm, vxbuf.at[0:D * 3 // 16], sems.at[1])
    wo_cp = pltpu.make_async_copy(wo_hbm, wo, sems.at[2])
    w3_cp = pltpu.make_async_copy(w3_hbm, w3, sems.at[3])
    w4_rows, r0 = [], 0
    for n in W4_CHUNKS:
        w4_rows.append((r0, r0 + n))
        r0 += n
    w4_cp = [pltpu.make_async_copy(w4_hbm.at[a:b], w4.at[a:b], sems.at[4 + c])
             for c, (a, b) in enumerate(w4_rows)]
    S0 = 4 + len(W4_CHUNKS)

    def k_cp(i):
        return pltpu.make_async_copy(
            k_hbm.at[pl.ds(i * GP, GP), pl.ds(t0 * 8, wt * 8), :],
            kbuf.at[pl.ds(i * GP, GP)], sems.at[S0 + i])

    def v_cp(i):
        return pltpu.make_async_copy(
            v_hbm.at[pl.ds(i * GP, GP), pl.ds(t0 * 8, wt * 8), :],
            vbuf.at[pl.ds(i * GP, GP)], sems.at[S0 + NP + i])

    for c in (wq_cp, x_cp, wo_cp):
        c.start()
    for i in range(NP):
        k_cp(i).start()
        v_cp(i).start()
    for c in [w3_cp] + w4_cp:
        c.start()

    zs[0] = 0
    qa[_vr(5), :] = jnp.zeros((8, 128), u32)

    lane = lax.broadcasted_iota(jnp.int32, (8, 128), 1)
    sub = lax.broadcasted_iota(jnp.int32, (8, 128), 0)
    lane_lo = lane < 64
    sub_lo = sub < 4

    def tile(ref, g0, G, t):
        g, r = _slot(G, t)
        return ref[g0 + g, r:r + 8, :]

    def retile(ref, i, expand):
        def body(c, carry):
            g0 = i * GP + 8 * c
            for G in range(4):
                for J in range(4):
                    xs = [[ref[g0 + 2 * G + e, _vr(4 * J + jj), :] for jj in range(4)]
                          for e in range(2)]
                    for jj in range(4):
                        x0, x1 = xs[0][jj], xs[1][jj]
                        ys = (jnp.where(sub_lo, x0, pltpu.roll(x1, 4, 0)),
                              jnp.where(sub_lo, pltpu.roll(x0, 4, 0), x1))
                        for e in range(2):
                            t = 8 * J + 2 * jj + e
                            g, r = _slot(G, t)
                            if expand and G % 2 and e:
                                ref[g0 + g, r:r + 8, :] = ys[e] << 16
                                g, r = _xslot(G, t)
                                vx[i * (GP // 4) + 2 * c + g, r:r + 8, :] = ys[e] & jnp.uint32(HI)
                            else:
                                ref[g0 + g, r:r + 8, :] = ys[e]
            return carry
        lax.fori_loop(0, GP // 8, body, 0)

    def merge_halves(get, nt, n):
        lo, hi = get(n // 2), get((nt + n) // 2)
        if n % 2:
            lo = pltpu.roll(lo, 4, 0)
        if (nt + n) % 2 == 0:
            hi = pltpu.roll(hi, 4, 0)
        return jnp.where(sub_lo, lo, hi)

    def retile_wq(G, carry):
        for n in range(3 * NP):
            wqu[n // 3 * (D // 16) + G, n % 3] = merge_halves(
                lambda v: vx[3 * G + v // 16, _vr(v % 16), :], 3 * NP, n)
        return carry

    def retile_wo(c, carry):
        for G in range(8):
            xs = [wou[8 * c + G, n] for n in range(5)]
            for n in range(5):
                wou[8 * c + G, n] = merge_halves(lambda v: xs[v], 5, n)
        return carry

    def lhs_at(ref, n):
        return pltpu.bitcast(ref[_vr(n), :], bf16)

    cur = [None]

    def new_block():
        cur[0] = -32 * jnp.clip(zs[0], 0, 1)

    def tick(ref, n, val):
        if val.dtype != ref.dtype:
            val = pltpu.bitcast(val, ref.dtype)
        ref[pl.ds(pl.multiple_of(cur[0] + 8 * n, 8), 8), :] = val

    def q_dots(i, st, qref, lhs=None, mean=None):
        def step(k):
            def run(tied=False):
                w = _wcols(wqu, pl.ds(i * (D // 16) + 8 * k, 8), range(3))
                if lhs is None:
                    r = jnp.dot(lhs_at(lref, L_Y + k), w, preferred_element_type=f32)[0:8]
                else:
                    r = jnp.dot(lhs[:, 128 * k:128 * k + 128], w, preferred_element_type=f32)
                st["q"] = r if k == 0 else st["q"] + r
                if k == 4:
                    q = st["q"] if lhs is None else st["q"][0:8] - mean * st["q"][8:16]
                    qq = pltpu.bitcast(q.astype(bf16).astype(f32), u32)
                    q0, q1, q2 = qq[:, 0:128], qq[:, 128:256], qq[:, 256:384]
                    for n, v in enumerate((q0 >> 16, q0, q2 >> 16, q2, q1)):
                        qref[_vr(n), :] = v
                return r[0:8, 256:384]
            return 3, lref, L_DUMMY, run
        return [step(k) for k in range(5)]

    def o_dots(slot, i, st, chunks=range(3)):
        def step(b):
            def run(tied=False):
                w = _wcols(wou, pl.ds(i * (GP // 2) + 8 * b, 8), range(5))
                lhs = obuf[pl.ds(pl.multiple_of(24 * slot + 8 * b, 8), 8), :]
                r = jnp.dot(pltpu.bitcast(lhs, bf16), w, preferred_element_type=f32)[0:8]
                st["acc"] = st["acc"] + r if "acc" in st else r
                return r[:, 512:640]
            return 5, obuf, 3 * (NP + 1), run
        return [step(b) for b in chunks]

    def mid_q(st, qref):
        q1 = qref[_vr(4), :]
        q1r = pltpu.roll(q1, 64, 1)
        st["u", 0] = jnp.where(lane_lo, q1 >> 16, q1r)
        st["u", 1] = jnp.where(lane_lo, q1r >> 16, q1)

    def k_dots(i, hh, st, qref, order=tuple(range(12))):
        g0 = i * GP
        gf, gh = ((0, 8), (16, 12))[hh]

        def step(r):
            def run(tied=False):
                if r < 8:
                    cols = [[tile(ku, g0, gf + G, 8 * T + r) for G in range(8)] for T in range(4)]
                    base, row = qref[_vr(2 * hh + r % 2), :], r // 2
                else:
                    cols = [[tile(ku, g0, gh + G % 4, 8 * T + 2 * (r - 8) + G // 4)
                             for G in range(8)] for T in range(4)]
                    if r == 8 and hh == 0 and "pre" not in st:
                        mid_q(st, qref)
                    base, row = st["u", hh], r - 8
                    if tied:
                        base = base | qref[_vr(5), :]
                lhs = jnp.where(sub == row, base, jnp.zeros((8, 128), u32))
                w = jnp.concatenate([jnp.concatenate(c, axis=0) for c in cols], axis=1)
                res = jnp.dot(pltpu.bitcast(lhs, bf16), pltpu.bitcast(w, bf16),
                              preferred_element_type=f32)[0:8]
                st["s", hh] = res if r == order[0] else st["s", hh] + res
                return res[:, 384:512]
            return 4, qref, 6, run
        return [step(r) for r in order]

    def col(s, T):
        return s[:, 128 * T:128 * T + 128]

    def row_max(s):
        m = jnp.maximum(jnp.maximum(col(s, 0), col(s, 1)), jnp.maximum(col(s, 2), col(s, 3)))
        return jnp.max(jnp.max(m, axis=1, keepdims=True), axis=0, keepdims=True)

    def prob(s, m):
        return jnp.exp2((s - m) * scl[_vr(0), :])

    def put_p(hh, T, p, ks=range(8)):
        for k in ks:
            pT[4 * hh + T][pl.ds(k, 8, stride=8), :] = p

    def part_sum(p):
        return (p[0] + p[1]) + (p[2] + p[3])

    def inv_sum(l):
        l = jnp.sum(jnp.sum(l, axis=1, keepdims=True), axis=0, keepdims=True)
        r = pl.reciprocal(l, approx=True)
        return jnp.broadcast_to(r * (2.0 - l * r), (8, 128))

    def softmax(s, hh):
        m = row_max(s)
        p = [prob(col(s, T), m) for T in range(4)]
        for T in range(4):
            put_p(hh, T, p[T])
        return p, part_sum(p)

    def get_state(i, n):
        return pltpu.bitcast(ku[i * GP + 3, _vr(n), :], f32)

    def set_state(i, n, v):
        ku[i * GP + 3, _vr(n), :] = pltpu.bitcast(v, u32)

    def stash_b(i, s):
        for T in range(4):
            set_state(i, T, col(s, T))
        m = jnp.broadcast_to(row_max(s), (8, 128))
        set_state(i, S_MAXB, m)
        return m

    def pack8(v):
        return pltpu.bitcast(v.astype(bf16), u32)

    def x_dots(i, hh, ts, get_lhs):
        st = {}
        rows = sorted({t % 8 for t in ts})

        def step(n, rho):
            def run(tied=False):
                res = []
                for T in [t // 8 for t in ts if t % 8 == rho]:
                    w = jnp.concatenate(
                        [tile(vu, i * GP, GX[hh] + G, 8 * T + rho) for G in range(8)], axis=0)
                    lhs = get_lhs(T) | obuf[_vr(0), :] if tied else get_lhs(T)
                    res.append(jnp.dot(pltpu.bitcast(lhs, bf16), pltpu.bitcast(w, bf16),
                                       preferred_element_type=f32)[0:8])
                st["x"] = jnp.where(sub == rho, sum(res[1:], res[0]), st["x"] if n else 0.0)
                if n == len(rows) - 1:
                    set_state(i, S_X + hh, st["x"])
                return res[-1]
            return sum(1 for t in ts if t % 8 == rho), obuf, 3 * (NP + 1), run
        return [step(n, rho) for n, rho in enumerate(rows)]

    def transpose_x(i, xrows):
        for hh in range(2):
            for t in xrows[hh]:
                w = jnp.concatenate([tile(vu, i * GP, GX[hh] + G, t) for G in range(8)], axis=0)
                w = pltpu.bitcast(pltpu.bitcast(w, bf16).astype(f32).T.astype(bf16), u32)
                for G in range(8):
                    g, r = _slot(GX[hh] + G, t)
                    vu[i * GP + g, r:r + 8, :] = w[_vr(G), :]

    def reduce_o(blocks, inva, invb, extra=(None, None, None)):
        out = []
        for b, inv in enumerate((inva, jnp.where(lane_lo, inva, invb), invb)):
            z = jnp.sum(pltpu.bitcast(blocks[b], f32).T.reshape(16, 8, 128), axis=0)
            if extra[b] is not None:
                z = z + extra[b]
            out.append(pack8(z * inv))
        return out

    def put_o(slot, o):
        for b in range(3):
            obuf[pl.ds(pl.multiple_of(24 * slot + 8 * b, 8), 4), :] = o[b]

    def mac(acc, n, c, G, t, pv):
        w = tile(vu, 8 * c, G, t)
        if G % 2 and t % 2:
            g, r = _xslot(G, t)
            halves = (w, vx[2 * c + g, r:r + 8, :])
        else:
            halves = (w << 16, w & jnp.uint32(HI))
        for k in range(2):
            a = pltpu.bitcast(halves[k], f32) * pv
            acc[n + k] = a if acc[n + k] is None else acc[n + k] + a

    def seg_rows(xrows, seg):
        hh, gp, T = seg // 24, seg % 24 // 4, seg % 4
        on_mxu = GX[hh] <= 12 * hh + 2 * gp < GX[hh] + 8
        return [rho for rho in range(8) if not (on_mxu and 8 * T + rho in xrows[hh])]

    def run_block(i, xrows, dots, hooks, plan):
        tie, clk = plan
        clock = []

        def emit(upto):
            while len(clock) < upto:
                n = len(clock)
                for h in hooks.get(("dot", n), ()):
                    h()
                clock.append(dots[n][3](n in tie.values()))

        zero = jnp.zeros((8, 128), f32)
        used = {}
        for seg in range(48):
            hh, gp, T = seg // 24, seg % 24 // 4, seg % 4
            if T == 0:
                a4 = [None] * 4
            pref = pT[4 * hh + T]
            upto = min([v for k, v in tie.items() if k >= seg]
                       + [k[1] for k, v in hooks.items() if k[0] == "after" and v >= seg]
                       + [len(dots) if tie else clk[seg] + 6])
            free = not any(k in tie for k in range(seg, seg - T + 4))
            if free or ("seg", seg) in hooks:
                upto = max(upto, clk[seg] + 1)
            emit(min(len(dots), max(upto, hooks.get(("need", seg), 0))))
            if free:
                tick(pref, 8, clock[clk[seg]])
            elif gp:
                tick(pref, 8, zero)
            for h in hooks.get(("seg", seg), ()):
                h(clock[clk[seg]])
            for rho in seg_rows(xrows, seg):
                pv = pref[_vr(rho), :]
                for e in range(2):
                    mac(a4, 2 * e, i * 6, 12 * hh + 2 * gp + e, 8 * T + rho, pv)
            if seg in tie:
                _, ref, slot, _ = dots[tie[seg]]
                used[tie[seg]] = used.get(tie[seg], -1) + 1
                for k in range(4):
                    tick(ref, slot + 4 * used[tie[seg]] + k, a4[k])
            if T == 3:
                for n in range(4):
                    G = 12 * hh + 2 * gp + n // 2
                    ku[i * GP + G // 8, pl.ds(16 * (G % 8) + n % 2, 8, stride=2), :] = (
                        pltpu.bitcast(a4[n], u32))
        emit(len(dots))

    def run_all(dots):
        for d in dots:
            d[3]()

    def set_input(c, scale):
        cp = pltpu.bitcast(_rows16(c, c), u32)
        for k in range(5):
            lref[_vr(L_Y + k), :] = cp[:, 128 * k:128 * k + 128]
        scl[_vr(0), :] = jnp.broadcast_to(scale, (8, 128))

    x_cp.wait()
    x = jnp.broadcast_to(xbuf[...].astype(f32), (8, D))
    set_input(_ln(x), jnp.full((8, 1), CEXP, f32))
    wq_cp.wait()
    lax.fori_loop(0, D // 16, retile_wq, 0)
    wo_cp.wait()
    lax.fori_loop(0, H * DH // 128, retile_wo, 0)

    def row_sum(a):
        return jnp.broadcast_to(jnp.sum(a, axis=0, keepdims=True), a.shape)

    obuf[24 * NP:24 * NP + 24, :] = jnp.zeros((24, 128), u32)

    def body1(i, acc):
        st = {"acc": acc}
        k_cp(i).wait()
        retile(ku, i, False)
        run_all(q_dots(i, st, qa))
        inv = []
        for hh in range(2):
            run_all(k_dots(i, hh, st, qa))
            inv.append(inv_sum(softmax(st["s", hh], hh)[1]))

        @pl.when(i > 1)
        def _():
            transpose_x(i - 1, XROWS)

        v_cp(i).wait()
        retile(vu, i, True)
        for hh in range(2):
            def pv_step(c, carry, hh=hh):
                acc8 = [None] * 8
                for t in range(32):
                    pv = pT[4 * hh + t // 8][_vr(t % 8), :]
                    for G in range(4):
                        mac(acc8, 2 * G, i * 6 + c, G, t, pv)
                for n in range(8):
                    obuf[pl.ds(64 * c + 16 * (n // 2) + n % 2, 8, stride=2), :] = (
                        pltpu.bitcast(acc8[n], u32))
                return carry
            lax.fori_loop(3 * hh, 3 * hh + 3, pv_step, 0)
        put_o(NP, reduce_o([obuf[128 * b:128 * b + 128, :] for b in range(3)], inv[0], inv[1]))
        run_all(o_dots(NP, i, st))
        return st["acc"]

    x = x + row_sum(lax.fori_loop(0, NP, body1, jnp.zeros((8, D), f32)))

    y = _ln(x)
    zz = _ln(y).astype(bf16)
    w3_cp.wait()
    h = jnp.dot(zz, w3[...], preferred_element_type=f32)
    h = jax.nn.gelu(h, approximate=True).astype(bf16)
    x = x + y
    transpose_x(NP - 1, XROWS_LAST)
    for cp, (a, b) in zip(w4_cp, w4_rows):
        cp.wait()
        x = x + jnp.dot(h[:, a:b], w4[a:b, :], preferred_element_type=f32)

    ones = jnp.ones((8, D), f32)
    xl = _rows16(x, ones)
    xb = xl[0:8].astype(f32)
    mean = _mean(xb)
    c = xb - mean
    set_input(c, lax.rsqrt(_mean(c * c) + EPS) * CEXP)
    obuf[0:24, :] = jnp.zeros((24, 128), u32)
    abuf[...] = jnp.where(lax.broadcasted_iota(jnp.int32, (8, D), 0) == 0, x, 0.0)

    def tail_hooks(i, st, hooks, seg0):
        def first(_):
            m = row_max(st["s", 0])
            st["pa"] = [prob(col(st["s", 0], T), m) for T in range(4)]
            set_state(i, S_INVA, inv_sum(part_sum(st["pa"])))
            for T in range(4):
                ku[i * GP + 3, 8 * (S_PA + T):8 * (S_PA + T) + 4, :] = pack8(st["pa"][T])

        def put(T, half):
            def run(clk):
                tick(pT[T], 8, clk)
                put_p(0, T, st["pa"][T], range(4 * half, 4 * half + 4))
            return run
        hooks.setdefault(("seg", seg0), []).append(first)
        for n in range(8):
            hooks.setdefault(("seg", seg0 + n), []).append(put(n // 2, n % 2))

    def head_b_hooks(i, segs, pb, final=False):
        def put_b(T):
            def run(clk):
                tick(scl, 4, clk)
                pb.append(prob(get_state(i, T), get_state(i, S_MAXB)))
                put_p(1, T, pb[T])
                if T == 3:
                    set_state(i, S_LB, inv_sum(part_sum(pb)) if final else part_sum(pb))
            return run
        return {("seg", segs[T]): [put_b(T)] for T in range(4)}

    def reduce_pair(i, xrows, final=False):
        xa, xb = (get_state(i, S_X + hh) if xrows[hh] else None for hh in range(2))
        invb = get_state(i, S_LB) if final else inv_sum(get_state(i, S_LB))
        return reduce_o([ku[i * GP + b] for b in range(3)],
                        get_state(i, S_INVA), invb, (xa, None, xb))

    st = {}
    new_block()
    late = tuple(range(8, 12)) + tuple(range(8))
    d0 = q_dots(0, st, qb, xl, mean) + q_dots(1, st, qa, xl, mean)
    d1 = k_dots(0, 0, st, qb) + k_dots(0, 1, st, qb, late) + k_dots(1, 0, st, qa, late) \
        + k_dots(1, 1, st, qa) + q_dots(2, st, qa)

    def sm_a0():
        m = row_max(st["s", 0])
        p = [prob(col(st["s", 0], T), m) for T in range(4)]
        tick(qb, 6, part_sum(p))
        put_p(0, 0, p[0])
        st["p0"] = p
        set_state(0, S_INVA, inv_sum(part_sum(p)))

    def put_a0(T):
        def run(clk):
            tick(pT[T], 8, clk)
            put_p(0, T, st["p0"][T])
        return run

    def sm_b0():
        tick(qa, 6, stash_b(0, st["s", 1]))

    hooks = head_b_hooks(0, range(B0_SEG, 48, 3), [])
    hooks.update({("dot", DA0): [sm_a0], ("dot", DB0): [sm_b0],
                  ("need", 0): DA0 + 1, ("need", B0_SEG): DB0 + 1, ("need", A1_SEG): 46})
    hooks.update({("seg", T): [put_a0(T + 1)] for T in range(3)})
    tail_hooks(1, st, hooks, A1_SEG)
    run_block(0, ((), ()), d0 + d1, hooks, PLAN_FIRST)
    set_state(0, S_X, jnp.zeros((8, 128), f32))
    stash_b(1, st["s", 1])

    def body2(j, carry, last=False):
        new_block()
        st = {"pre": True}
        if not last:
            mid_q(st, qa)
        o = reduce_pair(j, XROWS)
        pb = []
        hooks = head_b_hooks(j + 1, range(B_SEGL, 48, 3) if last else B_SEGS, pb, last)
        xrows = XROWS_LAST if last else XROWS
        xa = x_dots(j + 1, 0, xrows[0], lambda T: ku[(j + 1) * GP + 3, _vr(S_PA + T), :])
        if last:
            dots = o_dots(NP - 2, NP - 3, st)
            for n in range(NP - 3):
                dots += o_dots(n + 1, n, st, [2])
            hooks["after", len(dots)] = B_SEGL + 9
            dots += x_dots(j + 1, 1, xrows[1], lambda T: pltpu.bitcast(_rows16(pb[T], pb[T]), u32))
        else:
            dots = k_dots(j + 2, 0, st, qa, MIXA) + k_dots(j + 2, 1, st, qa, MIX) \
                + q_dots(jnp.minimum(j + 3, NP - 1), st, qa) \
                + o_dots(j, jnp.maximum(j - 1, 0), st, [0, 1]) + xa
            tail_hooks(j + 2, st, hooks, A_SEG0)
            hooks["need", A_SEG0] = 12
            hooks["dot", 24] = [lambda: stash_b(j + 2, st["s", 1])]
        run_block(j + 1, xrows, dots, hooks, PLAN_LAST if last else PLAN_BODY)
        put_o(j + 1, o)
        abuf[...] += st["acc"]
        return carry

    lax.fori_loop(0, NP - 2, body2, 0)

    @pl.when(zs[0] == 0)
    def _():
        body2(NP - 2, 0, True)

    st = {"acc": abuf[...]}
    run_all(x_dots(NP - 1, 0, XROWS_LAST[0], lambda T: ku[(NP - 1) * GP + 3, _vr(S_PA + T), :]))
    o = reduce_pair(NP - 1, XROWS_LAST, True)
    run_all(o_dots(NP - 1, NP - 2, st))
    put_o(NP, o)
    run_all(o_dots(NP, NP - 1, st))
    x = row_sum(st["acc"])

    xl = _rows16(x, ones)
    d = xl[0:8].astype(f32) - mean
    md = _mean(d)
    r1 = lax.rsqrt(jnp.maximum(_mean(d * d) - md * md, 0.0) + EPS)
    mean = mean + md
    y = (d - md) * r1
    my = _mean(y)
    r2 = lax.rsqrt(jnp.maximum(_mean(y * y) - my * my, 0.0) + EPS)
    h = jnp.dot(xl, w3[...], preferred_element_type=f32)
    h = h[0:8] * (r1 * r2) - h[8:16] * ((mean * r1 + my) * r2)
    h = jax.nn.gelu(h, approximate=True).astype(bf16)
    x = x + y
    for k in range(0, F, 128):
        x = x + jnp.dot(h[:, k:k + 128], w4[k:k + 128, :], preferred_element_type=f32)
    o_ref[...] = x[0:1].astype(o_ref.dtype)


def _cache_view(c):
    s = c.shape[2]
    c = jnp.transpose(c, (0, 1, 3, 2)).reshape(H * DH // 8, 8, s // 128, 128)
    return jnp.transpose(c, (0, 2, 1, 3)).reshape(H * DH // 8, s // 128 * 8, 128)


def _weight_view(w):
    k, n = w.shape
    w = jnp.transpose(w.reshape(k // 16, 2, 8, n // 128, 128), (0, 1, 3, 2, 4))
    return w.reshape(k // 16, n // 128, 16, 128)


@jax.jit
def pallas_interleave_layers__sliding_block_cached__mixer_s_mlp__decode_kernel(
    A_x: jax.Array,
    A_k_cache: jax.Array,
    A_v_cache: jax.Array,
    A_wq: jax.Array,
    A_wo: jax.Array,
    B_x: jax.Array,
    B_w1: jax.Array,
    B_w2: jax.Array,
    B_w3: jax.Array,
    B_w4: jax.Array,
):
    sk = A_k_cache.shape[2]
    win = min(4096, max(256, sk // 4))
    assert win == 4096 and sk % 128 == 0
    assert A_x.shape == (1, 1, D) and A_k_cache.shape == (1, H, sk, DH)
    wt = win // 128
    t0 = sk // 128 - wt
    ng = H * DH // 8
    hbm = pl.BlockSpec(memory_space=pl.ANY)
    out = pl.pallas_call(
        functools.partial(_kernel, t0=t0, wt=wt),
        out_shape=jax.ShapeDtypeStruct((1, D), A_x.dtype),
        in_specs=[hbm] * 7,
        out_specs=pl.BlockSpec(memory_space=pltpu.VMEM),
        scratch_shapes=[
            pltpu.VMEM((ng, wt * 8, 128), bf16),
            pltpu.VMEM((ng, wt * 8, 128), bf16),
            pltpu.VMEM((ng // 4, 256, 128), bf16),
            pltpu.VMEM((NP * D // 16, 3, 8, 128), u32),
            pltpu.VMEM((H * DH // 16, D // 128, 16, 128), bf16),
            pltpu.VMEM((D, F), bf16),
            pltpu.VMEM((F, D), bf16),
            pltpu.VMEM((1, D), bf16),
            pltpu.VMEM((136, 128), u32),
            pltpu.VMEM((24 * (NP + 1) + 96, 128), u32),
            pltpu.VMEM((144, 128), u32),
            pltpu.VMEM((144, 128), u32),
            pltpu.VMEM((40, 128), f32),
            pltpu.VMEM((8, D), f32),
            pltpu.SMEM((1,), jnp.int32),
        ] + [pltpu.VMEM((72, 128), f32)] * 8,
        compiler_params=pltpu.CompilerParams(vmem_limit_bytes=128 * 1024 * 1024),
    )(A_x.reshape(1, D), _cache_view(A_k_cache), _cache_view(A_v_cache),
      _weight_view(A_wq).reshape(D * 3 // 16, 256, 128), _weight_view(A_wo), B_w3, B_w4)
    return out.reshape(1, 1, D)
```

```python
import functools

import jax
import jax.numpy as jnp
from jax import lax
import jax.experimental.pallas as pl
import jax.experimental.pallas.tpu as pltpu

D = 640
H = 32
DH = 192
F = 1536
EPS = 1e-5
NP = H // 2
GP = 2 * DH // 8
HI = 0xFFFF0000
CEXP = DH ** -0.5 * 1.4426950408889634

f32 = jnp.float32
bf16 = jnp.bfloat16
u32 = jnp.uint32

L_Y = 0
L_DUMMY = 6
S_MAXB, S_LB, S_INVA, S_X, S_PA = 4, 5, 6, 7, 9
XROWS = ((2, 10, 18, 26), (4, 12, 20))
XROWS_LAST = (tuple(range(0, 32, 2)), tuple(t for t in range(0, 32, 2) if t % 8))
XNONE = ((), ())
GX = (0, 16)
PLANS = {
    "first": (
        {},
        (27, 27, 28, 29, 30, 29, 31, 32, 31, 33, 34, 34, 35, 36, 37, 37, 38, 39, 40, 40, 41, 42,
        42, 43, 44, 44, 45, 46, 47, 47, 48, 49, 50, 50, 51, 52, 52, 53, 54, 55, 55, 56, 57, 58,
        59, 59, 60, 61)),
    "second": (
        {1: 0, 3: 2, 5: 4, 7: 6, 9: 6, 11: 8, 13: 10, 15: 11, 17: 12, 19: 14, 21: 16, 23: 17,
        25: 19, 27: 21, 29: 21, 31: 26, 32: 28, 35: 29, 37: 30, 39: 33},
        (0, 0, 0, 0, 0, 0, 0, 0, 0, 0, 0, 2, 3, 5, 3, 4, 6, 7, 10, 7, 8, 9, 10, 10, 12, 13, 14,
        14, 15, 16, 17, 18, 18, 19, 20, 21, 21, 21, 22, 24, 24, 25, 26, 28, 29, 29, 30, 31)),
    "body": (
        {1: 0, 3: 1, 5: 3, 7: 4, 9: 5, 11: 8, 12: 10, 15: 10, 19: 12, 21: 14, 23: 16, 25: 17,
        27: 19, 29: 22, 31: 23, 33: 23, 35: 26, 37: 26, 39: 28, 40: 33, 41: 33, 43: 34, 45: 34,
        47: 34, 49: 35, 51: 37, 53: 38, 55: 39, 57: 40, 59: 42, 61: 43, 63: 46, 67: 49, 70: 51,
        71: 52, 72: 53, 75: 55, 77: 56, 79: 58, 81: 59, 83: 62, 84: 62},
        (0, 0, 0, 0, 0, 0, 0, 0, 0, 0, 0, 1, 2, 2, 3, 4, 4, 5, 6, 7, 7, 8, 9, 10, 10, 12, 12,
        13, 14, 15, 15, 16, 16, 17, 17, 18, 20, 21, 21, 24, 25, 23, 24, 27, 27, 33, 29, 29, 28,
        30, 30, 31, 31, 32, 33, 33, 34, 35, 35, 36, 36, 35, 35, 36, 37, 39, 43, 41, 43, 40, 45,
        45, 46, 48, 48, 48, 49, 50, 50, 51, 52, 51, 51, 54, 53, 54, 56, 58, 57, 59, 61, 59, 61,
        62, 63, 64)),
    "third": (
        {1: 0, 3: 3, 6: 3, 7: 4, 9: 5, 11: 8, 15: 10, 18: 12, 19: 14, 21: 14, 23: 15, 25: 17,
        26: 19, 27: 19, 30: 22},
        (0, 0, 0, 0, 0, 0, 0, 0, 0, 0, 1, 0, 0, 3, 3, 5, 2, 5, 4, 8, 7, 8, 10, 10, 10, 12, 12,
        13, 15, 17, 15, 16, 17, 17, 18, 19, 20, 18, 21, 22, 22, 24, 25, 26, 25, 24, 25, 25)),
    "last": (
        {0: 0, 3: 0, 7: 0, 9: 2, 11: 2, 15: 2, 17: 5, 19: 5, 21: 8, 23: 8, 25: 11, 27: 11,
        29: 13, 31: 13},
        (0, 0, 0, 0, 0, 0, 0, 1, 0, 1, 2, 1, 0, 0, 0, 0, 0, 0, 0, 0, 0, 0, 1, 3, 4, 5, 5, 6, 7,
        7, 6, 6, 9, 9, 10, 10, 11, 11, 12, 12, 13, 13, 14, 13, 14, 14, 16, 16)),
}
MIX = (0, 1, 8, 2, 3, 9, 4, 5, 10, 6, 7, 11)
MIXA = (0, 1, 2, 3, 4, 8, 5, 9, 6, 10, 7, 11)
B_SEGS = (9, 12, 15, 18)
B_SEGL = 7
DA0 = 31
DB0 = 45
B0_SEG = 13
A1_SEG = 34
A_SEG0 = 40
A_SEG2 = 39
A_SEG3 = 38
B_SEGS2 = (8, 11, 14, 17)
B_SEGS3 = (9, 11, 15, 19)
XA_AT = 8
AD_SEG = 32
BD_SEG = 12
NALT = 2
W4_CHUNKS = (1024, 384, 128)


def _mean(x):
    return jnp.mean(x, axis=-1, keepdims=True)


def _ln(x):
    c = x - _mean(x)
    return c * lax.rsqrt(_mean(c * c) + EPS)


def _wtile(wu, rows, nt):
    blk = wu[rows, nt]
    return pltpu.bitcast(blk.reshape(blk.shape[0] * 8, 128), bf16)


def _wcols(wu, rows, nts):
    return jnp.concatenate([_wtile(wu, rows, n) for n in nts], axis=1)


def _rows16(a, b):
    return jnp.concatenate([a, b], axis=0).astype(bf16)


def _slot(G, t):
    j = 4 * (t >> 3) + ((((t >> 1) & 3) + G + 2 * (t & 1) + (t >> 3)) & 3)
    return 2 * G + (t & 1), 8 * j


def _xslot(G, t):
    return G // 2, 8 * (4 * (t >> 3) + ((((t >> 1) & 3) + G + (t >> 3)) & 3))


def _vr(n):
    return slice(8 * n, 8 * n + 8)


def _kernel(*refs, t0, wt):
    pl.run_scoped(functools.partial(_body, refs, t0, wt),
                  pltpu.SemaphoreType.DMA((4 + len(W4_CHUNKS) + 2 * NP,)))


def _body(refs, t0, wt, sems):
    (x_hbm, k_hbm, v_hbm, wq_hbm, wo_hbm, w3_hbm, w4_hbm, o_ref,
     kbuf, vbuf, vxbuf, wqu, wo, w3, w4, xbuf, lref, obuf, qa, qb, qx, scl, abuf, zs) = refs[:24]
    pT = refs[24:]
    ku = kbuf.bitcast(u32)
    vu = vbuf.bitcast(u32)
    vx = vxbuf.bitcast(u32)
    wou = wo.bitcast(u32)

    x_cp = pltpu.make_async_copy(x_hbm, xbuf, sems.at[0])
    wq_cp = pltpu.make_async_copy(wq_hbm, vxbuf.at[0:D * 3 // 16], sems.at[1])
    wo_cp = pltpu.make_async_copy(wo_hbm, wo, sems.at[2])
    w3_cp = pltpu.make_async_copy(w3_hbm, w3, sems.at[3])
    w4_rows, r0 = [], 0
    for n in W4_CHUNKS:
        w4_rows.append((r0, r0 + n))
        r0 += n
    w4_cp = [pltpu.make_async_copy(w4_hbm.at[a:b], w4.at[a:b], sems.at[4 + c])
             for c, (a, b) in enumerate(w4_rows)]
    S0 = 4 + len(W4_CHUNKS)

    def k_cp(i):
        return pltpu.make_async_copy(
            k_hbm.at[pl.ds(i * GP, GP), pl.ds(t0 * 8, wt * 8), :],
            kbuf.at[pl.ds(i * GP, GP)], sems.at[S0 + i])

    def v_cp(i):
        return pltpu.make_async_copy(
            v_hbm.at[pl.ds(i * GP, GP), pl.ds(t0 * 8, wt * 8), :],
            vbuf.at[pl.ds(i * GP, GP)], sems.at[S0 + NP + i])

    for c in (wq_cp, x_cp, wo_cp):
        c.start()
    for i in range(NP):
        k_cp(i).start()
        v_cp(i).start()
    for c in [w3_cp] + w4_cp:
        c.start()

    zs[0] = 0
    for ref in (qa, qb, qx, lref):
        ref[_vr(5), :] = jnp.zeros((8, 128), u32)

    lane = lax.broadcasted_iota(jnp.int32, (8, 128), 1)
    sub = lax.broadcasted_iota(jnp.int32, (8, 128), 0)
    lane_lo = lane < 64
    sub_lo = sub < 4

    def tile(ref, g0, G, t):
        g, r = _slot(G, t)
        return ref[g0 + g, r:r + 8, :]

    def retile(ref, i, expand):
        def body(c, carry):
            g0 = i * GP + 8 * c
            for G in range(4):
                for J in range(4):
                    xs = [[ref[g0 + 2 * G + e, _vr(4 * J + jj), :] for jj in range(4)]
                          for e in range(2)]
                    for jj in range(4):
                        x0, x1 = xs[0][jj], xs[1][jj]
                        ys = (jnp.where(sub_lo, x0, pltpu.roll(x1, 4, 0)),
                              jnp.where(sub_lo, pltpu.roll(x0, 4, 0), x1))
                        for e in range(2):
                            t = 8 * J + 2 * jj + e
                            g, r = _slot(G, t)
                            if expand and G % 2 and e:
                                ref[g0 + g, r:r + 8, :] = ys[e] << 16
                                g, r = _xslot(G, t)
                                vx[i * (GP // 4) + 2 * c + g, r:r + 8, :] = ys[e] & jnp.uint32(HI)
                            else:
                                ref[g0 + g, r:r + 8, :] = ys[e]
            return carry
        lax.fori_loop(0, GP // 8, body, 0)

    def merge_halves(get, nt, n):
        lo, hi = get(n // 2), get((nt + n) // 2)
        if n % 2:
            lo = pltpu.roll(lo, 4, 0)
        if (nt + n) % 2 == 0:
            hi = pltpu.roll(hi, 4, 0)
        return jnp.where(sub_lo, lo, hi)

    def retile_wq(G, carry):
        for n in range(3 * NP):
            wqu[n // 3 * (D // 16) + G, n % 3] = merge_halves(
                lambda v: vx[3 * G + v // 16, _vr(v % 16), :], 3 * NP, n)
        return carry

    def retile_wo(c, carry):
        for G in range(8):
            xs = [wou[8 * c + G, n] for n in range(5)]
            for n in range(5):
                wou[8 * c + G, n] = merge_halves(lambda v: xs[v], 5, n)
        return carry

    def lhs_at(ref, n):
        return pltpu.bitcast(ref[_vr(n), :], bf16)

    cur = [None]

    def new_block():
        cur[0] = -32 * jnp.clip(zs[0], 0, 1)

    def tick(ref, n, val):
        if val.dtype != ref.dtype:
            val = pltpu.bitcast(val, ref.dtype)
        ref[pl.ds(pl.multiple_of(cur[0] + 8 * n, 8), 8), :] = val

    def q_dots(i, st, qref, lhs=None, mean=None):
        def step(k):
            def run(tied=False):
                w = _wcols(wqu, pl.ds(i * (D // 16) + 8 * k, 8), range(3))
                if lhs is None:
                    r = jnp.dot(lhs_at(lref, L_Y + k), w, preferred_element_type=f32)[0:8]
                else:
                    r = jnp.dot(lhs[:, 128 * k:128 * k + 128], w, preferred_element_type=f32)
                st["q"] = r if k == 0 else st["q"] + r
                if k == 4:
                    q = st["q"] if lhs is None else st["q"][0:8] - mean * st["q"][8:16]
                    qq = pltpu.bitcast(q.astype(bf16).astype(f32), u32)
                    q0, q1, q2 = qq[:, 0:128], qq[:, 128:256], qq[:, 256:384]
                    for n, v in enumerate((q0 >> 16, q0, q2 >> 16, q2, q1)):
                        qref[_vr(n), :] = v
                        if n < 2 and qref is qb:
                            qx[_vr(n), :] = v
                return r[0:8, 256:384]
            return 3, lref, L_DUMMY, run
        return [step(k) for k in range(5)]

    def o_dot(i, b, st, get_lhs, tref=None):
        def run(tied=False):
            w = _wcols(wou, pl.ds(i * (GP // 2) + 8 * b, 8), range(5))
            lhs = get_lhs() | tref[_vr(5), :] if tied and tref is not obuf else get_lhs()
            r = jnp.dot(pltpu.bitcast(lhs, bf16), w, preferred_element_type=f32)[0:8]
            st["acc"] = st["acc"] + r if "acc" in st else r
            return r[:, 512:640]
        return 5, tref, (32 if tref is obuf else 6), run

    def mid_q(st, qref):
        q1 = qref[_vr(4), :]
        q1r = pltpu.roll(q1, 64, 1)
        st["u", 0, qref is qa] = jnp.where(lane_lo, q1 >> 16, q1r)
        st["u", 1, qref is qa] = jnp.where(lane_lo, q1r >> 16, q1)

    def k_dots(i, hh, st, qref, order=tuple(range(12)), nalt=0):
        g0 = i * GP
        gf, gh = ((0, 8), (16, 12))[hh]

        def step(r):
            src = qx if r in order[:nalt] else qref

            def run(tied=False):
                if r < 8:
                    cols = [[tile(ku, g0, gf + G, 8 * T + r) for G in range(8)] for T in range(4)]
                    base, row = src[_vr(2 * hh + r % 2), :], r // 2
                else:
                    cols = [[tile(ku, g0, gh + G % 4, 8 * T + 2 * (r - 8) + G // 4)
                             for G in range(8)] for T in range(4)]
                    if ("u", hh, qref is qa) not in st:
                        mid_q(st, qref)
                    base, row = st["u", hh, qref is qa], r - 8
                    if tied:
                        base = base | src[_vr(5), :]
                lhs = jnp.where(sub == row, base, jnp.zeros((8, 128), u32))
                w = jnp.concatenate([jnp.concatenate(c, axis=0) for c in cols], axis=1)
                res = jnp.dot(pltpu.bitcast(lhs, bf16), pltpu.bitcast(w, bf16),
                              preferred_element_type=f32)[0:8]
                st["s", hh] = res if r == order[0] else st["s", hh] + res
                return res[:, 384:512]
            return 4, src, 6, run
        return [step(r) for r in order]

    def col(s, T):
        return s[:, 128 * T:128 * T + 128]

    def row_max(s):
        m = jnp.maximum(jnp.maximum(col(s, 0), col(s, 1)), jnp.maximum(col(s, 2), col(s, 3)))
        return jnp.max(jnp.max(m, axis=1, keepdims=True), axis=0, keepdims=True)

    def prob(s, m):
        return jnp.exp2((s - m) * scl[_vr(0), :])

    def put_p(hh, T, p, ks=range(8)):
        for k in ks:
            pT[4 * hh + T][pl.ds(k, 8, stride=8), :] = p

    def part_sum(p):
        return (p[0] + p[1]) + (p[2] + p[3])

    def inv_sum(l):
        l = jnp.sum(jnp.sum(l, axis=1, keepdims=True), axis=0, keepdims=True)
        r = pl.reciprocal(l, approx=True)
        return jnp.broadcast_to(r * (2.0 - l * r), (8, 128))

    def softmax(s, hh):
        m = row_max(s)
        p = [prob(col(s, T), m) for T in range(4)]
        for T in range(4):
            put_p(hh, T, p[T])
        return p, part_sum(p)

    def get_state(i, n):
        return pltpu.bitcast(ku[i * GP + 3, _vr(n), :], f32)

    def set_state(i, n, v):
        ku[i * GP + 3, _vr(n), :] = pltpu.bitcast(v, u32)

    def stash_b(i, s):
        for T in range(4):
            set_state(i, T, col(s, T))
        m = jnp.broadcast_to(row_max(s), (8, 128))
        set_state(i, S_MAXB, m)
        return m

    def pack8(v):
        return pltpu.bitcast(v.astype(bf16), u32)

    def x_dots(i, hh, ts, get_lhs, tref=None):
        st = {}
        rows = sorted({t % 8 for t in ts})

        def step(n, rho):
            def run(tied=False):
                res = []
                for T in [t // 8 for t in ts if t % 8 == rho]:
                    w = jnp.concatenate(
                        [tile(vu, i * GP, GX[hh] + G, 8 * T + rho) for G in range(8)], axis=0)
                    lhs = get_lhs(T) | tref[_vr(5), :] if tied else get_lhs(T)
                    res.append(jnp.dot(pltpu.bitcast(lhs, bf16), pltpu.bitcast(w, bf16),
                                       preferred_element_type=f32)[0:8])
                st["x"] = jnp.where(sub == rho, sum(res[1:], res[0]), st["x"] if n else 0.0)
                if n == len(rows) - 1:
                    set_state(i, S_X + hh, st["x"])
                return res[-1]
            return sum(1 for t in ts if t % 8 == rho), tref, 6, run
        return [step(n, rho) for n, rho in enumerate(rows)]

    def transpose_x(i, xrows):
        for hh in range(2):
            for t in xrows[hh]:
                w = jnp.concatenate([tile(vu, i * GP, GX[hh] + G, t) for G in range(8)], axis=0)
                w = pltpu.bitcast(pltpu.bitcast(w, bf16).astype(f32).T.astype(bf16), u32)
                for G in range(8):
                    g, r = _slot(GX[hh] + G, t)
                    vu[i * GP + g, r:r + 8, :] = w[_vr(G), :]

    def reduce_o(blocks, inva, invb, extra=(None, None, None)):
        out = []
        for b, inv in enumerate((inva, jnp.where(lane_lo, inva, invb), invb)):
            z = jnp.sum(pltpu.bitcast(blocks[b], f32).T.reshape(16, 8, 128), axis=0)
            if extra[b] is not None:
                z = z + extra[b]
            out.append(z * inv)
        return out

    def pack16(v):
        return pltpu.bitcast(_rows16(v, v), u32)

    def mac(acc, n, c, G, t, pv):
        w = tile(vu, 8 * c, G, t)
        if G % 2 and t % 2:
            g, r = _xslot(G, t)
            halves = (w, vx[2 * c + g, r:r + 8, :])
        else:
            halves = (w << 16, w & jnp.uint32(HI))
        for k in range(2):
            a = pltpu.bitcast(halves[k], f32) * pv
            acc[n + k] = a if acc[n + k] is None else acc[n + k] + a

    def seg_rows(xrows, seg):
        hh, gp, T = seg // 24 % 2, seg % 24 // 4, seg % 4
        on_mxu = GX[hh] <= 12 * hh + 2 * gp < GX[hh] + 8
        return [rho for rho in range(8) if not (on_mxu and 8 * T + rho in xrows[hh])]

    def run_block(pairs, xrows, dots, hooks, plan):
        tie, clk = plan
        clock = []

        def emit(upto):
            while len(clock) < upto:
                n = len(clock)
                for h in hooks.get(("dot", n), ()):
                    h()
                clock.append(dots[n][3](n in tie.values()))

        zero = jnp.zeros((8, 128), f32)
        used = {}
        for seg in range(48 * len(pairs)):
            i, hh, gp, T = pairs[seg // 48], seg // 24 % 2, seg % 24 // 4, seg % 4
            if T == 0:
                a4 = [None] * 4
            pref = pT[4 * hh + T]
            upto = min([v for k, v in tie.items() if k >= seg]
                       + [k[1] for k, v in hooks.items() if k[0] == "after" and v >= seg]
                       + [len(dots) if tie else clk[seg] + 6])
            free = not any(k in tie for k in range(seg, seg - T + 4))
            if free or ("seg", seg) in hooks:
                upto = max(upto, clk[seg] + 1)
            emit(min(len(dots), max(upto, hooks.get(("need", seg), 0))))
            if free:
                tick(pref, 8, clock[clk[seg]])
            elif gp:
                tick(pref, 8, zero)
            for h in hooks.get(("seg", seg), ()):
                h(clock[clk[seg]])
            for rho in seg_rows(xrows, seg):
                pv = pref[_vr(rho), :]
                for e in range(2):
                    mac(a4, 2 * e, i * 6, 12 * hh + 2 * gp + e, 8 * T + rho, pv)
            if seg in tie:
                ref, slot = dots[tie[seg]][1:3]
                used[tie[seg]] = used.get(tie[seg], -1) + 1
                for k in range(4):
                    tick(ref, slot + 4 * used[tie[seg]] + k, a4[k])
            if T == 3:
                for n in range(4):
                    G = 12 * hh + 2 * gp + n // 2
                    ku[i * GP + G // 8, pl.ds(16 * (G % 8) + n % 2, 8, stride=2), :] = (
                        pltpu.bitcast(a4[n], u32))
        emit(len(dots))

    def run_all(dots):
        for d in dots:
            d[3]()

    def set_input(c, scale):
        cp = pltpu.bitcast(_rows16(c, c), u32)
        for k in range(5):
            lref[_vr(L_Y + k), :] = cp[:, 128 * k:128 * k + 128]
        scl[_vr(0), :] = jnp.broadcast_to(scale, (8, 128))

    x_cp.wait()
    x = jnp.broadcast_to(xbuf[...].astype(f32), (8, D))
    set_input(_ln(x), jnp.full((8, 1), CEXP, f32))
    wq_cp.wait()
    lax.fori_loop(0, D // 16, retile_wq, 0)
    wo_cp.wait()
    lax.fori_loop(0, H * DH // 128, retile_wo, 0)

    def row_sum(a):
        return jnp.broadcast_to(jnp.sum(a, axis=0, keepdims=True), a.shape)

    def body1(i, acc):
        st = {"acc": acc}
        k_cp(i).wait()
        retile(ku, i, False)
        run_all(q_dots(i, st, qa))
        inv = []
        for hh in range(2):
            run_all(k_dots(i, hh, st, qa))
            inv.append(inv_sum(softmax(st["s", hh], hh)[1]))

        @pl.when(i > 2)
        def _():
            transpose_x(i - 1, XROWS)

        v_cp(i).wait()
        retile(vu, i, True)
        for hh in range(2):
            def pv_step(c, carry, hh=hh):
                acc8 = [None] * 8
                for t in range(32):
                    pv = pT[4 * hh + t // 8][_vr(t % 8), :]
                    for G in range(4):
                        mac(acc8, 2 * G, i * 6 + c, G, t, pv)
                for n in range(8):
                    obuf[pl.ds(64 * c + 16 * (n // 2) + n % 2, 8, stride=2), :] = (
                        pltpu.bitcast(acc8[n], u32))
                return carry
            lax.fori_loop(3 * hh, 3 * hh + 3, pv_step, 0)
        o = reduce_o([obuf[128 * b:128 * b + 128, :] for b in range(3)], inv[0], inv[1])
        run_all([o_dot(i, b, st, lambda b=b: pack16(o[b])) for b in range(3)])
        return st["acc"]

    x = x + row_sum(lax.fori_loop(0, NP, body1, jnp.zeros((8, D), f32)))

    y = _ln(x)
    zz = _ln(y).astype(bf16)
    w3_cp.wait()
    h = jnp.dot(zz, w3[...], preferred_element_type=f32)
    h = jax.nn.gelu(h, approximate=True).astype(bf16)
    x = x + y
    transpose_x(NP - 1, XROWS_LAST)
    for cp, (a, b) in zip(w4_cp, w4_rows):
        cp.wait()
        x = x + jnp.dot(h[:, a:b], w4[a:b, :], preferred_element_type=f32)

    ones = jnp.ones((8, D), f32)
    xl = _rows16(x, ones)
    xb = xl[0:8].astype(f32)
    mean = _mean(xb)
    c = xb - mean
    set_input(c, lax.rsqrt(_mean(c * c) + EPS) * CEXP)
    abuf[...] = jnp.where(lax.broadcasted_iota(jnp.int32, (8, D), 0) == 0, x, 0.0)

    def tail_hooks(i, st, hooks, seg0):
        def first(_):
            m = row_max(st["s", 0])
            st["pa"] = [prob(col(st["s", 0], T), m) for T in range(4)]
            set_state(i, S_INVA, inv_sum(part_sum(st["pa"])))
            for T in range(4):
                ku[i * GP + 3, 8 * (S_PA + T):8 * (S_PA + T) + 4, :] = pack8(st["pa"][T])

        def put(T, half):
            def run(clk):
                tick(pT[T], 8, clk)
                put_p(0, T, st["pa"][T], range(4 * half, 4 * half + 4))
            return run
        hooks.setdefault(("seg", seg0), []).append(first)
        for n in range(8):
            hooks.setdefault(("seg", seg0 + n), []).append(put(n // 2, n % 2))

    def head_b_hooks(i, segs, pb, final=False):
        def put_b(T):
            def run(clk):
                tick(scl, 4, clk)
                pb.append(prob(get_state(i, T), get_state(i, S_MAXB)))
                put_p(1, T, pb[T])
                if T == 3:
                    set_state(i, S_LB, inv_sum(part_sum(pb)) if final else part_sum(pb))
            return run
        return {("seg", segs[T]): [put_b(T)] for T in range(4)}

    def reduce_pair(i, xrows, final=False):
        xa, xb = (get_state(i, S_X + hh) if xrows[hh] else None for hh in range(2))
        invb = get_state(i, S_LB) if final else inv_sum(get_state(i, S_LB))
        return reduce_o([ku[i * GP + b] for b in range(3)],
                        get_state(i, S_INVA), invb, (xa, None, xb))

    st = {}
    new_block()
    late = tuple(range(8, 12)) + tuple(range(8))
    d0 = q_dots(0, st, qb, xl, mean) + q_dots(1, st, qa, xl, mean)
    d1 = k_dots(0, 0, st, qb) + k_dots(0, 1, st, qb, late) + k_dots(1, 0, st, qa, late) \
        + k_dots(1, 1, st, qa) + q_dots(2, st, qb)

    def sm_a0():
        m = row_max(st["s", 0])
        p = [prob(col(st["s", 0], T), m) for T in range(4)]
        tick(qb, 6, part_sum(p))
        put_p(0, 0, p[0])
        st["p0"] = p
        set_state(0, S_INVA, inv_sum(part_sum(p)))

    def put_a0(T):
        def run(clk):
            tick(pT[T], 8, clk)
            put_p(0, T, st["p0"][T])
        return run

    def sm_b0():
        tick(qa, 6, stash_b(0, st["s", 1]))

    hooks = head_b_hooks(0, range(B0_SEG, 48, 3), [])
    hooks.update({("dot", DA0): [sm_a0], ("dot", DB0): [sm_b0],
                  ("need", 0): DA0 + 1, ("need", B0_SEG): DB0 + 1, ("need", A1_SEG): 46})
    hooks.update({("seg", T): [put_a0(T + 1)] for T in range(3)})
    tail_hooks(1, st, hooks, A1_SEG)
    run_block([0], XNONE, d0 + d1, hooks, PLANS["first"])
    for n in range(4):
        set_state(n // 2, S_X + n % 2, jnp.zeros((8, 128), f32))
    stash_b(1, st["s", 1])

    qs = (qb, qa)

    def block(name, j, ks, reds, qn, xrows):
        last = ks == [NP - 1]
        a_seg = {"second": A_SEG2, "third": A_SEG3}.get(name, A_SEG0)
        b_segs = {"second": B_SEGS2, "third": B_SEGS3,
                  "last": range(B_SEGL, 48, 3)}.get(name, B_SEGS)
        new_block()
        st = {}
        for k in ks if not last else []:
            mid_q(st, qs[(k + 1) % 2])
        outs = [reduce_pair(j + r, XROWS) for r in reds]

        def kept(n):
            return (0, 1, 2) if last else (1, 2) if reds[n] == NP - 3 else (2,)

        def keep():
            for n, r in enumerate(reds):
                for b in kept(n):
                    obuf[pl.ds(pl.multiple_of(8 * (j + r + (2 - b) * 6), 8), 4), :] = (
                        pack8(outs[n][b]))

        if not last:
            keep()
        pb = []
        hooks = head_b_hooks(j + ks[0], b_segs, pb, last)
        dots = []

        def hook(key, fn):
            hooks.setdefault(key, []).append(fn)

        def direct(i, hh, seg0, tref):
            p = []

            def run():
                m = row_max(st["s", hh])
                p.extend(prob(col(st["s", hh], T), m) for T in range(4))
                l = part_sum(p)
                set_state(i, (S_INVA, S_LB)[hh], l if hh else inv_sum(l))

            def put(T, half):
                def go(clk):
                    tick(pT[4 * hh + T], 8, clk)
                    put_p(hh, T, p[T], range(4 * half, 4 * half + 4))
                return go
            hook(("dot", len(dots)), run)
            dots.extend(x_dots(i, hh, xrows[hh], lambda T: pack16(p[T]), tref))
            hooks["need", seg0] = len(dots)
            for n in range(8):
                hook(("seg", seg0 + n), put(n // 2, n % 2))

        def wo_of(n):
            return [o_dot(j + reds[n], b, st, lambda b=b: pack16(outs[n][b]), lref)
                    for b in range(3) if b not in kept(n)]

        def wq_of(n):
            nq = j + qn[n]
            return q_dots(nq if isinstance(nq, int) else jnp.minimum(nq, NP - 1), st, qs[qn[n] % 2])

        if last:
            dots += [o_dot(m, 2, st, lambda m=m: obuf[_vr(m), :], obuf) for m in range(NP - 2)]
            dots.append(o_dot(NP - 3, 1, st, lambda: obuf[_vr(NP + 3), :], obuf))
            hooks["after", len(dots)] = b_segs[3]
            dots += x_dots(j + ks[0], 1, xrows[1], lambda T: pack16(pb[T]), lref)
        for n, k in enumerate(ks if not last else []):
            q = qs[(k + 1) % 2]
            dots += k_dots(j + (k + 1), 0, st, q, MIX if n else MIXA, NALT if n else 0)
            if n == 0:
                if xrows[1]:
                    hooks["after", len(dots)] = b_segs[3]
                dots += x_dots(j + ks[0], 1, xrows[1], lambda T: pack16(pb[T]), q)
            else:
                direct(j + k, 1, 48 * n + BD_SEG, q)
            kb = k_dots(j + (k + 1), 1, st, q, MIX)
            if n < len(ks) - 1:
                dots += kb[:XA_AT]
                direct(j + (k + 1), 0, 48 * n + AD_SEG, q)
                dots += kb[XA_AT:] + wq_of(n) + wo_of(n)
            else:
                hooks["need", 48 * n + a_seg] = len(dots)
                tail_hooks(j + (k + 1), st, hooks, 48 * n + a_seg)
                dots += kb
                hook(("dot", len(dots)), lambda k=k: stash_b(j + (k + 1), st["s", 1]))
                for m in range(n, len(qn)):
                    dots += wq_of(m)
                for m in range(n, len(reds)):
                    dots += wo_of(m)
                dots += x_dots(j + ks[0], 0, xrows[0],
                               lambda T: ku[(j + ks[0]) * GP + 3, _vr(S_PA + T), :], lref)
        run_block([j + k for k in ks], xrows, dots, hooks, PLANS[name])
        if last:
            keep()
        if reds:
            abuf[...] += st["acc"]

    def body2(n, carry):
        block("body", 2 * n, [2, 3], [0, 1], [5, 6], XROWS)
        return carry

    pl.when(zs[0] == 0)(lambda: block("second", 0, [1], [], [3, 4], XNONE))
    lax.fori_loop(0, NP // 2 - 2, body2, 0)
    pl.when(zs[0] == 0)(lambda: block("third", 0, [NP - 2], [NP - 4, NP - 3], [], XROWS))
    pl.when(zs[0] <= 0)(lambda: block("last", 0, [NP - 1], [NP - 2], [], XROWS_LAST))

    st = {"acc": abuf[...]}
    run_all(x_dots(NP - 1, 0, XROWS_LAST[0], lambda T: ku[(NP - 1) * GP + 3, _vr(S_PA + T), :]))
    o = reduce_pair(NP - 1, XROWS_LAST, True)
    run_all([o_dot(NP - 2, b, st, lambda b=b: obuf[_vr(NP - 2 + (2 - b) * 6), :]) for b in range(3)])
    run_all([o_dot(NP - 1, b, st, lambda b=b: pack16(o[b])) for b in range(3)])
    x = row_sum(st["acc"])

    xl = _rows16(x, ones)
    d = xl[0:8].astype(f32) - mean
    md = _mean(d)
    r1 = lax.rsqrt(jnp.maximum(_mean(d * d) - md * md, 0.0) + EPS)
    mean = mean + md
    y = (d - md) * r1
    my = _mean(y)
    r2 = lax.rsqrt(jnp.maximum(_mean(y * y) - my * my, 0.0) + EPS)
    h = jnp.dot(xl, w3[...], preferred_element_type=f32)
    h = h[0:8] * (r1 * r2) - h[8:16] * ((mean * r1 + my) * r2)
    h = jax.nn.gelu(h, approximate=True).astype(bf16)
    x = x + y
    for k in range(0, F, 128):
        x = x + jnp.dot(h[:, k:k + 128], w4[k:k + 128, :], preferred_element_type=f32)
    o_ref[...] = x[0:1].astype(o_ref.dtype)


def _cache_view(c):
    s = c.shape[2]
    c = jnp.transpose(c, (0, 1, 3, 2)).reshape(H * DH // 8, 8, s // 128, 128)
    return jnp.transpose(c, (0, 2, 1, 3)).reshape(H * DH // 8, s // 128 * 8, 128)


def _weight_view(w):
    k, n = w.shape
    w = jnp.transpose(w.reshape(k // 16, 2, 8, n // 128, 128), (0, 1, 3, 2, 4))
    return w.reshape(k // 16, n // 128, 16, 128)


@jax.jit
def pallas_interleave_layers__sliding_block_cached__mixer_s_mlp__decode_kernel(
    A_x: jax.Array,
    A_k_cache: jax.Array,
    A_v_cache: jax.Array,
    A_wq: jax.Array,
    A_wo: jax.Array,
    B_x: jax.Array,
    B_w1: jax.Array,
    B_w2: jax.Array,
    B_w3: jax.Array,
    B_w4: jax.Array,
):
    sk = A_k_cache.shape[2]
    win = min(4096, max(256, sk // 4))
    assert win == 4096 and sk % 128 == 0
    assert A_x.shape == (1, 1, D) and A_k_cache.shape == (1, H, sk, DH)
    wt = win // 128
    t0 = sk // 128 - wt
    ng = H * DH // 8
    hbm = pl.BlockSpec(memory_space=pl.ANY)
    out = pl.pallas_call(
        functools.partial(_kernel, t0=t0, wt=wt),
        out_shape=jax.ShapeDtypeStruct((1, D), A_x.dtype),
        in_specs=[hbm] * 7,
        out_specs=pl.BlockSpec(memory_space=pltpu.VMEM),
        scratch_shapes=[
            pltpu.VMEM((ng, wt * 8, 128), bf16),
            pltpu.VMEM((ng, wt * 8, 128), bf16),
            pltpu.VMEM((ng // 4, 256, 128), bf16),
            pltpu.VMEM((NP * D // 16, 3, 8, 128), u32),
            pltpu.VMEM((H * DH // 16, D // 128, 16, 128), bf16),
            pltpu.VMEM((D, F), bf16),
            pltpu.VMEM((F, D), bf16),
            pltpu.VMEM((1, D), bf16),
            pltpu.VMEM((144, 128), u32),
            pltpu.VMEM((384, 128), u32),
            pltpu.VMEM((144, 128), u32),
            pltpu.VMEM((144, 128), u32),
            pltpu.VMEM((144, 128), u32),
            pltpu.VMEM((40, 128), f32),
            pltpu.VMEM((8, D), f32),
            pltpu.SMEM((1,), jnp.int32),
        ] + [pltpu.VMEM((72, 128), f32)] * 8,
        compiler_params=pltpu.CompilerParams(vmem_limit_bytes=128 * 1024 * 1024),
    )(A_x.reshape(1, D), _cache_view(A_k_cache), _cache_view(A_v_cache),
      _weight_view(A_wq).reshape(D * 3 // 16, 256, 128), _weight_view(A_wo), B_w3, B_w4)
    return out.reshape(1, 1, D)
```

```python
import functools

import jax
import jax.numpy as jnp
from jax import lax
import jax.experimental.pallas as pl
import jax.experimental.pallas.tpu as pltpu

D = 640
H = 32
DH = 192
F = 1536
EPS = 1e-5
NP = H // 2
GP = 2 * DH // 8
HI = 0xFFFF0000
CEXP = DH ** -0.5 * 1.4426950408889634

f32 = jnp.float32
bf16 = jnp.bfloat16
u32 = jnp.uint32

L_Y = 0
L_DUMMY = 6
S_MAXB, S_LB, S_INVA, S_X, S_PA, S_PB = 4, 5, 6, 7, 9, 13
XROWS = ((2, 10, 18, 26), (4, 12, 20))
XROWS_LAST = (tuple(range(0, 32, 2)), tuple(t for t in range(0, 32, 2) if t % 8))
GX = (0, 16)
PLANS = {
    "first": (
        {},
        (23, 23, 23, 25, 25, 25, 26, 26, 27, 28, 28, 29, 30, 29, 31, 32, 32, 33, 35, 34, 35, 37,
        38, 38, 39, 39, 39, 40, 40, 41, 42, 42, 43, 44, 44, 45, 46, 46, 46, 47, 48, 49, 50, 50,
        51, 52, 52, 53, 54, 54, 55, 56, 56, 57, 58, 58, 59, 60, 60, 61, 62, 62, 63, 64, 63, 65,
        66, 66, 67, 68, 68, 69, 70, 70, 71, 72, 72, 74, 75, 75, 76, 77, 77, 78, 79, 79, 80, 81,
        81, 81, 82, 82, 83, 83, 84, 85)),
    "body": (
        {1: 0, 3: 1, 5: 3, 7: 4, 9: 5, 11: 8, 12: 10, 15: 10, 19: 12, 21: 14, 23: 16, 25: 17,
        27: 19, 29: 22, 31: 23, 33: 23, 35: 26, 37: 26, 39: 28, 40: 33, 41: 33, 43: 34, 45: 34,
        47: 34, 49: 35, 51: 37, 53: 38, 55: 39, 57: 40, 59: 42, 61: 43, 63: 46, 67: 49, 70: 51,
        71: 52, 72: 53, 75: 55, 77: 56, 79: 58, 81: 59, 83: 62, 84: 62},
        (0, 0, 0, 0, 0, 0, 0, 0, 0, 0, 0, 1, 2, 2, 3, 4, 4, 5, 6, 7, 7, 8, 9, 10, 10, 12, 12,
        13, 14, 15, 15, 16, 16, 17, 17, 18, 20, 21, 21, 24, 25, 23, 24, 27, 27, 33, 29, 29, 28,
        30, 30, 31, 31, 32, 33, 33, 34, 35, 35, 36, 36, 35, 35, 36, 37, 39, 43, 41, 43, 40, 45,
        45, 46, 48, 48, 48, 49, 50, 50, 51, 52, 51, 51, 54, 53, 54, 56, 58, 57, 59, 61, 59, 61,
        62, 63, 64)),
    "third": (
        {1: 0, 3: 3, 6: 3, 7: 4, 9: 5, 11: 8, 15: 10, 18: 12, 19: 14, 21: 14, 23: 15, 25: 17,
        26: 19, 27: 19, 30: 22},
        (0, 0, 0, 0, 0, 0, 0, 0, 0, 0, 1, 0, 0, 3, 3, 5, 2, 5, 4, 8, 7, 8, 10, 10, 10, 12, 12,
        13, 15, 17, 15, 16, 17, 17, 18, 19, 20, 18, 21, 22, 22, 24, 25, 26, 25, 24, 25, 25)),
    "last": (
        {0: 0, 3: 0, 7: 0, 9: 2, 11: 2, 15: 2, 17: 5, 19: 5, 21: 8, 23: 8, 25: 11, 27: 11,
        29: 13, 31: 13},
        (0, 0, 0, 0, 0, 0, 0, 1, 0, 1, 2, 1, 0, 0, 0, 0, 0, 0, 0, 0, 0, 0, 1, 3, 4, 5, 5, 6, 7,
        7, 6, 6, 9, 9, 10, 10, 11, 11, 12, 12, 13, 13, 14, 13, 14, 14, 16, 16)),
}
MIX = (0, 1, 8, 2, 3, 9, 4, 5, 10, 6, 7, 11)
MIXA = (0, 1, 2, 3, 4, 8, 5, 9, 6, 10, 7, 11)
B_SEGS = (9, 12, 15, 18)
B_SEGL = 7
DA0 = 27
DW0 = 32
DB0 = 41
DA1 = 55
DB1 = 67
DQ = (26, 29, 33)
NQV = 3
B0_SEG = 18
A1_SEG = 40
B1_SEG = 12
A2_SEG = 40
A_SEG0 = 40
A_SEG3 = 38
B_SEGS3 = (9, 11, 15, 19)
XA_AT = 8
AD_SEG = 32
BD_SEG = 12
NALT = 2
W4_CHUNKS = (1024, 256, 160, 64, 32)
W4_MXU = 1280


def _mean(x):
    return jnp.mean(x, axis=-1, keepdims=True)


def _ln(x):
    c = x - _mean(x)
    return c * lax.rsqrt(_mean(c * c) + EPS)


def _wtile(wu, rows, nt):
    blk = wu[rows, nt]
    return pltpu.bitcast(blk.reshape(blk.shape[0] * 8, 128), bf16)


def _wcols(wu, rows, nts):
    return jnp.concatenate([_wtile(wu, rows, n) for n in nts], axis=1)


def _rows16(a, b):
    return jnp.concatenate([a, b], axis=0).astype(bf16)


def _slot(G, t):
    j = 4 * (t >> 3) + ((((t >> 1) & 3) + G + 2 * (t & 1) + (t >> 3)) & 3)
    return 2 * G + (t & 1), 8 * j


def _xslot(G, t):
    return G // 2, 8 * (4 * (t >> 3) + ((((t >> 1) & 3) + G + (t >> 3)) & 3))


def _vr(n):
    return slice(8 * n, 8 * n + 8)


def _kernel(*refs, t0, wt):
    pl.run_scoped(functools.partial(_body, refs, t0, wt),
                  pltpu.SemaphoreType.DMA((4 + len(W4_CHUNKS) + 2 * NP,)))


def _body(refs, t0, wt, sems):
    (x_hbm, k_hbm, v_hbm, wq_hbm, wo_hbm, w3_hbm, w4_hbm, o_ref,
     kbuf, vbuf, vxbuf, wqu, wo, w3, w4, xbuf, lref, obuf, qa, qb, qx, scl, abuf, zs) = refs[:24]
    qt, pT = refs[24:27], refs[27:]
    ku = kbuf.bitcast(u32)
    vu = vbuf.bitcast(u32)
    vx = vxbuf.bitcast(u32)
    wou = wo.bitcast(u32)

    x_cp = pltpu.make_async_copy(x_hbm, xbuf, sems.at[0])
    wq_cp = pltpu.make_async_copy(wq_hbm, vxbuf.at[0:D * 3 // 16], sems.at[1])
    wo_cp = pltpu.make_async_copy(wo_hbm, wo, sems.at[2])
    w3_cp = pltpu.make_async_copy(w3_hbm, w3, sems.at[3])
    w4_rows, r0 = [], 0
    for n in W4_CHUNKS:
        w4_rows.append((r0, r0 + n))
        r0 += n
    w4_cp = [pltpu.make_async_copy(w4_hbm.at[a:b], w4.at[a:b], sems.at[4 + c])
             for c, (a, b) in enumerate(w4_rows)]
    S0 = 4 + len(W4_CHUNKS)

    def k_cp(i):
        return pltpu.make_async_copy(
            k_hbm.at[pl.ds(i * GP, GP), pl.ds(t0 * 8, wt * 8), :],
            kbuf.at[pl.ds(i * GP, GP)], sems.at[S0 + i])

    def v_cp(i):
        return pltpu.make_async_copy(
            v_hbm.at[pl.ds(i * GP, GP), pl.ds(t0 * 8, wt * 8), :],
            vbuf.at[pl.ds(i * GP, GP)], sems.at[S0 + NP + i])

    for c in (wq_cp, x_cp, wo_cp):
        c.start()
    for i in range(NP):
        k_cp(i).start()
        v_cp(i).start()
    for c in [w3_cp] + w4_cp:
        c.start()

    zs[0] = 0
    for ref in (qa, qb, qx, lref):
        ref[_vr(5), :] = jnp.zeros((8, 128), u32)

    lane = lax.broadcasted_iota(jnp.int32, (8, 128), 1)
    sub = lax.broadcasted_iota(jnp.int32, (8, 128), 0)
    lane_lo = lane < 64
    sub_lo = sub < 4

    def tile(ref, g0, G, t):
        g, r = _slot(G, t)
        return ref[g0 + g, r:r + 8, :]

    def retile(ref, i, expand):
        def body(c, carry):
            g0 = i * GP + 8 * c
            for G in range(4):
                for J in range(4):
                    xs = [[ref[g0 + 2 * G + e, _vr(4 * J + jj), :] for jj in range(4)]
                          for e in range(2)]
                    for jj in range(4):
                        x0, x1 = xs[0][jj], xs[1][jj]
                        ys = (jnp.where(sub_lo, x0, pltpu.roll(x1, 4, 0)),
                              jnp.where(sub_lo, pltpu.roll(x0, 4, 0), x1))
                        for e in range(2):
                            t = 8 * J + 2 * jj + e
                            g, r = _slot(G, t)
                            if expand and G % 2 and e:
                                ref[g0 + g, r:r + 8, :] = ys[e] << 16
                                g, r = _xslot(G, t)
                                vx[i * (GP // 4) + 2 * c + g, r:r + 8, :] = ys[e] & jnp.uint32(HI)
                            else:
                                ref[g0 + g, r:r + 8, :] = ys[e]
            return carry
        lax.fori_loop(0, GP // 8, body, 0)

    def merge_halves(get, nt, n):
        lo, hi = get(n // 2), get((nt + n) // 2)
        if n % 2:
            lo = pltpu.roll(lo, 4, 0)
        if (nt + n) % 2 == 0:
            hi = pltpu.roll(hi, 4, 0)
        return jnp.where(sub_lo, lo, hi)

    def retile_wq(G, carry):
        for n in range(3 * NP):
            wqu[n // 3 * (D // 16) + G, n % 3] = merge_halves(
                lambda v: vx[3 * G + v // 16, _vr(v % 16), :], 3 * NP, n)
        return carry

    def retile_wo(c, carry):
        for G in range(8):
            xs = [wou[8 * c + G, n] for n in range(5)]
            for n in range(5):
                wou[8 * c + G, n] = merge_halves(lambda v: xs[v], 5, n)
        return carry

    def lhs_at(ref, n):
        return pltpu.bitcast(ref[_vr(n), :], bf16)

    cur = [None]

    def new_block():
        cur[0] = -32 * jnp.clip(zs[0], 0, 1)

    def tick(ref, n, val):
        if val.dtype != ref.dtype:
            val = pltpu.bitcast(val, ref.dtype)
        ref[pl.ds(pl.multiple_of(cur[0] + 8 * n, 8), 8), :] = val

    def put_q(q, qref):
        qq = pltpu.bitcast(q.astype(bf16).astype(f32), u32)
        q0, q1, q2 = qq[:, 0:128], qq[:, 128:256], qq[:, 256:384]
        for n, v in enumerate((q0 >> 16, q0, q2 >> 16, q2, q1)):
            qref[_vr(n), :] = v
            if n < 2 and qref is qb:
                qx[_vr(n), :] = v

    def transpose_wq(i):
        for k in range(5):
            for n in range(3):
                rows = pl.ds(i * (D // 16) + 8 * k, 8)
                w = pltpu.bitcast(_wtile(wqu, rows, n).astype(f32).T, u32)
                for G in range(8):
                    wqu[i * (D // 16) + 8 * k + G, n] = (w[_vr(2 * G), :] >> 16) | w[_vr(2 * G + 1), :]

    def q_vpu(i, c, qref):
        cols = []
        for n in range(3):
            acc = []
            for G in range(8):
                ws = [wqu[i * (D // 16) + 8 * k + G, n] for k in range(5)]
                for half in (lambda w: w << 16, lambda w: w & jnp.uint32(HI)):
                    t = [pltpu.bitcast(half(ws[k]), f32) * col(c, k) for k in range(5)]
                    acc.append((t[0] + t[1]) + (t[2] + t[3]) + t[4])
            z = jnp.sum(jnp.concatenate(acc, axis=0).T.reshape(16, 8, 128), axis=0)
            cols.append(row_sum(z))
        put_q(jnp.concatenate(cols, axis=1), qref)
        return cols[0] + cols[1] + cols[2]

    def row_sum(a):
        return jnp.broadcast_to(jnp.sum(a, axis=0, keepdims=True), a.shape)

    def q_dots(i, st, qref, lhs=None, mean=None):
        def step(k):
            def run(tied=False):
                w = _wcols(wqu, pl.ds(i * (D // 16) + 8 * k, 8), range(3))
                if lhs is None:
                    r = jnp.dot(lhs_at(lref, L_Y + k), w, preferred_element_type=f32)[0:8]
                else:
                    r = jnp.dot(lhs[:, 128 * k:128 * k + 128], w, preferred_element_type=f32)
                st["q"] = r if k == 0 else st["q"] + r
                if k == 4:
                    q = st["q"] if lhs is None else st["q"][0:8] - mean * st["q"][8:16]
                    put_q(q, qref)
                return r[0:8, 256:384]
            return 3, lref, L_DUMMY, run
        return [step(k) for k in range(5)]

    def o_dot(i, b, st, get_lhs, tref=None):
        def run(tied=False):
            w = _wcols(wou, pl.ds(i * (GP // 2) + 8 * b, 8), range(5))
            lhs = get_lhs() | tref[_vr(5), :] if tied and tref is not obuf else get_lhs()
            r = jnp.dot(pltpu.bitcast(lhs, bf16), w, preferred_element_type=f32)[0:8]
            st["acc"] = st["acc"] + r if "acc" in st else r
            return r[:, 512:640]
        return 5, tref, (32 if tref is obuf else 6), run

    def mid_q(st, qref):
        q1 = qref[_vr(4), :]
        q1r = pltpu.roll(q1, 64, 1)
        st["u", 0, id(qref)] = jnp.where(lane_lo, q1 >> 16, q1r)
        st["u", 1, id(qref)] = jnp.where(lane_lo, q1r >> 16, q1)

    def k_dots(i, hh, st, qref, order=tuple(range(12)), nalt=0):
        g0 = i * GP
        gf, gh = ((0, 8), (16, 12))[hh]

        def step(r):
            src = qx if r in order[:nalt] else qref

            def run(tied=False):
                if r < 8:
                    cols = [[tile(ku, g0, gf + G, 8 * T + r) for G in range(8)] for T in range(4)]
                    base, row = src[_vr(2 * hh + r % 2), :], r // 2
                else:
                    cols = [[tile(ku, g0, gh + G % 4, 8 * T + 2 * (r - 8) + G // 4)
                             for G in range(8)] for T in range(4)]
                    if ("u", hh, id(qref)) not in st:
                        mid_q(st, qref)
                    base, row = st["u", hh, id(qref)], r - 8
                    if tied:
                        base = base | src[_vr(5), :]
                lhs = jnp.where(sub == row, base, jnp.zeros((8, 128), u32))
                w = jnp.concatenate([jnp.concatenate(c, axis=0) for c in cols], axis=1)
                res = jnp.dot(pltpu.bitcast(lhs, bf16), pltpu.bitcast(w, bf16),
                              preferred_element_type=f32)[0:8]
                st["s", hh] = res if r == order[0] else st["s", hh] + res
                return res[:, 384:512]
            return 4, src, 6, run
        return [step(r) for r in order]

    def col(s, T):
        return s[:, 128 * T:128 * T + 128]

    def row_max(s):
        m = jnp.maximum(jnp.maximum(col(s, 0), col(s, 1)), jnp.maximum(col(s, 2), col(s, 3)))
        return jnp.max(jnp.max(m, axis=1, keepdims=True), axis=0, keepdims=True)

    def prob(s, m):
        return jnp.exp2((s - m) * scl[_vr(0), :])

    def put_p(hh, T, p, ks=range(8)):
        for k in ks:
            pT[4 * hh + T][pl.ds(k, 8, stride=8), :] = p

    def part_sum(p):
        return (p[0] + p[1]) + (p[2] + p[3])

    def inv_sum(l):
        l = jnp.sum(jnp.sum(l, axis=1, keepdims=True), axis=0, keepdims=True)
        r = pl.reciprocal(l, approx=True)
        return jnp.broadcast_to(r * (2.0 - l * r), (8, 128))

    def softmax(s, hh):
        m = row_max(s)
        p = [prob(col(s, T), m) for T in range(4)]
        for T in range(4):
            put_p(hh, T, p[T])
        return p, part_sum(p)

    def get_state(i, n):
        return pltpu.bitcast(ku[i * GP + 3, _vr(n), :], f32)

    def set_state(i, n, v):
        ku[i * GP + 3, _vr(n), :] = pltpu.bitcast(v, u32)

    def stash_b(i, s):
        for T in range(4):
            set_state(i, T, col(s, T))
        m = jnp.broadcast_to(row_max(s), (8, 128))
        set_state(i, S_MAXB, m)
        return m

    def pack8(v):
        return pltpu.bitcast(v.astype(bf16), u32)

    def park_p(i, n, p):
        ku[i * GP + 3, 8 * n:8 * n + 4, :] = pack8(p)

    def parked(i, n):
        return lambda T: ku[i * GP + 3, _vr(n + T), :]

    def x_dots(i, hh, ts, get_lhs, tref=None):
        st = {}
        rows = sorted({t % 8 for t in ts})

        def step(n, rho):
            def run(tied=False):
                res = []
                for T in [t // 8 for t in ts if t % 8 == rho]:
                    w = jnp.concatenate(
                        [tile(vu, i * GP, GX[hh] + G, 8 * T + rho) for G in range(8)], axis=0)
                    lhs = get_lhs(T) | tref[_vr(5), :] if tied else get_lhs(T)
                    res.append(jnp.dot(pltpu.bitcast(lhs, bf16), pltpu.bitcast(w, bf16),
                                       preferred_element_type=f32)[0:8])
                st["x"] = jnp.where(sub == rho, sum(res[1:], res[0]), st["x"] if n else 0.0)
                if n == len(rows) - 1:
                    set_state(i, S_X + hh, st["x"])
                return res[-1]
            return sum(1 for t in ts if t % 8 == rho), tref, 6, run
        return [step(n, rho) for n, rho in enumerate(rows)]

    def transpose_x(i, xrows):
        for hh in range(2):
            for t in xrows[hh]:
                w = jnp.concatenate([tile(vu, i * GP, GX[hh] + G, t) for G in range(8)], axis=0)
                w = pltpu.bitcast(pltpu.bitcast(w, bf16).astype(f32).T.astype(bf16), u32)
                for G in range(8):
                    g, r = _slot(GX[hh] + G, t)
                    vu[i * GP + g, r:r + 8, :] = w[_vr(G), :]

    def reduce_o(blocks, inva, invb, extra=(None, None, None)):
        out = []
        for b, inv in enumerate((inva, jnp.where(lane_lo, inva, invb), invb)):
            z = jnp.sum(pltpu.bitcast(blocks[b], f32).T.reshape(16, 8, 128), axis=0)
            if extra[b] is not None:
                z = z + extra[b]
            out.append(z * inv)
        return out

    def pack16(v):
        return pltpu.bitcast(_rows16(v, v), u32)

    def mac(acc, n, c, G, t, pv):
        w = tile(vu, 8 * c, G, t)
        if G % 2 and t % 2:
            g, r = _xslot(G, t)
            halves = (w, vx[2 * c + g, r:r + 8, :])
        else:
            halves = (w << 16, w & jnp.uint32(HI))
        for k in range(2):
            a = pltpu.bitcast(halves[k], f32) * pv
            acc[n + k] = a if acc[n + k] is None else acc[n + k] + a

    def seg_rows(xrows, seg):
        hh, gp, T = seg // 24 % 2, seg % 24 // 4, seg % 4
        on_mxu = GX[hh] <= 12 * hh + 2 * gp < GX[hh] + 8
        return [rho for rho in range(8) if not (on_mxu and 8 * T + rho in xrows[hh])]

    def run_block(pairs, xrows, dots, hooks, plan):
        tie, clk = plan
        clock = []

        def emit(upto):
            while len(clock) < upto:
                n = len(clock)
                for h in hooks.get(("dot", n), ()):
                    h()
                clock.append(dots[n][3](n in tie.values()))

        zero = jnp.zeros((8, 128), f32)
        used = {}
        for seg in range(48 * len(pairs)):
            i, hh, gp, T = pairs[seg // 48], seg // 24 % 2, seg % 24 // 4, seg % 4
            if T == 0:
                a4 = [None] * 4
            pref = pT[4 * hh + T]
            upto = min([v for k, v in tie.items() if k >= seg]
                       + [k[1] for k, v in hooks.items() if k[0] == "after" and v >= seg]
                       + [len(dots) if tie else clk[seg] + 6])
            free = not any(k in tie for k in range(seg, seg - T + 4))
            if free or ("seg", seg) in hooks:
                upto = max(upto, clk[seg] + 1)
            emit(min(len(dots), max(upto, hooks.get(("need", seg), 0))))
            if free:
                tick(pref, 8, clock[clk[seg]])
            elif gp:
                tick(pref, 8, zero)
            for h in hooks.get(("seg", seg), ()):
                h(clock[clk[seg]])
            for rho in seg_rows(xrows, seg):
                pv = pref[_vr(rho), :]
                for e in range(2):
                    mac(a4, 2 * e, i * 6, 12 * hh + 2 * gp + e, 8 * T + rho, pv)
            if seg in tie:
                ref, slot = dots[tie[seg]][1:3]
                used[tie[seg]] = used.get(tie[seg], -1) + 1
                for k in range(4):
                    tick(ref, slot + 4 * used[tie[seg]] + k, a4[k])
            if T == 3:
                for n in range(4):
                    G = 12 * hh + 2 * gp + n // 2
                    v = a4[n] * hooks["scale", seg // 24]() if ("scale", seg // 24) in hooks else a4[n]
                    ku[i * GP + G // 8, pl.ds(16 * (G % 8) + n % 2, 8, stride=2), :] = (
                        pltpu.bitcast(v, u32))
        emit(len(dots))

    def run_all(dots):
        for d in dots:
            d[3]()

    def set_input(c, scale):
        cp = pltpu.bitcast(_rows16(c, c), u32)
        for k in range(5):
            lref[_vr(L_Y + k), :] = cp[:, 128 * k:128 * k + 128]
        scl[_vr(0), :] = jnp.broadcast_to(scale, (8, 128))

    x_cp.wait()
    x = jnp.broadcast_to(xbuf[...].astype(f32), (8, D))
    set_input(_ln(x), jnp.full((8, 1), CEXP, f32))
    wq_cp.wait()
    lax.fori_loop(0, D // 16, retile_wq, 0)
    wo_cp.wait()
    lax.fori_loop(0, H * DH // 128, retile_wo, 0)

    def body1(i, acc):
        st = {"acc": acc}
        k_cp(i).wait()
        retile(ku, i, False)
        run_all(q_dots(i, st, qa))
        inv = []
        for hh in range(2):
            run_all(k_dots(i, hh, st, qa))
            inv.append(inv_sum(softmax(st["s", hh], hh)[1]))

        @pl.when(i > 0)
        def _():
            transpose_x(i - 1, XROWS)

        @pl.when(jnp.logical_and(i >= 5 - NQV, i < 5))
        def _():
            transpose_wq(i)

        v_cp(i).wait()
        retile(vu, i, True)
        for hh in range(2):
            def pv_step(c, carry, hh=hh):
                acc8 = [None] * 8
                for t in range(32):
                    pv = pT[4 * hh + t // 8][_vr(t % 8), :]
                    for G in range(4):
                        mac(acc8, 2 * G, i * 6 + c, G, t, pv)
                for n in range(8):
                    obuf[pl.ds(64 * c + 16 * (n // 2) + n % 2, 8, stride=2), :] = (
                        pltpu.bitcast(acc8[n], u32))
                return carry
            lax.fori_loop(3 * hh, 3 * hh + 3, pv_step, 0)
        o = reduce_o([obuf[128 * b:128 * b + 128, :] for b in range(3)], inv[0], inv[1])
        run_all([o_dot(i, b, st, lambda b=b: pack16(o[b])) for b in range(3)])
        return st["acc"]

    x = x + row_sum(lax.fori_loop(0, NP, body1, jnp.zeros((8, D), f32)))

    y = _ln(x)
    zz = _ln(y).astype(bf16)
    w3_cp.wait()
    h = jnp.dot(zz, w3[...], preferred_element_type=f32)
    h = jax.nn.gelu(h, approximate=True).astype(bf16)
    x = x + y
    transpose_x(NP - 1, XROWS_LAST)
    for k in range(W4_MXU, F, 128):
        hk = jnp.broadcast_to(h[0:1, k:k + 128].astype(f32), (128, 128))
        obuf[k - W4_MXU:k - W4_MXU + 128, :] = pltpu.bitcast(hk.T, u32)
    part = jnp.zeros((8, D), f32)
    for cp, (a, b) in zip(w4_cp, w4_rows):
        cp.wait()
        if a < W4_MXU:
            x = x + jnp.dot(h[:, a:b], w4[a:b, :], preferred_element_type=f32)
        else:
            for k in range(a, b, 16):
                hk = pltpu.bitcast(obuf[k - W4_MXU:k - W4_MXU + 16, :], f32)
                t = w4[k:k + 16, :].astype(f32) * jnp.concatenate([hk] * 5, axis=1)
                part = part + (t[0:8] + t[8:16])
    x = x + row_sum(part)

    ones = jnp.ones((8, D), f32)
    xl = _rows16(x, ones)
    xb = xl[0:8].astype(f32)
    mean = _mean(xb)
    c = xb - mean
    set_input(c, lax.rsqrt(_mean(c * c) + EPS) * CEXP)
    abuf[...] = jnp.where(lax.broadcasted_iota(jnp.int32, (8, D), 0) == 0, x, 0.0)

    def tail_hooks(i, st, hooks, seg0, compute=True):
        def first(_):
            m = row_max(st["s", 0])
            st["pa"] = [prob(col(st["s", 0], T), m) for T in range(4)]
            set_state(i, S_INVA, inv_sum(part_sum(st["pa"])))
            for T in range(4):
                park_p(i, S_PA + T, st["pa"][T])

        def put(T, half):
            def run(clk):
                tick(pT[T], 8, clk)
                put_p(0, T, st["pa"][T], range(4 * half, 4 * half + 4))
            return run
        if compute:
            hooks.setdefault(("seg", seg0), []).append(first)
        for n in range(8):
            hooks.setdefault(("seg", seg0 + n), []).append(put(n // 2, n % 2))

    def head_b_hooks(i, segs, pb, final=False, park=False):
        def put_b(T):
            def run(clk):
                tick(scl, 4, clk)
                pb.append(prob(get_state(i, T), get_state(i, S_MAXB)))
                put_p(1, T, pb[T])
                if park and T < 3:
                    park_p(i, S_PB + T, pb[T])
                if T == 3:
                    set_state(i, S_LB, inv_sum(part_sum(pb)) if final else part_sum(pb))
            return run
        return {("seg", segs[T]): [put_b(T)] for T in range(4)}

    def reduce_pair(i, xrows, final=False):
        xa, xb = (get_state(i, S_X + hh) if xrows[hh] else None for hh in range(2))
        invb = get_state(i, S_LB) if final else inv_sum(get_state(i, S_LB))
        return reduce_o([ku[i * GP + b] for b in range(3)],
                        get_state(i, S_INVA), invb, (xa, None, xb))

    st = {}
    new_block()
    late = tuple(range(8, 12)) + tuple(range(8))
    q0, q1, q2 = qt
    dots = q_dots(0, st, q0, xl, mean) + q_dots(1, st, q1, xl, mean) \
        + k_dots(0, 0, st, q0) + k_dots(0, 1, st, q0, late) + k_dots(1, 0, st, q1, late) \
        + k_dots(1, 1, st, q1, late) + k_dots(2, 0, st, q2, late) + k_dots(2, 1, st, q2)
    for n in range(4):
        dots += x_dots(n // 2, n % 2, XROWS[n % 2], parked(n // 2, (S_PA, S_PB)[n % 2]))

    def sm_a0():
        s0 = st["s", 0]
        m = jnp.maximum(jnp.maximum(col(s0, 0), col(s0, 1)), jnp.maximum(col(s0, 2), col(s0, 3)))
        m = jnp.max(m, axis=0, keepdims=True)
        p = [prob(col(s0, T), m) for T in range(4)]
        tick(q0, 6, part_sum(p))
        put_p(0, 0, p[0])
        st["p0"] = p
        st["w"] = prob(m, jnp.max(m, axis=1, keepdims=True))
        set_state(0, S_INVA, inv_sum(part_sum(p) * st["w"]))
        for T in range(4):
            park_p(0, S_PA + T, p[T] * st["w"])

    def put_a0(T):
        def run(clk):
            tick(pT[T], 8, clk)
            put_p(0, T, st["p0"][T])
        return run

    def sm_a1():
        m = row_max(st["s", 0])
        st["pa"] = [prob(col(st["s", 0], T), m) for T in range(4)]
        tick(q1, 6, part_sum(st["pa"]))
        set_state(1, S_INVA, inv_sum(part_sum(st["pa"])))
        for T in range(4):
            park_p(1, S_PA + T, st["pa"][T])

    hooks = head_b_hooks(0, range(B0_SEG, 48, 2), [], park=True)
    hooks.update(head_b_hooks(1, range(48 + B1_SEG, 96, 3), [], park=True))
    hooks.update({("scale", 0): lambda: st["w"],
                  ("need", 0): DA0 + 1, ("need", B0_SEG): DB0 + 1, ("need", A1_SEG): DA1 + 1,
                  ("need", 48 + B1_SEG): DB1 + 1, ("need", 48 + A2_SEG): 70,
                  ("after", 82): 48 + B1_SEG + 9})
    for n, fn in ((10, lambda: mid_q(st, q0)),
                  (DQ[0], lambda: tick(q0, 5, q_vpu(2, c, q2))),
                  (DQ[1], lambda: tick(q0, 5, q_vpu(3, c, qa))),
                  (DQ[2], lambda: tick(q0, 5, q_vpu(4, c, qb))),
                  (DA0, sm_a0), (DW0, lambda: tick(q0, 7, st["w"])),
                  (DB0, lambda: tick(q1, 6, stash_b(0, st["s", 1]))), (DA1, sm_a1),
                  (DB1, lambda: tick(q2, 6, stash_b(1, st["s", 1]))),
                  (82, lambda: stash_b(2, st["s", 1]))):
        hooks.setdefault(("dot", n), []).append(fn)
    hooks.update({("seg", T): [put_a0(T + 1)] for T in range(3)})
    tail_hooks(1, st, hooks, A1_SEG, False)
    tail_hooks(2, st, hooks, 48 + A2_SEG)
    run_block([0, 1], XROWS, dots, hooks, PLANS["first"])

    qs = (qb, qa)

    def block(name, j, ks, reds, qn, xrows):
        last = ks == [NP - 1]
        a_seg = A_SEG3 if name == "third" else A_SEG0
        b_segs = {"third": B_SEGS3,
                  "last": range(B_SEGL, 48, 3)}.get(name, B_SEGS)
        new_block()
        st = {}
        for k in ks if not last else []:
            mid_q(st, qs[(k + 1) % 2])
        outs = [reduce_pair(j + r, XROWS) for r in reds]

        def kept(n):
            return (0, 1, 2) if last else (1, 2) if reds[n] == NP - 3 else (2,)

        def keep():
            for n, r in enumerate(reds):
                for b in kept(n):
                    obuf[pl.ds(pl.multiple_of(8 * (j + r + (2 - b) * 6), 8), 4), :] = (
                        pack8(outs[n][b]))

        if not last:
            keep()
        pb = []
        hooks = head_b_hooks(j + ks[0], b_segs, pb, last)
        dots = []

        def hook(key, fn):
            hooks.setdefault(key, []).append(fn)

        def direct(i, hh, seg0, tref):
            p = []

            def run():
                m = row_max(st["s", hh])
                p.extend(prob(col(st["s", hh], T), m) for T in range(4))
                l = part_sum(p)
                set_state(i, (S_INVA, S_LB)[hh], l if hh else inv_sum(l))

            def put(T, half):
                def go(clk):
                    tick(pT[4 * hh + T], 8, clk)
                    put_p(hh, T, p[T], range(4 * half, 4 * half + 4))
                return go
            hook(("dot", len(dots)), run)
            dots.extend(x_dots(i, hh, xrows[hh], lambda T: pack16(p[T]), tref))
            hooks["need", seg0] = len(dots)
            for n in range(8):
                hook(("seg", seg0 + n), put(n // 2, n % 2))

        def wo_of(n):
            return [o_dot(j + reds[n], b, st, lambda b=b: pack16(outs[n][b]), lref)
                    for b in range(3) if b not in kept(n)]

        def wq_of(n):
            nq = j + qn[n]
            return q_dots(nq if isinstance(nq, int) else jnp.minimum(nq, NP - 1), st, qs[qn[n] % 2])

        if last:
            dots += [o_dot(m, 2, st, lambda m=m: obuf[_vr(m), :], obuf) for m in range(NP - 2)]
            dots.append(o_dot(NP - 3, 1, st, lambda: obuf[_vr(NP + 3), :], obuf))
            hooks["after", len(dots)] = b_segs[3]
            dots += x_dots(j + ks[0], 1, xrows[1], lambda T: pack16(pb[T]), lref)
        for n, k in enumerate(ks if not last else []):
            q = qs[(k + 1) % 2]
            dots += k_dots(j + (k + 1), 0, st, q, MIX if n else MIXA, NALT if n else 0)
            if n == 0:
                if xrows[1]:
                    hooks["after", len(dots)] = b_segs[3]
                dots += x_dots(j + ks[0], 1, xrows[1], lambda T: pack16(pb[T]), q)
            else:
                direct(j + k, 1, 48 * n + BD_SEG, q)
            kb = k_dots(j + (k + 1), 1, st, q, MIX)
            if n < len(ks) - 1:
                dots += kb[:XA_AT]
                direct(j + (k + 1), 0, 48 * n + AD_SEG, q)
                dots += kb[XA_AT:] + wq_of(n) + wo_of(n)
            else:
                hooks["need", 48 * n + a_seg] = len(dots)
                tail_hooks(j + (k + 1), st, hooks, 48 * n + a_seg)
                dots += kb
                hook(("dot", len(dots)), lambda k=k: stash_b(j + (k + 1), st["s", 1]))
                for m in range(n, len(qn)):
                    dots += wq_of(m)
                for m in range(n, len(reds)):
                    dots += wo_of(m)
                dots += x_dots(j + ks[0], 0, xrows[0],
                               parked(j + ks[0], S_PA), lref)
        run_block([j + k for k in ks], xrows, dots, hooks, PLANS[name])
        if last:
            keep()
        if reds:
            abuf[...] += st["acc"]

    def body2(n, carry):
        block("body", 2 * n, [2, 3], [0, 1], [5, 6], XROWS)
        return carry

    lax.fori_loop(0, NP // 2 - 2, body2, 0)
    pl.when(zs[0] == 0)(lambda: block("third", 0, [NP - 2], [NP - 4, NP - 3], [], XROWS))
    pl.when(zs[0] <= 0)(lambda: block("last", 0, [NP - 1], [NP - 2], [], XROWS_LAST))

    st = {"acc": abuf[...]}
    run_all(x_dots(NP - 1, 0, XROWS_LAST[0], parked(NP - 1, S_PA)))
    o = reduce_pair(NP - 1, XROWS_LAST, True)
    run_all([o_dot(NP - 2, b, st, lambda b=b: obuf[_vr(NP - 2 + (2 - b) * 6), :]) for b in range(3)])
    run_all([o_dot(NP - 1, b, st, lambda b=b: pack16(o[b])) for b in range(3)])
    x = row_sum(st["acc"])

    xl = _rows16(x, ones)
    d = xl[0:8].astype(f32) - mean
    md = _mean(d)
    r1 = lax.rsqrt(jnp.maximum(_mean(d * d) - md * md, 0.0) + EPS)
    mean = mean + md
    y = (d - md) * r1
    my = _mean(y)
    r2 = lax.rsqrt(jnp.maximum(_mean(y * y) - my * my, 0.0) + EPS)
    h = jnp.dot(xl, w3[...], preferred_element_type=f32)
    h = h[0:8] * (r1 * r2) - h[8:16] * ((mean * r1 + my) * r2)
    h = jax.nn.gelu(h, approximate=True).astype(bf16)
    x = x + y
    for k in range(0, F, 128):
        x = x + jnp.dot(h[:, k:k + 128], w4[k:k + 128, :], preferred_element_type=f32)
    o_ref[...] = x[0:1].astype(o_ref.dtype)


def _cache_view(c):
    s = c.shape[2]
    c = jnp.transpose(c, (0, 1, 3, 2)).reshape(H * DH // 8, 8, s // 128, 128)
    return jnp.transpose(c, (0, 2, 1, 3)).reshape(H * DH // 8, s // 128 * 8, 128)


def _weight_view(w):
    k, n = w.shape
    w = jnp.transpose(w.reshape(k // 16, 2, 8, n // 128, 128), (0, 1, 3, 2, 4))
    return w.reshape(k // 16, n // 128, 16, 128)


@jax.jit
def pallas_interleave_layers__sliding_block_cached__mixer_s_mlp__decode_kernel(
    A_x: jax.Array,
    A_k_cache: jax.Array,
    A_v_cache: jax.Array,
    A_wq: jax.Array,
    A_wo: jax.Array,
    B_x: jax.Array,
    B_w1: jax.Array,
    B_w2: jax.Array,
    B_w3: jax.Array,
    B_w4: jax.Array,
):
    sk = A_k_cache.shape[2]
    win = min(4096, max(256, sk // 4))
    assert win == 4096 and sk % 128 == 0
    assert A_x.shape == (1, 1, D) and A_k_cache.shape == (1, H, sk, DH)
    wt = win // 128
    t0 = sk // 128 - wt
    ng = H * DH // 8
    hbm = pl.BlockSpec(memory_space=pl.ANY)
    out = pl.pallas_call(
        functools.partial(_kernel, t0=t0, wt=wt),
        out_shape=jax.ShapeDtypeStruct((1, D), A_x.dtype),
        in_specs=[hbm] * 7,
        out_specs=pl.BlockSpec(memory_space=pltpu.VMEM),
        scratch_shapes=[
            pltpu.VMEM((ng, wt * 8, 128), bf16),
            pltpu.VMEM((ng, wt * 8, 128), bf16),
            pltpu.VMEM((ng // 4, 256, 128), bf16),
            pltpu.VMEM((NP * D // 16, 3, 8, 128), u32),
            pltpu.VMEM((H * DH // 16, D // 128, 16, 128), bf16),
            pltpu.VMEM((D, F), bf16),
            pltpu.VMEM((F, D), bf16),
            pltpu.VMEM((1, D), bf16),
            pltpu.VMEM((144, 128), u32),
            pltpu.VMEM((384, 128), u32),
            pltpu.VMEM((144, 128), u32),
            pltpu.VMEM((144, 128), u32),
            pltpu.VMEM((144, 128), u32),
            pltpu.VMEM((40, 128), f32),
            pltpu.VMEM((8, D), f32),
            pltpu.SMEM((1,), jnp.int32),
        ] + [pltpu.VMEM((64, 128), u32)] * 3
        + [pltpu.VMEM((72, 128), f32)] * 8,
        compiler_params=pltpu.CompilerParams(vmem_limit_bytes=128 * 1024 * 1024),
    )(A_x.reshape(1, D), _cache_view(A_k_cache), _cache_view(A_v_cache),
      _weight_view(A_wq).reshape(D * 3 // 16, 256, 128), _weight_view(A_wo), B_w3, B_w4)
    return out.reshape(1, 1, D)
```

```python
import functools

import jax
import jax.numpy as jnp
from jax import lax
import jax.experimental.pallas as pl
import jax.experimental.pallas.tpu as pltpu

D = 640
H = 32
DH = 192
F = 1536
EPS = 1e-5
NP = H // 2
GP = 2 * DH // 8
HI = 0xFFFF0000
CEXP = DH ** -0.5 * 1.4426950408889634

f32 = jnp.float32
bf16 = jnp.bfloat16
u32 = jnp.uint32

L_Y = 0
L_DUMMY = 6
S_MAXB, S_LB, S_INVA, S_X, S_PA, S_PB = 4, 5, 6, 7, 9, 13
XROWS = ((2, 10, 18, 26), (4, 12, 20))
XROWS_LAST = ((2, 10, 18, 26, 6, 14, 22, 30, 4, 12, 20, 28), ())
GX = (0, 16)
PLANS = {
    "first": (
        {},
        (23, 23, 23, 25, 25, 25, 26, 26, 27, 28, 28, 29, 30, 29, 31, 32, 32, 33, 35, 34, 35, 37,
        38, 38, 39, 39, 39, 40, 40, 41, 42, 42, 43, 44, 44, 45, 46, 46, 47, 48, 49, 50, 51, 51,
        52, 53, 53, 54, 55, 55, 56, 57, 57, 58, 58, 58, 59, 60, 60, 61, 62, 62, 63, 64, 63, 65,
        66, 66, 67, 68, 68, 69, 70, 70, 71, 71, 71, 74, 75, 75, 76, 77, 77, 78, 79, 79, 80, 81,
        81, 81, 82, 82, 83, 83, 84, 85)),
    "body": (
        {1: 0, 3: 1, 5: 3, 7: 4, 9: 5, 11: 8, 12: 10, 15: 10, 19: 12, 21: 14, 23: 16, 25: 17,
        27: 19, 29: 22, 31: 23, 33: 23, 35: 26, 37: 26, 39: 28, 40: 33, 41: 33, 43: 34, 45: 34,
        47: 34, 49: 35, 51: 37, 53: 38, 55: 39, 57: 40, 59: 42, 61: 43, 63: 46, 67: 49, 70: 51,
        71: 52, 72: 53, 75: 55, 77: 56, 79: 58, 81: 59, 83: 62, 84: 62},
        (0, 0, 0, 0, 0, 0, 0, 0, 0, 0, 0, 1, 2, 2, 3, 4, 4, 5, 6, 7, 7, 8, 9, 10, 10, 12, 12,
        13, 14, 15, 15, 16, 16, 17, 17, 18, 20, 21, 21, 24, 25, 23, 24, 27, 27, 33, 29, 29, 28,
        30, 30, 31, 31, 32, 33, 33, 34, 35, 35, 36, 36, 35, 35, 36, 37, 39, 43, 41, 43, 40, 45,
        45, 46, 48, 48, 48, 49, 50, 50, 51, 52, 51, 51, 54, 53, 54, 56, 58, 57, 59, 61, 59, 61,
        62, 63, 64)),
    "third": (
        {1: 0, 3: 3, 6: 3, 7: 4, 9: 5, 11: 8, 15: 10, 18: 12, 19: 14, 21: 14, 23: 15, 25: 17,
        26: 19, 27: 19, 30: 22},
        (0, 0, 0, 0, 0, 0, 0, 0, 0, 0, 1, 0, 0, 3, 3, 5, 2, 5, 4, 8, 7, 8, 10, 10, 10, 12, 12,
        13, 15, 17, 15, 16, 17, 17, 18, 19, 20, 18, 21, 22, 22, 24, 25, 26, 25, 24, 25, 25)),
    "last": (
        {1: 0, 3: 1, 7: 2, 11: 3, 15: 4, 17: 6, 19: 7, 21: 10, 23: 11, 27: 13},
        (0, 0, 0, 0, 0, 0, 0, 0, 0, 0, 0, 0, 0, 0, 0, 0, 1, 1, 2, 3, 4, 6, 6, 6, 7, 7, 8, 6, 8,
        9, 9, 10, 10, 11, 11, 11)),
    "final": (
        {37: 0, 39: 1, 40: 2, 41: 3, 42: 3, 43: 4, 45: 5},
        (0, 0, 0, 0, 0, 0, 0, 0, 0, 0, 0, 0, 0, 0, 0, 0, 0, 0, 0, 0, 0, 0, 0, 0, 0, 0, 0, 0, 0,
        0, 0, 0, 0, 0, 0, 0, 0, 0, 0, 0, 0, 0, 5, 2, 0, 1, 0, 0)),
}
MIX = (0, 1, 8, 2, 3, 9, 4, 5, 10, 6, 7, 11)
MIXA = (0, 1, 2, 3, 4, 8, 5, 9, 6, 10, 7, 11)
NLATE = 12
NSPLIT = 36
B_SEGS = (9, 12, 15, 18)
B_SEGL = 8
DA0 = 27
DW0 = 32
DB0 = 41
DA1 = 55
DB1 = 67
DQ = (26, 29, 33)
NQV = 3
B0_SEG = 18
A1_SEG = 40
B1_SEG = 12
A2_SEG = 40
A_SEG0 = 40
A_SEG3 = 38
B_SEGS3 = (9, 11, 15, 19)
XA_AT = 8
AD_SEG = 32
BD_SEG = 12
NALT = 2
W4_CHUNKS = (1024, 256, 160, 64, 32)
W4_MXU = 1280


def _mean(x):
    return jnp.mean(x, axis=-1, keepdims=True)


def _ln(x):
    c = x - _mean(x)
    return c * lax.rsqrt(_mean(c * c) + EPS)


def _wtile(wu, rows, nt):
    blk = wu[rows, nt]
    return pltpu.bitcast(blk.reshape(blk.shape[0] * 8, 128), bf16)


def _wcols(wu, rows, nts):
    return jnp.concatenate([_wtile(wu, rows, n) for n in nts], axis=1)


def _rows16(a, b):
    return jnp.concatenate([a, b], axis=0).astype(bf16)


def _slot(G, t):
    j = 4 * (t >> 3) + ((((t >> 1) & 3) + G + 2 * (t & 1) + (t >> 3)) & 3)
    return 2 * G + (t & 1), 8 * j


def _xslot(G, t):
    return G // 2, 8 * (4 * (t >> 3) + ((((t >> 1) & 3) + G + (t >> 3)) & 3))


def _vr(n):
    return slice(8 * n, 8 * n + 8)


def _kernel(*refs, t0, wt):
    pl.run_scoped(functools.partial(_body, refs, t0, wt),
                  pltpu.SemaphoreType.DMA((4 + len(W4_CHUNKS) + 2 * NP,)))


def _body(refs, t0, wt, sems):
    (x_hbm, k_hbm, v_hbm, wq_hbm, wo_hbm, w3_hbm, w4_hbm, o_ref,
     kbuf, vbuf, vxbuf, wqu, wo, w3, w4, xbuf, lref, obuf, qa, qb, qx, scl, abuf, zs) = refs[:24]
    qt, pT = refs[24:27], refs[27:]
    ku = kbuf.bitcast(u32)
    vu = vbuf.bitcast(u32)
    vx = vxbuf.bitcast(u32)
    wou = wo.bitcast(u32)

    x_cp = pltpu.make_async_copy(x_hbm, xbuf, sems.at[0])
    wq_cp = pltpu.make_async_copy(wq_hbm, vxbuf.at[0:D * 3 // 16], sems.at[1])
    wo_cp = pltpu.make_async_copy(wo_hbm, wo, sems.at[2])
    w3_cp = pltpu.make_async_copy(w3_hbm, w3, sems.at[3])
    w4_rows, r0 = [], 0
    for n in W4_CHUNKS:
        w4_rows.append((r0, r0 + n))
        r0 += n
    w4_cp = [pltpu.make_async_copy(w4_hbm.at[a:b], w4.at[a:b], sems.at[4 + c])
             for c, (a, b) in enumerate(w4_rows)]
    S0 = 4 + len(W4_CHUNKS)

    def k_cp(i):
        return pltpu.make_async_copy(
            k_hbm.at[pl.ds(i * GP, GP), pl.ds(t0 * 8, wt * 8), :],
            kbuf.at[pl.ds(i * GP, GP)], sems.at[S0 + i])

    def v_cp(i):
        return pltpu.make_async_copy(
            v_hbm.at[pl.ds(i * GP, GP), pl.ds(t0 * 8, wt * 8), :],
            vbuf.at[pl.ds(i * GP, GP)], sems.at[S0 + NP + i])

    for c in (wq_cp, x_cp, wo_cp):
        c.start()
    for i in range(NP):
        k_cp(i).start()
        v_cp(i).start()
    for c in [w3_cp] + w4_cp:
        c.start()

    zs[0] = 0
    for ref in (qa, qb, qx, lref):
        ref[_vr(5), :] = jnp.zeros((8, 128), u32)

    lane = lax.broadcasted_iota(jnp.int32, (8, 128), 1)
    sub = lax.broadcasted_iota(jnp.int32, (8, 128), 0)
    lane_lo = lane < 64
    sub_lo = sub < 4

    def tile(ref, g0, G, t):
        g, r = _slot(G, t)
        return ref[g0 + g, r:r + 8, :]

    def retile(ref, i, expand):
        def body(c, carry):
            g0 = i * GP + 8 * c
            for G in range(4):
                for J in range(4):
                    xs = [[ref[g0 + 2 * G + e, _vr(4 * J + jj), :] for jj in range(4)]
                          for e in range(2)]
                    for jj in range(4):
                        x0, x1 = xs[0][jj], xs[1][jj]
                        ys = (jnp.where(sub_lo, x0, pltpu.roll(x1, 4, 0)),
                              jnp.where(sub_lo, pltpu.roll(x0, 4, 0), x1))
                        for e in range(2):
                            t = 8 * J + 2 * jj + e
                            g, r = _slot(G, t)
                            if expand and G % 2 and e:
                                ref[g0 + g, r:r + 8, :] = ys[e] << 16
                                g, r = _xslot(G, t)
                                vx[i * (GP // 4) + 2 * c + g, r:r + 8, :] = ys[e] & jnp.uint32(HI)
                            else:
                                ref[g0 + g, r:r + 8, :] = ys[e]
            return carry
        lax.fori_loop(0, GP // 8, body, 0)

    def merge_halves(get, nt, n):
        lo, hi = get(n // 2), get((nt + n) // 2)
        if n % 2:
            lo = pltpu.roll(lo, 4, 0)
        if (nt + n) % 2 == 0:
            hi = pltpu.roll(hi, 4, 0)
        return jnp.where(sub_lo, lo, hi)

    def retile_wq(G, carry):
        for n in range(3 * NP):
            wqu[n // 3 * (D // 16) + G, n % 3] = merge_halves(
                lambda v: vx[3 * G + v // 16, _vr(v % 16), :], 3 * NP, n)
        return carry

    def retile_wo(c, carry):
        for G in range(8):
            xs = [wou[8 * c + G, n] for n in range(5)]
            for n in range(5):
                wou[8 * c + G, n] = merge_halves(lambda v: xs[v], 5, n)
        return carry

    def lhs_at(ref, n):
        return pltpu.bitcast(ref[_vr(n), :], bf16)

    cur = [None]

    def new_block():
        cur[0] = -32 * jnp.clip(zs[0], 0, 1)

    def tick(ref, n, val):
        if val.dtype != ref.dtype:
            val = pltpu.bitcast(val, ref.dtype)
        ref[pl.ds(pl.multiple_of(cur[0] + 8 * n, 8), 8), :] = val

    def put_q(q, qref):
        qq = pltpu.bitcast(q.astype(bf16).astype(f32), u32)
        q0, q1, q2 = qq[:, 0:128], qq[:, 128:256], qq[:, 256:384]
        for n, v in enumerate((q0 >> 16, q0, q2 >> 16, q2, q1)):
            qref[_vr(n), :] = v
            if n < 2 and qref is qb:
                qx[_vr(n), :] = v

    def transpose_wq(i):
        for k in range(5):
            for n in range(3):
                rows = pl.ds(i * (D // 16) + 8 * k, 8)
                w = pltpu.bitcast(_wtile(wqu, rows, n).astype(f32).T, u32)
                for G in range(8):
                    wqu[i * (D // 16) + 8 * k + G, n] = (w[_vr(2 * G), :] >> 16) | w[_vr(2 * G + 1), :]

    def q_vpu(i, c, qref):
        cols = []
        for n in range(3):
            acc = []
            for G in range(8):
                ws = [wqu[i * (D // 16) + 8 * k + G, n] for k in range(5)]
                for half in (lambda w: w << 16, lambda w: w & jnp.uint32(HI)):
                    t = [pltpu.bitcast(half(ws[k]), f32) * col(c, k) for k in range(5)]
                    acc.append((t[0] + t[1]) + (t[2] + t[3]) + t[4])
            z = jnp.sum(jnp.concatenate(acc, axis=0).T.reshape(16, 8, 128), axis=0)
            cols.append(row_sum(z))
        put_q(jnp.concatenate(cols, axis=1), qref)
        return cols[0] + cols[1] + cols[2]

    def row_sum(a):
        return jnp.broadcast_to(jnp.sum(a, axis=0, keepdims=True), a.shape)

    def q_dots(i, st, qref, lhs=None, mean=None):
        def step(k):
            def run(tied=False):
                w = _wcols(wqu, pl.ds(i * (D // 16) + 8 * k, 8), range(3))
                if lhs is None:
                    r = jnp.dot(lhs_at(lref, L_Y + k), w, preferred_element_type=f32)[0:8]
                else:
                    r = jnp.dot(lhs[:, 128 * k:128 * k + 128], w, preferred_element_type=f32)
                st["q"] = r if k == 0 else st["q"] + r
                if k == 4:
                    q = st["q"] if lhs is None else st["q"][0:8] - mean * st["q"][8:16]
                    put_q(q, qref)
                return r[0:8, 256:384]
            return 3, lref, L_DUMMY, run
        return [step(k) for k in range(5)]

    def o_dot(i, b, st, get_lhs, tref=None):
        def run(tied=False):
            w = _wcols(wou, pl.ds(i * (GP // 2) + 8 * b, 8), range(5))
            lhs = get_lhs() | tref[_vr(5), :] if tied and tref is not obuf else get_lhs()
            r = jnp.dot(pltpu.bitcast(lhs, bf16), w, preferred_element_type=f32)[0:8]
            st["acc"] = st["acc"] + r if "acc" in st else r
            return r[:, 512:640]
        return 5, tref, (32 if tref is obuf else 6), run

    def mid_q(st, qref):
        q1 = qref[_vr(4), :]
        q1r = pltpu.roll(q1, 64, 1)
        st["u", 0, id(qref)] = jnp.where(lane_lo, q1 >> 16, q1r)
        st["u", 1, id(qref)] = jnp.where(lane_lo, q1r >> 16, q1)

    def k_dots(i, hh, st, qref, order=tuple(range(12)), nalt=0):
        g0 = i * GP
        gf, gh = ((0, 8), (16, 12))[hh]

        def step(r):
            src = qx if r in order[:nalt] else qref

            def run(tied=False):
                if r < 8:
                    cols = [[tile(ku, g0, gf + G, 8 * T + r) for G in range(8)] for T in range(4)]
                    base, row = src[_vr(2 * hh + r % 2), :], r // 2
                else:
                    cols = [[tile(ku, g0, gh + G % 4, 8 * T + 2 * (r - 8) + G // 4)
                             for G in range(8)] for T in range(4)]
                    if ("u", hh, id(qref)) not in st:
                        mid_q(st, qref)
                    base, row = st["u", hh, id(qref)], r - 8
                    if tied:
                        base = base | src[_vr(5), :]
                lhs = jnp.where(sub == row, base, jnp.zeros((8, 128), u32))
                w = jnp.concatenate([jnp.concatenate(c, axis=0) for c in cols], axis=1)
                res = jnp.dot(pltpu.bitcast(lhs, bf16), pltpu.bitcast(w, bf16),
                              preferred_element_type=f32)[0:8]
                st["s", hh] = res if r == order[0] else st["s", hh] + res
                return res[:, 384:512]
            return 4, src, 6, run
        return [step(r) for r in order]

    def col(s, T):
        return s[:, 128 * T:128 * T + 128]

    def row_max(s):
        m = jnp.maximum(jnp.maximum(col(s, 0), col(s, 1)), jnp.maximum(col(s, 2), col(s, 3)))
        return jnp.max(jnp.max(m, axis=1, keepdims=True), axis=0, keepdims=True)

    def prob(s, m):
        return jnp.exp2((s - m) * scl[_vr(0), :])

    def put_p(hh, T, p, ks=range(8)):
        for k in ks:
            pT[4 * hh + T][pl.ds(k, 8, stride=8), :] = p

    def part_sum(p):
        return (p[0] + p[1]) + (p[2] + p[3])

    def inv_sum(l):
        l = jnp.sum(jnp.sum(l, axis=1, keepdims=True), axis=0, keepdims=True)
        r = pl.reciprocal(l, approx=True)
        return jnp.broadcast_to(r * (2.0 - l * r), (8, 128))

    def softmax(s, hh):
        m = row_max(s)
        p = [prob(col(s, T), m) for T in range(4)]
        for T in range(4):
            put_p(hh, T, p[T])
        return p, part_sum(p)

    def get_state(i, n):
        return pltpu.bitcast(ku[i * GP + 3, _vr(n), :], f32)

    def set_state(i, n, v):
        ku[i * GP + 3, _vr(n), :] = pltpu.bitcast(v, u32)

    def stash_b(i, s):
        for T in range(4):
            set_state(i, T, col(s, T))
        m = jnp.broadcast_to(row_max(s), (8, 128))
        set_state(i, S_MAXB, m)
        return m

    def pack8(v):
        return pltpu.bitcast(v.astype(bf16), u32)

    def park_p(i, n, p):
        ku[i * GP + 3, 8 * n:8 * n + 4, :] = pack8(p)

    def parked(i, n):
        return lambda T: ku[i * GP + 3, _vr(n + T), :]

    def x_dots(i, hh, ts, get_lhs, tref=None):
        st = {}
        rows = sorted({t % 8 for t in ts})

        def step(n, rho):
            def run(tied=False):
                res = []
                for T in [t // 8 for t in ts if t % 8 == rho]:
                    w = jnp.concatenate(
                        [tile(vu, i * GP, GX[hh] + G, 8 * T + rho) for G in range(8)], axis=0)
                    lhs = get_lhs(T) | tref[_vr(5), :] if tied else get_lhs(T)
                    res.append(jnp.dot(pltpu.bitcast(lhs, bf16), pltpu.bitcast(w, bf16),
                                       preferred_element_type=f32)[0:8])
                st["x"] = jnp.where(sub == rho, sum(res[1:], res[0]), st["x"] if n else 0.0)
                if n == len(rows) - 1:
                    set_state(i, S_X + hh, st["x"])
                return res[-1]
            return sum(1 for t in ts if t % 8 == rho), tref, 6, run
        return [step(n, rho) for n, rho in enumerate(rows)]

    def transpose_x(i, xrows):
        for hh in range(2):
            for t in xrows[hh]:
                w = jnp.concatenate([tile(vu, i * GP, GX[hh] + G, t) for G in range(8)], axis=0)
                w = pltpu.bitcast(pltpu.bitcast(w, bf16).astype(f32).T.astype(bf16), u32)
                for G in range(8):
                    g, r = _slot(GX[hh] + G, t)
                    vu[i * GP + g, r:r + 8, :] = w[_vr(G), :]

    def reduce_o(blocks, inva, invb, extra=(None, None, None)):
        out = []
        for b, inv in enumerate((inva, jnp.where(lane_lo, inva, invb), invb)[:len(blocks)]):
            z = jnp.sum(pltpu.bitcast(blocks[b], f32).T.reshape(16, 8, 128), axis=0)
            if extra[b] is not None:
                z = z + extra[b]
            out.append(z * inv)
        return out

    def pack16(v):
        return pltpu.bitcast(_rows16(v, v), u32)

    def mac(acc, n, c, G, t, pv):
        w = tile(vu, 8 * c, G, t)
        if G % 2 and t % 2:
            g, r = _xslot(G, t)
            halves = (w, vx[2 * c + g, r:r + 8, :])
        else:
            halves = (w << 16, w & jnp.uint32(HI))
        for k in range(2):
            a = pltpu.bitcast(halves[k], f32) * pv
            acc[n + k] = a if acc[n + k] is None else acc[n + k] + a

    def seg_rows(xrows, seg):
        hh, gp, T = seg // 24 % 2, seg % 24 // 4, seg % 4
        on_mxu = GX[hh] <= 12 * hh + 2 * gp < GX[hh] + 8
        return [rho for rho in range(8) if not (on_mxu and 8 * T + rho in xrows[hh])]

    def run_block(pairs, xrows, dots, hooks, plan, segs=None):
        tie, clk = plan
        clock = []

        def emit(upto):
            while len(clock) < upto:
                n = len(clock)
                for h in hooks.get(("dot", n), ()):
                    h()
                clock.append(dots[n][3](n in tie.values()))

        zero = jnp.zeros((8, 128), f32)
        used = {}
        for seg in segs or range(48 * len(pairs)):
            i, hh, gp, T = pairs[seg // 48], seg // 24 % 2, seg % 24 // 4, seg % 4
            if T == 0:
                a4 = [None] * 4
            pref = pT[4 * hh + T]
            upto = min([v for k, v in tie.items() if k >= seg]
                       + [k[1] for k, v in hooks.items() if k[0] == "after" and v >= seg]
                       + [len(dots) if tie else clk[seg] + 6])
            free = not any(k in tie for k in range(seg, seg - T + 4))
            if free or ("seg", seg) in hooks:
                upto = max(upto, clk[seg] + 1)
            emit(min(len(dots), max(upto, hooks.get(("need", seg), 0))))
            if free:
                tick(pref, 8, clock[clk[seg]])
            elif gp:
                tick(pref, 8, zero)
            for h in hooks.get(("seg", seg), ()):
                h(clock[clk[seg]])
            for rho in seg_rows(xrows, seg):
                pv = pref[_vr(rho), :]
                for e in range(2):
                    mac(a4, 2 * e, i * 6, 12 * hh + 2 * gp + e, 8 * T + rho, pv)
            if seg in tie:
                ref, slot = dots[tie[seg]][1:3]
                used[tie[seg]] = used.get(tie[seg], -1) + 1
                for k in range(4):
                    tick(ref, slot + 4 * used[tie[seg]] + k, a4[k])
            if T == 3 and ("end", 0) in hooks and seg >= 32:
                hooks["end", 0](12 * hh + 2 * gp, a4)
            elif T == 3:
                for n in range(4):
                    G = 12 * hh + 2 * gp + n // 2
                    v = a4[n] * hooks["scale", seg // 24]() if ("scale", seg // 24) in hooks else a4[n]
                    ku[i * GP + G // 8, pl.ds(16 * (G % 8) + n % 2, 8, stride=2), :] = (
                        pltpu.bitcast(v, u32))
        emit(len(dots))

    def run_all(dots):
        for d in dots:
            d[3]()

    def set_input(c, scale):
        cp = pltpu.bitcast(_rows16(c, c), u32)
        for k in range(5):
            lref[_vr(L_Y + k), :] = cp[:, 128 * k:128 * k + 128]
        scl[_vr(0), :] = jnp.broadcast_to(scale, (8, 128))

    x_cp.wait()
    x = jnp.broadcast_to(xbuf[...].astype(f32), (8, D))
    set_input(_ln(x), jnp.full((8, 1), CEXP, f32))
    wq_cp.wait()
    lax.fori_loop(0, D // 16, retile_wq, 0)
    wo_cp.wait()
    lax.fori_loop(0, H * DH // 128, retile_wo, 0)

    def body1(i, acc):
        st = {"acc": acc}
        k_cp(i).wait()
        retile(ku, i, False)
        run_all(q_dots(i, st, qa))
        inv = []
        for hh in range(2):
            run_all(k_dots(i, hh, st, qa))
            inv.append(inv_sum(softmax(st["s", hh], hh)[1]))

        @pl.when(i > 0)
        def _():
            transpose_x(i - 1, XROWS)

        @pl.when(jnp.logical_and(i >= 5 - NQV, i < 5))
        def _():
            transpose_wq(i)

        v_cp(i).wait()
        retile(vu, i, True)
        for hh in range(2):
            def pv_step(c, carry, hh=hh):
                acc8 = [None] * 8
                for t in range(32):
                    pv = pT[4 * hh + t // 8][_vr(t % 8), :]
                    for G in range(4):
                        mac(acc8, 2 * G, i * 6 + c, G, t, pv)
                for n in range(8):
                    obuf[pl.ds(64 * c + 16 * (n // 2) + n % 2, 8, stride=2), :] = (
                        pltpu.bitcast(acc8[n], u32))
                return carry
            lax.fori_loop(3 * hh, 3 * hh + 3, pv_step, 0)
        o = reduce_o([obuf[128 * b:128 * b + 128, :] for b in range(3)], inv[0], inv[1])
        run_all([o_dot(i, b, st, lambda b=b: pack16(o[b])) for b in range(3)])
        return st["acc"]

    x = x + row_sum(lax.fori_loop(0, NP, body1, jnp.zeros((8, D), f32)))

    y = _ln(x)
    zz = _ln(y).astype(bf16)
    w3_cp.wait()
    h = jnp.dot(zz, w3[...], preferred_element_type=f32)
    h = jax.nn.gelu(h, approximate=True).astype(bf16)
    x = x + y
    transpose_x(NP - 1, XROWS_LAST)
    for k in range(W4_MXU, F, 128):
        hk = jnp.broadcast_to(h[0:1, k:k + 128].astype(f32), (128, 128))
        obuf[k - W4_MXU:k - W4_MXU + 128, :] = pltpu.bitcast(hk.T, u32)
    part = jnp.zeros((8, D), f32)
    for cp, (a, b) in zip(w4_cp, w4_rows):
        cp.wait()
        if a < W4_MXU:
            x = x + jnp.dot(h[:, a:b], w4[a:b, :], preferred_element_type=f32)
        else:
            for k in range(a, b, 16):
                hk = pltpu.bitcast(obuf[k - W4_MXU:k - W4_MXU + 16, :], f32)
                t = w4[k:k + 16, :].astype(f32) * jnp.concatenate([hk] * 5, axis=1)
                part = part + (t[0:8] + t[8:16])
    x = x + row_sum(part)

    ones = jnp.ones((8, D), f32)
    xl = _rows16(x, ones)
    xb = xl[0:8].astype(f32)
    mean = _mean(xb)
    c = xb - mean
    set_input(c, lax.rsqrt(_mean(c * c) + EPS) * CEXP)
    abuf[...] = jnp.where(lax.broadcasted_iota(jnp.int32, (8, D), 0) == 0, x, 0.0)

    def tail_hooks(i, st, hooks, seg0, compute=True):
        def first(_):
            m = row_max(st["s", 0])
            st["pa"] = [prob(col(st["s", 0], T), m) for T in range(4)]
            set_state(i, S_INVA, inv_sum(part_sum(st["pa"])))
            for T in range(4):
                park_p(i, S_PA + T, st["pa"][T])

        def put(T, half):
            def run(clk):
                tick(pT[T], 8, clk)
                put_p(0, T, st["pa"][T], range(4 * half, 4 * half + 4))
            return run
        if compute:
            hooks.setdefault(("seg", seg0), []).append(first)
        for n in range(8):
            hooks.setdefault(("seg", seg0 + n), []).append(put(n // 2, n % 2))

    def head_b_hooks(i, segs, pb, final=False, park=False):
        def put_b(T):
            def run(clk):
                tick(scl, 4, clk)
                pb.append(prob(get_state(i, T), get_state(i, S_MAXB)))
                put_p(1, T, pb[T])
                if park and T < 3:
                    park_p(i, S_PB + T, pb[T])
                if T == 3:
                    set_state(i, S_LB, inv_sum(part_sum(pb)) if final else part_sum(pb))
            return run
        return {("seg", segs[T]): [put_b(T)] for T in range(4)}

    def reduce_pair(i):
        xa, xb = get_state(i, S_X), get_state(i, S_X + 1)
        invb = inv_sum(get_state(i, S_LB))
        return reduce_o([ku[i * GP + b] for b in range(3)],
                        get_state(i, S_INVA), invb, (xa, None, xb))

    st = {}
    new_block()
    late = tuple(range(8, 12)) + tuple(range(8))
    q0, q1, q2 = qt
    dots = q_dots(0, st, q0, xl, mean) + q_dots(1, st, q1, xl, mean) \
        + k_dots(0, 0, st, q0) + k_dots(0, 1, st, q0, late) + k_dots(1, 0, st, q1, late) \
        + k_dots(1, 1, st, q1, late) + k_dots(2, 0, st, q2, late) + k_dots(2, 1, st, q2)
    for n in range(4):
        dots += x_dots(n // 2, n % 2, XROWS[n % 2], parked(n // 2, (S_PA, S_PB)[n % 2]))

    def sm_a0():
        s0 = st["s", 0]
        m = jnp.maximum(jnp.maximum(col(s0, 0), col(s0, 1)), jnp.maximum(col(s0, 2), col(s0, 3)))
        m = jnp.max(m, axis=0, keepdims=True)
        p = [prob(col(s0, T), m) for T in range(4)]
        tick(q0, 6, part_sum(p))
        put_p(0, 0, p[0])
        st["p0"] = p
        st["w"] = prob(m, jnp.max(m, axis=1, keepdims=True))
        set_state(0, S_INVA, inv_sum(part_sum(p) * st["w"]))
        for T in range(4):
            park_p(0, S_PA + T, p[T] * st["w"])

    def put_a0(T):
        def run(clk):
            tick(pT[T], 8, clk)
            put_p(0, T, st["p0"][T])
        return run

    def sm_a1():
        m = row_max(st["s", 0])
        st["pa"] = [prob(col(st["s", 0], T), m) for T in range(4)]
        tick(q1, 6, part_sum(st["pa"]))
        set_state(1, S_INVA, inv_sum(part_sum(st["pa"])))
        for T in range(4):
            park_p(1, S_PA + T, st["pa"][T])

    hooks = head_b_hooks(0, range(B0_SEG, 48, 2), [], park=True)
    hooks.update(head_b_hooks(1, range(48 + B1_SEG, 96, 3), [], park=True))
    hooks.update({("scale", 0): lambda: st["w"],
                  ("need", 0): DA0 + 1, ("need", B0_SEG): DB0 + 1, ("need", A1_SEG): DA1 + 1,
                  ("need", 48 + B1_SEG): DB1 + 1, ("need", 48 + A2_SEG): 70,
                  ("after", 82): 48 + B1_SEG + 9})
    for n, fn in ((10, lambda: mid_q(st, q0)),
                  (DQ[0], lambda: tick(q0, 5, q_vpu(2, c, q2))),
                  (DQ[1], lambda: tick(q0, 5, q_vpu(3, c, qa))),
                  (DQ[2], lambda: tick(q0, 5, q_vpu(4, c, qb))),
                  (DA0, sm_a0), (DW0, lambda: tick(q0, 7, st["w"])),
                  (DB0, lambda: tick(q1, 6, stash_b(0, st["s", 1]))), (DA1, sm_a1),
                  (DB1, lambda: tick(q2, 6, stash_b(1, st["s", 1]))),
                  (82, lambda: stash_b(2, st["s", 1]))):
        hooks.setdefault(("dot", n), []).append(fn)
    hooks.update({("seg", T): [put_a0(T + 1)] for T in range(3)})
    tail_hooks(1, st, hooks, A1_SEG, False)
    tail_hooks(2, st, hooks, 48 + A2_SEG)
    run_block([0, 1], XROWS, dots, hooks, PLANS["first"])

    qs = (qb, qa)

    def late_dots(st):
        todo = [(m, 2) for m in range(NP - 2)] + [(NP - 3, 1)] + [(NP - 2, b) for b in range(3)]
        return [o_dot(m, b, st, lambda n=m + (2 - b) * 6: obuf[_vr(n), :], obuf) for m, b in todo]

    def block(name, j, ks, reds, qn, xrows):
        last = ks == [NP - 1]
        a_seg = A_SEG3 if name == "third" else A_SEG0
        b_segs = {"third": B_SEGS3,
                  "last": range(B_SEGL, 48, 3)}.get(name, B_SEGS)
        new_block()
        st = {}
        for k in ks if not last else []:
            mid_q(st, qs[(k + 1) % 2])
        outs = [reduce_pair(j + r) for r in reds]

        def kept(n):
            return (0, 1, 2) if last else (1, 2) if reds[n] == NP - 3 else (2,)

        def keep():
            for n, r in enumerate(reds):
                for b in kept(n):
                    obuf[pl.ds(pl.multiple_of(8 * (j + r + (2 - b) * 6), 8), 4), :] = (
                        pack8(outs[n][b]))

        if not last:
            keep()
        pb = []
        hooks = head_b_hooks(j + ks[0], b_segs, pb, last)
        dots = []

        def hook(key, fn):
            hooks.setdefault(key, []).append(fn)

        def direct(i, hh, seg0, tref):
            p = []

            def run():
                m = row_max(st["s", hh])
                p.extend(prob(col(st["s", hh], T), m) for T in range(4))
                l = part_sum(p)
                set_state(i, (S_INVA, S_LB)[hh], l if hh else inv_sum(l))

            def put(T, half):
                def go(clk):
                    tick(pT[4 * hh + T], 8, clk)
                    put_p(hh, T, p[T], range(4 * half, 4 * half + 4))
                return go
            hook(("dot", len(dots)), run)
            dots.extend(x_dots(i, hh, xrows[hh], lambda T: pack16(p[T]), tref))
            hooks["need", seg0] = len(dots)
            for n in range(8):
                hook(("seg", seg0 + n), put(n // 2, n % 2))

        def wo_of(n):
            return [o_dot(j + reds[n], b, st, lambda b=b: pack16(outs[n][b]), lref)
                    for b in range(3) if b not in kept(n)]

        def wq_of(n):
            nq = j + qn[n]
            return q_dots(nq if isinstance(nq, int) else jnp.minimum(nq, NP - 1), st, qs[qn[n] % 2])

        if last:
            dots += late_dots(st)[:NLATE] + x_dots(NP - 1, 0, xrows[0], parked(NP - 1, S_PA), lref)

            def park_acc(G, a4):
                for n in range(4):
                    ku[(NP - 1) * GP + 2, _vr(2 * (G - 16) + n), :] = pltpu.bitcast(a4[n], u32)
            hooks["end", 0] = park_acc
        for n, k in enumerate(ks if not last else []):
            q = qs[(k + 1) % 2]
            dots += k_dots(j + (k + 1), 0, st, q, MIX if n else MIXA, NALT if n else 0)
            if n == 0:
                if xrows[1]:
                    hooks["after", len(dots)] = b_segs[3]
                dots += x_dots(j + ks[0], 1, xrows[1], lambda T: pack16(pb[T]), q)
            else:
                direct(j + k, 1, 48 * n + BD_SEG, q)
            kb = k_dots(j + (k + 1), 1, st, q, MIX)
            if n < len(ks) - 1:
                dots += kb[:XA_AT]
                direct(j + (k + 1), 0, 48 * n + AD_SEG, q)
                dots += kb[XA_AT:] + wq_of(n) + wo_of(n)
            else:
                hooks["need", 48 * n + a_seg] = len(dots)
                tail_hooks(j + (k + 1), st, hooks, 48 * n + a_seg)
                dots += kb
                hook(("dot", len(dots)), lambda k=k: stash_b(j + (k + 1), st["s", 1]))
                for m in range(n, len(qn)):
                    dots += wq_of(m)
                for m in range(n, len(reds)):
                    dots += wo_of(m)
                dots += x_dots(j + ks[0], 0, xrows[0],
                               parked(j + ks[0], S_PA), lref)
        run_block([j + k for k in ks], xrows, dots, hooks,
                  PLANS[name], range(NSPLIT) if last else None)
        if last:
            keep()
        if reds:
            abuf[...] += st["acc"]

    def body2(n, carry):
        block("body", 2 * n, [2, 3], [0, 1], [5, 6], XROWS)
        return carry

    lax.fori_loop(0, NP // 2 - 2, body2, 0)
    pl.when(zs[0] == 0)(lambda: block("third", 0, [NP - 2], [NP - 4, NP - 3], [], XROWS))
    pl.when(zs[0] <= 0)(lambda: block("last", 0, [NP - 1], [NP - 2], [], XROWS_LAST))

    new_block()
    st = {"acc": abuf[...]}
    invb = get_state(NP - 1, S_LB)
    o = reduce_o([ku[(NP - 1) * GP + b] for b in range(2)], get_state(NP - 1, S_INVA), invb,
                 (get_state(NP - 1, S_X), None))
    part = [None] * 5

    def finish(G, a4):
        for k in range(4):
            tick(lref, L_DUMMY + k, a4[k])
        z = lref[_vr(5), :]
        project(G, [pltpu.bitcast(v, u32) | z for v in a4])

    def project(G, a4):
        for n in range(4):
            v = jnp.sum(pltpu.bitcast(a4[n], f32), axis=1, keepdims=True)
            for nt in range(5):
                w = wou[(NP - 1) * (GP // 2) + G + n // 2, nt]
                t = pltpu.bitcast(w & jnp.uint32(HI) if n % 2 else w << 16, f32) * v
                part[nt] = t if part[nt] is None else part[nt] + t

    for G in range(16, NSPLIT // 2, 2):
        project(G, [ku[(NP - 1) * GP + 2, _vr(2 * (G - 16) + n), :] for n in range(4)])
    dots = late_dots(st)[NLATE:] + [o_dot(NP - 1, b, st, lambda b=b: pack16(o[b]), lref)
                                    for b in range(2)]
    run_block([NP - 1], XROWS_LAST, dots, {("end", 0): finish},
              PLANS["final"], range(NSPLIT, 48))
    x = row_sum(st["acc"] + jnp.concatenate([v * invb for v in part], axis=1))

    xl = _rows16(x, ones)
    d = xl[0:8].astype(f32) - mean
    md = _mean(d)
    r1 = lax.rsqrt(jnp.maximum(_mean(d * d) - md * md, 0.0) + EPS)
    mean = mean + md
    y = (d - md) * r1
    my = _mean(y)
    r2 = lax.rsqrt(jnp.maximum(_mean(y * y) - my * my, 0.0) + EPS)
    h = jnp.dot(xl, w3[...], preferred_element_type=f32)
    h = h[0:8] * (r1 * r2) - h[8:16] * ((mean * r1 + my) * r2)
    h = jax.nn.gelu(h, approximate=True).astype(bf16)
    x = x + y
    for k in range(0, F, 128):
        x = x + jnp.dot(h[:, k:k + 128], w4[k:k + 128, :], preferred_element_type=f32)
    o_ref[...] = x[0:1].astype(o_ref.dtype)


def _cache_view(c):
    s = c.shape[2]
    c = jnp.transpose(c, (0, 1, 3, 2)).reshape(H * DH // 8, 8, s // 128, 128)
    return jnp.transpose(c, (0, 2, 1, 3)).reshape(H * DH // 8, s // 128 * 8, 128)


def _weight_view(w):
    k, n = w.shape
    w = jnp.transpose(w.reshape(k // 16, 2, 8, n // 128, 128), (0, 1, 3, 2, 4))
    return w.reshape(k // 16, n // 128, 16, 128)


@jax.jit
def pallas_interleave_layers__sliding_block_cached__mixer_s_mlp__decode_kernel(
    A_x: jax.Array,
    A_k_cache: jax.Array,
    A_v_cache: jax.Array,
    A_wq: jax.Array,
    A_wo: jax.Array,
    B_x: jax.Array,
    B_w1: jax.Array,
    B_w2: jax.Array,
    B_w3: jax.Array,
    B_w4: jax.Array,
):
    sk = A_k_cache.shape[2]
    win = min(4096, max(256, sk // 4))
    assert win == 4096 and sk % 128 == 0
    assert A_x.shape == (1, 1, D) and A_k_cache.shape == (1, H, sk, DH)
    wt = win // 128
    t0 = sk // 128 - wt
    ng = H * DH // 8
    hbm = pl.BlockSpec(memory_space=pl.ANY)
    out = pl.pallas_call(
        functools.partial(_kernel, t0=t0, wt=wt),
        out_shape=jax.ShapeDtypeStruct((1, D), A_x.dtype),
        in_specs=[hbm] * 7,
        out_specs=pl.BlockSpec(memory_space=pltpu.VMEM),
        scratch_shapes=[
            pltpu.VMEM((ng, wt * 8, 128), bf16),
            pltpu.VMEM((ng, wt * 8, 128), bf16),
            pltpu.VMEM((ng // 4, 256, 128), bf16),
            pltpu.VMEM((NP * D // 16, 3, 8, 128), u32),
            pltpu.VMEM((H * DH // 16, D // 128, 16, 128), bf16),
            pltpu.VMEM((D, F), bf16),
            pltpu.VMEM((F, D), bf16),
            pltpu.VMEM((1, D), bf16),
            pltpu.VMEM((144, 128), u32),
            pltpu.VMEM((384, 128), u32),
            pltpu.VMEM((144, 128), u32),
            pltpu.VMEM((144, 128), u32),
            pltpu.VMEM((144, 128), u32),
            pltpu.VMEM((40, 128), f32),
            pltpu.VMEM((8, D), f32),
            pltpu.SMEM((1,), jnp.int32),
        ] + [pltpu.VMEM((64, 128), u32)] * 3
        + [pltpu.VMEM((72, 128), f32)] * 8,
        compiler_params=pltpu.CompilerParams(vmem_limit_bytes=128 * 1024 * 1024),
    )(A_x.reshape(1, D), _cache_view(A_k_cache), _cache_view(A_v_cache),
      _weight_view(A_wq).reshape(D * 3 // 16, 256, 128), _weight_view(A_wo), B_w3, B_w4)
    return out.reshape(1, 1, D)
```

```python
import functools

import jax
import jax.numpy as jnp
from jax import lax
import jax.experimental.pallas as pl
import jax.experimental.pallas.tpu as pltpu

D = 640
H = 32
DH = 192
F = 1536
EPS = 1e-5
NP = H // 2
GP = 2 * DH // 8
HI = 0xFFFF0000
CEXP = DH ** -0.5 * 1.4426950408889634

f32 = jnp.float32
bf16 = jnp.bfloat16
u32 = jnp.uint32

L_Y = 0
L_DUMMY = 6
S_MAXB, S_LB, S_INVA, S_X, S_PA, S_PB = 4, 5, 6, 7, 9, 13
XROWS = ((2, 10, 18, 26), (4, 12, 20))
XROWS_LAST = ((2, 10, 18, 26, 6, 14, 22, 30, 4, 12, 20, 28), ())
GX = (0, 16)
PLANS = {
    "first": (
        {},
        (21, 23, 23, 23, 24, 25, 27, 27, 27, 28, 29, 29, 30, 31, 30, 31, 32, 32, 33, 34, 34, 35,
        36, 36, 37, 38, 38, 39, 40, 40, 41, 42, 43, 43, 44, 44, 45, 46, 46, 47, 48, 48, 49, 49,
        50, 51, 51, 52, 52, 52, 53, 54, 54, 56, 56, 56, 57, 58, 58, 59, 60, 60, 61, 62, 62, 63,
        64, 64, 65, 66, 66, 67, 68, 68, 69, 70, 70, 71, 72, 72, 73, 74, 74, 75, 76, 76, 77, 78,
        78, 79, 80, 81, 82, 82, 83, 82)),
    "body": (
        {1: 0, 3: 1, 5: 3, 7: 4, 9: 5, 11: 8, 12: 10, 15: 10, 19: 12, 21: 14, 23: 16, 25: 17,
        27: 19, 29: 22, 31: 23, 33: 23, 35: 26, 37: 26, 39: 28, 40: 33, 41: 33, 43: 34, 45: 34,
        47: 34, 49: 35, 51: 37, 53: 38, 55: 39, 57: 40, 59: 42, 61: 43, 63: 46, 67: 49, 70: 51,
        71: 52, 72: 53, 75: 55, 77: 56, 79: 58, 81: 59, 83: 62, 84: 62},
        (0, 0, 0, 0, 0, 0, 0, 0, 0, 0, 0, 1, 2, 2, 3, 4, 4, 5, 6, 7, 7, 8, 9, 10, 10, 12, 12,
        13, 14, 15, 15, 16, 16, 17, 17, 18, 20, 21, 21, 24, 25, 23, 24, 27, 27, 33, 29, 29, 28,
        30, 30, 31, 31, 32, 33, 33, 34, 35, 35, 36, 36, 35, 35, 36, 37, 39, 43, 41, 43, 40, 45,
        45, 46, 48, 48, 48, 49, 50, 50, 51, 52, 51, 51, 54, 53, 54, 56, 58, 57, 59, 61, 59, 61,
        62, 63, 64)),
    "third": (
        {1: 0, 3: 3, 6: 3, 7: 4, 9: 5, 11: 8, 15: 10, 18: 12, 19: 14, 21: 14, 23: 15, 25: 17,
        26: 19, 27: 19, 30: 21},
        (0, 0, 0, 0, 0, 0, 0, 0, 0, 0, 1, 0, 0, 3, 3, 5, 2, 5, 4, 8, 7, 8, 10, 10, 10, 12, 12,
        13, 15, 17, 15, 16, 17, 17, 18, 19, 20, 18, 21, 22, 22, 24, 25, 26, 25, 24, 25, 26)),
    "last": (
        {1: 0, 3: 1, 7: 2, 11: 3, 15: 4, 17: 6, 19: 7, 21: 10, 23: 11, 27: 13},
        (0, 0, 0, 0, 0, 0, 0, 0, 0, 0, 0, 0, 0, 0, 0, 0, 1, 1, 2, 3, 4, 6, 6, 6, 7, 7, 8, 6, 8,
        9, 9, 10, 10, 11, 11, 11)),
    "final": (
        {37: 0, 39: 1, 40: 2, 41: 3, 42: 3, 43: 4, 45: 5},
        (0, 0, 0, 0, 0, 0, 0, 0, 0, 0, 0, 0, 0, 0, 0, 0, 0, 0, 0, 0, 0, 0, 0, 0, 0, 0, 0, 0, 0,
        0, 0, 0, 0, 0, 0, 0, 0, 0, 0, 0, 0, 0, 5, 2, 0, 1, 0, 0)),
}
MIX = (0, 1, 8, 2, 3, 9, 4, 5, 10, 6, 7, 11)
MIXA = (0, 1, 2, 3, 4, 8, 5, 9, 6, 10, 7, 11)
NLATE = 12
NSPLIT = 36
W4_VPU = 256
W4_AT = 896
B_SEGS = (9, 12, 15, 18)
B_SEGL = 8
DA0 = 16
NOTICK = 3
DW0 = 32
DB0 = 44
DA1 = 56
DB1 = 67
DQ = (26, 29, 33)
NQV = 3
B0_SEG = 17
A1_SEG = 39
B1_SEG = 12
A2_SEG = 40
A_SEG0 = 40
A_SEG3 = 38
B_SEGS3 = (9, 11, 15, 19)
XA_AT = 8
AD_SEG = 32
BD_SEG = 12
NALT = 2
W4_CHUNKS = (1024, 256, 160, 64, 32)
W4_MXU = 1280


def _mean(x):
    return jnp.mean(x, axis=-1, keepdims=True)


def _ln(x):
    c = x - _mean(x)
    return c * lax.rsqrt(_mean(c * c) + EPS)


def _wtile(wu, rows, nt):
    blk = wu[rows, nt]
    return pltpu.bitcast(blk.reshape(blk.shape[0] * 8, 128), bf16)


def _wcols(wu, rows, nts):
    return jnp.concatenate([_wtile(wu, rows, n) for n in nts], axis=1)


def _rows16(a, b):
    return jnp.concatenate([a, b], axis=0).astype(bf16)


def _slot(G, t):
    j = 4 * (t >> 3) + ((((t >> 1) & 3) + G + 2 * (t & 1) + (t >> 3)) & 3)
    return 2 * G + (t & 1), 8 * j


def _xslot(G, t):
    return G // 2, 8 * (4 * (t >> 3) + ((((t >> 1) & 3) + G + (t >> 3)) & 3))


def _vr(n):
    return slice(8 * n, 8 * n + 8)


def _kernel(*refs, t0, wt):
    pl.run_scoped(functools.partial(_body, refs, t0, wt),
                  pltpu.SemaphoreType.DMA((4 + len(W4_CHUNKS) + 2 * NP,)))


def _body(refs, t0, wt, sems):
    (x_hbm, k_hbm, v_hbm, wq_hbm, wo_hbm, w3_hbm, w4_hbm, o_ref,
     kbuf, vbuf, vxbuf, wqu, wo, w3, w4, xbuf, lref, obuf, qa, qb, qx, scl, abuf, zs) = refs[:24]
    qt, pT = refs[24:27], refs[27:]
    ku = kbuf.bitcast(u32)
    vu = vbuf.bitcast(u32)
    vx = vxbuf.bitcast(u32)
    wou = wo.bitcast(u32)

    x_cp = pltpu.make_async_copy(x_hbm, xbuf, sems.at[0])
    wq_cp = pltpu.make_async_copy(wq_hbm, vxbuf.at[0:D * 3 // 16], sems.at[1])
    wo_cp = pltpu.make_async_copy(wo_hbm, wo, sems.at[2])
    w3_cp = pltpu.make_async_copy(w3_hbm, w3, sems.at[3])
    w4_rows, r0 = [], 0
    for n in W4_CHUNKS:
        w4_rows.append((r0, r0 + n))
        r0 += n
    w4_cp = [pltpu.make_async_copy(w4_hbm.at[a:b], w4.at[a:b], sems.at[4 + c])
             for c, (a, b) in enumerate(w4_rows)]
    S0 = 4 + len(W4_CHUNKS)

    def k_cp(i):
        return pltpu.make_async_copy(
            k_hbm.at[pl.ds(i * GP, GP), pl.ds(t0 * 8, wt * 8), :],
            kbuf.at[pl.ds(i * GP, GP)], sems.at[S0 + i])

    def v_cp(i):
        return pltpu.make_async_copy(
            v_hbm.at[pl.ds(i * GP, GP), pl.ds(t0 * 8, wt * 8), :],
            vbuf.at[pl.ds(i * GP, GP)], sems.at[S0 + NP + i])

    for c in (wq_cp, x_cp, wo_cp):
        c.start()
    for i in range(NP):
        k_cp(i).start()
        v_cp(i).start()
    for c in [w3_cp] + w4_cp:
        c.start()

    zs[0] = 0
    for ref in (qa, qb, qx, lref):
        ref[_vr(5), :] = jnp.zeros((8, 128), u32)

    lane = lax.broadcasted_iota(jnp.int32, (8, 128), 1)
    sub = lax.broadcasted_iota(jnp.int32, (8, 128), 0)
    lane_lo = lane < 64
    sub_lo = sub < 4

    def tile(ref, g0, G, t):
        g, r = _slot(G, t)
        return ref[g0 + g, r:r + 8, :]

    def retile(ref, i, expand):
        def body(c, carry):
            g0 = i * GP + 8 * c
            for G in range(4):
                for J in range(4):
                    xs = [[ref[g0 + 2 * G + e, _vr(4 * J + jj), :] for jj in range(4)]
                          for e in range(2)]
                    for jj in range(4):
                        x0, x1 = xs[0][jj], xs[1][jj]
                        ys = (jnp.where(sub_lo, x0, pltpu.roll(x1, 4, 0)),
                              jnp.where(sub_lo, pltpu.roll(x0, 4, 0), x1))
                        for e in range(2):
                            t = 8 * J + 2 * jj + e
                            g, r = _slot(G, t)
                            if expand and G % 2 and e:
                                ref[g0 + g, r:r + 8, :] = ys[e] << 16
                                g, r = _xslot(G, t)
                                vx[i * (GP // 4) + 2 * c + g, r:r + 8, :] = ys[e] & jnp.uint32(HI)
                            else:
                                ref[g0 + g, r:r + 8, :] = ys[e]
            return carry
        lax.fori_loop(0, GP // 8, body, 0)

    def merge_halves(get, nt, n):
        lo, hi = get(n // 2), get((nt + n) // 2)
        if n % 2:
            lo = pltpu.roll(lo, 4, 0)
        if (nt + n) % 2 == 0:
            hi = pltpu.roll(hi, 4, 0)
        return jnp.where(sub_lo, lo, hi)

    def retile_wq(G, carry):
        for n in range(3 * NP):
            wqu[n // 3 * (D // 16) + G, n % 3] = merge_halves(
                lambda v: vx[3 * G + v // 16, _vr(v % 16), :], 3 * NP, n)
        return carry

    def retile_wo(c, carry):
        for G in range(8):
            xs = [wou[8 * c + G, n] for n in range(5)]
            for n in range(5):
                wou[8 * c + G, n] = merge_halves(lambda v: xs[v], 5, n)
        return carry

    def lhs_at(ref, n):
        return pltpu.bitcast(ref[_vr(n), :], bf16)

    cur = [None]

    def new_block():
        cur[0] = -32 * jnp.clip(zs[0], 0, 1)

    def tick(ref, n, val):
        if val.dtype != ref.dtype:
            val = pltpu.bitcast(val, ref.dtype)
        ref[pl.ds(pl.multiple_of(cur[0] + 8 * n, 8), 8), :] = val

    def put_q(q, qref):
        qq = pltpu.bitcast(q.astype(bf16).astype(f32), u32)
        q0, q1, q2 = qq[:, 0:128], qq[:, 128:256], qq[:, 256:384]
        for n, v in enumerate((q0 >> 16, q0, q2 >> 16, q2, q1)):
            qref[_vr(n), :] = v
            if n < 2 and qref is qb:
                qx[_vr(n), :] = v

    def transpose_wq(i):
        for k in range(5):
            for n in range(3):
                rows = pl.ds(i * (D // 16) + 8 * k, 8)
                w = pltpu.bitcast(_wtile(wqu, rows, n).astype(f32).T, u32)
                for G in range(8):
                    wqu[i * (D // 16) + 8 * k + G, n] = (w[_vr(2 * G), :] >> 16) | w[_vr(2 * G + 1), :]

    def q_vpu(i, c, qref):
        cols = []
        for n in range(3):
            acc = []
            for G in range(8):
                ws = [wqu[i * (D // 16) + 8 * k + G, n] for k in range(5)]
                for half in (lambda w: w << 16, lambda w: w & jnp.uint32(HI)):
                    t = [pltpu.bitcast(half(ws[k]), f32) * col(c, k) for k in range(5)]
                    acc.append((t[0] + t[1]) + (t[2] + t[3]) + t[4])
            z = jnp.sum(jnp.concatenate(acc, axis=0).T.reshape(16, 8, 128), axis=0)
            cols.append(row_sum(z))
        put_q(jnp.concatenate(cols, axis=1), qref)
        return cols[0] + cols[1] + cols[2]

    def row_sum(a):
        return jnp.broadcast_to(jnp.sum(a, axis=0, keepdims=True), a.shape)

    def q_dots(i, st, qref, lhs=None, mean=None):
        def step(k):
            def run(tied=False):
                w = _wcols(wqu, pl.ds(i * (D // 16) + 8 * k, 8), range(3))
                if lhs is None:
                    r = jnp.dot(lhs_at(lref, L_Y + k), w, preferred_element_type=f32)[0:8]
                else:
                    r = jnp.dot(lhs[:, 128 * k:128 * k + 128], w, preferred_element_type=f32)
                st["q"] = r if k == 0 else st["q"] + r
                if k == 4:
                    q = st["q"] if lhs is None else st["q"][0:8] - mean * st["q"][8:16]
                    put_q(q, qref)
                return r[0:8, 256:384]
            return 3, lref, L_DUMMY, run
        return [step(k) for k in range(5)]

    def o_dot(i, b, st, get_lhs, tref=None):
        def run(tied=False):
            w = _wcols(wou, pl.ds(i * (GP // 2) + 8 * b, 8), range(5))
            lhs = get_lhs() | tref[_vr(5), :] if tied and tref is not obuf else get_lhs()
            r = jnp.dot(pltpu.bitcast(lhs, bf16), w, preferred_element_type=f32)[0:8]
            st["acc"] = st["acc"] + r if "acc" in st else r
            return r[:, 512:640]
        return 5, tref, (32 if tref is obuf else 6), run

    def mid_q(st, qref):
        q1 = qref[_vr(4), :]
        q1r = pltpu.roll(q1, 64, 1)
        st["u", 0, id(qref)] = jnp.where(lane_lo, q1 >> 16, q1r)
        st["u", 1, id(qref)] = jnp.where(lane_lo, q1r >> 16, q1)

    def k_dots(i, hh, st, qref, order=tuple(range(12)), nalt=0):
        g0 = i * GP
        gf, gh = ((0, 8), (16, 12))[hh]

        def step(r):
            src = qx if r in order[:nalt] else qref

            def run(tied=False):
                if r < 8:
                    cols = [[tile(ku, g0, gf + G, 8 * T + r) for G in range(8)] for T in range(4)]
                    base, row = src[_vr(2 * hh + r % 2), :], r // 2
                else:
                    cols = [[tile(ku, g0, gh + G % 4, 8 * T + 2 * (r - 8) + G // 4)
                             for G in range(8)] for T in range(4)]
                    if ("u", hh, id(qref)) not in st:
                        mid_q(st, qref)
                    base, row = st["u", hh, id(qref)], r - 8
                    if tied:
                        base = base | src[_vr(5), :]
                lhs = jnp.where(sub == row, base, jnp.zeros((8, 128), u32))
                w = jnp.concatenate([jnp.concatenate(c, axis=0) for c in cols], axis=1)
                res = jnp.dot(pltpu.bitcast(lhs, bf16), pltpu.bitcast(w, bf16),
                              preferred_element_type=f32)[0:8]
                st["s", hh] = res if r == order[0] else st["s", hh] + res
                return res[:, 384:512]
            return 4, src, 6, run
        return [step(r) for r in order]

    def col(s, T):
        return s[:, 128 * T:128 * T + 128]

    def row_max(s):
        m = jnp.maximum(jnp.maximum(col(s, 0), col(s, 1)), jnp.maximum(col(s, 2), col(s, 3)))
        return jnp.max(jnp.max(m, axis=1, keepdims=True), axis=0, keepdims=True)

    def prob(s, m):
        return jnp.exp2((s - m) * scl[_vr(0), :])

    def put_p(hh, T, p, ks=range(8)):
        for k in ks:
            pT[4 * hh + T][pl.ds(k, 8, stride=8), :] = p

    def part_sum(p):
        return (p[0] + p[1]) + (p[2] + p[3])

    def inv_sum(l):
        l = jnp.sum(jnp.sum(l, axis=1, keepdims=True), axis=0, keepdims=True)
        r = pl.reciprocal(l, approx=True)
        return jnp.broadcast_to(r * (2.0 - l * r), (8, 128))

    def softmax(s, hh):
        m = row_max(s)
        p = [prob(col(s, T), m) for T in range(4)]
        for T in range(4):
            put_p(hh, T, p[T])
        return p, part_sum(p)

    def get_state(i, n):
        return pltpu.bitcast(ku[i * GP + 3, _vr(n), :], f32)

    def set_state(i, n, v):
        ku[i * GP + 3, _vr(n), :] = pltpu.bitcast(v, u32)

    def stash_b(i, s):
        for T in range(4):
            set_state(i, T, col(s, T))
        m = jnp.broadcast_to(row_max(s), (8, 128))
        set_state(i, S_MAXB, m)
        return m

    def pack8(v):
        return pltpu.bitcast(v.astype(bf16), u32)

    def park_p(i, n, p):
        ku[i * GP + 3, 8 * n:8 * n + 4, :] = pack8(p)

    def parked(i, n):
        return lambda T: ku[i * GP + 3, _vr(n + T), :]

    def x_dots(i, hh, ts, get_lhs, tref=None):
        st = {}
        rows = sorted({t % 8 for t in ts})

        def step(n, rho):
            def run(tied=False):
                res = []
                for T in [t // 8 for t in ts if t % 8 == rho]:
                    w = jnp.concatenate(
                        [tile(vu, i * GP, GX[hh] + G, 8 * T + rho) for G in range(8)], axis=0)
                    lhs = get_lhs(T) | tref[_vr(5), :] if tied else get_lhs(T)
                    res.append(jnp.dot(pltpu.bitcast(lhs, bf16), pltpu.bitcast(w, bf16),
                                       preferred_element_type=f32)[0:8])
                st["x"] = jnp.where(sub == rho, sum(res[1:], res[0]), st["x"] if n else 0.0)
                if n == len(rows) - 1:
                    set_state(i, S_X + hh, st["x"])
                return res[-1]
            return sum(1 for t in ts if t % 8 == rho), tref, 6, run
        return [step(n, rho) for n, rho in enumerate(rows)]

    def transpose_x(i, xrows):
        for hh in range(2):
            for t in xrows[hh]:
                w = jnp.concatenate([tile(vu, i * GP, GX[hh] + G, t) for G in range(8)], axis=0)
                w = pltpu.bitcast(pltpu.bitcast(w, bf16).astype(f32).T.astype(bf16), u32)
                for G in range(8):
                    g, r = _slot(GX[hh] + G, t)
                    vu[i * GP + g, r:r + 8, :] = w[_vr(G), :]

    def reduce_o(blocks, inva, invb, extra=(None, None, None)):
        out = []
        for b, inv in enumerate((inva, jnp.where(lane_lo, inva, invb), invb)[:len(blocks)]):
            z = jnp.sum(pltpu.bitcast(blocks[b], f32).T.reshape(16, 8, 128), axis=0)
            if extra[b] is not None:
                z = z + extra[b]
            out.append(z * inv)
        return out

    def pack16(v):
        return pltpu.bitcast(_rows16(v, v), u32)

    def mac(acc, n, c, G, t, pv):
        w = tile(vu, 8 * c, G, t)
        if G % 2 and t % 2:
            g, r = _xslot(G, t)
            halves = (w, vx[2 * c + g, r:r + 8, :])
        else:
            halves = (w << 16, w & jnp.uint32(HI))
        for k in range(2):
            a = pltpu.bitcast(halves[k], f32) * pv
            acc[n + k] = a if acc[n + k] is None else acc[n + k] + a

    def seg_rows(xrows, seg):
        hh, gp, T = seg // 24 % 2, seg % 24 // 4, seg % 4
        on_mxu = GX[hh] <= 12 * hh + 2 * gp < GX[hh] + 8
        return [rho for rho in range(8) if not (on_mxu and 8 * T + rho in xrows[hh])]

    def run_block(pairs, xrows, dots, hooks, plan, segs=None):
        tie, clk = plan
        clock = []

        def emit(upto):
            while len(clock) < upto:
                n = len(clock)
                for h in hooks.get(("dot", n), ()):
                    h()
                clock.append(dots[n][3](n in tie.values()))

        zero = jnp.zeros((8, 128), f32)
        used = {}
        for seg in segs or range(48 * len(pairs)):
            i, hh, gp, T = pairs[seg // 48], seg // 24 % 2, seg % 24 // 4, seg % 4
            if T == 0:
                a4 = [None] * 4
            pref = pT[4 * hh + T]
            upto = min([v for k, v in tie.items() if k >= seg]
                       + [k[1] for k, v in hooks.items() if k[0] == "after" and v >= seg]
                       + [len(dots) if tie else clk[seg] + 6])
            free = not any(k in tie for k in range(seg, seg - T + 4))
            if free or ("seg", seg) in hooks:
                upto = max(upto, clk[seg] + 1)
            emit(min(len(dots), max(upto, hooks.get(("need", seg), 0))))
            if seg < hooks.get(("notick", 0), 0):
                pass
            elif free:
                tick(pref, 8, clock[clk[seg]])
            elif gp:
                tick(pref, 8, zero)
            for h in hooks.get(("seg", seg), ()):
                h(clock[clk[seg]])
            for rho in seg_rows(xrows, seg):
                pv = pref[_vr(rho), :]
                for e in range(2):
                    mac(a4, 2 * e, i * 6, 12 * hh + 2 * gp + e, 8 * T + rho, pv)
            if seg in tie:
                ref, slot = dots[tie[seg]][1:3]
                used[tie[seg]] = used.get(tie[seg], -1) + 1
                for k in range(4):
                    tick(ref, slot + 4 * used[tie[seg]] + k, a4[k])
            if T == 3 and ("end", 0) in hooks and seg >= 32:
                hooks["end", 0](12 * hh + 2 * gp, a4)
            elif T == 3:
                for n in range(4):
                    G = 12 * hh + 2 * gp + n // 2
                    v = a4[n] * hooks["scale", seg // 24]() if ("scale", seg // 24) in hooks else a4[n]
                    ku[i * GP + G // 8, pl.ds(16 * (G % 8) + n % 2, 8, stride=2), :] = (
                        pltpu.bitcast(v, u32))
        emit(len(dots))

    def run_all(dots):
        for d in dots:
            d[3]()

    def set_input(c, scale):
        cp = pltpu.bitcast(_rows16(c, c), u32)
        for k in range(5):
            lref[_vr(L_Y + k), :] = cp[:, 128 * k:128 * k + 128]
        scl[_vr(0), :] = jnp.broadcast_to(scale, (8, 128))

    x_cp.wait()
    x = jnp.broadcast_to(xbuf[...].astype(f32), (8, D))
    set_input(_ln(x), jnp.full((8, 1), CEXP, f32))
    wq_cp.wait()
    lax.fori_loop(0, D // 16, retile_wq, 0)
    wo_cp.wait()
    lax.fori_loop(0, H * DH // 128, retile_wo, 0)

    def body1(i, acc):
        st = {"acc": acc}
        k_cp(i).wait()
        retile(ku, i, False)
        run_all(q_dots(i, st, qa))
        inv = []
        for hh in range(2):
            run_all(k_dots(i, hh, st, qa))
            inv.append(inv_sum(softmax(st["s", hh], hh)[1]))

        @pl.when(i > 0)
        def _():
            transpose_x(i - 1, XROWS)

        @pl.when(jnp.logical_and(i >= 5 - NQV, i < 5))
        def _():
            transpose_wq(i)

        v_cp(i).wait()
        retile(vu, i, True)
        for hh in range(2):
            def pv_step(c, carry, hh=hh):
                acc8 = [None] * 8
                for t in range(32):
                    pv = pT[4 * hh + t // 8][_vr(t % 8), :]
                    for G in range(4):
                        mac(acc8, 2 * G, i * 6 + c, G, t, pv)
                for n in range(8):
                    obuf[pl.ds(64 * c + 16 * (n // 2) + n % 2, 8, stride=2), :] = (
                        pltpu.bitcast(acc8[n], u32))
                return carry
            lax.fori_loop(3 * hh, 3 * hh + 3, pv_step, 0)
        o = reduce_o([obuf[128 * b:128 * b + 128, :] for b in range(3)], inv[0], inv[1])
        run_all([o_dot(i, b, st, lambda b=b: pack16(o[b])) for b in range(3)])
        return st["acc"]

    x = x + row_sum(lax.fori_loop(0, NP, body1, jnp.zeros((8, D), f32)))

    y = _ln(x)
    zz = _ln(y).astype(bf16)
    w3_cp.wait()
    h = jnp.dot(zz, w3[...], preferred_element_type=f32)
    h = jax.nn.gelu(h, approximate=True).astype(bf16)
    x = x + y
    transpose_x(NP - 1, XROWS_LAST)
    for k in range(W4_MXU, F, 128):
        hk = jnp.broadcast_to(h[0:1, k:k + 128].astype(f32), (128, 128))
        obuf[k - W4_MXU:k - W4_MXU + 128, :] = pltpu.bitcast(hk.T, u32)
    part = jnp.zeros((8, D), f32)
    for cp, (a, b) in zip(w4_cp, w4_rows):
        cp.wait()
        if a < W4_MXU:
            x = x + jnp.dot(h[:, a:b], w4[a:b, :], preferred_element_type=f32)
        else:
            for k in range(a, b, 16):
                hk = pltpu.bitcast(obuf[k - W4_MXU:k - W4_MXU + 16, :], f32)
                t = w4[k:k + 16, :].astype(f32) * jnp.concatenate([hk] * 5, axis=1)
                part = part + (t[0:8] + t[8:16])
    x = x + row_sum(part)

    ones = jnp.ones((8, D), f32)
    xl = _rows16(x, ones)
    xb = xl[0:8].astype(f32)
    mean = _mean(xb)
    c = xb - mean
    set_input(c, lax.rsqrt(_mean(c * c) + EPS) * CEXP)
    abuf[...] = jnp.where(lax.broadcasted_iota(jnp.int32, (8, D), 0) == 0, x, 0.0)

    def tail_hooks(i, st, hooks, seg0):
        def first(_):
            m = row_max(st["s", 0])
            st["pa"] = [prob(col(st["s", 0], T), m) for T in range(4)]
            set_state(i, S_INVA, inv_sum(part_sum(st["pa"])))
            for T in range(4):
                park_p(i, S_PA + T, st["pa"][T])

        def put(T, half):
            def run(clk):
                tick(pT[T], 8, clk)
                put_p(0, T, st["pa"][T], range(4 * half, 4 * half + 4))
            return run
        hooks.setdefault(("seg", seg0), []).append(first)
        for n in range(8):
            hooks.setdefault(("seg", seg0 + n), []).append(put(n // 2, n % 2))

    def head_b_hooks(i, segs, pb, final=False, park=False):
        def put_b(T):
            def run(clk):
                tick(scl, 4, clk)
                pb.append(prob(get_state(i, T), get_state(i, S_MAXB)))
                put_p(1, T, pb[T])
                if park and T < 3:
                    park_p(i, S_PB + T, pb[T])
                if T == 3:
                    set_state(i, S_LB, inv_sum(part_sum(pb)) if final else part_sum(pb))
            return run
        return {("seg", segs[T]): [put_b(T)] for T in range(4)}

    def reduce_pair(i):
        xa, xb = get_state(i, S_X), get_state(i, S_X + 1)
        invb = inv_sum(get_state(i, S_LB))
        return reduce_o([ku[i * GP + b] for b in range(3)],
                        get_state(i, S_INVA), invb, (xa, None, xb))

    st = {}
    new_block()
    late = tuple(range(8, 12)) + tuple(range(8))
    q0, q1, q2 = qt
    dots = q_dots(0, st, q0, xl, mean) + q_dots(1, st, q1, xl, mean) \
        + k_dots(0, 0, st, q0) + k_dots(0, 1, st, q0, late) + k_dots(1, 0, st, q1, late) \
        + k_dots(1, 1, st, q1, late) + k_dots(2, 0, st, q2, late) + k_dots(2, 1, st, q2)
    for n in range(4):
        dots += x_dots(n // 2, n % 2, XROWS[n % 2], parked(n // 2, (S_PA, S_PB)[n % 2]))

    def lane_softmax(h, first=False):
        i, hh = h // 2, h % 2

        def run():
            s0 = st["s", hh]
            m = jnp.maximum(jnp.maximum(col(s0, 0), col(s0, 1)),
                            jnp.maximum(col(s0, 2), col(s0, 3)))
            m = jnp.max(m, axis=0, keepdims=True)
            p = st["p", h] = [prob(col(s0, T), m) for T in range(4)]
            if first:
                for T in range(4):
                    for rho in range(8):
                        pT[T][_vr(rho), :] = jnp.broadcast_to(p[T][rho:rho + 1], (8, 128))
            w = st["w", h] = prob(m, jnp.max(m, axis=1, keepdims=True))
            l = part_sum(p) * w
            set_state(i, (S_INVA, S_LB)[hh], l if hh else inv_sum(l))
            for T in range(4 - hh):
                park_p(i, (S_PA, S_PB)[hh] + T, p[T] * w)
        return run

    def put_lane(h, T):
        def run(clk):
            tick(pT[4 * (h % 2) + T], 8, clk)
            put_p(h % 2, T, st["p", h][T])
        return run

    hooks = head_b_hooks(1, range(48 + B1_SEG, 96, 3), [], park=True)
    hooks.update({("need", 0): 23, ("need", B0_SEG): 35, ("need", A1_SEG): 47,
                  ("need", 48 + B1_SEG): DB1 + 1, ("need", 48 + A2_SEG): 70,
                  ("after", 82): 48 + B1_SEG + 9})
    for n, fn in ((10, lambda: mid_q(st, q0)),
                  (DQ[0], lambda: tick(q0, 5, q_vpu(2, c, q2))),
                  (DQ[1], lambda: tick(q0, 5, q_vpu(3, c, qa))),
                  (DQ[2], lambda: tick(q0, 5, q_vpu(4, c, qb))),
                  (DA0, lambda: tick(q0, 6, scl[_vr(0), :])), (22, lane_softmax(0, True)),
                   (DW0, lambda: tick(q0, 7, st["w", 0])),
                  (34, lane_softmax(1)), (DB0, lambda: tick(q1, 6, st["w", 1])),
                  (46, lane_softmax(2)), (DA1, lambda: tick(q1, 6, st["w", 2])),
                  (DB1, lambda: tick(q2, 6, stash_b(1, st["s", 1]))),
                  (82, lambda: stash_b(2, st["s", 1]))):
        hooks.setdefault(("dot", n), []).append(fn)
    for h in range(3):
        hooks["scale", h] = lambda h=h: st["w", h]
    hooks["notick", 0] = NOTICK
    hooks.update({("seg", B0_SEG + 2 * T): [put_lane(1, T)] for T in range(4)})
    hooks.update({("seg", A1_SEG + 2 * T): [put_lane(2, T)] for T in range(4)})
    tail_hooks(2, st, hooks, 48 + A2_SEG)
    run_block([0, 1], XROWS, dots, hooks, PLANS["first"])

    qs = (qb, qa)

    def late_dots(st):
        todo = [(m, 2) for m in range(NP - 2)] + [(NP - 3, 1)] + [(NP - 2, b) for b in range(3)]
        return [o_dot(m, b, st, lambda n=m + (2 - b) * 6: obuf[_vr(n), :], obuf) for m, b in todo]

    def block(name, j, ks, reds, qn, xrows):
        last = ks == [NP - 1]
        a_seg = A_SEG3 if name == "third" else A_SEG0
        b_segs = {"third": B_SEGS3,
                  "last": range(B_SEGL, 48, 3)}.get(name, B_SEGS)
        new_block()
        st = {}
        for k in ks if not last else []:
            mid_q(st, qs[(k + 1) % 2])
        outs = [reduce_pair(j + r) for r in reds]

        def kept(n):
            return (0, 1, 2) if last else (1, 2) if reds[n] == NP - 3 else (2,)

        def keep():
            for n, r in enumerate(reds):
                for b in kept(n):
                    obuf[pl.ds(pl.multiple_of(8 * (j + r + (2 - b) * 6), 8), 4), :] = (
                        pack8(outs[n][b]))

        if not last:
            keep()
        pb = []
        hooks = head_b_hooks(j + ks[0], b_segs, pb, last)
        dots = []

        def hook(key, fn):
            hooks.setdefault(key, []).append(fn)

        def direct(i, hh, seg0, tref):
            p = []

            def run():
                m = row_max(st["s", hh])
                p.extend(prob(col(st["s", hh], T), m) for T in range(4))
                l = part_sum(p)
                set_state(i, (S_INVA, S_LB)[hh], l if hh else inv_sum(l))

            def put(T, half):
                def go(clk):
                    tick(pT[4 * hh + T], 8, clk)
                    put_p(hh, T, p[T], range(4 * half, 4 * half + 4))
                return go
            hook(("dot", len(dots)), run)
            dots.extend(x_dots(i, hh, xrows[hh], lambda T: pack16(p[T]), tref))
            hooks["need", seg0] = len(dots)
            for n in range(8):
                hook(("seg", seg0 + n), put(n // 2, n % 2))

        def wo_of(n):
            return [o_dot(j + reds[n], b, st, lambda b=b: pack16(outs[n][b]), lref)
                    for b in range(3) if b not in kept(n)]

        def wq_of(n):
            nq = j + qn[n]
            return q_dots(nq if isinstance(nq, int) else jnp.minimum(nq, NP - 1), st, qs[qn[n] % 2])

        if last:
            dots += late_dots(st)[:NLATE] + x_dots(NP - 1, 0, xrows[0], parked(NP - 1, S_PA), lref)

            def park_acc(G, a4):
                for n in range(4):
                    ku[(NP - 1) * GP + 2, _vr(2 * (G - 16) + n), :] = pltpu.bitcast(a4[n], u32)
            hooks["end", 0] = park_acc
        for n, k in enumerate(ks if not last else []):
            q = qs[(k + 1) % 2]
            dots += k_dots(j + (k + 1), 0, st, q, MIX if n else MIXA, NALT if n else 0)
            if n == 0:
                if xrows[1]:
                    hooks["after", len(dots)] = b_segs[3]
                dots += x_dots(j + ks[0], 1, xrows[1], lambda T: pack16(pb[T]), q)
            else:
                direct(j + k, 1, 48 * n + BD_SEG, q)
            kb = k_dots(j + (k + 1), 1, st, q, MIX)
            if n < len(ks) - 1:
                dots += kb[:XA_AT]
                direct(j + (k + 1), 0, 48 * n + AD_SEG, q)
                dots += kb[XA_AT:] + wq_of(n) + wo_of(n)
            else:
                hooks["need", 48 * n + a_seg] = len(dots)
                tail_hooks(j + (k + 1), st, hooks, 48 * n + a_seg)
                dots += kb
                hook(("dot", len(dots)), lambda k=k: stash_b(j + (k + 1), st["s", 1]))
                for m in range(n, len(qn)):
                    dots += wq_of(m)
                for m in range(n, len(reds)):
                    dots += wo_of(m)
                dots += x_dots(j + ks[0], 0, xrows[0],
                               parked(j + ks[0], S_PA), lref)
        run_block([j + k for k in ks], xrows, dots, hooks,
                  PLANS[name], range(NSPLIT) if last else None)
        if last:
            keep()
        if reds:
            abuf[...] += st["acc"]

    def body2(n, carry):
        block("body", 2 * n, [2, 3], [0, 1], [5, 6], XROWS)
        return carry

    lax.fori_loop(0, NP // 2 - 2, body2, 0)
    pl.when(zs[0] == 0)(lambda: block("third", 0, [NP - 2], [NP - 4, NP - 3], [], XROWS))
    pl.when(zs[0] <= 0)(lambda: block("last", 0, [NP - 1], [NP - 2], [], XROWS_LAST))

    new_block()
    st = {"acc": abuf[...]}
    invb = get_state(NP - 1, S_LB)
    o = reduce_o([ku[(NP - 1) * GP + b] for b in range(2)], get_state(NP - 1, S_INVA), invb,
                 (get_state(NP - 1, S_X), None))
    part = [None] * 5

    def finish(G, a4):
        for k in range(4):
            tick(lref, L_DUMMY + k, a4[k])
        z = lref[_vr(5), :]
        project(G, [pltpu.bitcast(v, u32) | z for v in a4])

    def project(G, a4):
        for n in range(4):
            v = jnp.sum(pltpu.bitcast(a4[n], f32), axis=1, keepdims=True)
            for nt in range(5):
                w = wou[(NP - 1) * (GP // 2) + G + n // 2, nt]
                t = pltpu.bitcast(w & jnp.uint32(HI) if n % 2 else w << 16, f32) * v
                part[nt] = t if part[nt] is None else part[nt] + t

    for G in range(16, NSPLIT // 2, 2):
        project(G, [ku[(NP - 1) * GP + 2, _vr(2 * (G - 16) + n), :] for n in range(4)])
    dots = late_dots(st)[NLATE:] + [o_dot(NP - 1, b, st, lambda b=b: pack16(o[b]), lref)
                                    for b in range(2)]
    run_block([NP - 1], XROWS_LAST, dots, {("end", 0): finish},
              PLANS["final"], range(NSPLIT, 48))
    x = row_sum(st["acc"] + jnp.concatenate([v * invb for v in part], axis=1))

    xl = _rows16(x, ones)
    d = xl[0:8].astype(f32) - mean
    md = _mean(d)
    r1 = lax.rsqrt(jnp.maximum(_mean(d * d) - md * md, 0.0) + EPS)
    mean = mean + md
    y = (d - md) * r1
    my = _mean(y)
    r2 = lax.rsqrt(jnp.maximum(_mean(y * y) - my * my, 0.0) + EPS)
    h = jnp.dot(xl, w3[...], preferred_element_type=f32)
    h = h[0:8] * (r1 * r2) - h[8:16] * ((mean * r1 + my) * r2)
    h = jax.nn.gelu(h, approximate=True).astype(bf16)
    x = x + y
    parts = []
    for k in range(0, W4_VPU, 128):
        hk = jnp.broadcast_to(h[0:1, k:k + 128].astype(f32), (128, 128)).T
        t = w4[k:k + 128, :].astype(f32) * jnp.concatenate([hk] * 5, axis=1)
        parts.append(jnp.sum(t.reshape(16, 8, D), axis=0))
    for k in range(W4_VPU, F, 128):
        if k == W4_AT:
            x = x + row_sum(sum(parts[1:], parts[0]))
        x = x + jnp.dot(h[:, k:k + 128], w4[k:k + 128, :], preferred_element_type=f32)
    o_ref[...] = x[0:1].astype(o_ref.dtype)


def _cache_view(c):
    s = c.shape[2]
    c = jnp.transpose(c, (0, 1, 3, 2)).reshape(H * DH // 8, 8, s // 128, 128)
    return jnp.transpose(c, (0, 2, 1, 3)).reshape(H * DH // 8, s // 128 * 8, 128)


def _weight_view(w):
    k, n = w.shape
    w = jnp.transpose(w.reshape(k // 16, 2, 8, n // 128, 128), (0, 1, 3, 2, 4))
    return w.reshape(k // 16, n // 128, 16, 128)


@jax.jit
def pallas_interleave_layers__sliding_block_cached__mixer_s_mlp__decode_kernel(
    A_x: jax.Array,
    A_k_cache: jax.Array,
    A_v_cache: jax.Array,
    A_wq: jax.Array,
    A_wo: jax.Array,
    B_x: jax.Array,
    B_w1: jax.Array,
    B_w2: jax.Array,
    B_w3: jax.Array,
    B_w4: jax.Array,
):
    sk = A_k_cache.shape[2]
    win = min(4096, max(256, sk // 4))
    assert win == 4096 and sk % 128 == 0
    assert A_x.shape == (1, 1, D) and A_k_cache.shape == (1, H, sk, DH)
    wt = win // 128
    t0 = sk // 128 - wt
    ng = H * DH // 8
    hbm = pl.BlockSpec(memory_space=pl.ANY)
    out = pl.pallas_call(
        functools.partial(_kernel, t0=t0, wt=wt),
        out_shape=jax.ShapeDtypeStruct((1, D), A_x.dtype),
        in_specs=[hbm] * 7,
        out_specs=pl.BlockSpec(memory_space=pltpu.VMEM),
        scratch_shapes=[
            pltpu.VMEM((ng, wt * 8, 128), bf16),
            pltpu.VMEM((ng, wt * 8, 128), bf16),
            pltpu.VMEM((ng // 4, 256, 128), bf16),
            pltpu.VMEM((NP * D // 16, 3, 8, 128), u32),
            pltpu.VMEM((H * DH // 16, D // 128, 16, 128), bf16),
            pltpu.VMEM((D, F), bf16),
            pltpu.VMEM((F, D), bf16),
            pltpu.VMEM((1, D), bf16),
            pltpu.VMEM((144, 128), u32),
            pltpu.VMEM((384, 128), u32),
            pltpu.VMEM((144, 128), u32),
            pltpu.VMEM((144, 128), u32),
            pltpu.VMEM((144, 128), u32),
            pltpu.VMEM((40, 128), f32),
            pltpu.VMEM((8, D), f32),
            pltpu.SMEM((1,), jnp.int32),
        ] + [pltpu.VMEM((64, 128), u32)] * 3
        + [pltpu.VMEM((72, 128), f32)] * 8,
        compiler_params=pltpu.CompilerParams(vmem_limit_bytes=128 * 1024 * 1024),
    )(A_x.reshape(1, D), _cache_view(A_k_cache), _cache_view(A_v_cache),
      _weight_view(A_wq).reshape(D * 3 // 16, 256, 128), _weight_view(A_wo), B_w3, B_w4)
    return out.reshape(1, 1, D)
```

```python
import functools

import jax
import jax.numpy as jnp
from jax import lax
import jax.experimental.pallas as pl
import jax.experimental.pallas.tpu as pltpu

D = 640
H = 32
DH = 192
F = 1536
EPS = 1e-5
NP = H // 2
GP = 2 * DH // 8
HI = 0xFFFF0000
CEXP = DH ** -0.5 * 1.4426950408889634

f32 = jnp.float32
bf16 = jnp.bfloat16
u32 = jnp.uint32

L_Y = 0
L_DUMMY = 6
S_MAXB, S_LB, S_INVA, S_X, S_PA, S_PB = 4, 5, 6, 7, 9, 13
XROWS = ((2, 10, 18, 26), (4, 12, 20))
XROWS_LAST = ((2, 10, 18, 26, 6, 14, 22, 30, 4, 12, 20, 28), ())
GX = (0, 16)
PLANS = {
    "first": (
        {},
        (21, 23, 23, 23, 24, 25, 27, 27, 27, 28, 29, 29, 30, 31, 30, 31, 32, 32, 33, 34, 34, 35,
        36, 36, 37, 38, 38, 39, 40, 40, 41, 42, 43, 43, 44, 44, 45, 46, 46, 47, 48, 48, 49, 49,
        50, 51, 51, 52, 52, 52, 53, 54, 54, 56, 56, 56, 57, 58, 58, 59, 60, 60, 61, 62, 62, 63,
        64, 64, 65, 66, 66, 67, 68, 68, 69, 70, 70, 71, 72, 72, 73, 74, 74, 75, 76, 76, 77, 78,
        78, 79, 80, 81, 82, 82, 83, 82)),
    "body": (
        {1: 0, 3: 1, 5: 3, 7: 4, 9: 5, 11: 8, 12: 10, 15: 10, 19: 12, 21: 14, 23: 16, 25: 17,
        27: 19, 29: 22, 31: 23, 33: 23, 35: 26, 37: 26, 39: 28, 40: 33, 41: 33, 43: 34, 45: 34,
        47: 34, 49: 35, 51: 37, 53: 38, 55: 39, 57: 40, 59: 42, 61: 43, 63: 46, 67: 49, 70: 51,
        71: 52, 72: 53, 75: 55, 77: 56, 79: 58, 81: 59, 83: 62, 84: 62},
        (0, 0, 0, 0, 0, 0, 0, 0, 0, 0, 0, 1, 2, 2, 3, 4, 4, 5, 6, 7, 7, 8, 9, 10, 10, 12, 12,
        13, 14, 15, 15, 16, 16, 17, 17, 18, 20, 21, 21, 24, 25, 23, 24, 27, 27, 33, 29, 29, 28,
        30, 30, 31, 31, 32, 33, 33, 34, 35, 35, 36, 36, 35, 35, 36, 37, 39, 43, 41, 43, 40, 45,
        45, 46, 48, 48, 48, 49, 50, 50, 51, 52, 51, 51, 54, 53, 54, 56, 58, 57, 59, 61, 59, 61,
        62, 63, 64)),
    "third": (
        {1: 0, 3: 3, 6: 3, 7: 4, 9: 5, 11: 8, 15: 10, 18: 12, 19: 14, 21: 14, 23: 15, 25: 17,
        26: 19, 27: 19, 30: 21},
        (0, 0, 0, 0, 0, 0, 0, 0, 0, 0, 1, 0, 0, 3, 3, 5, 2, 5, 4, 8, 7, 8, 10, 10, 10, 12, 12,
        13, 15, 17, 15, 16, 17, 17, 18, 19, 20, 18, 21, 22, 22, 24, 25, 26, 25, 24, 25, 26)),
    "last": (
        {1: 0, 3: 1, 7: 2, 11: 3, 15: 4, 17: 6, 19: 7, 21: 10, 23: 11, 27: 13},
        (0, 0, 0, 0, 0, 0, 0, 0, 0, 0, 0, 0, 0, 0, 0, 0, 1, 1, 2, 3, 4, 6, 6, 6, 7, 7, 8, 6, 8,
        9, 9, 10, 10, 11, 11, 11)),
    "final": (
        {37: 0, 39: 1, 40: 2, 41: 3, 42: 3, 43: 4, 45: 5},
        (0, 0, 0, 0, 0, 0, 0, 0, 0, 0, 0, 0, 0, 0, 0, 0, 0, 0, 0, 0, 0, 0, 0, 0, 0, 0, 0, 0, 0,
        0, 0, 0, 0, 0, 0, 0, 0, 0, 0, 0, 0, 0, 5, 2, 0, 1, 0, 0)),
}
MIX = (0, 1, 8, 2, 3, 9, 4, 5, 10, 6, 7, 11)
MIXA = (0, 1, 2, 3, 4, 8, 5, 9, 6, 10, 7, 11)
NLATE = 12
NSPLIT = 36
W4_VPU = 256
W4_AT = 896
B_SEGS = (9, 12, 15, 18)
B_SEGL = 8
DA0 = 16
NOTICK = 3
DW0 = 32
DB0 = 44
DA1 = 56
DB1 = 67
DQ = (26, 29, 33)
NQV = 3
B0_SEG = 17
A1_SEG = 39
B1_SEG = 12
A2_SEG = 40
A_SEG0 = 40
A_SEG3 = 38
B_SEGS3 = (9, 11, 15, 19)
XA_AT = 8
AD_SEG = 32
BD_SEG = 12
NALT = 2
W4_CHUNKS = (1024, 256, 160, 64, 32)
W4_MXU = 1280


def _mean(x):
    return jnp.mean(x, axis=-1, keepdims=True)


def _ln(x):
    c = x - _mean(x)
    return c * lax.rsqrt(_mean(c * c) + EPS)


def _wtile(wu, rows, nt):
    blk = wu[rows, nt]
    return pltpu.bitcast(blk.reshape(blk.shape[0] * 8, 128), bf16)


def _wcols(wu, rows, nts):
    return jnp.concatenate([_wtile(wu, rows, n) for n in nts], axis=1)


def _rows16(a, b):
    return jnp.concatenate([a, b], axis=0).astype(bf16)


def _slot(G, t):
    j = 4 * (t >> 3) + ((((t >> 1) & 3) + G + 2 * (t & 1) + (t >> 3)) & 3)
    return 2 * G + (t & 1), 8 * j


def _xslot(G, t):
    return G // 2, 8 * (4 * (t >> 3) + ((((t >> 1) & 3) + G + (t >> 3)) & 3))


def _vr(n):
    return slice(8 * n, 8 * n + 8)


def _kernel(*refs, t0, wt):
    pl.run_scoped(functools.partial(_body, refs, t0, wt),
                  pltpu.SemaphoreType.DMA((4 + len(W4_CHUNKS) + 2 * NP,)))


def _body(refs, t0, wt, sems):
    (x_hbm, k_hbm, v_hbm, wq_hbm, wo_hbm, w3_hbm, w4_hbm, o_ref,
     kbuf, vbuf, vx, wqu, wo, w3, w4, xbuf, lref, obuf, qa, qb, qx, scl, abuf, zs) = refs[:24]
    qt, pT = refs[24:27], refs[27:]
    ku = kbuf.bitcast(u32)
    vu = vbuf.bitcast(u32)
    wou = wo.bitcast(u32)

    x_cp = pltpu.make_async_copy(x_hbm, xbuf, sems.at[0])
    wq_cp = pltpu.make_async_copy(wq_hbm, wo, sems.at[1])
    wo_cp = pltpu.make_async_copy(wo_hbm, wo, sems.at[2])
    w3_cp = pltpu.make_async_copy(w3_hbm, w3, sems.at[3])
    w4_rows, r0 = [], 0
    for n in W4_CHUNKS:
        w4_rows.append((r0, r0 + n))
        r0 += n
    w4_cp = [pltpu.make_async_copy(w4_hbm.at[a:b], w4.at[a:b], sems.at[4 + c])
             for c, (a, b) in enumerate(w4_rows)]
    S0 = 4 + len(W4_CHUNKS)

    def k_cp(i):
        return pltpu.make_async_copy(
            k_hbm.at[pl.ds(i * GP, GP), pl.ds(t0 * 8, wt * 8), :],
            kbuf.at[pl.ds(i * GP, GP)], sems.at[S0 + i])

    def v_cp(i):
        return pltpu.make_async_copy(
            v_hbm.at[pl.ds(i * GP, GP), pl.ds(t0 * 8, wt * 8), :],
            vbuf.at[pl.ds(i * GP, GP)], sems.at[S0 + NP + i])

    for c in (wq_cp, x_cp, k_cp(0), v_cp(0)):
        c.start()

    zs[0] = 0
    for ref in (qa, qb, qx, lref):
        ref[_vr(5), :] = jnp.zeros((8, 128), u32)

    lane = lax.broadcasted_iota(jnp.int32, (8, 128), 1)
    sub = lax.broadcasted_iota(jnp.int32, (8, 128), 0)
    lane_lo = lane < 64
    sub_lo = sub < 4

    def pair_view(buf, i):
        return buf.at[pl.ds(i * GP, GP)].bitcast(u32)

    def tile(ref, g0, G, t):
        g, r = _slot(G, t)
        return ref[g0 + g, r:r + 8, :]

    def retile(ref, i, expand):
        def body(c, carry):
            g0 = 8 * c
            for G in range(4):
                for J in range(4):
                    xs = [[ref[g0 + 2 * G + e, _vr(4 * J + jj), :] for jj in range(4)]
                          for e in range(2)]
                    for jj in range(4):
                        x0, x1 = xs[0][jj], xs[1][jj]
                        ys = (jnp.where(sub_lo, x0, pltpu.roll(x1, 4, 0)),
                              jnp.where(sub_lo, pltpu.roll(x0, 4, 0), x1))
                        for e in range(2):
                            t = 8 * J + 2 * jj + e
                            g, r = _slot(G, t)
                            if expand and G % 2 and e:
                                ref[g0 + g, r:r + 8, :] = ys[e] << 16
                                g, r = _xslot(G, t)
                                vx[i * (GP // 4) + 2 * c + g, r:r + 8, :] = ys[e] & jnp.uint32(HI)
                            else:
                                ref[g0 + g, r:r + 8, :] = ys[e]
            return carry
        lax.fori_loop(0, GP // 8, body, 0)

    def merge_halves(get, nt, n):
        lo, hi = get(n // 2), get((nt + n) // 2)
        if n % 2:
            lo = pltpu.roll(lo, 4, 0)
        if (nt + n) % 2 == 0:
            hi = pltpu.roll(hi, 4, 0)
        return jnp.where(sub_lo, lo, hi)

    def retile_wq(c, carry):
        for G in range(5):
            for n in range(3 * NP):
                wqu[n // 3 * (D // 16) + 5 * c + G, n % 3] = merge_halves(
                    lambda v: wou[48 * c + (48 * G + v) // 5, (48 * G + v) % 5], 3 * NP, n)
        return carry

    def retile_wo(c, carry):
        for G in range(8):
            xs = [wou[8 * c + G, n] for n in range(5)]
            for n in range(5):
                wou[8 * c + G, n] = merge_halves(lambda v: xs[v], 5, n)
        return carry

    def lhs_at(ref, n):
        return pltpu.bitcast(ref[_vr(n), :], bf16)

    cur = [None]

    def new_block():
        cur[0] = -32 * jnp.clip(zs[0], 0, 1)

    def tick(ref, n, val):
        if val.dtype != ref.dtype:
            val = pltpu.bitcast(val, ref.dtype)
        ref[pl.ds(pl.multiple_of(cur[0] + 8 * n, 8), 8), :] = val

    def put_q(q, qref):
        qq = pltpu.bitcast(q.astype(bf16).astype(f32), u32)
        q0, q1, q2 = qq[:, 0:128], qq[:, 128:256], qq[:, 256:384]
        for n, v in enumerate((q0 >> 16, q0, q2 >> 16, q2, q1)):
            qref[_vr(n), :] = v
            if n < 2 and qref is qb:
                qx[_vr(n), :] = v

    def transpose_wq(i):
        for k in range(5):
            for n in range(3):
                rows = pl.ds(i * (D // 16) + 8 * k, 8)
                w = pltpu.bitcast(_wtile(wqu, rows, n).astype(f32).T, u32)
                for G in range(8):
                    wqu[i * (D // 16) + 8 * k + G, n] = (w[_vr(2 * G), :] >> 16) | w[_vr(2 * G + 1), :]

    def q_vpu(i, c, qref):
        cols = []
        for n in range(3):
            acc = []
            for G in range(8):
                ws = [wqu[i * (D // 16) + 8 * k + G, n] for k in range(5)]
                for half in (lambda w: w << 16, lambda w: w & jnp.uint32(HI)):
                    t = [pltpu.bitcast(half(ws[k]), f32) * col(c, k) for k in range(5)]
                    acc.append((t[0] + t[1]) + (t[2] + t[3]) + t[4])
            z = jnp.sum(jnp.concatenate(acc, axis=0).T.reshape(16, 8, 128), axis=0)
            cols.append(row_sum(z))
        put_q(jnp.concatenate(cols, axis=1), qref)
        return cols[0] + cols[1] + cols[2]

    def row_sum(a):
        return jnp.broadcast_to(jnp.sum(a, axis=0, keepdims=True), a.shape)

    def q_dots(i, st, qref, lhs=None, mean=None):
        def step(k):
            def run(tied=False):
                w = _wcols(wqu, pl.ds(i * (D // 16) + 8 * k, 8), range(3))
                if lhs is None:
                    r = jnp.dot(lhs_at(lref, L_Y + k), w, preferred_element_type=f32)[0:8]
                else:
                    r = jnp.dot(lhs[:, 128 * k:128 * k + 128], w, preferred_element_type=f32)
                st["q"] = r if k == 0 else st["q"] + r
                if k == 4:
                    q = st["q"] if lhs is None else st["q"][0:8] - mean * st["q"][8:16]
                    put_q(q, qref)
                return r[0:8, 256:384]
            return 3, lref, L_DUMMY, run
        return [step(k) for k in range(5)]

    def o_dot(i, b, st, get_lhs, tref=None):
        def run(tied=False):
            w = _wcols(wou, pl.ds(i * (GP // 2) + 8 * b, 8), range(5))
            lhs = get_lhs() | tref[_vr(5), :] if tied and tref is not obuf else get_lhs()
            r = jnp.dot(pltpu.bitcast(lhs, bf16), w, preferred_element_type=f32)[0:8]
            st["acc"] = st["acc"] + r if "acc" in st else r
            return r[:, 512:640]
        return 5, tref, (32 if tref is obuf else 6), run

    def mid_q(st, qref):
        q1 = qref[_vr(4), :]
        q1r = pltpu.roll(q1, 64, 1)
        st["u", 0, id(qref)] = jnp.where(lane_lo, q1 >> 16, q1r)
        st["u", 1, id(qref)] = jnp.where(lane_lo, q1r >> 16, q1)

    def k_dots(i, hh, st, qref, order=tuple(range(12)), nalt=0, ku=ku):
        g0 = i * GP
        gf, gh = ((0, 8), (16, 12))[hh]

        def step(r):
            src = qx if r in order[:nalt] else qref

            def run(tied=False):
                if r < 8:
                    cols = [[tile(ku, g0, gf + G, 8 * T + r) for G in range(8)] for T in range(4)]
                    base, row = src[_vr(2 * hh + r % 2), :], r // 2
                else:
                    cols = [[tile(ku, g0, gh + G % 4, 8 * T + 2 * (r - 8) + G // 4)
                             for G in range(8)] for T in range(4)]
                    if ("u", hh, id(qref)) not in st:
                        mid_q(st, qref)
                    base, row = st["u", hh, id(qref)], r - 8
                    if tied:
                        base = base | src[_vr(5), :]
                lhs = jnp.where(sub == row, base, jnp.zeros((8, 128), u32))
                w = jnp.concatenate([jnp.concatenate(c, axis=0) for c in cols], axis=1)
                res = jnp.dot(pltpu.bitcast(lhs, bf16), pltpu.bitcast(w, bf16),
                              preferred_element_type=f32)[0:8]
                st["s", hh] = res if r == order[0] else st["s", hh] + res
                return res[:, 384:512]
            return 4, src, 6, run
        return [step(r) for r in order]

    def col(s, T):
        return s[:, 128 * T:128 * T + 128]

    def row_max(s):
        m = jnp.maximum(jnp.maximum(col(s, 0), col(s, 1)), jnp.maximum(col(s, 2), col(s, 3)))
        return jnp.max(jnp.max(m, axis=1, keepdims=True), axis=0, keepdims=True)

    def prob(s, m):
        return jnp.exp2((s - m) * scl[_vr(0), :])

    def put_p(hh, T, p, ks=range(8)):
        for k in ks:
            pT[4 * hh + T][pl.ds(k, 8, stride=8), :] = p

    def part_sum(p):
        return (p[0] + p[1]) + (p[2] + p[3])

    def inv_sum(l):
        l = jnp.sum(jnp.sum(l, axis=1, keepdims=True), axis=0, keepdims=True)
        r = pl.reciprocal(l, approx=True)
        return jnp.broadcast_to(r * (2.0 - l * r), (8, 128))

    def softmax(s, hh):
        m = row_max(s)
        p = [prob(col(s, T), m) for T in range(4)]
        for T in range(4):
            put_p(hh, T, p[T])
        return p, part_sum(p)

    def get_state(i, n):
        return pltpu.bitcast(ku[i * GP + 3, _vr(n), :], f32)

    def set_state(i, n, v):
        ku[i * GP + 3, _vr(n), :] = pltpu.bitcast(v, u32)

    def stash_b(i, s):
        for T in range(4):
            set_state(i, T, col(s, T))
        m = jnp.broadcast_to(row_max(s), (8, 128))
        set_state(i, S_MAXB, m)
        return m

    def pack8(v):
        return pltpu.bitcast(v.astype(bf16), u32)

    def park_p(i, n, p):
        ku[i * GP + 3, 8 * n:8 * n + 4, :] = pack8(p)

    def parked(i, n):
        return lambda T: ku[i * GP + 3, _vr(n + T), :]

    def x_dots(i, hh, ts, get_lhs, tref=None):
        st = {}
        rows = sorted({t % 8 for t in ts})

        def step(n, rho):
            def run(tied=False):
                res = []
                for T in [t // 8 for t in ts if t % 8 == rho]:
                    w = jnp.concatenate(
                        [tile(vu, i * GP, GX[hh] + G, 8 * T + rho) for G in range(8)], axis=0)
                    lhs = get_lhs(T) | tref[_vr(5), :] if tied else get_lhs(T)
                    res.append(jnp.dot(pltpu.bitcast(lhs, bf16), pltpu.bitcast(w, bf16),
                                       preferred_element_type=f32)[0:8])
                st["x"] = jnp.where(sub == rho, sum(res[1:], res[0]), st["x"] if n else 0.0)
                if n == len(rows) - 1:
                    set_state(i, S_X + hh, st["x"])
                return res[-1]
            return sum(1 for t in ts if t % 8 == rho), tref, 6, run
        return [step(n, rho) for n, rho in enumerate(rows)]

    def transpose_x(view, xrows):
        for hh in range(2):
            for t in xrows[hh]:
                w = jnp.concatenate([tile(view, 0, GX[hh] + G, t) for G in range(8)], axis=0)
                w = pltpu.bitcast(pltpu.bitcast(w, bf16).astype(f32).T.astype(bf16), u32)
                for G in range(8):
                    g, r = _slot(GX[hh] + G, t)
                    view[g, r:r + 8, :] = w[_vr(G), :]

    def reduce_o(blocks, inva, invb, extra=(None, None, None)):
        out = []
        for b, inv in enumerate((inva, jnp.where(lane_lo, inva, invb), invb)[:len(blocks)]):
            z = jnp.sum(pltpu.bitcast(blocks[b], f32).T.reshape(16, 8, 128), axis=0)
            if extra[b] is not None:
                z = z + extra[b]
            out.append(z * inv)
        return out

    def pack16(v):
        return pltpu.bitcast(_rows16(v, v), u32)

    def mac(acc, n, c, G, t, pv, view=None):
        w = tile(vu, 8 * c, G, t) if view is None else tile(view[0], view[1], G, t)
        if G % 2 and t % 2:
            g, r = _xslot(G, t)
            halves = (w, vx[2 * c + g, r:r + 8, :])
        else:
            halves = (w << 16, w & jnp.uint32(HI))
        for k in range(2):
            a = pltpu.bitcast(halves[k], f32) * pv
            acc[n + k] = a if acc[n + k] is None else acc[n + k] + a

    def seg_rows(xrows, seg):
        hh, gp, T = seg // 24 % 2, seg % 24 // 4, seg % 4
        on_mxu = GX[hh] <= 12 * hh + 2 * gp < GX[hh] + 8
        return [rho for rho in range(8) if not (on_mxu and 8 * T + rho in xrows[hh])]

    def run_block(pairs, xrows, dots, hooks, plan, segs=None):
        tie, clk = plan
        clock = []

        def emit(upto):
            while len(clock) < upto:
                n = len(clock)
                for h in hooks.get(("dot", n), ()):
                    h()
                clock.append(dots[n][3](n in tie.values()))

        zero = jnp.zeros((8, 128), f32)
        used = {}
        for seg in segs or range(48 * len(pairs)):
            i, hh, gp, T = pairs[seg // 48], seg // 24 % 2, seg % 24 // 4, seg % 4
            if T == 0:
                a4 = [None] * 4
            pref = pT[4 * hh + T]
            upto = min([v for k, v in tie.items() if k >= seg]
                       + [k[1] for k, v in hooks.items() if k[0] == "after" and v >= seg]
                       + [len(dots) if tie else clk[seg] + 6])
            free = not any(k in tie for k in range(seg, seg - T + 4))
            if free or ("seg", seg) in hooks:
                upto = max(upto, clk[seg] + 1)
            emit(min(len(dots), max(upto, hooks.get(("need", seg), 0))))
            if seg < hooks.get(("notick", 0), 0):
                pass
            elif free:
                tick(pref, 8, clock[clk[seg]])
            elif gp:
                tick(pref, 8, zero)
            for h in hooks.get(("seg", seg), ()):
                h(clock[clk[seg]])
            for rho in seg_rows(xrows, seg):
                pv = pref[_vr(rho), :]
                for e in range(2):
                    mac(a4, 2 * e, i * 6, 12 * hh + 2 * gp + e, 8 * T + rho, pv)
            if seg in tie:
                ref, slot = dots[tie[seg]][1:3]
                used[tie[seg]] = used.get(tie[seg], -1) + 1
                for k in range(4):
                    tick(ref, slot + 4 * used[tie[seg]] + k, a4[k])
            if T == 3 and ("end", 0) in hooks and seg >= 32:
                hooks["end", 0](12 * hh + 2 * gp, a4)
            elif T == 3:
                for n in range(4):
                    G = 12 * hh + 2 * gp + n // 2
                    v = a4[n] * hooks["scale", seg // 24]() if ("scale", seg // 24) in hooks else a4[n]
                    ku[i * GP + G // 8, pl.ds(16 * (G % 8) + n % 2, 8, stride=2), :] = (
                        pltpu.bitcast(v, u32))
        emit(len(dots))

    def run_all(dots):
        for d in dots:
            d[3]()

    def set_input(c, scale):
        cp = pltpu.bitcast(_rows16(c, c), u32)
        for k in range(5):
            lref[_vr(L_Y + k), :] = cp[:, 128 * k:128 * k + 128]
        scl[_vr(0), :] = jnp.broadcast_to(scale, (8, 128))

    x_cp.wait()
    x = jnp.broadcast_to(xbuf[...].astype(f32), (8, D))
    set_input(_ln(x), jnp.full((8, 1), CEXP, f32))
    wq_cp.wait()
    lax.fori_loop(0, D // 80, retile_wq, 0)
    wo_cp.start()
    for i in range(1, NP):
        k_cp(i).start()
        v_cp(i).start()
    for c in [w3_cp] + w4_cp:
        c.start()
    wo_cp.wait()
    lax.fori_loop(0, H * DH // 128, retile_wo, 0)

    def body1(i, acc):
        st = {"acc": acc}
        k_cp(i).wait()
        kv = pair_view(kbuf, i)
        retile(kv, i, False)
        run_all(q_dots(i, st, qa))
        inv = []
        for hh in range(2):
            run_all(k_dots(0, hh, st, qa, ku=kv))
            inv.append(inv_sum(softmax(st["s", hh], hh)[1]))

        @pl.when(i > 0)
        def _():
            transpose_x(pair_view(vbuf, i - 1), XROWS)

        @pl.when(jnp.logical_and(i >= 5 - NQV, i < 5))
        def _():
            transpose_wq(i)

        v_cp(i).wait()
        vv = pair_view(vbuf, i)
        retile(vv, i, True)
        for hh in range(2):
            def pv_step(c, carry, hh=hh):
                acc8 = [None] * 8
                for t in range(32):
                    pv = pT[4 * hh + t // 8][_vr(t % 8), :]
                    for G in range(4):
                        mac(acc8, 2 * G, i * 6 + c, G, t, pv, (vv, 8 * c))
                for n in range(8):
                    obuf[pl.ds(64 * c + 16 * (n // 2) + n % 2, 8, stride=2), :] = (
                        pltpu.bitcast(acc8[n], u32))
                return carry
            lax.fori_loop(3 * hh, 3 * hh + 3, pv_step, 0)
        o = reduce_o([obuf[128 * b:128 * b + 128, :] for b in range(3)], inv[0], inv[1])
        run_all([o_dot(i, b, st, lambda b=b: pack16(o[b])) for b in range(3)])
        return st["acc"]

    x = x + row_sum(lax.fori_loop(0, NP, body1, jnp.zeros((8, D), f32)))

    y = _ln(x)
    zz = _ln(y).astype(bf16)
    w3_cp.wait()
    h = jnp.dot(zz, w3[...], preferred_element_type=f32)
    h = jax.nn.gelu(h, approximate=True).astype(bf16)
    x = x + y
    transpose_x(pair_view(vbuf, NP - 1), XROWS_LAST)
    for k in range(W4_MXU, F, 128):
        hk = jnp.broadcast_to(h[0:1, k:k + 128].astype(f32), (128, 128))
        obuf[k - W4_MXU:k - W4_MXU + 128, :] = pltpu.bitcast(hk.T, u32)
    part = jnp.zeros((8, D), f32)
    for cp, (a, b) in zip(w4_cp, w4_rows):
        cp.wait()
        if a < W4_MXU:
            x = x + jnp.dot(h[:, a:b], w4[a:b, :], preferred_element_type=f32)
        else:
            for k in range(a, b, 16):
                hk = pltpu.bitcast(obuf[k - W4_MXU:k - W4_MXU + 16, :], f32)
                t = w4[k:k + 16, :].astype(f32) * jnp.concatenate([hk] * 5, axis=1)
                part = part + (t[0:8] + t[8:16])
    x = x + row_sum(part)

    ones = jnp.ones((8, D), f32)
    xl = _rows16(x, ones)
    xb = xl[0:8].astype(f32)
    mean = _mean(xb)
    c = xb - mean
    set_input(c, lax.rsqrt(_mean(c * c) + EPS) * CEXP)
    abuf[...] = jnp.where(lax.broadcasted_iota(jnp.int32, (8, D), 0) == 0, x, 0.0)

    def tail_hooks(i, st, hooks, seg0):
        def first(_):
            m = row_max(st["s", 0])
            st["pa"] = [prob(col(st["s", 0], T), m) for T in range(4)]
            set_state(i, S_INVA, inv_sum(part_sum(st["pa"])))
            for T in range(4):
                park_p(i, S_PA + T, st["pa"][T])

        def put(T, half):
            def run(clk):
                tick(pT[T], 8, clk)
                put_p(0, T, st["pa"][T], range(4 * half, 4 * half + 4))
            return run
        hooks.setdefault(("seg", seg0), []).append(first)
        for n in range(8):
            hooks.setdefault(("seg", seg0 + n), []).append(put(n // 2, n % 2))

    def head_b_hooks(i, segs, pb, final=False, park=False):
        def put_b(T):
            def run(clk):
                tick(scl, 4, clk)
                pb.append(prob(get_state(i, T), get_state(i, S_MAXB)))
                put_p(1, T, pb[T])
                if park and T < 3:
                    park_p(i, S_PB + T, pb[T])
                if T == 3:
                    set_state(i, S_LB, inv_sum(part_sum(pb)) if final else part_sum(pb))
            return run
        return {("seg", segs[T]): [put_b(T)] for T in range(4)}

    def reduce_pair(i):
        xa, xb = get_state(i, S_X), get_state(i, S_X + 1)
        invb = inv_sum(get_state(i, S_LB))
        return reduce_o([ku[i * GP + b] for b in range(3)],
                        get_state(i, S_INVA), invb, (xa, None, xb))

    st = {}
    new_block()
    late = tuple(range(8, 12)) + tuple(range(8))
    q0, q1, q2 = qt
    dots = q_dots(0, st, q0, xl, mean) + q_dots(1, st, q1, xl, mean) \
        + k_dots(0, 0, st, q0) + k_dots(0, 1, st, q0, late) + k_dots(1, 0, st, q1, late) \
        + k_dots(1, 1, st, q1, late) + k_dots(2, 0, st, q2, late) + k_dots(2, 1, st, q2)
    for n in range(4):
        dots += x_dots(n // 2, n % 2, XROWS[n % 2], parked(n // 2, (S_PA, S_PB)[n % 2]))

    def lane_softmax(h, first=False):
        i, hh = h // 2, h % 2

        def run():
            s0 = st["s", hh]
            m = jnp.maximum(jnp.maximum(col(s0, 0), col(s0, 1)),
                            jnp.maximum(col(s0, 2), col(s0, 3)))
            m = jnp.max(m, axis=0, keepdims=True)
            p = st["p", h] = [prob(col(s0, T), m) for T in range(4)]
            if first:
                for T in range(4):
                    for rho in range(8):
                        pT[T][_vr(rho), :] = jnp.broadcast_to(p[T][rho:rho + 1], (8, 128))
            w = st["w", h] = prob(m, jnp.max(m, axis=1, keepdims=True))
            l = part_sum(p) * w
            set_state(i, (S_INVA, S_LB)[hh], l if hh else inv_sum(l))
            for T in range(4 - hh):
                park_p(i, (S_PA, S_PB)[hh] + T, p[T] * w)
        return run

    def put_lane(h, T):
        def run(clk):
            tick(pT[4 * (h % 2) + T], 8, clk)
            put_p(h % 2, T, st["p", h][T])
        return run

    hooks = head_b_hooks(1, range(48 + B1_SEG, 96, 3), [], park=True)
    hooks.update({("need", 0): 23, ("need", B0_SEG): 35, ("need", A1_SEG): 47,
                  ("need", 48 + B1_SEG): DB1 + 1, ("need", 48 + A2_SEG): 70,
                  ("after", 82): 48 + B1_SEG + 9})
    for n, fn in ((10, lambda: mid_q(st, q0)),
                  (DQ[0], lambda: tick(q0, 5, q_vpu(2, c, q2))),
                  (DQ[1], lambda: tick(q0, 5, q_vpu(3, c, qa))),
                  (DQ[2], lambda: tick(q0, 5, q_vpu(4, c, qb))),
                  (DA0, lambda: tick(q0, 6, scl[_vr(0), :])), (22, lane_softmax(0, True)),
                   (DW0, lambda: tick(q0, 7, st["w", 0])),
                  (34, lane_softmax(1)), (DB0, lambda: tick(q1, 6, st["w", 1])),
                  (46, lane_softmax(2)), (DA1, lambda: tick(q1, 6, st["w", 2])),
                  (DB1, lambda: tick(q2, 6, stash_b(1, st["s", 1]))),
                  (82, lambda: stash_b(2, st["s", 1]))):
        hooks.setdefault(("dot", n), []).append(fn)
    for h in range(3):
        hooks["scale", h] = lambda h=h: st["w", h]
    hooks["notick", 0] = NOTICK
    hooks.update({("seg", B0_SEG + 2 * T): [put_lane(1, T)] for T in range(4)})
    hooks.update({("seg", A1_SEG + 2 * T): [put_lane(2, T)] for T in range(4)})
    tail_hooks(2, st, hooks, 48 + A2_SEG)
    run_block([0, 1], XROWS, dots, hooks, PLANS["first"])

    qs = (qb, qa)

    def late_dots(st):
        todo = [(m, 2) for m in range(NP - 2)] + [(NP - 3, 1)] + [(NP - 2, b) for b in range(3)]
        return [o_dot(m, b, st, lambda n=m + (2 - b) * 6: obuf[_vr(n), :], obuf) for m, b in todo]

    def block(name, j, ks, reds, qn, xrows):
        last = ks == [NP - 1]
        a_seg = A_SEG3 if name == "third" else A_SEG0
        b_segs = {"third": B_SEGS3,
                  "last": range(B_SEGL, 48, 3)}.get(name, B_SEGS)
        new_block()
        st = {}
        for k in ks if not last else []:
            mid_q(st, qs[(k + 1) % 2])
        outs = [reduce_pair(j + r) for r in reds]

        def kept(n):
            return (0, 1, 2) if last else (1, 2) if reds[n] == NP - 3 else (2,)

        def keep():
            for n, r in enumerate(reds):
                for b in kept(n):
                    obuf[pl.ds(pl.multiple_of(8 * (j + r + (2 - b) * 6), 8), 4), :] = (
                        pack8(outs[n][b]))

        if not last:
            keep()
        pb = []
        hooks = head_b_hooks(j + ks[0], b_segs, pb, last)
        dots = []

        def hook(key, fn):
            hooks.setdefault(key, []).append(fn)

        def direct(i, hh, seg0, tref):
            p = []

            def run():
                m = row_max(st["s", hh])
                p.extend(prob(col(st["s", hh], T), m) for T in range(4))
                l = part_sum(p)
                set_state(i, (S_INVA, S_LB)[hh], l if hh else inv_sum(l))

            def put(T, half):
                def go(clk):
                    tick(pT[4 * hh + T], 8, clk)
                    put_p(hh, T, p[T], range(4 * half, 4 * half + 4))
                return go
            hook(("dot", len(dots)), run)
            dots.extend(x_dots(i, hh, xrows[hh], lambda T: pack16(p[T]), tref))
            hooks["need", seg0] = len(dots)
            for n in range(8):
                hook(("seg", seg0 + n), put(n // 2, n % 2))

        def wo_of(n):
            return [o_dot(j + reds[n], b, st, lambda b=b: pack16(outs[n][b]), lref)
                    for b in range(3) if b not in kept(n)]

        def wq_of(n):
            nq = j + qn[n]
            return q_dots(nq if isinstance(nq, int) else jnp.minimum(nq, NP - 1), st, qs[qn[n] % 2])

        if last:
            dots += late_dots(st)[:NLATE] + x_dots(NP - 1, 0, xrows[0], parked(NP - 1, S_PA), lref)

            def park_acc(G, a4):
                for n in range(4):
                    ku[(NP - 1) * GP + 2, _vr(2 * (G - 16) + n), :] = pltpu.bitcast(a4[n], u32)
            hooks["end", 0] = park_acc
        for n, k in enumerate(ks if not last else []):
            q = qs[(k + 1) % 2]
            dots += k_dots(j + (k + 1), 0, st, q, MIX if n else MIXA, NALT if n else 0)
            if n == 0:
                if xrows[1]:
                    hooks["after", len(dots)] = b_segs[3]
                dots += x_dots(j + ks[0], 1, xrows[1], lambda T: pack16(pb[T]), q)
            else:
                direct(j + k, 1, 48 * n + BD_SEG, q)
            kb = k_dots(j + (k + 1), 1, st, q, MIX)
            if n < len(ks) - 1:
                dots += kb[:XA_AT]
                direct(j + (k + 1), 0, 48 * n + AD_SEG, q)
                dots += kb[XA_AT:] + wq_of(n) + wo_of(n)
            else:
                hooks["need", 48 * n + a_seg] = len(dots)
                tail_hooks(j + (k + 1), st, hooks, 48 * n + a_seg)
                dots += kb
                hook(("dot", len(dots)), lambda k=k: stash_b(j + (k + 1), st["s", 1]))
                for m in range(n, len(qn)):
                    dots += wq_of(m)
                for m in range(n, len(reds)):
                    dots += wo_of(m)
                dots += x_dots(j + ks[0], 0, xrows[0],
                               parked(j + ks[0], S_PA), lref)
        run_block([j + k for k in ks], xrows, dots, hooks,
                  PLANS[name], range(NSPLIT) if last else None)
        if last:
            keep()
        if reds:
            abuf[...] += st["acc"]

    def body2(n, carry):
        block("body", 2 * n, [2, 3], [0, 1], [5, 6], XROWS)
        return carry

    lax.fori_loop(0, NP // 2 - 2, body2, 0)
    pl.when(zs[0] == 0)(lambda: block("third", 0, [NP - 2], [NP - 4, NP - 3], [], XROWS))
    pl.when(zs[0] <= 0)(lambda: block("last", 0, [NP - 1], [NP - 2], [], XROWS_LAST))

    new_block()
    st = {"acc": abuf[...]}
    invb = get_state(NP - 1, S_LB)
    o = reduce_o([ku[(NP - 1) * GP + b] for b in range(2)], get_state(NP - 1, S_INVA), invb,
                 (get_state(NP - 1, S_X), None))
    part = [None] * 5

    def finish(G, a4):
        for k in range(4):
            tick(lref, L_DUMMY + k, a4[k])
        z = lref[_vr(5), :]
        project(G, [pltpu.bitcast(v, u32) | z for v in a4])

    def project(G, a4):
        for n in range(4):
            v = jnp.sum(pltpu.bitcast(a4[n], f32), axis=1, keepdims=True)
            for nt in range(5):
                w = wou[(NP - 1) * (GP // 2) + G + n // 2, nt]
                t = pltpu.bitcast(w & jnp.uint32(HI) if n % 2 else w << 16, f32) * v
                part[nt] = t if part[nt] is None else part[nt] + t

    for G in range(16, NSPLIT // 2, 2):
        project(G, [ku[(NP - 1) * GP + 2, _vr(2 * (G - 16) + n), :] for n in range(4)])
    dots = late_dots(st)[NLATE:] + [o_dot(NP - 1, b, st, lambda b=b: pack16(o[b]), lref)
                                    for b in range(2)]
    run_block([NP - 1], XROWS_LAST, dots, {("end", 0): finish},
              PLANS["final"], range(NSPLIT, 48))
    x = row_sum(st["acc"] + jnp.concatenate([v * invb for v in part], axis=1))

    xl = _rows16(x, ones)
    d = xl[0:8].astype(f32) - mean
    md = _mean(d)
    r1 = lax.rsqrt(jnp.maximum(_mean(d * d) - md * md, 0.0) + EPS)
    mean = mean + md
    y = (d - md) * r1
    my = _mean(y)
    r2 = lax.rsqrt(jnp.maximum(_mean(y * y) - my * my, 0.0) + EPS)
    h = jnp.dot(xl, w3[...], preferred_element_type=f32)
    h = h[0:8] * (r1 * r2) - h[8:16] * ((mean * r1 + my) * r2)
    h = jax.nn.gelu(h, approximate=True).astype(bf16)
    x = x + y
    parts = []
    for k in range(0, W4_VPU, 128):
        hk = jnp.broadcast_to(h[0:1, k:k + 128].astype(f32), (128, 128)).T
        t = w4[k:k + 128, :].astype(f32) * jnp.concatenate([hk] * 5, axis=1)
        parts.append(jnp.sum(t.reshape(16, 8, D), axis=0))
    for k in range(W4_VPU, F, 128):
        if k == W4_AT:
            x = x + row_sum(sum(parts[1:], parts[0]))
        x = x + jnp.dot(h[:, k:k + 128], w4[k:k + 128, :], preferred_element_type=f32)
    o_ref[...] = x[0:1].astype(o_ref.dtype)


def _cache_view(c):
    s = c.shape[2]
    c = jnp.transpose(c, (0, 1, 3, 2)).reshape(H * DH // 8, 8, s // 128, 128)
    return jnp.transpose(c, (0, 2, 1, 3)).reshape(H * DH // 8, s // 128 * 8, 128)


def _weight_view(w):
    k, n = w.shape
    w = jnp.transpose(w.reshape(k // 16, 2, 8, n // 128, 128), (0, 1, 3, 2, 4))
    return w.reshape(k // 16, n // 128, 16, 128)


@jax.jit
def pallas_interleave_layers__sliding_block_cached__mixer_s_mlp__decode_kernel(
    A_x: jax.Array,
    A_k_cache: jax.Array,
    A_v_cache: jax.Array,
    A_wq: jax.Array,
    A_wo: jax.Array,
    B_x: jax.Array,
    B_w1: jax.Array,
    B_w2: jax.Array,
    B_w3: jax.Array,
    B_w4: jax.Array,
):
    sk = A_k_cache.shape[2]
    win = min(4096, max(256, sk // 4))
    assert win == 4096 and sk % 128 == 0
    assert A_x.shape == (1, 1, D) and A_k_cache.shape == (1, H, sk, DH)
    wt = win // 128
    t0 = sk // 128 - wt
    ng = H * DH // 8
    hbm = pl.BlockSpec(memory_space=pl.ANY)
    out = pl.pallas_call(
        functools.partial(_kernel, t0=t0, wt=wt),
        out_shape=jax.ShapeDtypeStruct((1, D), A_x.dtype),
        in_specs=[hbm] * 7,
        out_specs=pl.BlockSpec(memory_space=pltpu.VMEM),
        scratch_shapes=[
            pltpu.VMEM((ng, wt * 8, 128), bf16),
            pltpu.VMEM((ng, wt * 8, 128), bf16),
            pltpu.VMEM((ng // 4, 128, 128), u32),
            pltpu.VMEM((NP * D // 16, 3, 8, 128), u32),
            pltpu.VMEM((H * DH // 16, D // 128, 16, 128), bf16),
            pltpu.VMEM((D, F), bf16),
            pltpu.VMEM((F, D), bf16),
            pltpu.VMEM((1, D), bf16),
            pltpu.VMEM((144, 128), u32),
            pltpu.VMEM((384, 128), u32),
            pltpu.VMEM((144, 128), u32),
            pltpu.VMEM((144, 128), u32),
            pltpu.VMEM((144, 128), u32),
            pltpu.VMEM((40, 128), f32),
            pltpu.VMEM((8, D), f32),
            pltpu.SMEM((1,), jnp.int32),
        ] + [pltpu.VMEM((64, 128), u32)] * 3
        + [pltpu.VMEM((72, 128), f32)] * 8,
        compiler_params=pltpu.CompilerParams(vmem_limit_bytes=128 * 1024 * 1024),
    )(A_x.reshape(1, D), _cache_view(A_k_cache), _cache_view(A_v_cache),
      _weight_view(A_wq).reshape(H * DH // 16, D // 128, 16, 128), _weight_view(A_wo), B_w3, B_w4)
    return out.reshape(1, 1, D)
```

```python
import functools

import jax
import jax.numpy as jnp
from jax import lax
import jax.experimental.pallas as pl
import jax.experimental.pallas.tpu as pltpu

D = 640
H = 32
DH = 192
F = 1536
EPS = 1e-5
NP = H // 2
GP = 2 * DH // 8
HI = 0xFFFF0000
CEXP = DH ** -0.5 * 1.4426950408889634

f32 = jnp.float32
bf16 = jnp.bfloat16
u32 = jnp.uint32

L_Y = 0
L_DUMMY = 6
S_MAXB, S_LB, S_INVA, S_X, S_PA, S_PB = 4, 5, 6, 7, 9, 13
XROWS = ((2, 10, 18, 26), (4, 12, 20))
XROWS_LAST = ((2, 10, 18, 26, 6, 14, 22, 30, 4, 12, 20, 28), ())
GX = (0, 16)
PLANS = {
    "first": (
        {},
        (21, 23, 23, 23, 24, 25, 27, 27, 27, 28, 29, 29, 30, 31, 30, 31, 32, 32, 33, 34, 34, 35,
        36, 36, 37, 38, 38, 39, 40, 40, 41, 42, 43, 43, 44, 44, 45, 46, 46, 47, 48, 48, 49, 49,
        50, 51, 51, 52, 52, 52, 53, 54, 54, 56, 56, 56, 57, 58, 58, 59, 60, 60, 61, 62, 62, 63,
        64, 64, 65, 66, 66, 67, 68, 68, 69, 70, 70, 71, 72, 72, 73, 74, 74, 75, 76, 76, 77, 78,
        78, 79, 80, 81, 82, 82, 83, 82)),
    "body": (
        {1: 0, 3: 2, 5: 4, 7: 4, 9: 5, 11: 8, 12: 10, 15: 13, 19: 14, 21: 14, 23: 16, 25: 17,
        27: 19, 29: 22, 31: 23, 33: 23, 35: 26, 37: 26, 39: 28, 40: 33, 41: 33, 43: 34, 45: 34,
        47: 34, 49: 35, 51: 37, 53: 38, 55: 39, 57: 40, 59: 42, 61: 43, 63: 48, 67: 50, 70: 51,
        71: 52, 72: 53, 75: 55, 77: 56, 79: 58, 81: 59, 83: 61, 84: 62},
        (0, 0, 0, 0, 0, 0, 0, 0, 0, 0, 0, 1, 2, 2, 3, 4, 4, 5, 6, 7, 7, 8, 9, 10, 10, 12, 12,
        13, 14, 15, 15, 16, 16, 17, 17, 18, 20, 21, 21, 24, 24, 24, 22, 23, 26, 29, 25, 25, 24,
        27, 28, 30, 30, 31, 32, 32, 33, 34, 35, 36, 36, 34, 35, 37, 37, 39, 43, 42, 41, 39, 44,
        45, 46, 48, 48, 47, 48, 49, 49, 50, 51, 49, 51, 52, 54, 56, 56, 58, 57, 59, 61, 59, 61,
        61, 63, 64)),
    "third": (
        {1: 0, 3: 3, 6: 3, 7: 4, 9: 5, 11: 8, 15: 10, 19: 14, 21: 14, 23: 15, 25: 17, 26: 19,
        27: 19, 30: 21},
        (0, 0, 0, 0, 0, 0, 0, 0, 0, 0, 1, 0, 0, 3, 3, 5, 3, 5, 4, 8, 8, 9, 11, 11, 10, 12, 12,
        12, 15, 17, 15, 16, 17, 17, 18, 19, 20, 18, 21, 22, 22, 24, 25, 26, 25, 24, 25, 26)),
    "last": (
        {1: 0, 3: 1, 7: 2, 11: 3, 15: 4, 17: 6, 19: 7, 21: 10, 23: 11, 27: 13},
        (0, 0, 0, 0, 0, 0, 0, 0, 0, 0, 0, 0, 0, 0, 0, 0, 1, 1, 2, 3, 4, 6, 6, 6, 7, 7, 8, 6, 8,
        9, 9, 10, 10, 11, 11, 11)),
    "final": (
        {37: 0, 39: 1, 40: 4, 43: 4, 45: 6},
        (0, 0, 0, 0, 0, 0, 0, 0, 0, 0, 0, 0, 0, 0, 0, 0, 0, 0, 0, 0, 0, 0, 0, 0, 0, 0, 0, 0, 0,
        0, 0, 0, 0, 0, 0, 0, 0, 0, 0, 0, 0, 0, 6, 3, 1, 2, 0, 0)),
}
MIX = (0, 1, 8, 2, 3, 9, 4, 5, 10, 6, 7, 11)
MIXA = (0, 1, 2, 3, 4, 8, 5, 9, 6, 10, 7, 11)
NLATE = 12
NSPLIT = 36
W4_VPU = 256
W4_AT = 896
B_SEGS = (9, 12, 15, 18)
B_SEGL = 8
DA0 = 16
NOTICK = 3
DW0 = 32
DB0 = 44
DA1 = 56
DB1 = 67
DQ = (26, 29, 33)
NQV = 3
B0_SEG = 17
A1_SEG = 39
B1_SEG = 12
A2_SEG = 40
A_SEG0 = 40
A_SEG3 = 38
B_SEGS3 = (9, 11, 15, 19)
XA_AT = 8
AD_SEG = 32
BD_SEG = 12
NALT = 2
W4_CHUNKS = (1024, 256, 160, 64, 32)
W4_MXU = 1280


def _mean(x):
    return jnp.mean(x, axis=-1, keepdims=True)


def _ln(x):
    c = x - _mean(x)
    return c * lax.rsqrt(_mean(c * c) + EPS)


def _wtile(wu, rows, nt):
    blk = wu[rows, nt]
    return pltpu.bitcast(blk.reshape(blk.shape[0] * 8, 128), bf16)


def _wcols(wu, rows, nts):
    return jnp.concatenate([_wtile(wu, rows, n) for n in nts], axis=1)


def _rows16(a, b):
    return jnp.concatenate([a, b], axis=0).astype(bf16)


def _slot(G, t):
    j = 4 * (t >> 3) + ((((t >> 1) & 3) + G + 2 * (t & 1) + (t >> 3)) & 3)
    return 2 * G + (t & 1), 8 * j


def _xslot(G, t):
    return G // 2, 8 * (4 * (t >> 3) + ((((t >> 1) & 3) + G + (t >> 3)) & 3))


def _vr(n):
    return slice(8 * n, 8 * n + 8)


def _kernel(*refs, t0, wt):
    pl.run_scoped(functools.partial(_body, refs, t0, wt),
                  pltpu.SemaphoreType.DMA((4 + len(W4_CHUNKS) + 2 * NP,)))


def _body(refs, t0, wt, sems):
    (x_hbm, k_hbm, v_hbm, wq_hbm, wo_hbm, w3_hbm, w4_hbm, o_ref,
     kbuf, vbuf, vx, wqu, wo, w3, w4, xbuf, lref, obuf, qa, qb, qx, scl, abuf, zs) = refs[:24]
    qt, pT = refs[24:27], refs[27:]
    ku = kbuf.bitcast(u32)
    vu = vbuf.bitcast(u32)
    wou = wo.bitcast(u32)

    x_cp = pltpu.make_async_copy(x_hbm, xbuf, sems.at[0])
    wq_cp = pltpu.make_async_copy(wq_hbm, wo, sems.at[1])
    wo_cp = pltpu.make_async_copy(wo_hbm, wo, sems.at[2])
    w3_cp = pltpu.make_async_copy(w3_hbm, w3, sems.at[3])
    w4_rows, r0 = [], 0
    for n in W4_CHUNKS:
        w4_rows.append((r0, r0 + n))
        r0 += n
    w4_cp = [pltpu.make_async_copy(w4_hbm.at[a:b], w4.at[a:b], sems.at[4 + c])
             for c, (a, b) in enumerate(w4_rows)]
    S0 = 4 + len(W4_CHUNKS)

    def k_cp(i):
        return pltpu.make_async_copy(
            k_hbm.at[pl.ds(i * GP, GP), pl.ds(t0 * 8, wt * 8), :],
            kbuf.at[pl.ds(i * GP, GP)], sems.at[S0 + i])

    def v_cp(i):
        return pltpu.make_async_copy(
            v_hbm.at[pl.ds(i * GP, GP), pl.ds(t0 * 8, wt * 8), :],
            vbuf.at[pl.ds(i * GP, GP)], sems.at[S0 + NP + i])

    for c in (wq_cp, x_cp, k_cp(0), v_cp(0)):
        c.start()

    zs[0] = 0
    for ref in (qa, qb, qx, lref):
        ref[_vr(5), :] = jnp.zeros((8, 128), u32)

    lane = lax.broadcasted_iota(jnp.int32, (8, 128), 1)
    sub = lax.broadcasted_iota(jnp.int32, (8, 128), 0)
    lane_lo = lane < 64
    sub_lo = sub < 4

    def pair_view(buf, i):
        return buf.at[pl.ds(i * GP, GP)].bitcast(u32)

    def tile(ref, g0, G, t):
        g, r = _slot(G, t)
        return ref[g0 + g, r:r + 8, :]

    def retile(ref, i, expand):
        def body(c, carry):
            g0 = 8 * c
            for G in range(4):
                for J in range(4):
                    xs = [[ref[g0 + 2 * G + e, _vr(4 * J + jj), :] for jj in range(4)]
                          for e in range(2)]
                    for jj in range(4):
                        x0, x1 = xs[0][jj], xs[1][jj]
                        ys = (jnp.where(sub_lo, x0, pltpu.roll(x1, 4, 0)),
                              jnp.where(sub_lo, pltpu.roll(x0, 4, 0), x1))
                        for e in range(2):
                            t = 8 * J + 2 * jj + e
                            g, r = _slot(G, t)
                            if expand and G % 2 and e:
                                ref[g0 + g, r:r + 8, :] = ys[e] << 16
                                g, r = _xslot(G, t)
                                vx[i * (GP // 4) + 2 * c + g, r:r + 8, :] = ys[e] & jnp.uint32(HI)
                            else:
                                ref[g0 + g, r:r + 8, :] = ys[e]
            return carry
        lax.fori_loop(0, GP // 8, body, 0)

    def merge_halves(get, nt, n):
        lo, hi = get(n // 2), get((nt + n) // 2)
        if n % 2:
            lo = pltpu.roll(lo, 4, 0)
        if (nt + n) % 2 == 0:
            hi = pltpu.roll(hi, 4, 0)
        return jnp.where(sub_lo, lo, hi)

    def retile_wq(c, carry):
        for G in range(5):
            for n in range(3 * NP):
                wqu[n // 3 * (D // 16) + 5 * c + G, n % 3] = merge_halves(
                    lambda v: wou[48 * c + (48 * G + v) // 5, (48 * G + v) % 5], 3 * NP, n)
        return carry

    def retile_wo(c, carry):
        for G in range(8):
            xs = [wou[8 * c + G, n] for n in range(5)]
            for n in range(5):
                wou[8 * c + G, n] = merge_halves(lambda v: xs[v], 5, n)
        return carry

    def lhs_at(ref, n):
        return pltpu.bitcast(ref[_vr(n), :], bf16)

    cur = [None]

    def new_block():
        cur[0] = -32 * jnp.clip(zs[0], 0, 1)

    def tick(ref, n, val):
        if val.dtype != ref.dtype:
            val = pltpu.bitcast(val, ref.dtype)
        ref[pl.ds(pl.multiple_of(cur[0] + 8 * n, 8), 8), :] = val

    def put_q(q, qref):
        qq = pltpu.bitcast(q.astype(bf16).astype(f32), u32)
        q0, q1, q2 = qq[:, 0:128], qq[:, 128:256], qq[:, 256:384]
        for n, v in enumerate((q0 >> 16, q0, q2 >> 16, q2, q1)):
            qref[_vr(n), :] = v
            if n < 2 and qref is qb:
                qx[_vr(n), :] = v

    def transpose_wq(i):
        for k in range(5):
            for n in range(3):
                rows = pl.ds(i * (D // 16) + 8 * k, 8)
                w = pltpu.bitcast(_wtile(wqu, rows, n).astype(f32).T, u32)
                for G in range(8):
                    wqu[i * (D // 16) + 8 * k + G, n] = (w[_vr(2 * G), :] >> 16) | w[_vr(2 * G + 1), :]

    def q_vpu(i, c, qref):
        cols = []
        for n in range(3):
            acc = []
            for G in range(8):
                ws = [wqu[i * (D // 16) + 8 * k + G, n] for k in range(5)]
                for half in (lambda w: w << 16, lambda w: w & jnp.uint32(HI)):
                    t = [pltpu.bitcast(half(ws[k]), f32) * col(c, k) for k in range(5)]
                    acc.append((t[0] + t[1]) + (t[2] + t[3]) + t[4])
            z = jnp.sum(jnp.concatenate(acc, axis=0).T.reshape(16, 8, 128), axis=0)
            cols.append(row_sum(z))
        put_q(jnp.concatenate(cols, axis=1), qref)
        return cols[0] + cols[1] + cols[2]

    def row_sum(a):
        return jnp.broadcast_to(jnp.sum(a, axis=0, keepdims=True), a.shape)

    def q_dots(i, st, qref, lhs=None, mean=None):
        def step(k):
            def run(tied=False):
                w = _wcols(wqu, pl.ds(i * (D // 16) + 8 * k, 8), range(3))
                if lhs is None:
                    r = jnp.dot(lhs_at(lref, L_Y + k), w, preferred_element_type=f32)[0:8]
                else:
                    r = jnp.dot(lhs[:, 128 * k:128 * k + 128], w, preferred_element_type=f32)
                st["q"] = r if k == 0 else st["q"] + r
                if k == 4:
                    q = st["q"] if lhs is None else st["q"][0:8] - mean * st["q"][8:16]
                    put_q(q, qref)
                return r[0:8, 256:384]
            return 3, lref, L_DUMMY, run
        return [step(k) for k in range(5)]

    def as_lhs(v, tref):
        if v.dtype == f32 and tref is None:
            return v.astype(bf16)
        if v.dtype == f32:
            v = pltpu.bitcast(_rows16(v, v), u32)
        return pltpu.bitcast(v if tref is None else v | tref[_vr(5), :], bf16)

    def o_dot(i, b, st, get_lhs, tref=None):
        def run(tied=False):
            w = _wcols(wou, pl.ds(i * (GP // 2) + 8 * b, 8), range(5))
            lhs = as_lhs(get_lhs(), tref if tied and tref is not obuf else None)
            r = jnp.dot(lhs, w, preferred_element_type=f32)[0:8]
            st["acc"] = st["acc"] + r if "acc" in st else r
            return r[:, 512:640]
        return 5, tref, (32 if tref is obuf else 6), run

    def mid_q(st, qref):
        q1 = qref[_vr(4), :]
        q1r = pltpu.roll(q1, 64, 1)
        st["u", 0, id(qref)] = jnp.where(lane_lo, q1 >> 16, q1r)
        st["u", 1, id(qref)] = jnp.where(lane_lo, q1r >> 16, q1)

    def k_dots(i, hh, st, qref, order=tuple(range(12)), nalt=0, ku=ku):
        g0 = i * GP
        gf, gh = ((0, 8), (16, 12))[hh]

        def step(r):
            src = qx if r in order[:nalt] else qref

            def run(tied=False):
                if r < 8:
                    cols = [[tile(ku, g0, gf + G, 8 * T + r) for G in range(8)] for T in range(4)]
                    base, row = src[_vr(2 * hh + r % 2), :], r // 2
                else:
                    cols = [[tile(ku, g0, gh + G % 4, 8 * T + 2 * (r - 8) + G // 4)
                             for G in range(8)] for T in range(4)]
                    if ("u", hh, id(qref)) not in st:
                        mid_q(st, qref)
                    base, row = st["u", hh, id(qref)], r - 8
                    if tied:
                        base = base | src[_vr(5), :]
                lhs = jnp.where(sub == row, base, jnp.zeros((8, 128), u32))
                w = jnp.concatenate([jnp.concatenate(c, axis=0) for c in cols], axis=1)
                res = jnp.dot(pltpu.bitcast(lhs, bf16), pltpu.bitcast(w, bf16),
                              preferred_element_type=f32)[0:8]
                st["s", hh] = res if r == order[0] else st["s", hh] + res
                return res[:, 384:512]
            return 4, src, 6, run
        return [step(r) for r in order]

    def col(s, T):
        return s[:, 128 * T:128 * T + 128]

    def row_max(s):
        m = jnp.maximum(jnp.maximum(col(s, 0), col(s, 1)), jnp.maximum(col(s, 2), col(s, 3)))
        return jnp.max(jnp.max(m, axis=1, keepdims=True), axis=0, keepdims=True)

    def prob(s, m):
        return jnp.exp2((s - m) * scl[_vr(0), :])

    def put_p(hh, T, p, ks=range(8)):
        for k in ks:
            pT[4 * hh + T][pl.ds(k, 8, stride=8), :] = p

    def part_sum(p):
        return (p[0] + p[1]) + (p[2] + p[3])

    def inv_sum(l):
        l = jnp.sum(jnp.sum(l, axis=1, keepdims=True), axis=0, keepdims=True)
        r = pl.reciprocal(l, approx=True)
        return jnp.broadcast_to(r * (2.0 - l * r), (8, 128))

    def softmax(s, hh):
        m = row_max(s)
        p = [prob(col(s, T), m) for T in range(4)]
        for T in range(4):
            put_p(hh, T, p[T])
        return p, part_sum(p)

    def get_state(i, n):
        return pltpu.bitcast(ku[i * GP + 3, _vr(n), :], f32)

    def set_state(i, n, v):
        ku[i * GP + 3, _vr(n), :] = pltpu.bitcast(v, u32)

    def stash_b(i, s):
        for T in range(4):
            set_state(i, T, col(s, T))
        m = jnp.broadcast_to(row_max(s), (8, 128))
        set_state(i, S_MAXB, m)
        return m

    def pack8(v):
        return pltpu.bitcast(v.astype(bf16), u32)

    def park_p(i, n, p):
        ku[i * GP + 3, 8 * n:8 * n + 4, :] = pack8(p)

    def parked(i, n):
        return lambda T: ku[i * GP + 3, _vr(n + T), :]

    def x_dots(i, hh, ts, get_lhs, tref=None):
        st = {}
        rows = sorted({t % 8 for t in ts})

        def step(n, rho):
            def run(tied=False):
                res = []
                for T in [t // 8 for t in ts if t % 8 == rho]:
                    w = jnp.concatenate(
                        [tile(vu, i * GP, GX[hh] + G, 8 * T + rho) for G in range(8)], axis=0)
                    lhs = as_lhs(get_lhs(T), tref if tied else None)
                    res.append(jnp.dot(lhs, pltpu.bitcast(w, bf16),
                                       preferred_element_type=f32)[0:8])
                st["x"] = jnp.where(sub == rho, sum(res[1:], res[0]), st["x"] if n else 0.0)
                if n == len(rows) - 1:
                    set_state(i, S_X + hh, st["x"])
                return res[-1]
            return sum(1 for t in ts if t % 8 == rho), tref, 6, run
        return [step(n, rho) for n, rho in enumerate(rows)]

    def transpose_x(view, xrows):
        for hh in range(2):
            for t in xrows[hh]:
                w = jnp.concatenate([tile(view, 0, GX[hh] + G, t) for G in range(8)], axis=0)
                w = pltpu.bitcast(pltpu.bitcast(w, bf16).astype(f32).T.astype(bf16), u32)
                for G in range(8):
                    g, r = _slot(GX[hh] + G, t)
                    view[g, r:r + 8, :] = w[_vr(G), :]

    def reduce_o(blocks, inva, invb, extra=(None, None, None)):
        out = []
        for b, inv in enumerate((inva, jnp.where(lane_lo, inva, invb), invb)[:len(blocks)]):
            z = jnp.sum(pltpu.bitcast(blocks[b], f32).T.reshape(16, 8, 128), axis=0)
            if extra[b] is not None:
                z = z + extra[b]
            out.append(z * inv)
        return out

    def mac(acc, n, c, G, t, pv, view=None):
        w = tile(vu, 8 * c, G, t) if view is None else tile(view[0], view[1], G, t)
        if G % 2 and t % 2:
            g, r = _xslot(G, t)
            halves = (w, vx[2 * c + g, r:r + 8, :])
        else:
            halves = (w << 16, w & jnp.uint32(HI))
        for k in range(2):
            a = pltpu.bitcast(halves[k], f32) * pv
            acc[n + k] = a if acc[n + k] is None else acc[n + k] + a

    def seg_rows(xrows, seg):
        hh, gp, T = seg // 24 % 2, seg % 24 // 4, seg % 4
        on_mxu = GX[hh] <= 12 * hh + 2 * gp < GX[hh] + 8
        return [rho for rho in range(8) if not (on_mxu and 8 * T + rho in xrows[hh])]

    def run_block(pairs, xrows, dots, hooks, plan, segs=None):
        tie, clk = plan
        clock = []

        def emit(upto):
            while len(clock) < upto:
                n = len(clock)
                for h in hooks.get(("dot", n), ()):
                    h()
                clock.append(dots[n][3](n in tie.values()))

        zero = jnp.zeros((8, 128), f32)
        used = {}
        for seg in segs or range(48 * len(pairs)):
            i, hh, gp, T = pairs[seg // 48], seg // 24 % 2, seg % 24 // 4, seg % 4
            if T == 0:
                a4 = [None] * 4
            pref = pT[4 * hh + T]
            upto = min([v for k, v in tie.items() if k >= seg]
                       + [k[1] for k, v in hooks.items() if k[0] == "after" and v >= seg]
                       + [len(dots) if tie else clk[seg] + 6])
            free = not any(k in tie for k in range(seg, seg - T + 4))
            if free or ("seg", seg) in hooks:
                upto = max(upto, clk[seg] + 1)
            emit(min(len(dots), max(upto, hooks.get(("need", seg), 0))))
            if seg < hooks.get(("notick", 0), 0):
                pass
            elif free:
                tick(pref, 8, clock[clk[seg]])
            elif gp:
                tick(pref, 8, zero)
            for h in hooks.get(("seg", seg), ()):
                h(clock[clk[seg]])
            for rho in seg_rows(xrows, seg):
                pv = pref[_vr(rho), :]
                for e in range(2):
                    mac(a4, 2 * e, i * 6, 12 * hh + 2 * gp + e, 8 * T + rho, pv)
            if seg in tie:
                ref, slot = dots[tie[seg]][1:3]
                used[tie[seg]] = used.get(tie[seg], -1) + 1
                for k in range(4):
                    tick(ref, slot + 4 * used[tie[seg]] + k, a4[k])
            if T == 3 and ("end", 0) in hooks and seg >= 32:
                hooks["end", 0](12 * hh + 2 * gp, a4)
            elif T == 3:
                for n in range(4):
                    G = 12 * hh + 2 * gp + n // 2
                    v = a4[n] * hooks["scale", seg // 24]() if ("scale", seg // 24) in hooks else a4[n]
                    ku[i * GP + G // 8, pl.ds(16 * (G % 8) + n % 2, 8, stride=2), :] = (
                        pltpu.bitcast(v, u32))
        emit(len(dots))

    def run_all(dots):
        for d in dots:
            d[3]()

    def set_input(c, scale):
        cp = pltpu.bitcast(_rows16(c, c), u32)
        for k in range(5):
            lref[_vr(L_Y + k), :] = cp[:, 128 * k:128 * k + 128]
        scl[_vr(0), :] = jnp.broadcast_to(scale, (8, 128))

    x_cp.wait()
    x = jnp.broadcast_to(xbuf[...].astype(f32), (8, D))
    set_input(_ln(x), jnp.full((8, 1), CEXP, f32))
    wq_cp.wait()
    lax.fori_loop(0, D // 80, retile_wq, 0)
    wo_cp.start()
    for i in range(1, NP):
        k_cp(i).start()
        v_cp(i).start()
    for c in [w3_cp] + w4_cp:
        c.start()
    wo_cp.wait()
    lax.fori_loop(0, H * DH // 128, retile_wo, 0)

    def body1(i, acc):
        st = {"acc": acc}
        k_cp(i).wait()
        kv = pair_view(kbuf, i)
        retile(kv, i, False)
        run_all(q_dots(i, st, qa))
        inv = []
        for hh in range(2):
            run_all(k_dots(0, hh, st, qa, ku=kv))
            inv.append(inv_sum(softmax(st["s", hh], hh)[1]))

        @pl.when(i > 0)
        def _():
            transpose_x(pair_view(vbuf, i - 1), XROWS)

        @pl.when(jnp.logical_and(i >= 5 - NQV, i < 5))
        def _():
            transpose_wq(i)

        v_cp(i).wait()
        vv = pair_view(vbuf, i)
        retile(vv, i, True)
        for hh in range(2):
            def pv_step(c, carry, hh=hh):
                acc8 = [None] * 8
                for t in range(32):
                    pv = pT[4 * hh + t // 8][_vr(t % 8), :]
                    for G in range(4):
                        mac(acc8, 2 * G, i * 6 + c, G, t, pv, (vv, 8 * c))
                for n in range(8):
                    obuf[pl.ds(64 * c + 16 * (n // 2) + n % 2, 8, stride=2), :] = (
                        pltpu.bitcast(acc8[n], u32))
                return carry
            lax.fori_loop(3 * hh, 3 * hh + 3, pv_step, 0)
        o = reduce_o([obuf[128 * b:128 * b + 128, :] for b in range(3)], inv[0], inv[1])
        run_all([o_dot(i, b, st, lambda b=b: o[b]) for b in range(3)])
        return st["acc"]

    x = x + row_sum(lax.fori_loop(0, NP, body1, jnp.zeros((8, D), f32)))

    y = _ln(x)
    zz = _ln(y).astype(bf16)
    w3_cp.wait()
    h = jnp.dot(zz, w3[...], preferred_element_type=f32)
    h = jax.nn.gelu(h, approximate=True).astype(bf16)
    x = x + y
    transpose_x(pair_view(vbuf, NP - 1), XROWS_LAST)
    for k in range(W4_MXU, F, 128):
        hk = jnp.broadcast_to(h[0:1, k:k + 128].astype(f32), (128, 128))
        obuf[k - W4_MXU:k - W4_MXU + 128, :] = pltpu.bitcast(hk.T, u32)
    part = jnp.zeros((8, D), f32)
    for cp, (a, b) in zip(w4_cp, w4_rows):
        cp.wait()
        if a < W4_MXU:
            x = x + jnp.dot(h[:, a:b], w4[a:b, :], preferred_element_type=f32)
        else:
            for k in range(a, b, 16):
                hk = pltpu.bitcast(obuf[k - W4_MXU:k - W4_MXU + 16, :], f32)
                t = w4[k:k + 16, :].astype(f32) * jnp.concatenate([hk] * 5, axis=1)
                part = part + (t[0:8] + t[8:16])
    x = x + row_sum(part)

    ones = jnp.ones((8, D), f32)
    xl = _rows16(x, ones)
    xb = xl[0:8].astype(f32)
    mean = _mean(xb)
    c = xb - mean
    set_input(c, lax.rsqrt(_mean(c * c) + EPS) * CEXP)
    abuf[...] = jnp.where(lax.broadcasted_iota(jnp.int32, (8, D), 0) == 0, x, 0.0)

    def tail_hooks(i, st, hooks, seg0):
        def first(_):
            m = row_max(st["s", 0])
            st["pa"] = [prob(col(st["s", 0], T), m) for T in range(4)]
            set_state(i, S_INVA, inv_sum(part_sum(st["pa"])))
            for T in range(4):
                park_p(i, S_PA + T, st["pa"][T])

        def put(T, half):
            def run(clk):
                tick(pT[T], 8, clk)
                put_p(0, T, st["pa"][T], range(4 * half, 4 * half + 4))
            return run
        hooks.setdefault(("seg", seg0), []).append(first)
        for n in range(8):
            hooks.setdefault(("seg", seg0 + n), []).append(put(n // 2, n % 2))

    def head_b_hooks(i, segs, pb, final=False, park=False):
        def put_b(T):
            def run(clk):
                tick(scl, 4, clk)
                pb.append(prob(get_state(i, T), get_state(i, S_MAXB)))
                put_p(1, T, pb[T])
                if park and T < 3:
                    park_p(i, S_PB + T, pb[T])
                if T == 3:
                    set_state(i, S_LB, inv_sum(part_sum(pb)) if final else part_sum(pb))
            return run
        return {("seg", segs[T]): [put_b(T)] for T in range(4)}

    def reduce_pair(i):
        xa, xb = get_state(i, S_X), get_state(i, S_X + 1)
        invb = inv_sum(get_state(i, S_LB))
        return reduce_o([ku[i * GP + b] for b in range(3)],
                        get_state(i, S_INVA), invb, (xa, None, xb))

    st = {}
    new_block()
    late = tuple(range(8, 12)) + tuple(range(8))
    q0, q1, q2 = qt
    dots = q_dots(0, st, q0, xl, mean) + q_dots(1, st, q1, xl, mean) \
        + k_dots(0, 0, st, q0) + k_dots(0, 1, st, q0, late) + k_dots(1, 0, st, q1, late) \
        + k_dots(1, 1, st, q1, late) + k_dots(2, 0, st, q2, late) + k_dots(2, 1, st, q2)
    for n in range(4):
        dots += x_dots(n // 2, n % 2, XROWS[n % 2], parked(n // 2, (S_PA, S_PB)[n % 2]))

    def lane_softmax(h, first=False):
        i, hh = h // 2, h % 2

        def run():
            s0 = st["s", hh]
            m = jnp.maximum(jnp.maximum(col(s0, 0), col(s0, 1)),
                            jnp.maximum(col(s0, 2), col(s0, 3)))
            m = jnp.max(m, axis=0, keepdims=True)
            p = st["p", h] = [prob(col(s0, T), m) for T in range(4)]
            if first:
                for T in range(4):
                    for rho in range(8):
                        pT[T][_vr(rho), :] = jnp.broadcast_to(p[T][rho:rho + 1], (8, 128))
            w = st["w", h] = prob(m, jnp.max(m, axis=1, keepdims=True))
            l = part_sum(p) * w
            set_state(i, (S_INVA, S_LB)[hh], l if hh else inv_sum(l))
            for T in range(4 - hh):
                park_p(i, (S_PA, S_PB)[hh] + T, p[T] * w)
        return run

    def put_lane(h, T):
        def run(clk):
            tick(pT[4 * (h % 2) + T], 8, clk)
            put_p(h % 2, T, st["p", h][T])
        return run

    hooks = head_b_hooks(1, range(48 + B1_SEG, 96, 3), [], park=True)
    hooks.update({("need", 0): 23, ("need", B0_SEG): 35, ("need", A1_SEG): 47,
                  ("need", 48 + B1_SEG): DB1 + 1, ("need", 48 + A2_SEG): 70,
                  ("after", 82): 48 + B1_SEG + 9})
    for n, fn in ((10, lambda: mid_q(st, q0)),
                  (DQ[0], lambda: tick(q0, 5, q_vpu(2, c, q2))),
                  (DQ[1], lambda: tick(q0, 5, q_vpu(3, c, qa))),
                  (DQ[2], lambda: tick(q0, 5, q_vpu(4, c, qb))),
                  (DA0, lambda: tick(q0, 6, scl[_vr(0), :])), (22, lane_softmax(0, True)),
                   (DW0, lambda: tick(q0, 7, st["w", 0])),
                  (34, lane_softmax(1)), (DB0, lambda: tick(q1, 6, st["w", 1])),
                  (46, lane_softmax(2)), (DA1, lambda: tick(q1, 6, st["w", 2])),
                  (DB1, lambda: tick(q2, 6, stash_b(1, st["s", 1]))),
                  (82, lambda: stash_b(2, st["s", 1]))):
        hooks.setdefault(("dot", n), []).append(fn)
    for h in range(3):
        hooks["scale", h] = lambda h=h: st["w", h]
    hooks["notick", 0] = NOTICK
    hooks.update({("seg", B0_SEG + 2 * T): [put_lane(1, T)] for T in range(4)})
    hooks.update({("seg", A1_SEG + 2 * T): [put_lane(2, T)] for T in range(4)})
    tail_hooks(2, st, hooks, 48 + A2_SEG)
    run_block([0, 1], XROWS, dots, hooks, PLANS["first"])

    qs = (qb, qa)

    def late_dots(st):
        todo = [(m, 2) for m in range(NP - 2)] + [(NP - 3, 1)] + [(NP - 2, b) for b in range(3)]
        return [o_dot(m, b, st, lambda n=m + (2 - b) * 6: obuf[_vr(n), :], obuf) for m, b in todo]

    def block(name, j, ks, reds, qn, xrows):
        last = ks == [NP - 1]
        a_seg = A_SEG3 if name == "third" else A_SEG0
        b_segs = {"third": B_SEGS3,
                  "last": range(B_SEGL, 48, 3)}.get(name, B_SEGS)
        new_block()
        st = {}
        for k in ks if not last else []:
            mid_q(st, qs[(k + 1) % 2])
        outs = [reduce_pair(j + r) for r in reds]

        def kept(n):
            return (0, 1, 2) if last else (1, 2) if reds[n] == NP - 3 else (2,)

        def keep():
            for n, r in enumerate(reds):
                for b in kept(n):
                    obuf[pl.ds(pl.multiple_of(8 * (j + r + (2 - b) * 6), 8), 4), :] = (
                        pack8(outs[n][b]))

        if not last:
            keep()
        pb = []
        hooks = head_b_hooks(j + ks[0], b_segs, pb, last)
        dots = []

        def hook(key, fn):
            hooks.setdefault(key, []).append(fn)

        def direct(i, hh, seg0, tref):
            p = []

            def run():
                m = row_max(st["s", hh])
                p.extend(prob(col(st["s", hh], T), m) for T in range(4))
                l = part_sum(p)
                set_state(i, (S_INVA, S_LB)[hh], l if hh else inv_sum(l))

            def put(T, half):
                def go(clk):
                    tick(pT[4 * hh + T], 8, clk)
                    put_p(hh, T, p[T], range(4 * half, 4 * half + 4))
                return go
            hook(("dot", len(dots)), run)
            dots.extend(x_dots(i, hh, xrows[hh], lambda T: p[T], tref))
            hooks["need", seg0] = len(dots)
            for n in range(8):
                hook(("seg", seg0 + n), put(n // 2, n % 2))

        def wo_of(n):
            return [o_dot(j + reds[n], b, st, lambda b=b: outs[n][b], lref)
                    for b in range(3) if b not in kept(n)]

        def wq_of(n):
            nq = j + qn[n]
            return q_dots(nq if isinstance(nq, int) else jnp.minimum(nq, NP - 1), st, qs[qn[n] % 2])

        if last:
            dots += late_dots(st)[:NLATE] + x_dots(NP - 1, 0, xrows[0], parked(NP - 1, S_PA), lref)

            def park_acc(G, a4):
                for n in range(4):
                    ku[(NP - 1) * GP + 2, _vr(2 * (G - 16) + n), :] = pltpu.bitcast(a4[n], u32)
            hooks["end", 0] = park_acc
        for n, k in enumerate(ks if not last else []):
            q = qs[(k + 1) % 2]
            dots += k_dots(j + (k + 1), 0, st, q, MIX if n else MIXA, NALT if n else 0)
            if n == 0:
                if xrows[1]:
                    hooks["after", len(dots)] = b_segs[3]
                dots += x_dots(j + ks[0], 1, xrows[1], lambda T: pb[T], q)
            else:
                direct(j + k, 1, 48 * n + BD_SEG, q)
            kb = k_dots(j + (k + 1), 1, st, q, MIX)
            if n < len(ks) - 1:
                dots += kb[:XA_AT]
                direct(j + (k + 1), 0, 48 * n + AD_SEG, q)
                dots += kb[XA_AT:] + wq_of(n) + wo_of(n)
            else:
                hooks["need", 48 * n + a_seg] = len(dots)
                tail_hooks(j + (k + 1), st, hooks, 48 * n + a_seg)
                dots += kb
                hook(("dot", len(dots)), lambda k=k: stash_b(j + (k + 1), st["s", 1]))
                for m in range(n, len(qn)):
                    dots += wq_of(m)
                for m in range(n, len(reds)):
                    dots += wo_of(m)
                dots += x_dots(j + ks[0], 0, xrows[0],
                               parked(j + ks[0], S_PA), lref)
        run_block([j + k for k in ks], xrows, dots, hooks,
                  PLANS[name], range(NSPLIT) if last else None)
        if last:
            keep()
        if reds:
            abuf[...] += st["acc"]

    def body2(n, carry):
        block("body", 2 * n, [2, 3], [0, 1], [5, 6], XROWS)
        return carry

    zero = zs[0]
    lax.fori_loop(0, NP // 2 - 2, body2, 0)
    pl.when(zero == 0)(lambda: block("third", 0, [NP - 2], [NP - 4, NP - 3], [], XROWS))
    pl.when(zero <= 0)(lambda: block("last", 0, [NP - 1], [NP - 2], [], XROWS_LAST))

    new_block()
    st = {"acc": abuf[...]}
    invb = get_state(NP - 1, S_LB)
    o = reduce_o([ku[(NP - 1) * GP + b] for b in range(2)], get_state(NP - 1, S_INVA), invb,
                 (get_state(NP - 1, S_X), None))
    part = [None] * 5

    def finish(G, a4):
        for k in range(4):
            tick(lref, L_DUMMY + k, a4[k])
        z = lref[_vr(5), :]
        project(G, [pltpu.bitcast(v, u32) | z for v in a4])

    def project(G, a4):
        for n in range(4):
            v = jnp.sum(pltpu.bitcast(a4[n], f32), axis=1, keepdims=True)
            for nt in range(5):
                w = wou[(NP - 1) * (GP // 2) + G + n // 2, nt]
                t = pltpu.bitcast(w & jnp.uint32(HI) if n % 2 else w << 16, f32) * v
                part[nt] = t if part[nt] is None else part[nt] + t

    for G in range(16, NSPLIT // 2, 2):
        project(G, [ku[(NP - 1) * GP + 2, _vr(2 * (G - 16) + n), :] for n in range(4)])
    dots = late_dots(st)[NLATE:] + [o_dot(NP - 1, b, st, lambda b=b: o[b], lref)
                                    for b in range(2)]
    run_block([NP - 1], XROWS_LAST, dots, {("end", 0): finish},
              PLANS["final"], range(NSPLIT, 48))
    x = row_sum(st["acc"] + jnp.concatenate([v * invb for v in part], axis=1))

    xl = _rows16(x, ones)
    d = xl[0:8].astype(f32) - mean
    md = _mean(d)
    r1 = lax.rsqrt(jnp.maximum(_mean(d * d) - md * md, 0.0) + EPS)
    mean = mean + md
    y = (d - md) * r1
    my = _mean(y)
    r2 = lax.rsqrt(jnp.maximum(_mean(y * y) - my * my, 0.0) + EPS)
    h = jnp.dot(xl, w3[...], preferred_element_type=f32)
    h = h[0:8] * (r1 * r2) - h[8:16] * ((mean * r1 + my) * r2)
    h = jax.nn.gelu(h, approximate=True).astype(bf16)
    x = x + y
    parts = []
    for k in range(0, W4_VPU, 128):
        hk = jnp.broadcast_to(h[0:1, k:k + 128].astype(f32), (128, 128)).T
        t = w4[k:k + 128, :].astype(f32) * jnp.concatenate([hk] * 5, axis=1)
        parts.append(jnp.sum(t.reshape(16, 8, D), axis=0))
    for k in range(W4_VPU, F, 128):
        if k == W4_AT:
            x = x + row_sum(sum(parts[1:], parts[0]))
        x = x + jnp.dot(h[:, k:k + 128], w4[k:k + 128, :], preferred_element_type=f32)
    o_ref[...] = x[0:1].astype(o_ref.dtype)


def _cache_view(c):
    s = c.shape[2]
    c = jnp.transpose(c, (0, 1, 3, 2)).reshape(H * DH // 8, 8, s // 128, 128)
    return jnp.transpose(c, (0, 2, 1, 3)).reshape(H * DH // 8, s // 128 * 8, 128)


def _weight_view(w):
    k, n = w.shape
    w = jnp.transpose(w.reshape(k // 16, 2, 8, n // 128, 128), (0, 1, 3, 2, 4))
    return w.reshape(k // 16, n // 128, 16, 128)


@jax.jit
def pallas_interleave_layers__sliding_block_cached__mixer_s_mlp__decode_kernel(
    A_x: jax.Array,
    A_k_cache: jax.Array,
    A_v_cache: jax.Array,
    A_wq: jax.Array,
    A_wo: jax.Array,
    B_x: jax.Array,
    B_w1: jax.Array,
    B_w2: jax.Array,
    B_w3: jax.Array,
    B_w4: jax.Array,
):
    sk = A_k_cache.shape[2]
    win = min(4096, max(256, sk // 4))
    assert win == 4096 and sk % 128 == 0
    assert A_x.shape == (1, 1, D) and A_k_cache.shape == (1, H, sk, DH)
    wt = win // 128
    t0 = sk // 128 - wt
    ng = H * DH // 8
    hbm = pl.BlockSpec(memory_space=pl.ANY)
    out = pl.pallas_call(
        functools.partial(_kernel, t0=t0, wt=wt),
        out_shape=jax.ShapeDtypeStruct((1, D), A_x.dtype),
        in_specs=[hbm] * 7,
        out_specs=pl.BlockSpec(memory_space=pltpu.VMEM),
        scratch_shapes=[
            pltpu.VMEM((ng, wt * 8, 128), bf16),
            pltpu.VMEM((ng, wt * 8, 128), bf16),
            pltpu.VMEM((ng // 4, 128, 128), u32),
            pltpu.VMEM((NP * D // 16, 3, 8, 128), u32),
            pltpu.VMEM((H * DH // 16, D // 128, 16, 128), bf16),
            pltpu.VMEM((D, F), bf16),
            pltpu.VMEM((F, D), bf16),
            pltpu.VMEM((1, D), bf16),
            pltpu.VMEM((144, 128), u32),
            pltpu.VMEM((384, 128), u32),
            pltpu.VMEM((144, 128), u32),
            pltpu.VMEM((144, 128), u32),
            pltpu.VMEM((144, 128), u32),
            pltpu.VMEM((40, 128), f32),
            pltpu.VMEM((8, D), f32),
            pltpu.SMEM((1,), jnp.int32),
        ] + [pltpu.VMEM((64, 128), u32)] * 3
        + [pltpu.VMEM((72, 128), f32)] * 8,
        compiler_params=pltpu.CompilerParams(vmem_limit_bytes=128 * 1024 * 1024),
    )(A_x.reshape(1, D), _cache_view(A_k_cache), _cache_view(A_v_cache),
      _weight_view(A_wq).reshape(H * DH // 16, D // 128, 16, 128), _weight_view(A_wo), B_w3, B_w4)
    return out.reshape(1, 1, D)
```

```python
import functools

import jax
import jax.numpy as jnp
from jax import lax
import jax.experimental.pallas as pl
import jax.experimental.pallas.tpu as pltpu

D = 640
H = 32
DH = 192
F = 1536
EPS = 1e-5
NP = H // 2
GP = 2 * DH // 8
HI = 0xFFFF0000
CEXP = DH ** -0.5 * 1.4426950408889634

f32 = jnp.float32
bf16 = jnp.bfloat16
u32 = jnp.uint32

L_Y = 0
L_DUMMY = 6
S_MAXB, S_LB, S_INVA, S_X, S_PA, S_PB = 4, 5, 6, 7, 9, 13
XROWS = ((2, 10, 18, 26), (4, 12, 20))
XROWS_LAST = ((2, 10, 18, 26, 6, 14, 22, 30, 4, 12, 20, 28), ())
GX = (0, 16)
PLANS = {
    "first": (
        {},
        (21, 22, 22, 23, 24, 23, 26, 27, 26, 27, 28, 28, 29, 29, 30, 31, 32, 31, 33, 34, 34, 35,
        36, 36, 37, 38, 38, 39, 40, 40, 41, 42, 42, 43, 44, 44, 45, 46, 46, 47, 48, 48, 49, 49,
        50, 51, 51, 53, 51, 52, 54, 55, 54, 55, 56, 56, 57, 58, 58, 59, 60, 59, 60, 62, 62, 63,
        64, 64, 65, 66, 66, 67, 68, 68, 69, 70, 70, 71, 72, 71, 73, 74, 74, 75, 76, 73, 77, 78,
        77, 79, 80, 81, 82, 82, 82, 76)),
    "body": (
        {1: 0, 3: 2, 5: 4, 7: 4, 9: 5, 11: 8, 14: 10, 15: 13, 19: 14, 21: 14, 23: 16, 25: 17,
        27: 19, 29: 22, 31: 23, 33: 23, 35: 26, 37: 26, 39: 28, 40: 33, 41: 33, 43: 34, 47: 34,
        49: 35, 51: 37, 53: 38, 55: 39, 57: 40, 59: 42, 61: 43, 63: 48, 67: 50, 70: 51, 71: 52,
        72: 53, 75: 55, 77: 56, 79: 58, 81: 59, 83: 61, 84: 62},
        (0, 0, 0, 0, 0, 0, 0, 0, 0, 0, 0, 1, 2, 2, 3, 4, 4, 5, 6, 7, 7, 8, 9, 10, 10, 12, 12,
        13, 14, 15, 15, 16, 16, 17, 17, 18, 20, 21, 21, 24, 24, 24, 21, 22, 26, 30, 24, 25, 23,
        26, 27, 29, 29, 30, 31, 31, 33, 34, 35, 36, 36, 34, 34, 37, 37, 39, 43, 42, 40, 37, 41,
        41, 43, 46, 46, 45, 46, 47, 47, 49, 50, 51, 50, 51, 52, 57, 56, 58, 57, 59, 61, 60, 62,
        62, 63, 63)),
    "third": (
        {1: 0, 3: 3, 6: 3, 7: 4, 9: 5, 11: 8, 15: 10, 19: 14, 21: 14, 23: 15, 25: 17, 26: 19,
        27: 19, 30: 21},
        (0, 0, 0, 0, 0, 0, 0, 0, 0, 0, 1, 0, 0, 3, 3, 5, 3, 5, 4, 8, 8, 9, 11, 11, 10, 12, 12,
        12, 15, 17, 15, 16, 17, 17, 18, 19, 20, 18, 21, 22, 22, 24, 25, 26, 25, 24, 25, 26)),
    "last": (
        {1: 0, 3: 1, 7: 2, 11: 3, 15: 4, 17: 6, 19: 7, 21: 10, 23: 11, 27: 13},
        (0, 0, 0, 0, 0, 0, 0, 0, 0, 0, 0, 0, 0, 0, 0, 0, 1, 1, 2, 3, 4, 6, 6, 6, 7, 7, 8, 6, 8,
        9, 9, 10, 10, 11, 11, 11)),
    "final": (
        {37: 0, 39: 1, 40: 4, 43: 4, 45: 6},
        (0, 0, 0, 0, 0, 0, 0, 0, 0, 0, 0, 0, 0, 0, 0, 0, 0, 0, 0, 0, 0, 0, 0, 0, 0, 0, 0, 0, 0,
        0, 0, 0, 0, 0, 0, 0, 0, 0, 0, 0, 0, 0, 6, 3, 1, 2, 0, 0)),
}
MIX = (0, 1, 8, 2, 3, 9, 4, 5, 10, 6, 7, 11)
MIXA = (0, 1, 2, 3, 4, 8, 5, 9, 6, 10, 7, 11)
NLATE = 12
NSPLIT = 36
W4_VPU = 256
W4_AT = 896
B_SEGS = (9, 12, 15, 18)
B_SEGL = 8
DA0 = 17
DW0 = 32
DB0 = 44
DA1 = 55
DB1 = 67
DQ = (26, 29, 33)
NQV = 3
B0_SEG = 20
A1_SEG = 39
B1_SEG = 12
A2_SEG = 36
A_SEG0 = 40
A_SEG3 = 38
B_SEGS3 = (9, 11, 15, 19)
XA_AT = 8
AD_SEG = 32
BD_SEG = 12
NALT = 2
W4_CHUNKS = (1024, 256, 160, 64, 32)
W4_MXU = 1280


def _mean(x):
    return jnp.mean(x, axis=-1, keepdims=True)


def _ln(x):
    c = x - _mean(x)
    return c * lax.rsqrt(_mean(c * c) + EPS)


def _wtile(wu, rows, nt):
    blk = wu[rows, nt]
    return pltpu.bitcast(blk.reshape(blk.shape[0] * 8, 128), bf16)


def _wcols(wu, rows, nts):
    return jnp.concatenate([_wtile(wu, rows, n) for n in nts], axis=1)


def _rows16(a, b):
    return jnp.concatenate([a, b], axis=0).astype(bf16)


def _slot(G, t):
    j = 4 * (t >> 3) + ((((t >> 1) & 3) + G + 2 * (t & 1) + (t >> 3)) & 3)
    return 2 * G + (t & 1), 8 * j


def _xslot(G, t):
    return G // 2, 8 * (4 * (t >> 3) + ((((t >> 1) & 3) + G + (t >> 3)) & 3))


def _vr(n):
    return slice(8 * n, 8 * n + 8)


def _kernel(*refs, t0, wt):
    pl.run_scoped(functools.partial(_body, refs, t0, wt),
                  pltpu.SemaphoreType.DMA((4 + len(W4_CHUNKS) + 2 * NP,)))


def _body(refs, t0, wt, sems):
    (x_hbm, k_hbm, v_hbm, wq_hbm, wo_hbm, w3_hbm, w4_hbm, o_ref,
     kbuf, vbuf, vx, wqu, wo, w3, w4, xbuf, lref, obuf, qa, qb, qx, scl, abuf, zs) = refs[:24]
    qt, pT = refs[24:27], refs[27:]
    ku = kbuf.bitcast(u32)
    vu = vbuf.bitcast(u32)
    wou = wo.bitcast(u32)

    x_cp = pltpu.make_async_copy(x_hbm, xbuf, sems.at[0])
    wq_cp = pltpu.make_async_copy(wq_hbm, wo, sems.at[1])
    wo_cp = pltpu.make_async_copy(wo_hbm, wo, sems.at[2])
    w3_cp = pltpu.make_async_copy(w3_hbm, w3, sems.at[3])
    w4_rows, r0 = [], 0
    for n in W4_CHUNKS:
        w4_rows.append((r0, r0 + n))
        r0 += n
    w4_cp = [pltpu.make_async_copy(w4_hbm.at[a:b], w4.at[a:b], sems.at[4 + c])
             for c, (a, b) in enumerate(w4_rows)]
    S0 = 4 + len(W4_CHUNKS)

    def k_cp(i):
        return pltpu.make_async_copy(
            k_hbm.at[pl.ds(i * GP, GP), pl.ds(t0 * 8, wt * 8), :],
            kbuf.at[pl.ds(i * GP, GP)], sems.at[S0 + i])

    def v_cp(i):
        return pltpu.make_async_copy(
            v_hbm.at[pl.ds(i * GP, GP), pl.ds(t0 * 8, wt * 8), :],
            vbuf.at[pl.ds(i * GP, GP)], sems.at[S0 + NP + i])

    for c in (wq_cp, x_cp, k_cp(0), v_cp(0)):
        c.start()

    zs[0] = 0
    for ref in (qa, qb, qx, lref):
        ref[_vr(5), :] = jnp.zeros((8, 128), u32)

    lane = lax.broadcasted_iota(jnp.int32, (8, 128), 1)
    sub = lax.broadcasted_iota(jnp.int32, (8, 128), 0)
    lane_lo = lane < 64
    sub_lo = sub < 4

    def pair_view(buf, i):
        return buf.at[pl.ds(i * GP, GP)].bitcast(u32)

    def tile(ref, g0, G, t):
        g, r = _slot(G, t)
        return ref[g0 + g, r:r + 8, :]

    def retile(ref, i, expand):
        def body(c, carry):
            g0 = 8 * c
            for G in range(4):
                for J in range(4):
                    xs = [[ref[g0 + 2 * G + e, _vr(4 * J + jj), :] for jj in range(4)]
                          for e in range(2)]
                    for jj in range(4):
                        x0, x1 = xs[0][jj], xs[1][jj]
                        ys = (jnp.where(sub_lo, x0, pltpu.roll(x1, 4, 0)),
                              jnp.where(sub_lo, pltpu.roll(x0, 4, 0), x1))
                        for e in range(2):
                            t = 8 * J + 2 * jj + e
                            g, r = _slot(G, t)
                            if expand and G % 2 and e:
                                ref[g0 + g, r:r + 8, :] = ys[e] << 16
                                g, r = _xslot(G, t)
                                vx[i * (GP // 4) + 2 * c + g, r:r + 8, :] = ys[e] & jnp.uint32(HI)
                            else:
                                ref[g0 + g, r:r + 8, :] = ys[e]
            return carry
        lax.fori_loop(0, GP // 8, body, 0)

    def merge_halves(get, nt, n):
        lo, hi = get(n // 2), get((nt + n) // 2)
        if n % 2:
            lo = pltpu.roll(lo, 4, 0)
        if (nt + n) % 2 == 0:
            hi = pltpu.roll(hi, 4, 0)
        return jnp.where(sub_lo, lo, hi)

    def retile_wq(c, carry):
        for G in range(5):
            for n in range(3 * NP):
                wqu[n // 3 * (D // 16) + 5 * c + G, n % 3] = merge_halves(
                    lambda v: wou[48 * c + (48 * G + v) // 5, (48 * G + v) % 5], 3 * NP, n)
        return carry

    def retile_wo(c, carry):
        for G in range(8):
            xs = [wou[8 * c + G, n] for n in range(5)]
            for n in range(5):
                wou[8 * c + G, n] = merge_halves(lambda v: xs[v], 5, n)
        return carry

    def lhs_at(ref, n):
        return pltpu.bitcast(ref[_vr(n), :], bf16)

    cur = [None]

    def new_block():
        cur[0] = -32 * jnp.clip(zs[0], 0, 1)

    def tick(ref, n, val):
        assert 4 <= n < ref.shape[0] // 8
        if val.dtype != ref.dtype:
            val = pltpu.bitcast(val, ref.dtype)
        ref[pl.ds(pl.multiple_of(cur[0] + 8 * n, 8), 8), :] = val

    def put_q(q, qref):
        qq = pltpu.bitcast(q.astype(bf16).astype(f32), u32)
        q0, q1, q2 = qq[:, 0:128], qq[:, 128:256], qq[:, 256:384]
        for n, v in enumerate((q0 >> 16, q0, q2 >> 16, q2, q1)):
            qref[_vr(n), :] = v
            if n < 2 and qref is qb:
                qx[_vr(n), :] = v

    def transpose_wq(i):
        for k in range(5):
            for n in range(3):
                rows = pl.ds(i * (D // 16) + 8 * k, 8)
                w = pltpu.bitcast(_wtile(wqu, rows, n).astype(f32).T, u32)
                for G in range(8):
                    wqu[i * (D // 16) + 8 * k + G, n] = (w[_vr(2 * G), :] >> 16) | w[_vr(2 * G + 1), :]

    def q_vpu(i, c, qref):
        cols = []
        for n in range(3):
            acc = []
            for G in range(8):
                ws = [wqu[i * (D // 16) + 8 * k + G, n] for k in range(5)]
                for half in (lambda w: w << 16, lambda w: w & jnp.uint32(HI)):
                    t = [pltpu.bitcast(half(ws[k]), f32) * col(c, k) for k in range(5)]
                    acc.append((t[0] + t[1]) + (t[2] + t[3]) + t[4])
            z = jnp.sum(jnp.concatenate(acc, axis=0).T.reshape(16, 8, 128), axis=0)
            cols.append(row_sum(z))
        put_q(jnp.concatenate(cols, axis=1), qref)
        return cols[0] + cols[1] + cols[2]

    def row_sum(a):
        return jnp.broadcast_to(jnp.sum(a, axis=0, keepdims=True), a.shape)

    def q_dots(i, st, qref, lhs=None, mean=None):
        def step(k):
            def run(tied=False):
                w = _wcols(wqu, pl.ds(i * (D // 16) + 8 * k, 8), range(3))
                if lhs is None:
                    r = jnp.dot(lhs_at(lref, L_Y + k), w, preferred_element_type=f32)[0:8]
                else:
                    r = jnp.dot(lhs[:, 128 * k:128 * k + 128], w, preferred_element_type=f32)
                st["q"] = r if k == 0 else st["q"] + r
                if k == 4:
                    q = st["q"] if lhs is None else st["q"][0:8] - mean * st["q"][8:16]
                    put_q(q, qref)
                return r[0:8, 256:384]
            return 3, lref, L_DUMMY, run
        return [step(k) for k in range(5)]

    def as_lhs(v, tref):
        if v.dtype == f32 and tref is None:
            return v.astype(bf16)
        if v.dtype == f32:
            v = pltpu.bitcast(_rows16(v, v), u32)
        return pltpu.bitcast(v if tref is None else v | tref[_vr(5), :], bf16)

    def o_dot(i, b, st, get_lhs, tref=None):
        def run(tied=False):
            w = _wcols(wou, pl.ds(i * (GP // 2) + 8 * b, 8), range(5))
            lhs = as_lhs(get_lhs(), tref if tied and tref is not obuf else None)
            r = jnp.dot(lhs, w, preferred_element_type=f32)[0:8]
            st["acc"] = st["acc"] + r if "acc" in st else r
            return r[:, 512:640]
        return 5, tref, (32 if tref is obuf else 6), run

    def mid_q(st, qref):
        q1 = qref[_vr(4), :]
        q1r = pltpu.roll(q1, 64, 1)
        st["u", 0, id(qref)] = jnp.where(lane_lo, q1 >> 16, q1r)
        st["u", 1, id(qref)] = jnp.where(lane_lo, q1r >> 16, q1)

    def k_dots(i, hh, st, qref, order=tuple(range(12)), nalt=0, ku=ku):
        g0 = i * GP
        gf, gh = ((0, 8), (16, 12))[hh]

        def step(r):
            src = qx if r in order[:nalt] else qref

            def run(tied=False):
                if r < 8:
                    cols = [[tile(ku, g0, gf + G, 8 * T + r) for G in range(8)] for T in range(4)]
                    base, row = src[_vr(2 * hh + r % 2), :], r // 2
                else:
                    cols = [[tile(ku, g0, gh + G % 4, 8 * T + 2 * (r - 8) + G // 4)
                             for G in range(8)] for T in range(4)]
                    if ("u", hh, id(qref)) not in st:
                        mid_q(st, qref)
                    base, row = st["u", hh, id(qref)], r - 8
                    if tied:
                        base = base | src[_vr(5), :]
                lhs = jnp.where(sub == row, base, jnp.zeros((8, 128), u32))
                w = jnp.concatenate([jnp.concatenate(c, axis=0) for c in cols], axis=1)
                res = jnp.dot(pltpu.bitcast(lhs, bf16), pltpu.bitcast(w, bf16),
                              preferred_element_type=f32)[0:8]
                st["s", hh] = res if r == order[0] else st["s", hh] + res
                return res[:, 384:512]
            return 4, src, 6, run
        return [step(r) for r in order]

    def col(s, T):
        return s[:, 128 * T:128 * T + 128]

    def row_max(s):
        m = jnp.maximum(jnp.maximum(col(s, 0), col(s, 1)), jnp.maximum(col(s, 2), col(s, 3)))
        return jnp.max(jnp.max(m, axis=1, keepdims=True), axis=0, keepdims=True)

    def prob(s, m):
        return jnp.exp2((s - m) * scl[_vr(0), :])

    def put_p(hh, T, p, ks=range(8)):
        for k in ks:
            pT[4 * hh + T][pl.ds(k, 8, stride=8), :] = p

    def part_sum(p):
        return (p[0] + p[1]) + (p[2] + p[3])

    def inv_sum(l):
        l = jnp.sum(jnp.sum(l, axis=1, keepdims=True), axis=0, keepdims=True)
        r = pl.reciprocal(l, approx=True)
        return jnp.broadcast_to(r * (2.0 - l * r), (8, 128))

    def softmax(s, hh):
        m = row_max(s)
        p = [prob(col(s, T), m) for T in range(4)]
        for T in range(4):
            put_p(hh, T, p[T])
        return p, part_sum(p)

    def get_state(i, n):
        return pltpu.bitcast(ku[i * GP + 3, _vr(n), :], f32)

    def set_state(i, n, v):
        ku[i * GP + 3, _vr(n), :] = pltpu.bitcast(v, u32)

    def stash_b(i, s):
        for T in range(4):
            set_state(i, T, col(s, T))
        m = jnp.broadcast_to(row_max(s), (8, 128))
        set_state(i, S_MAXB, m)
        return m

    def pack8(v):
        return pltpu.bitcast(v.astype(bf16), u32)

    def park_p(i, n, p):
        ku[i * GP + 3, 8 * n:8 * n + 4, :] = pack8(p)

    def parked(i, n):
        return lambda T: ku[i * GP + 3, _vr(n + T), :]

    def x_dots(i, hh, ts, get_lhs, tref=None):
        st = {}
        rows = sorted({t % 8 for t in ts})

        def step(n, rho):
            def run(tied=False):
                res = []
                for T in [t // 8 for t in ts if t % 8 == rho]:
                    w = jnp.concatenate(
                        [tile(vu, i * GP, GX[hh] + G, 8 * T + rho) for G in range(8)], axis=0)
                    lhs = as_lhs(get_lhs(T), tref if tied else None)
                    res.append(jnp.dot(lhs, pltpu.bitcast(w, bf16),
                                       preferred_element_type=f32)[0:8])
                st["x"] = jnp.where(sub == rho, sum(res[1:], res[0]), st["x"] if n else 0.0)
                if n == len(rows) - 1:
                    set_state(i, S_X + hh, st["x"])
                return res[-1]
            return sum(1 for t in ts if t % 8 == rho), tref, 6, run
        return [step(n, rho) for n, rho in enumerate(rows)]

    def transpose_x(view, xrows):
        for hh in range(2):
            for t in xrows[hh]:
                w = jnp.concatenate([tile(view, 0, GX[hh] + G, t) for G in range(8)], axis=0)
                w = pltpu.bitcast(pltpu.bitcast(w, bf16).astype(f32).T.astype(bf16), u32)
                for G in range(8):
                    g, r = _slot(GX[hh] + G, t)
                    view[g, r:r + 8, :] = w[_vr(G), :]

    def reduce_o(blocks, inva, invb, extra=(None, None, None)):
        out = []
        for b, inv in enumerate((inva, jnp.where(lane_lo, inva, invb), invb)[:len(blocks)]):
            z = jnp.sum(pltpu.bitcast(blocks[b], f32).T.reshape(16, 8, 128), axis=0)
            if extra[b] is not None:
                z = z + extra[b]
            out.append(z * inv)
        return out

    def mac(acc, n, c, G, t, pv, view=None):
        w = tile(vu, 8 * c, G, t) if view is None else tile(view[0], view[1], G, t)
        if G % 2 and t % 2:
            g, r = _xslot(G, t)
            halves = (w, vx[2 * c + g, r:r + 8, :])
        else:
            halves = (w << 16, w & jnp.uint32(HI))
        for k in range(2):
            a = pltpu.bitcast(halves[k], f32) * pv
            acc[n + k] = a if acc[n + k] is None else acc[n + k] + a

    def seg_rows(xrows, seg):
        hh, gp, T = seg // 24 % 2, seg % 24 // 4, seg % 4
        on_mxu = GX[hh] <= 12 * hh + 2 * gp < GX[hh] + 8
        return [rho for rho in range(8) if not (on_mxu and 8 * T + rho in xrows[hh])]

    def run_block(pairs, xrows, dots, hooks, plan, segs=None):
        tie, clk = plan
        clock = []

        def emit(upto):
            while len(clock) < upto:
                n = len(clock)
                for h in hooks.get(("dot", n), ()):
                    h()
                clock.append(dots[n][3](n in tie.values()))

        zero = jnp.zeros((8, 128), f32)
        used = {}
        for seg in segs or range(48 * len(pairs)):
            i, hh, gp, T = pairs[seg // 48], seg // 24 % 2, seg % 24 // 4, seg % 4
            if T == 0:
                a4 = [None] * 4
            pref = pT[4 * hh + T]
            upto = min([v for k, v in tie.items() if k >= seg]
                       + [k[1] for k, v in hooks.items() if k[0] == "after" and v >= seg]
                       + [len(dots) if tie else clk[seg] + 6])
            free = not any(k in tie for k in range(seg, seg - T + 4))
            if free or ("seg", seg) in hooks:
                upto = max(upto, clk[seg] + 1)
            emit(min(len(dots), max(upto, hooks.get(("need", seg), 0))))
            if free:
                tick(pref, 8, clock[clk[seg]])
            elif gp:
                tick(pref, 8, zero)
            for h in hooks.get(("seg", seg), ()):
                h(clock[clk[seg]])
            for rho in seg_rows(xrows, seg):
                pv = pref[_vr(rho), :]
                for e in range(2):
                    mac(a4, 2 * e, i * 6, 12 * hh + 2 * gp + e, 8 * T + rho, pv)
            if seg in tie:
                ref, slot = dots[tie[seg]][1:3]
                used[tie[seg]] = used.get(tie[seg], -1) + 1
                for k in range(4):
                    tick(ref, slot + 4 * used[tie[seg]] + k, a4[k])
            if T == 3 and ("end", 0) in hooks and seg >= 32:
                hooks["end", 0](12 * hh + 2 * gp, a4)
            elif T == 3:
                for n in range(4):
                    G = 12 * hh + 2 * gp + n // 2
                    v = a4[n] * hooks["scale", seg // 24]() if ("scale", seg // 24) in hooks else a4[n]
                    ku[i * GP + G // 8, pl.ds(16 * (G % 8) + n % 2, 8, stride=2), :] = (
                        pltpu.bitcast(v, u32))
        emit(len(dots))

    def run_all(dots):
        for d in dots:
            d[3]()

    def set_input(c, scale):
        cp = pltpu.bitcast(_rows16(c, c), u32)
        for k in range(5):
            lref[_vr(L_Y + k), :] = cp[:, 128 * k:128 * k + 128]
        scl[_vr(0), :] = jnp.broadcast_to(scale, (8, 128))

    x_cp.wait()
    x = jnp.broadcast_to(xbuf[...].astype(f32), (8, D))
    set_input(_ln(x), jnp.full((8, 1), CEXP, f32))
    wq_cp.wait()
    lax.fori_loop(0, D // 80, retile_wq, 0)
    wo_cp.start()
    for i in range(1, NP):
        k_cp(i).start()
        v_cp(i).start()
    for c in [w3_cp] + w4_cp:
        c.start()
    wo_cp.wait()
    lax.fori_loop(0, H * DH // 128, retile_wo, 0)

    def body1(i, acc):
        st = {"acc": acc}
        k_cp(i).wait()
        kv = pair_view(kbuf, i)
        retile(kv, i, False)
        run_all(q_dots(i, st, qa))
        inv = []
        for hh in range(2):
            run_all(k_dots(0, hh, st, qa, ku=kv))
            inv.append(inv_sum(softmax(st["s", hh], hh)[1]))

        @pl.when(i > 0)
        def _():
            transpose_x(pair_view(vbuf, i - 1), XROWS)

        @pl.when(jnp.logical_and(i >= 5 - NQV, i < 5))
        def _():
            transpose_wq(i)

        v_cp(i).wait()
        vv = pair_view(vbuf, i)
        retile(vv, i, True)
        for hh in range(2):
            def pv_step(c, carry, hh=hh):
                acc8 = [None] * 8
                for t in range(32):
                    pv = pT[4 * hh + t // 8][_vr(t % 8), :]
                    for G in range(4):
                        mac(acc8, 2 * G, i * 6 + c, G, t, pv, (vv, 8 * c))
                for n in range(8):
                    obuf[pl.ds(64 * c + 16 * (n // 2) + n % 2, 8, stride=2), :] = (
                        pltpu.bitcast(acc8[n], u32))
                return carry
            lax.fori_loop(3 * hh, 3 * hh + 3, pv_step, 0)
        o = reduce_o([obuf[128 * b:128 * b + 128, :] for b in range(3)], inv[0], inv[1])
        run_all([o_dot(i, b, st, lambda b=b: o[b]) for b in range(3)])
        return st["acc"]

    x = x + row_sum(lax.fori_loop(0, NP, body1, jnp.zeros((8, D), f32)))

    y = _ln(x)
    zz = _ln(y).astype(bf16)
    w3_cp.wait()
    h = jnp.dot(zz, w3[...], preferred_element_type=f32)
    h = jax.nn.gelu(h, approximate=True).astype(bf16)
    x = x + y
    transpose_x(pair_view(vbuf, NP - 1), XROWS_LAST)
    for k in range(W4_MXU, F, 128):
        hk = jnp.broadcast_to(h[0:1, k:k + 128].astype(f32), (128, 128))
        obuf[k - W4_MXU:k - W4_MXU + 128, :] = pltpu.bitcast(hk.T, u32)
    part = jnp.zeros((8, D), f32)
    for cp, (a, b) in zip(w4_cp, w4_rows):
        cp.wait()
        if a < W4_MXU:
            x = x + jnp.dot(h[:, a:b], w4[a:b, :], preferred_element_type=f32)
        else:
            for k in range(a, b, 16):
                hk = pltpu.bitcast(obuf[k - W4_MXU:k - W4_MXU + 16, :], f32)
                t = w4[k:k + 16, :].astype(f32) * jnp.concatenate([hk] * 5, axis=1)
                part = part + (t[0:8] + t[8:16])
    x = x + row_sum(part)

    ones = jnp.ones((8, D), f32)
    xl = _rows16(x, ones)
    xb = xl[0:8].astype(f32)
    mean = _mean(xb)
    c = xb - mean
    set_input(c, lax.rsqrt(_mean(c * c) + EPS) * CEXP)
    abuf[...] = jnp.where(lax.broadcasted_iota(jnp.int32, (8, D), 0) == 0, x, 0.0)

    def tail_hooks(i, st, hooks, seg0):
        def first(_):
            m = row_max(st["s", 0])
            st["pa"] = [prob(col(st["s", 0], T), m) for T in range(4)]
            set_state(i, S_INVA, inv_sum(part_sum(st["pa"])))
            for T in range(4):
                park_p(i, S_PA + T, st["pa"][T])

        def put(T, half):
            def run(clk):
                tick(pT[T], 8, clk)
                put_p(0, T, st["pa"][T], range(4 * half, 4 * half + 4))
            return run
        hooks.setdefault(("seg", seg0), []).append(first)
        for n in range(8):
            hooks.setdefault(("seg", seg0 + n), []).append(put(n // 2, n % 2))

    def head_b_hooks(i, segs, pb, final=False, park=False):
        def put_b(T):
            def run(clk):
                tick(scl, 4, clk)
                pb.append(prob(get_state(i, T), get_state(i, S_MAXB)))
                put_p(1, T, pb[T])
                if park and T < 3:
                    park_p(i, S_PB + T, pb[T])
                if T == 3:
                    set_state(i, S_LB, inv_sum(part_sum(pb)) if final else part_sum(pb))
            return run
        return {("seg", segs[T]): [put_b(T)] for T in range(4)}

    def reduce_pair(i):
        xa, xb = get_state(i, S_X), get_state(i, S_X + 1)
        invb = inv_sum(get_state(i, S_LB))
        return reduce_o([ku[i * GP + b] for b in range(3)],
                        get_state(i, S_INVA), invb, (xa, None, xb))

    st = {}
    new_block()
    late = tuple(range(8, 12)) + tuple(range(8))
    q0, q1, q2 = qt
    dots = q_dots(0, st, q0, xl, mean) + q_dots(1, st, q1, xl, mean) \
        + k_dots(0, 0, st, q0) + k_dots(0, 1, st, q0, late) + k_dots(1, 0, st, q1, late) \
        + k_dots(1, 1, st, q1, late) + k_dots(2, 0, st, q2, late) + k_dots(2, 1, st, q2)
    for n in range(4):
        dots += x_dots(n // 2, n % 2, XROWS[n % 2], parked(n // 2, (S_PA, S_PB)[n % 2]))

    def lane_softmax(h):
        i, hh = h // 2, h % 2

        def run():
            s0 = st["s", hh]
            m = jnp.maximum(jnp.maximum(col(s0, 0), col(s0, 1)),
                            jnp.maximum(col(s0, 2), col(s0, 3)))
            m = jnp.max(m, axis=0, keepdims=True)
            p = st["p", h] = [prob(col(s0, T), m) for T in range(4)]
            w = st["w", h] = prob(m, jnp.max(m, axis=1, keepdims=True))
            l = part_sum(p) * w
            set_state(i, (S_INVA, S_LB)[hh], l if hh else inv_sum(l))
            for T in range(4 - hh):
                park_p(i, (S_PA, S_PB)[hh] + T, p[T] * w)
        return run

    def put_lane(h, T):
        def run(clk):
            tick(pT[4 * (h % 2) + T], 8, clk)
            put_p(h % 2, T, st["p", h][T])
        return run

    hooks = head_b_hooks(1, range(48 + B1_SEG, 96, 3), [], park=True)
    hooks.update({("need", 0): 23, ("need", B0_SEG): 35, ("need", A1_SEG): 47,
                  ("need", 48 + B1_SEG): DB1 + 1, ("need", 48 + A2_SEG): 70,
                  ("after", 82): 48 + B1_SEG + 9})
    for n, fn in ((10, lambda: mid_q(st, q0)),
                  (DQ[0], lambda: tick(q0, 5, q_vpu(2, c, q2))),
                  (DQ[1], lambda: tick(q0, 5, q_vpu(3, c, qa))),
                  (DQ[2], lambda: tick(q0, 5, q_vpu(4, c, qb))),
                  (DA0, lambda: tick(q0, 6, scl[_vr(0), :])), (22, lane_softmax(0)),
                   (DW0, lambda: tick(q0, 7, st["w", 0])),
                  (34, lane_softmax(1)), (DB0, lambda: tick(q1, 6, st["w", 1])),
                  (46, lane_softmax(2)), (DA1, lambda: tick(q1, 6, st["w", 2])),
                  (DB1, lambda: tick(q2, 6, stash_b(1, st["s", 1]))),
                  (82, lambda: stash_b(2, st["s", 1]))):
        hooks.setdefault(("dot", n), []).append(fn)
    for h in range(3):
        hooks["scale", h] = lambda h=h: st["w", h]

    def put_first(T):
        def run(_):
            for rho in range(8):
                pT[T][_vr(rho), :] = jnp.broadcast_to(st["p", 0][T][rho:rho + 1], (8, 128))
        return run

    hooks.update({("seg", T): [put_first(T)] for T in range(4)})
    hooks.update({("seg", B0_SEG + 2 * T): [put_lane(1, T)] for T in range(4)})
    hooks.update({("seg", A1_SEG + 2 * T): [put_lane(2, T)] for T in range(4)})
    tail_hooks(2, st, hooks, 48 + A2_SEG)
    run_block([0, 1], XROWS, dots, hooks, PLANS["first"])

    qs = (qb, qa)

    def late_dots(st):
        todo = [(m, 2) for m in range(NP - 2)] + [(NP - 3, 1)] + [(NP - 2, b) for b in range(3)]
        return [o_dot(m, b, st, lambda n=m + (2 - b) * 6: obuf[_vr(n), :], obuf) for m, b in todo]

    def block(name, j, ks, reds, qn, xrows):
        last = ks == [NP - 1]
        a_seg = A_SEG3 if name == "third" else A_SEG0
        b_segs = {"third": B_SEGS3,
                  "last": range(B_SEGL, 48, 3)}.get(name, B_SEGS)
        new_block()
        st = {}
        for k in ks if not last else []:
            mid_q(st, qs[(k + 1) % 2])
        outs = [reduce_pair(j + r) for r in reds]

        def kept(n):
            return (0, 1, 2) if last else (1, 2) if reds[n] == NP - 3 else (2,)

        def keep():
            for n, r in enumerate(reds):
                for b in kept(n):
                    obuf[pl.ds(pl.multiple_of(8 * (j + r + (2 - b) * 6), 8), 4), :] = (
                        pack8(outs[n][b]))

        if not last:
            keep()
        pb = []
        hooks = head_b_hooks(j + ks[0], b_segs, pb, last)
        dots = []

        def hook(key, fn):
            hooks.setdefault(key, []).append(fn)

        def direct(i, hh, seg0, tref):
            p = []

            def run():
                m = row_max(st["s", hh])
                p.extend(prob(col(st["s", hh], T), m) for T in range(4))
                l = part_sum(p)
                set_state(i, (S_INVA, S_LB)[hh], l if hh else inv_sum(l))

            def put(T, half):
                def go(clk):
                    tick(pT[4 * hh + T], 8, clk)
                    put_p(hh, T, p[T], range(4 * half, 4 * half + 4))
                return go
            hook(("dot", len(dots)), run)
            dots.extend(x_dots(i, hh, xrows[hh], lambda T: p[T], tref))
            hooks["need", seg0] = len(dots)
            for n in range(8):
                hook(("seg", seg0 + n), put(n // 2, n % 2))

        def wo_of(n):
            return [o_dot(j + reds[n], b, st, lambda b=b: outs[n][b], lref)
                    for b in range(3) if b not in kept(n)]

        def wq_of(n):
            nq = j + qn[n]
            return q_dots(nq if isinstance(nq, int) else jnp.minimum(nq, NP - 1), st, qs[qn[n] % 2])

        if last:
            dots += late_dots(st)[:NLATE] + x_dots(NP - 1, 0, xrows[0], parked(NP - 1, S_PA), lref)

            def park_acc(G, a4):
                for n in range(4):
                    ku[(NP - 1) * GP + 2, _vr(2 * (G - 16) + n), :] = pltpu.bitcast(a4[n], u32)
            hooks["end", 0] = park_acc
        for n, k in enumerate(ks if not last else []):
            q = qs[(k + 1) % 2]
            dots += k_dots(j + (k + 1), 0, st, q, MIX if n else MIXA, NALT if n else 0)
            if n == 0:
                if xrows[1]:
                    hooks["after", len(dots)] = b_segs[3]
                dots += x_dots(j + ks[0], 1, xrows[1], lambda T: pb[T], q)
            else:
                direct(j + k, 1, 48 * n + BD_SEG, q)
            kb = k_dots(j + (k + 1), 1, st, q, MIX)
            if n < len(ks) - 1:
                dots += kb[:XA_AT]
                direct(j + (k + 1), 0, 48 * n + AD_SEG, q)
                dots += kb[XA_AT:] + wq_of(n) + wo_of(n)
            else:
                hooks["need", 48 * n + a_seg] = len(dots)
                tail_hooks(j + (k + 1), st, hooks, 48 * n + a_seg)
                dots += kb
                hook(("dot", len(dots)), lambda k=k: stash_b(j + (k + 1), st["s", 1]))
                for m in range(n, len(qn)):
                    dots += wq_of(m)
                for m in range(n, len(reds)):
                    dots += wo_of(m)
                dots += x_dots(j + ks[0], 0, xrows[0],
                               parked(j + ks[0], S_PA), lref)
        run_block([j + k for k in ks], xrows, dots, hooks,
                  PLANS[name], range(NSPLIT) if last else None)
        if last:
            keep()
        if reds:
            abuf[...] += st["acc"]

    def body2(n, carry):
        block("body", 2 * n, [2, 3], [0, 1], [5, 6], XROWS)
        return carry

    zero = zs[0]
    lax.fori_loop(0, NP // 2 - 2, body2, 0)
    pl.when(zero == 0)(lambda: block("third", 0, [NP - 2], [NP - 4, NP - 3], [], XROWS))
    pl.when(zero <= 0)(lambda: block("last", 0, [NP - 1], [NP - 2], [], XROWS_LAST))

    new_block()
    st = {"acc": abuf[...]}
    invb = get_state(NP - 1, S_LB)
    o = reduce_o([ku[(NP - 1) * GP + b] for b in range(2)], get_state(NP - 1, S_INVA), invb,
                 (get_state(NP - 1, S_X), None))
    part = [None] * 5

    def finish(G, a4):
        for k in range(4):
            tick(lref, L_DUMMY + k, a4[k])
        z = lref[_vr(5), :]
        project(G, [pltpu.bitcast(v, u32) | z for v in a4])

    def project(G, a4):
        for n in range(4):
            v = jnp.sum(pltpu.bitcast(a4[n], f32), axis=1, keepdims=True)
            for nt in range(5):
                w = wou[(NP - 1) * (GP // 2) + G + n // 2, nt]
                t = pltpu.bitcast(w & jnp.uint32(HI) if n % 2 else w << 16, f32) * v
                part[nt] = t if part[nt] is None else part[nt] + t

    for G in range(16, NSPLIT // 2, 2):
        project(G, [ku[(NP - 1) * GP + 2, _vr(2 * (G - 16) + n), :] for n in range(4)])
    dots = late_dots(st)[NLATE:] + [o_dot(NP - 1, b, st, lambda b=b: o[b], lref)
                                    for b in range(2)]
    run_block([NP - 1], XROWS_LAST, dots, {("end", 0): finish},
              PLANS["final"], range(NSPLIT, 48))
    x = row_sum(st["acc"] + jnp.concatenate([v * invb for v in part], axis=1))

    xl = _rows16(x, ones)
    d = xl[0:8].astype(f32) - mean
    md = _mean(d)
    r1 = lax.rsqrt(jnp.maximum(_mean(d * d) - md * md, 0.0) + EPS)
    mean = mean + md
    y = (d - md) * r1
    my = _mean(y)
    r2 = lax.rsqrt(jnp.maximum(_mean(y * y) - my * my, 0.0) + EPS)
    h = jnp.dot(xl, w3[...], preferred_element_type=f32)
    h = h[0:8] * (r1 * r2) - h[8:16] * ((mean * r1 + my) * r2)
    h = jax.nn.gelu(h, approximate=True).astype(bf16)
    x = x + y
    parts = []
    for k in range(0, W4_VPU, 128):
        hk = jnp.broadcast_to(h[0:1, k:k + 128].astype(f32), (128, 128)).T
        t = w4[k:k + 128, :].astype(f32) * jnp.concatenate([hk] * 5, axis=1)
        parts.append(jnp.sum(t.reshape(16, 8, D), axis=0))
    for k in range(W4_VPU, F, 128):
        if k == W4_AT:
            x = x + row_sum(sum(parts[1:], parts[0]))
        x = x + jnp.dot(h[:, k:k + 128], w4[k:k + 128, :], preferred_element_type=f32)
    o_ref[...] = x[0:1].astype(o_ref.dtype)


def _cache_view(c):
    s = c.shape[2]
    c = jnp.transpose(c, (0, 1, 3, 2)).reshape(H * DH // 8, 8, s // 128, 128)
    return jnp.transpose(c, (0, 2, 1, 3)).reshape(H * DH // 8, s // 128 * 8, 128)


def _weight_view(w):
    k, n = w.shape
    w = jnp.transpose(w.reshape(k // 16, 2, 8, n // 128, 128), (0, 1, 3, 2, 4))
    return w.reshape(k // 16, n // 128, 16, 128)


@jax.jit
def pallas_interleave_layers__sliding_block_cached__mixer_s_mlp__decode_kernel(
    A_x: jax.Array,
    A_k_cache: jax.Array,
    A_v_cache: jax.Array,
    A_wq: jax.Array,
    A_wo: jax.Array,
    B_x: jax.Array,
    B_w1: jax.Array,
    B_w2: jax.Array,
    B_w3: jax.Array,
    B_w4: jax.Array,
):
    sk = A_k_cache.shape[2]
    win = min(4096, max(256, sk // 4))
    assert win == 4096 and sk % 128 == 0
    assert A_x.shape == (1, 1, D) and A_k_cache.shape == (1, H, sk, DH)
    wt = win // 128
    t0 = sk // 128 - wt
    ng = H * DH // 8
    hbm = pl.BlockSpec(memory_space=pl.ANY)
    out = pl.pallas_call(
        functools.partial(_kernel, t0=t0, wt=wt),
        out_shape=jax.ShapeDtypeStruct((1, D), A_x.dtype),
        in_specs=[hbm] * 7,
        out_specs=pl.BlockSpec(memory_space=pltpu.VMEM),
        scratch_shapes=[
            pltpu.VMEM((ng, wt * 8, 128), bf16),
            pltpu.VMEM((ng, wt * 8, 128), bf16),
            pltpu.VMEM((ng // 4, 128, 128), u32),
            pltpu.VMEM((NP * D // 16, 3, 8, 128), u32),
            pltpu.VMEM((H * DH // 16, D // 128, 16, 128), bf16),
            pltpu.VMEM((D, F), bf16),
            pltpu.VMEM((F, D), bf16),
            pltpu.VMEM((1, D), bf16),
            pltpu.VMEM((144, 128), u32),
            pltpu.VMEM((384, 128), u32),
            pltpu.VMEM((144, 128), u32),
            pltpu.VMEM((144, 128), u32),
            pltpu.VMEM((144, 128), u32),
            pltpu.VMEM((40, 128), f32),
            pltpu.VMEM((8, D), f32),
            pltpu.SMEM((1,), jnp.int32),
        ] + [pltpu.VMEM((64, 128), u32)] * 3
        + [pltpu.VMEM((72, 128), f32)] * 8,
        compiler_params=pltpu.CompilerParams(vmem_limit_bytes=128 * 1024 * 1024),
    )(A_x.reshape(1, D), _cache_view(A_k_cache), _cache_view(A_v_cache),
      _weight_view(A_wq).reshape(H * DH // 16, D // 128, 16, 128), _weight_view(A_wo), B_w3, B_w4)
    return out.reshape(1, 1, D)
```

```python
import functools

import jax
import jax.numpy as jnp
from jax import lax
import jax.experimental.pallas as pl
import jax.experimental.pallas.tpu as pltpu

D = 640
H = 32
DH = 192
F = 1536
EPS = 1e-5
NP = H // 2
GP = 2 * DH // 8
HI = 0xFFFF0000
CEXP = DH ** -0.5 * 1.4426950408889634

f32 = jnp.float32
bf16 = jnp.bfloat16
u32 = jnp.uint32

L_Y = 0
L_DUMMY = 6
S_MAXB, S_LB, S_INVA, S_X, S_PA, S_PB = 4, 5, 6, 7, 9, 13
XROWS = ((2, 10, 18, 26), (4, 12, 20))
XROWS_LAST = ((2, 10, 18, 26, 6, 14, 22, 30, 4, 12, 20, 28), ())
GX = (0, 16)
PLANS = {
    "first": (
        {},
        (21, 22, 22, 23, 24, 23, 26, 27, 26, 27, 28, 28, 29, 29, 30, 31, 32, 31, 33, 34, 34, 35,
        36, 36, 37, 38, 38, 39, 40, 40, 41, 42, 42, 43, 44, 44, 45, 46, 46, 47, 48, 48, 49, 49,
        50, 51, 51, 53, 51, 52, 54, 55, 54, 55, 56, 56, 57, 58, 58, 59, 60, 59, 60, 62, 62, 63,
        64, 64, 65, 66, 66, 67, 68, 68, 69, 70, 70, 71, 72, 71, 73, 74, 74, 75, 76, 73, 77, 78,
        77, 79, 80, 81, 82, 82, 82, 76)),
    "body": (
        {1: 0, 3: 2, 5: 4, 7: 4, 9: 5, 11: 8, 14: 10, 15: 13, 19: 14, 21: 14, 23: 16, 25: 17,
        27: 19, 29: 22, 31: 23, 33: 23, 35: 26, 37: 26, 39: 28, 40: 33, 41: 33, 43: 34, 47: 34,
        49: 35, 51: 37, 53: 38, 55: 39, 57: 40, 59: 42, 61: 43, 63: 48, 67: 50, 70: 51, 71: 52,
        72: 53, 75: 55, 77: 56, 79: 58, 81: 59, 83: 61, 84: 62},
        (0, 0, 0, 0, 0, 0, 0, 0, 0, 0, 0, 1, 2, 2, 3, 4, 4, 5, 6, 7, 7, 8, 9, 10, 10, 12, 12,
        13, 14, 15, 15, 16, 16, 17, 17, 18, 20, 21, 21, 24, 24, 24, 21, 22, 26, 30, 24, 25, 23,
        26, 27, 29, 29, 30, 31, 31, 33, 34, 35, 36, 36, 34, 34, 37, 37, 39, 43, 42, 40, 37, 41,
        41, 43, 46, 46, 45, 46, 47, 47, 49, 50, 51, 50, 51, 52, 57, 56, 58, 57, 59, 61, 60, 62,
        62, 63, 63)),
    "third": (
        {1: 0, 3: 3, 5: 3, 6: 3, 7: 4, 9: 5, 11: 8, 15: 11, 19: 14, 21: 14, 23: 15, 25: 17,
        26: 18, 27: 19, 30: 21},
        (0, 0, 0, 0, 0, 0, 0, 0, 0, 0, 0, 0, 0, 2, 2, 4, 3, 4, 3, 10, 9, 10, 12, 13, 12, 13, 13,
        12, 14, 17, 15, 16, 17, 17, 18, 19, 20, 18, 21, 22, 22, 24, 25, 26, 24, 25, 25, 27)),
    "last": (
        {1: 0, 3: 1, 5: 1, 7: 2, 11: 3, 15: 4, 17: 6, 19: 7, 21: 9, 23: 10, 26: 12},
        (0, 0, 0, 0, 0, 1, 1, 0, 0, 0, 0, 0, 0, 0, 0, 0, 1, 1, 0, 1, 2, 8, 5, 5, 6, 7, 10, 5, 8,
        8, 9, 10, 11, 11, 12, 10)),
    "final": (
        {37: 0, 39: 1, 40: 4, 43: 4, 45: 6},
        (0, 0, 0, 0, 0, 0, 0, 0, 0, 0, 0, 0, 0, 0, 0, 0, 0, 0, 0, 0, 0, 0, 0, 0, 0, 0, 0, 0, 0,
        0, 0, 0, 0, 0, 0, 0, 0, 0, 0, 0, 0, 0, 6, 3, 1, 2, 0, 0)),
}
MIX = (0, 1, 8, 2, 3, 9, 4, 5, 10, 6, 7, 11)
MIXA = (0, 1, 2, 3, 4, 8, 5, 9, 6, 10, 7, 11)
NLATE = 12
NSPLIT = 36
W4_VPU = 256
W4_AT = 896
B_SEGS = (9, 12, 15, 18)
B_SEGL = 8
DA0 = 17
DW0 = 32
DB0 = 44
DA1 = 55
DB1 = 67
DQ = (26, 29, 33)
NQV = 3
B0_SEG = 20
A1_SEG = 39
B1_SEG = 12
A2_SEG = 36
A_SEG0 = 40
A_SEG3 = 40
B_SEGS3 = (9, 11, 15, 19)
XA_AT = 8
AD_SEG = 32
BD_SEG = 12
NALT = 2
W4_CHUNKS = (1024, 256, 160, 64, 32)
W4_MXU = 1280


def _mean(x):
    return jnp.mean(x, axis=-1, keepdims=True)


def _ln(x):
    c = x - _mean(x)
    return c * lax.rsqrt(_mean(c * c) + EPS)


def _wtile(wu, rows, nt):
    blk = wu[rows, nt]
    return pltpu.bitcast(blk.reshape(blk.shape[0] * 8, 128), bf16)


def _wcols(wu, rows, nts):
    return jnp.concatenate([_wtile(wu, rows, n) for n in nts], axis=1)


def _rows16(a, b):
    return jnp.concatenate([a, b], axis=0).astype(bf16)


def _slot(G, t):
    j = 4 * (t >> 3) + ((((t >> 1) & 3) + G + 2 * (t & 1) + (t >> 3)) & 3)
    return 2 * G + (t & 1), 8 * j


def _xslot(G, t):
    return G // 2, 8 * (4 * (t >> 3) + ((((t >> 1) & 3) + G + (t >> 3)) & 3))


def _vr(n):
    return slice(8 * n, 8 * n + 8)


def _kernel(*refs, t0, wt):
    pl.run_scoped(functools.partial(_body, refs, t0, wt),
                  pltpu.SemaphoreType.DMA((4 + len(W4_CHUNKS) + 2 * NP,)))


def _body(refs, t0, wt, sems):
    (x_hbm, k_hbm, v_hbm, wq_hbm, wo_hbm, w3_hbm, w4_hbm, o_ref,
     kbuf, vbuf, vx, wqu, wo, w3, w4, xbuf, lref, obuf, qa, qb, qx, scl, abuf, zs) = refs[:24]
    qt, pT = refs[24:27], refs[27:]
    ku = kbuf.bitcast(u32)
    vu = vbuf.bitcast(u32)
    wou = wo.bitcast(u32)

    x_cp = pltpu.make_async_copy(x_hbm, xbuf, sems.at[0])
    wq_cp = pltpu.make_async_copy(wq_hbm, wo, sems.at[1])
    wo_cp = pltpu.make_async_copy(wo_hbm, wo, sems.at[2])
    w3_cp = pltpu.make_async_copy(w3_hbm, w3, sems.at[3])
    w4_rows, r0 = [], 0
    for n in W4_CHUNKS:
        w4_rows.append((r0, r0 + n))
        r0 += n
    w4_cp = [pltpu.make_async_copy(w4_hbm.at[a:b], w4.at[a:b], sems.at[4 + c])
             for c, (a, b) in enumerate(w4_rows)]
    S0 = 4 + len(W4_CHUNKS)

    def k_cp(i):
        return pltpu.make_async_copy(
            k_hbm.at[pl.ds(i * GP, GP), pl.ds(t0 * 8, wt * 8), :],
            kbuf.at[pl.ds(i * GP, GP)], sems.at[S0 + i])

    def v_cp(i):
        return pltpu.make_async_copy(
            v_hbm.at[pl.ds(i * GP, GP), pl.ds(t0 * 8, wt * 8), :],
            vbuf.at[pl.ds(i * GP, GP)], sems.at[S0 + NP + i])

    for c in (wq_cp, x_cp, k_cp(0), v_cp(0)):
        c.start()

    zs[0] = 0
    for ref in (qa, qb, qx, lref):
        ref[_vr(5), :] = jnp.zeros((8, 128), u32)

    lane = lax.broadcasted_iota(jnp.int32, (8, 128), 1)
    sub = lax.broadcasted_iota(jnp.int32, (8, 128), 0)
    lane_lo = lane < 64
    sub_lo = sub < 4

    def pair_view(buf, i):
        return buf.at[pl.ds(i * GP, GP)].bitcast(u32)

    def tile(ref, g0, G, t):
        g, r = _slot(G, t)
        return ref[g0 + g, r:r + 8, :]

    def retile(ref, i, expand):
        def body(c, carry):
            g0 = 8 * c
            for G in range(4):
                for J in range(4):
                    xs = [[ref[g0 + 2 * G + e, _vr(4 * J + jj), :] for jj in range(4)]
                          for e in range(2)]
                    for jj in range(4):
                        x0, x1 = xs[0][jj], xs[1][jj]
                        ys = (jnp.where(sub_lo, x0, pltpu.roll(x1, 4, 0)),
                              jnp.where(sub_lo, pltpu.roll(x0, 4, 0), x1))
                        for e in range(2):
                            t = 8 * J + 2 * jj + e
                            g, r = _slot(G, t)
                            if expand and G % 2 and e:
                                ref[g0 + g, r:r + 8, :] = ys[e] << 16
                                g, r = _xslot(G, t)
                                vx[i * (GP // 4) + 2 * c + g, r:r + 8, :] = ys[e] & jnp.uint32(HI)
                            else:
                                ref[g0 + g, r:r + 8, :] = ys[e]
            return carry
        lax.fori_loop(0, GP // 8, body, 0)

    def merge_halves(get, nt, n):
        lo, hi = get(n // 2), get((nt + n) // 2)
        if n % 2:
            lo = pltpu.roll(lo, 4, 0)
        if (nt + n) % 2 == 0:
            hi = pltpu.roll(hi, 4, 0)
        return jnp.where(sub_lo, lo, hi)

    def retile_wq(c, carry):
        for G in range(5):
            for n in range(3 * NP):
                wqu[n // 3 * (D // 16) + 5 * c + G, n % 3] = merge_halves(
                    lambda v: wou[48 * c + (48 * G + v) // 5, (48 * G + v) % 5], 3 * NP, n)
        return carry

    def retile_wo(c, carry):
        for G in range(8):
            xs = [wou[8 * c + G, n] for n in range(5)]
            for n in range(5):
                wou[8 * c + G, n] = merge_halves(lambda v: xs[v], 5, n)
        return carry

    def lhs_at(ref, n):
        return pltpu.bitcast(ref[_vr(n), :], bf16)

    cur = [None]

    def new_block():
        cur[0] = -32 * jnp.clip(zs[0], 0, 1)

    def tick(ref, n, val):
        assert 4 <= n < ref.shape[0] // 8
        if val.dtype != ref.dtype:
            val = pltpu.bitcast(val, ref.dtype)
        ref[pl.ds(pl.multiple_of(cur[0] + 8 * n, 8), 8), :] = val

    def put_q(q, qref):
        qq = pltpu.bitcast(q.astype(bf16).astype(f32), u32)
        q0, q1, q2 = qq[:, 0:128], qq[:, 128:256], qq[:, 256:384]
        for n, v in enumerate((q0 >> 16, q0, q2 >> 16, q2, q1)):
            qref[_vr(n), :] = v
            if n < 2 and qref is qb:
                qx[_vr(n), :] = v

    def transpose_wq(i):
        for k in range(5):
            for n in range(3):
                rows = pl.ds(i * (D // 16) + 8 * k, 8)
                w = pltpu.bitcast(_wtile(wqu, rows, n).astype(f32).T, u32)
                for G in range(8):
                    wqu[i * (D // 16) + 8 * k + G, n] = (w[_vr(2 * G), :] >> 16) | w[_vr(2 * G + 1), :]

    def q_vpu(i, c, qref):
        cols = []
        for n in range(3):
            acc = []
            for G in range(8):
                ws = [wqu[i * (D // 16) + 8 * k + G, n] for k in range(5)]
                for half in (lambda w: w << 16, lambda w: w & jnp.uint32(HI)):
                    t = [pltpu.bitcast(half(ws[k]), f32) * col(c, k) for k in range(5)]
                    acc.append((t[0] + t[1]) + (t[2] + t[3]) + t[4])
            z = jnp.sum(jnp.concatenate(acc, axis=0).T.reshape(16, 8, 128), axis=0)
            cols.append(row_sum(z))
        put_q(jnp.concatenate(cols, axis=1), qref)
        return cols[0] + cols[1] + cols[2]

    def row_sum(a):
        return jnp.broadcast_to(jnp.sum(a, axis=0, keepdims=True), a.shape)

    def q_dots(i, st, qref, lhs=None, mean=None):
        def step(k):
            def run(tied=False):
                w = _wcols(wqu, pl.ds(i * (D // 16) + 8 * k, 8), range(3))
                if lhs is None:
                    r = jnp.dot(lhs_at(lref, L_Y + k), w, preferred_element_type=f32)[0:8]
                else:
                    r = jnp.dot(lhs[:, 128 * k:128 * k + 128], w, preferred_element_type=f32)
                st["q"] = r if k == 0 else st["q"] + r
                if k == 4:
                    q = st["q"] if lhs is None else st["q"][0:8] - mean * st["q"][8:16]
                    put_q(q, qref)
                return r[0:8, 256:384]
            return 3, lref, L_DUMMY, run
        return [step(k) for k in range(5)]

    def as_lhs(v, tref):
        if v.dtype == f32 and tref is None:
            return v.astype(bf16)
        if v.dtype == f32:
            v = pltpu.bitcast(_rows16(v, v), u32)
        return pltpu.bitcast(v if tref is None else v | tref[_vr(5), :], bf16)

    def o_dot(i, b, st, get_lhs, tref=None):
        def run(tied=False):
            w = _wcols(wou, pl.ds(i * (GP // 2) + 8 * b, 8), range(5))
            lhs = as_lhs(get_lhs(), tref if tied and tref is not obuf else None)
            r = jnp.dot(lhs, w, preferred_element_type=f32)[0:8]
            st["acc"] = st["acc"] + r if "acc" in st else r
            return r[:, 512:640]
        return 5, tref, (32 if tref is obuf else 6), run

    def mid_q(st, qref):
        q1 = qref[_vr(4), :]
        q1r = pltpu.roll(q1, 64, 1)
        st["u", 0, id(qref)] = jnp.where(lane_lo, q1 >> 16, q1r)
        st["u", 1, id(qref)] = jnp.where(lane_lo, q1r >> 16, q1)

    def k_dots(i, hh, st, qref, order=tuple(range(12)), nalt=0, ku=ku):
        g0 = i * GP
        gf, gh = ((0, 8), (16, 12))[hh]

        def step(r):
            src = qx if r in order[:nalt] else qref

            def run(tied=False):
                if r < 8:
                    cols = [[tile(ku, g0, gf + G, 8 * T + r) for G in range(8)] for T in range(4)]
                    base, row = src[_vr(2 * hh + r % 2), :], r // 2
                else:
                    cols = [[tile(ku, g0, gh + G % 4, 8 * T + 2 * (r - 8) + G // 4)
                             for G in range(8)] for T in range(4)]
                    if ("u", hh, id(qref)) not in st:
                        mid_q(st, qref)
                    base, row = st["u", hh, id(qref)], r - 8
                    if tied:
                        base = base | src[_vr(5), :]
                lhs = jnp.where(sub == row, base, jnp.zeros((8, 128), u32))
                w = jnp.concatenate([jnp.concatenate(c, axis=0) for c in cols], axis=1)
                res = jnp.dot(pltpu.bitcast(lhs, bf16), pltpu.bitcast(w, bf16),
                              preferred_element_type=f32)[0:8]
                st["s", hh] = res if r == order[0] else st["s", hh] + res
                return res[:, 384:512]
            return 4, src, 6, run
        return [step(r) for r in order]

    def col(s, T):
        return s[:, 128 * T:128 * T + 128]

    def row_max(s):
        m = jnp.maximum(jnp.maximum(col(s, 0), col(s, 1)), jnp.maximum(col(s, 2), col(s, 3)))
        return jnp.max(jnp.max(m, axis=1, keepdims=True), axis=0, keepdims=True)

    def prob(s, m):
        return jnp.exp2((s - m) * scl[_vr(0), :])

    def put_p(hh, T, p, ks=range(8)):
        for k in ks:
            pT[4 * hh + T][pl.ds(k, 8, stride=8), :] = p

    def part_sum(p):
        return (p[0] + p[1]) + (p[2] + p[3])

    def inv_sum(l):
        l = jnp.sum(jnp.sum(l, axis=1, keepdims=True), axis=0, keepdims=True)
        r = pl.reciprocal(l, approx=True)
        return jnp.broadcast_to(r * (2.0 - l * r), (8, 128))

    def softmax(s, hh):
        m = row_max(s)
        p = [prob(col(s, T), m) for T in range(4)]
        for T in range(4):
            put_p(hh, T, p[T])
        return p, part_sum(p)

    def get_state(i, n):
        return pltpu.bitcast(ku[i * GP + 3, _vr(n), :], f32)

    def set_state(i, n, v):
        ku[i * GP + 3, _vr(n), :] = pltpu.bitcast(v, u32)

    def stash_b(i, s):
        for T in range(4):
            set_state(i, T, col(s, T))
        m = jnp.broadcast_to(row_max(s), (8, 128))
        set_state(i, S_MAXB, m)
        return m

    def pack8(v):
        return pltpu.bitcast(v.astype(bf16), u32)

    def park_p(i, n, p):
        ku[i * GP + 3, 8 * n:8 * n + 4, :] = pack8(p)

    def parked(i, n):
        return lambda T: ku[i * GP + 3, _vr(n + T), :]

    def x_dots(i, hh, ts, get_lhs, tref=None):
        st = {}
        rows = sorted({t % 8 for t in ts})

        def step(n, rho):
            def run(tied=False):
                res = []
                for T in [t // 8 for t in ts if t % 8 == rho]:
                    w = jnp.concatenate(
                        [tile(vu, i * GP, GX[hh] + G, 8 * T + rho) for G in range(8)], axis=0)
                    lhs = as_lhs(get_lhs(T), tref if tied else None)
                    res.append(jnp.dot(lhs, pltpu.bitcast(w, bf16),
                                       preferred_element_type=f32)[0:8])
                st["x"] = jnp.where(sub == rho, sum(res[1:], res[0]), st["x"] if n else 0.0)
                if n == len(rows) - 1:
                    set_state(i, S_X + hh, st["x"])
                return res[-1]
            return sum(1 for t in ts if t % 8 == rho), tref, 6, run
        return [step(n, rho) for n, rho in enumerate(rows)]

    def transpose_x(view, xrows):
        for hh in range(2):
            for t in xrows[hh]:
                w = jnp.concatenate([tile(view, 0, GX[hh] + G, t) for G in range(8)], axis=0)
                w = pltpu.bitcast(pltpu.bitcast(w, bf16).astype(f32).T.astype(bf16), u32)
                for G in range(8):
                    g, r = _slot(GX[hh] + G, t)
                    view[g, r:r + 8, :] = w[_vr(G), :]

    def reduce_o(blocks, inva, invb, extra=(None, None, None)):
        out = []
        for b, inv in enumerate((inva, jnp.where(lane_lo, inva, invb), invb)[:len(blocks)]):
            z = jnp.sum(pltpu.bitcast(blocks[b], f32).T.reshape(16, 8, 128), axis=0)
            if extra[b] is not None:
                z = z + extra[b]
            out.append(z * inv)
        return out

    def mac(acc, n, c, G, t, pv, view=None):
        w = tile(vu, 8 * c, G, t) if view is None else tile(view[0], view[1], G, t)
        if G % 2 and t % 2:
            g, r = _xslot(G, t)
            halves = (w, vx[2 * c + g, r:r + 8, :])
        else:
            halves = (w << 16, w & jnp.uint32(HI))
        for k in range(2):
            a = pltpu.bitcast(halves[k], f32) * pv
            acc[n + k] = a if acc[n + k] is None else acc[n + k] + a

    def seg_rows(xrows, seg):
        hh, gp, T = seg // 24 % 2, seg % 24 // 4, seg % 4
        on_mxu = GX[hh] <= 12 * hh + 2 * gp < GX[hh] + 8
        return [rho for rho in range(8) if not (on_mxu and 8 * T + rho in xrows[hh])]

    def run_block(pairs, xrows, dots, hooks, plan, segs=None):
        tie, clk = plan
        clock = []

        def emit(upto):
            while len(clock) < upto:
                n = len(clock)
                for h in hooks.get(("dot", n), ()):
                    h()
                clock.append(dots[n][3](n in tie.values()))

        zero = jnp.zeros((8, 128), f32)
        used = {}
        for seg in segs or range(48 * len(pairs)):
            i, hh, gp, T = pairs[seg // 48], seg // 24 % 2, seg % 24 // 4, seg % 4
            if T == 0:
                a4 = [None] * 4
            pref = pT[4 * hh + T]
            upto = min([v for k, v in tie.items() if k >= seg]
                       + [k[1] for k, v in hooks.items() if k[0] == "after" and v >= seg]
                       + [len(dots) if tie else clk[seg] + 6])
            free = not any(k in tie for k in range(seg, seg - T + 4))
            if free or ("seg", seg) in hooks:
                upto = max(upto, clk[seg] + 1)
            emit(min(len(dots), max(upto, hooks.get(("need", seg), 0))))
            if free:
                tick(pref, 8, clock[clk[seg]])
            elif gp:
                tick(pref, 8, zero)
            for h in hooks.get(("seg", seg), ()):
                h(clock[clk[seg]])
            for rho in seg_rows(xrows, seg):
                pv = pref[_vr(rho), :]
                for e in range(2):
                    mac(a4, 2 * e, i * 6, 12 * hh + 2 * gp + e, 8 * T + rho, pv)
            if seg in tie:
                ref, slot = dots[tie[seg]][1:3]
                used[tie[seg]] = used.get(tie[seg], -1) + 1
                for k in range(4):
                    tick(ref, slot + 4 * used[tie[seg]] + k, a4[k])
            if T == 3 and ("end", 0) in hooks and seg >= 32:
                hooks["end", 0](12 * hh + 2 * gp, a4)
            elif T == 3:
                for n in range(4):
                    G = 12 * hh + 2 * gp + n // 2
                    v = a4[n] * hooks["scale", seg // 24]() if ("scale", seg // 24) in hooks else a4[n]
                    ku[i * GP + G // 8, pl.ds(16 * (G % 8) + n % 2, 8, stride=2), :] = (
                        pltpu.bitcast(v, u32))
        emit(len(dots))

    def run_all(dots):
        for d in dots:
            d[3]()

    def set_input(c, scale):
        cp = pltpu.bitcast(_rows16(c, c), u32)
        for k in range(5):
            lref[_vr(L_Y + k), :] = cp[:, 128 * k:128 * k + 128]
        scl[_vr(0), :] = jnp.broadcast_to(scale, (8, 128))

    x_cp.wait()
    x = jnp.broadcast_to(xbuf[...].astype(f32), (8, D))
    set_input(_ln(x), jnp.full((8, 1), CEXP, f32))
    wq_cp.wait()
    lax.fori_loop(0, D // 80, retile_wq, 0)
    wo_cp.start()
    for i in range(1, NP):
        k_cp(i).start()
        v_cp(i).start()
    for c in [w3_cp] + w4_cp:
        c.start()
    wo_cp.wait()
    lax.fori_loop(0, H * DH // 128, retile_wo, 0)

    def body1(i, acc):
        st = {"acc": acc}
        k_cp(i).wait()
        kv = pair_view(kbuf, i)
        retile(kv, i, False)
        run_all(q_dots(i, st, qa))
        inv = []
        for hh in range(2):
            run_all(k_dots(0, hh, st, qa, ku=kv))
            inv.append(inv_sum(softmax(st["s", hh], hh)[1]))

        @pl.when(i > 0)
        def _():
            transpose_x(pair_view(vbuf, i - 1), XROWS)

        @pl.when(jnp.logical_and(i >= 5 - NQV, i < 5))
        def _():
            transpose_wq(i)

        v_cp(i).wait()
        vv = pair_view(vbuf, i)
        retile(vv, i, True)
        for hh in range(2):
            def pv_step(c, carry, hh=hh):
                acc8 = [None] * 8
                for t in range(32):
                    pv = pT[4 * hh + t // 8][_vr(t % 8), :]
                    for G in range(4):
                        mac(acc8, 2 * G, i * 6 + c, G, t, pv, (vv, 8 * c))
                for n in range(8):
                    obuf[pl.ds(64 * c + 16 * (n // 2) + n % 2, 8, stride=2), :] = (
                        pltpu.bitcast(acc8[n], u32))
                return carry
            lax.fori_loop(3 * hh, 3 * hh + 3, pv_step, 0)
        o = reduce_o([obuf[128 * b:128 * b + 128, :] for b in range(3)], inv[0], inv[1])
        run_all([o_dot(i, b, st, lambda b=b: o[b]) for b in range(3)])
        return st["acc"]

    x = x + row_sum(lax.fori_loop(0, NP, body1, jnp.zeros((8, D), f32)))

    y = _ln(x)
    zz = _ln(y).astype(bf16)
    w3_cp.wait()
    h = jnp.dot(zz, w3[...], preferred_element_type=f32)
    h = jax.nn.gelu(h, approximate=True).astype(bf16)
    x = x + y
    transpose_x(pair_view(vbuf, NP - 1), XROWS_LAST)
    for k in range(W4_MXU, F, 128):
        hk = jnp.broadcast_to(h[0:1, k:k + 128].astype(f32), (128, 128))
        obuf[k - W4_MXU:k - W4_MXU + 128, :] = pltpu.bitcast(hk.T, u32)
    part = jnp.zeros((8, D), f32)
    for cp, (a, b) in zip(w4_cp, w4_rows):
        cp.wait()
        if a < W4_MXU:
            x = x + jnp.dot(h[:, a:b], w4[a:b, :], preferred_element_type=f32)
        else:
            for k in range(a, b, 16):
                hk = pltpu.bitcast(obuf[k - W4_MXU:k - W4_MXU + 16, :], f32)
                t = w4[k:k + 16, :].astype(f32) * jnp.concatenate([hk] * 5, axis=1)
                part = part + (t[0:8] + t[8:16])
    x = x + row_sum(part)

    ones = jnp.ones((8, D), f32)
    xl = _rows16(x, ones)
    xb = xl[0:8].astype(f32)
    mean = _mean(xb)
    c = xb - mean
    set_input(c, lax.rsqrt(_mean(c * c) + EPS) * CEXP)
    abuf[...] = jnp.where(lax.broadcasted_iota(jnp.int32, (8, D), 0) == 0, x, 0.0)

    def tail_hooks(i, st, hooks, seg0):
        def first(_):
            m = row_max(st["s", 0])
            st["pa"] = [prob(col(st["s", 0], T), m) for T in range(4)]
            set_state(i, S_INVA, inv_sum(part_sum(st["pa"])))
            for T in range(4):
                park_p(i, S_PA + T, st["pa"][T])

        def put(T, half):
            def run(clk):
                tick(pT[T], 8, clk)
                put_p(0, T, st["pa"][T], range(4 * half, 4 * half + 4))
            return run
        hooks.setdefault(("seg", seg0), []).append(first)
        for n in range(8):
            hooks.setdefault(("seg", seg0 + n), []).append(put(n // 2, n % 2))

    def head_b_hooks(i, segs, pb, final=False, park=False):
        def put_b(T):
            def run(clk):
                tick(scl, 4, clk)
                pb.append(prob(get_state(i, T), get_state(i, S_MAXB)))
                put_p(1, T, pb[T])
                if park and T < 3:
                    park_p(i, S_PB + T, pb[T])
                if T == 3:
                    set_state(i, S_LB, inv_sum(part_sum(pb)) if final else part_sum(pb))
            return run
        return {("seg", segs[T]): [put_b(T)] for T in range(4)}

    def reduce_pair(i):
        xa, xb = get_state(i, S_X), get_state(i, S_X + 1)
        invb = inv_sum(get_state(i, S_LB))
        return reduce_o([ku[i * GP + b] for b in range(3)],
                        get_state(i, S_INVA), invb, (xa, None, xb))

    st = {}
    new_block()
    late = tuple(range(8, 12)) + tuple(range(8))
    q0, q1, q2 = qt
    dots = q_dots(0, st, q0, xl, mean) + q_dots(1, st, q1, xl, mean) \
        + k_dots(0, 0, st, q0) + k_dots(0, 1, st, q0, late) + k_dots(1, 0, st, q1, late) \
        + k_dots(1, 1, st, q1, late) + k_dots(2, 0, st, q2, late) + k_dots(2, 1, st, q2)
    for n in range(4):
        dots += x_dots(n // 2, n % 2, XROWS[n % 2], parked(n // 2, (S_PA, S_PB)[n % 2]))

    def lane_softmax(h):
        i, hh = h // 2, h % 2

        def run():
            s0 = st["s", hh]
            m = jnp.maximum(jnp.maximum(col(s0, 0), col(s0, 1)),
                            jnp.maximum(col(s0, 2), col(s0, 3)))
            m = jnp.max(m, axis=0, keepdims=True)
            p = st["p", h] = [prob(col(s0, T), m) for T in range(4)]
            w = st["w", h] = prob(m, jnp.max(m, axis=1, keepdims=True))
            l = part_sum(p) * w
            set_state(i, (S_INVA, S_LB)[hh], l if hh else inv_sum(l))
            for T in range(4 - hh):
                park_p(i, (S_PA, S_PB)[hh] + T, p[T] * w)
        return run

    def put_lane(h, T):
        def run(clk):
            tick(pT[4 * (h % 2) + T], 8, clk)
            put_p(h % 2, T, st["p", h][T])
        return run

    hooks = head_b_hooks(1, range(48 + B1_SEG, 96, 3), [], park=True)
    hooks.update({("need", 0): 23, ("need", B0_SEG): 35, ("need", A1_SEG): 47,
                  ("need", 48 + B1_SEG): DB1 + 1, ("need", 48 + A2_SEG): 70,
                  ("after", 82): 48 + B1_SEG + 9})
    for n, fn in ((10, lambda: mid_q(st, q0)),
                  (DQ[0], lambda: tick(q0, 5, q_vpu(2, c, q2))),
                  (DQ[1], lambda: tick(q0, 5, q_vpu(3, c, qa))),
                  (DQ[2], lambda: tick(q0, 5, q_vpu(4, c, qb))),
                  (DA0, lambda: tick(q0, 6, scl[_vr(0), :])), (22, lane_softmax(0)),
                   (DW0, lambda: tick(q0, 7, st["w", 0])),
                  (34, lane_softmax(1)), (DB0, lambda: tick(q1, 6, st["w", 1])),
                  (46, lane_softmax(2)), (DA1, lambda: tick(q1, 6, st["w", 2])),
                  (DB1, lambda: tick(q2, 6, stash_b(1, st["s", 1]))),
                  (82, lambda: stash_b(2, st["s", 1]))):
        hooks.setdefault(("dot", n), []).append(fn)
    for h in range(3):
        hooks["scale", h] = lambda h=h: st["w", h]

    def put_first(T):
        def run(_):
            for rho in range(8):
                pT[T][_vr(rho), :] = jnp.broadcast_to(st["p", 0][T][rho:rho + 1], (8, 128))
        return run

    hooks.update({("seg", T): [put_first(T)] for T in range(4)})
    hooks.update({("seg", B0_SEG + 2 * T): [put_lane(1, T)] for T in range(4)})
    hooks.update({("seg", A1_SEG + 2 * T): [put_lane(2, T)] for T in range(4)})
    tail_hooks(2, st, hooks, 48 + A2_SEG)
    run_block([0, 1], XROWS, dots, hooks, PLANS["first"])

    qs = (qb, qa)

    def late_dots(st):
        todo = [(m, 2) for m in range(NP - 2)] + [(NP - 3, 1)] + [(NP - 2, b) for b in range(3)]
        return [o_dot(m, b, st, lambda n=m + (2 - b) * 6: obuf[_vr(n), :], obuf) for m, b in todo]

    def block(name, j, ks, reds, qn, xrows):
        last = ks == [NP - 1]
        a_seg = A_SEG3 if name == "third" else A_SEG0
        b_segs = {"third": B_SEGS3,
                  "last": range(B_SEGL, 48, 3)}.get(name, B_SEGS)
        new_block()
        st = {}
        for k in ks if not last else []:
            mid_q(st, qs[(k + 1) % 2])
        outs = [reduce_pair(j + r) for r in reds]

        def kept(n):
            return (0, 1, 2) if last else (1, 2) if reds[n] == NP - 3 else (2,)

        def keep():
            for n, r in enumerate(reds):
                for b in kept(n):
                    obuf[pl.ds(pl.multiple_of(8 * (j + r + (2 - b) * 6), 8), 4), :] = (
                        pack8(outs[n][b]))

        if not last:
            keep()
        pb = []
        hooks = head_b_hooks(j + ks[0], b_segs, pb, last)
        dots = []

        def hook(key, fn):
            hooks.setdefault(key, []).append(fn)

        def direct(i, hh, seg0, tref):
            p = []

            def run():
                m = row_max(st["s", hh])
                p.extend(prob(col(st["s", hh], T), m) for T in range(4))
                l = part_sum(p)
                set_state(i, (S_INVA, S_LB)[hh], l if hh else inv_sum(l))

            def put(T, half):
                def go(clk):
                    tick(pT[4 * hh + T], 8, clk)
                    put_p(hh, T, p[T], range(4 * half, 4 * half + 4))
                return go
            hook(("dot", len(dots)), run)
            dots.extend(x_dots(i, hh, xrows[hh], lambda T: p[T], tref))
            hooks["need", seg0] = len(dots)
            for n in range(8):
                hook(("seg", seg0 + n), put(n // 2, n % 2))

        def wo_of(n):
            return [o_dot(j + reds[n], b, st, lambda b=b: outs[n][b], lref)
                    for b in range(3) if b not in kept(n)]

        def wq_of(n):
            nq = j + qn[n]
            return q_dots(nq if isinstance(nq, int) else jnp.minimum(nq, NP - 1), st, qs[qn[n] % 2])

        if last:
            dots += late_dots(st)[:NLATE] + x_dots(NP - 1, 0, xrows[0], parked(NP - 1, S_PA), lref)

            def park_acc(G, a4):
                for n in range(4):
                    ku[(NP - 1) * GP + 2, _vr(2 * (G - 16) + n), :] = pltpu.bitcast(a4[n], u32)
            hooks["end", 0] = park_acc
        for n, k in enumerate(ks if not last else []):
            q = qs[(k + 1) % 2]
            dots += k_dots(j + (k + 1), 0, st, q, MIX if n else MIXA, NALT if n else 0)
            if n == 0:
                if xrows[1]:
                    hooks["after", len(dots)] = b_segs[3]
                dots += x_dots(j + ks[0], 1, xrows[1], lambda T: pb[T], q)
            else:
                direct(j + k, 1, 48 * n + BD_SEG, q)
            kb = k_dots(j + (k + 1), 1, st, q, MIX)
            if n < len(ks) - 1:
                dots += kb[:XA_AT]
                direct(j + (k + 1), 0, 48 * n + AD_SEG, q)
                dots += kb[XA_AT:] + wq_of(n) + wo_of(n)
            else:
                hooks["need", 48 * n + a_seg] = len(dots)
                tail_hooks(j + (k + 1), st, hooks, 48 * n + a_seg)
                dots += kb
                hook(("dot", len(dots)), lambda k=k: stash_b(j + (k + 1), st["s", 1]))
                for m in range(n, len(qn)):
                    dots += wq_of(m)
                for m in range(n, len(reds)):
                    dots += wo_of(m)
                dots += x_dots(j + ks[0], 0, xrows[0],
                               parked(j + ks[0], S_PA), lref)
        run_block([j + k for k in ks], xrows, dots, hooks,
                  PLANS[name], range(NSPLIT) if last else None)
        if last:
            keep()
        if reds:
            abuf[...] += st["acc"]

    def body2(n, carry):
        block("body", 2 * n, [2, 3], [0, 1], [5, 6], XROWS)
        return carry

    zero = zs[0]
    lax.fori_loop(0, NP // 2 - 2, body2, 0)
    pl.when(zero == 0)(lambda: block("third", 0, [NP - 2], [NP - 4, NP - 3], [], XROWS))
    pl.when(zero <= 0)(lambda: block("last", 0, [NP - 1], [NP - 2], [], XROWS_LAST))

    new_block()
    st = {"acc": abuf[...]}
    invb = get_state(NP - 1, S_LB)
    o = reduce_o([ku[(NP - 1) * GP + b] for b in range(2)], get_state(NP - 1, S_INVA), invb,
                 (get_state(NP - 1, S_X), None))
    part = [None] * 5

    def finish(G, a4):
        for k in range(4):
            tick(lref, L_DUMMY + k, a4[k])
        z = lref[_vr(5), :]
        project(G, [pltpu.bitcast(v, u32) | z for v in a4])

    def project(G, a4):
        for n in range(4):
            v = jnp.sum(pltpu.bitcast(a4[n], f32), axis=1, keepdims=True)
            for nt in range(5):
                w = wou[(NP - 1) * (GP // 2) + G + n // 2, nt]
                t = pltpu.bitcast(w & jnp.uint32(HI) if n % 2 else w << 16, f32) * v
                part[nt] = t if part[nt] is None else part[nt] + t

    for G in range(16, NSPLIT // 2, 2):
        project(G, [ku[(NP - 1) * GP + 2, _vr(2 * (G - 16) + n), :] for n in range(4)])
    dots = late_dots(st)[NLATE:] + [o_dot(NP - 1, b, st, lambda b=b: o[b], lref)
                                    for b in range(2)]
    run_block([NP - 1], XROWS_LAST, dots, {("end", 0): finish},
              PLANS["final"], range(NSPLIT, 48))
    x = row_sum(st["acc"] + jnp.concatenate([v * invb for v in part], axis=1))

    xl = _rows16(x, ones)
    d = xl[0:8].astype(f32) - mean
    md = _mean(d)
    r1 = lax.rsqrt(jnp.maximum(_mean(d * d) - md * md, 0.0) + EPS)
    mean = mean + md
    y = (d - md) * r1
    my = _mean(y)
    r2 = lax.rsqrt(jnp.maximum(_mean(y * y) - my * my, 0.0) + EPS)
    h = jnp.dot(xl, w3[...], preferred_element_type=f32)
    h = h[0:8] * (r1 * r2) - h[8:16] * ((mean * r1 + my) * r2)
    h = jax.nn.gelu(h, approximate=True).astype(bf16)
    x = x + y
    parts = []
    for k in range(0, W4_VPU, 128):
        hk = jnp.broadcast_to(h[0:1, k:k + 128].astype(f32), (128, 128)).T
        t = w4[k:k + 128, :].astype(f32) * jnp.concatenate([hk] * 5, axis=1)
        parts.append(jnp.sum(t.reshape(16, 8, D), axis=0))
    for k in range(W4_VPU, F, 128):
        if k == W4_AT:
            x = x + row_sum(sum(parts[1:], parts[0]))
        x = x + jnp.dot(h[:, k:k + 128], w4[k:k + 128, :], preferred_element_type=f32)
    o_ref[...] = x[0:1].astype(o_ref.dtype)


def _cache_view(c):
    s = c.shape[2]
    c = jnp.transpose(c, (0, 1, 3, 2)).reshape(H * DH // 8, 8, s // 128, 128)
    return jnp.transpose(c, (0, 2, 1, 3)).reshape(H * DH // 8, s // 128 * 8, 128)


def _weight_view(w):
    k, n = w.shape
    w = jnp.transpose(w.reshape(k // 16, 2, 8, n // 128, 128), (0, 1, 3, 2, 4))
    return w.reshape(k // 16, n // 128, 16, 128)


@jax.jit
def pallas_interleave_layers__sliding_block_cached__mixer_s_mlp__decode_kernel(
    A_x: jax.Array,
    A_k_cache: jax.Array,
    A_v_cache: jax.Array,
    A_wq: jax.Array,
    A_wo: jax.Array,
    B_x: jax.Array,
    B_w1: jax.Array,
    B_w2: jax.Array,
    B_w3: jax.Array,
    B_w4: jax.Array,
):
    sk = A_k_cache.shape[2]
    win = min(4096, max(256, sk // 4))
    assert win == 4096 and sk % 128 == 0
    assert A_x.shape == (1, 1, D) and A_k_cache.shape == (1, H, sk, DH)
    wt = win // 128
    t0 = sk // 128 - wt
    ng = H * DH // 8
    hbm = pl.BlockSpec(memory_space=pl.ANY)
    out = pl.pallas_call(
        functools.partial(_kernel, t0=t0, wt=wt),
        out_shape=jax.ShapeDtypeStruct((1, D), A_x.dtype),
        in_specs=[hbm] * 7,
        out_specs=pl.BlockSpec(memory_space=pltpu.VMEM),
        scratch_shapes=[
            pltpu.VMEM((ng, wt * 8, 128), bf16),
            pltpu.VMEM((ng, wt * 8, 128), bf16),
            pltpu.VMEM((ng // 4, 128, 128), u32),
            pltpu.VMEM((NP * D // 16, 3, 8, 128), u32),
            pltpu.VMEM((H * DH // 16, D // 128, 16, 128), bf16),
            pltpu.VMEM((D, F), bf16),
            pltpu.VMEM((F, D), bf16),
            pltpu.VMEM((1, D), bf16),
            pltpu.VMEM((144, 128), u32),
            pltpu.VMEM((384, 128), u32),
            pltpu.VMEM((144, 128), u32),
            pltpu.VMEM((144, 128), u32),
            pltpu.VMEM((144, 128), u32),
            pltpu.VMEM((40, 128), f32),
            pltpu.VMEM((8, D), f32),
            pltpu.SMEM((1,), jnp.int32),
        ] + [pltpu.VMEM((64, 128), u32)] * 3
        + [pltpu.VMEM((72, 128), f32)] * 8,
        compiler_params=pltpu.CompilerParams(vmem_limit_bytes=128 * 1024 * 1024),
    )(A_x.reshape(1, D), _cache_view(A_k_cache), _cache_view(A_v_cache),
      _weight_view(A_wq).reshape(H * DH // 16, D // 128, 16, 128), _weight_view(A_wo), B_w3, B_w4)
    return out.reshape(1, 1, D)
```

```python
import functools

import jax
import jax.numpy as jnp
from jax import lax
import jax.experimental.pallas as pl
import jax.experimental.pallas.tpu as pltpu

D = 640
H = 32
DH = 192
F = 1536
EPS = 1e-5
NP = H // 2
GP = 2 * DH // 8
HI = 0xFFFF0000
CEXP = DH ** -0.5 * 1.4426950408889634

f32 = jnp.float32
bf16 = jnp.bfloat16
u32 = jnp.uint32

L_Y = 0
L_DUMMY = 6
S_MAXB, S_LB, S_INVA, S_X, S_PA, S_PB = 4, 5, 6, 7, 9, 13
XROWS = ((2, 10, 18, 26), (4, 12, 20))
XROWS_LAST = ((2, 10, 18, 26, 6, 14, 22, 30, 4, 12, 20, 28), ())
GX = (0, 16)
PLANS = {
    "first": (
        {},
        (21, 22, 22, 23, 24, 23, 26, 27, 26, 27, 28, 28, 29, 29, 30, 31, 32, 31, 33, 34, 34, 35,
        36, 36, 37, 38, 38, 39, 40, 40, 41, 42, 42, 43, 44, 44, 45, 46, 46, 47, 48, 48, 49, 49,
        50, 51, 51, 53, 51, 52, 54, 55, 54, 55, 56, 56, 57, 58, 58, 59, 60, 59, 60, 62, 62, 63,
        64, 64, 65, 66, 66, 67, 68, 68, 69, 70, 70, 71, 72, 71, 73, 74, 74, 75, 76, 72, 77, 78,
        77, 79, 80, 81, 82, 82, 81, 76)),
    "body": (
        {1: 0, 3: 2, 5: 4, 7: 4, 9: 5, 11: 8, 14: 10, 15: 13, 19: 14, 21: 14, 23: 16, 25: 17,
        27: 19, 29: 22, 31: 23, 33: 23, 35: 26, 37: 26, 39: 28, 40: 33, 41: 33, 43: 34, 47: 34,
        49: 35, 51: 37, 53: 38, 55: 39, 57: 40, 59: 42, 61: 43, 63: 48, 67: 50, 70: 51, 71: 52,
        72: 53, 75: 55, 77: 56, 79: 58, 81: 59, 83: 61, 84: 62},
        (0, 0, 0, 0, 0, 0, 0, 0, 0, 0, 0, 1, 2, 2, 3, 4, 4, 5, 6, 7, 7, 8, 9, 10, 10, 12, 12,
        13, 14, 15, 15, 16, 16, 17, 17, 18, 20, 21, 21, 24, 24, 24, 21, 22, 26, 30, 24, 25, 23,
        26, 27, 29, 29, 30, 31, 31, 33, 34, 35, 36, 36, 34, 34, 37, 37, 39, 43, 42, 40, 37, 41,
        41, 43, 46, 46, 45, 46, 47, 47, 49, 50, 51, 50, 51, 52, 57, 56, 58, 57, 59, 61, 60, 62,
        62, 63, 63)),
    "third": (
        {1: 0, 3: 3, 5: 3, 6: 3, 7: 4, 9: 5, 11: 8, 15: 11, 19: 14, 21: 14, 23: 15, 25: 17,
        26: 18, 27: 19, 30: 21},
        (0, 0, 0, 0, 0, 0, 0, 0, 0, 0, 0, 0, 0, 2, 2, 4, 3, 4, 3, 10, 9, 10, 12, 13, 12, 13, 13,
        12, 14, 17, 15, 16, 17, 17, 18, 19, 20, 18, 21, 22, 22, 24, 25, 26, 24, 25, 25, 27)),
    "last": (
        {1: 0, 3: 1, 5: 1, 7: 2, 11: 3, 15: 4, 17: 6, 19: 7, 21: 9, 23: 10, 26: 12},
        (0, 0, 0, 0, 0, 1, 1, 0, 0, 0, 0, 0, 0, 0, 0, 0, 1, 1, 0, 1, 2, 8, 5, 5, 6, 7, 10, 5, 8,
        8, 9, 10, 11, 11, 12, 10)),
    "final": (
        {37: 0, 39: 1, 40: 4, 43: 4, 45: 6},
        (0, 0, 0, 0, 0, 0, 0, 0, 0, 0, 0, 0, 0, 0, 0, 0, 0, 0, 0, 0, 0, 0, 0, 0, 0, 0, 0, 0, 0,
        0, 0, 0, 0, 0, 0, 0, 0, 0, 0, 0, 0, 0, 6, 3, 1, 2, 0, 0)),
}
MIX = (0, 1, 8, 2, 3, 9, 4, 5, 10, 6, 7, 11)
MIXA = (0, 1, 2, 3, 4, 8, 5, 9, 6, 10, 7, 11)
NLATE = 12
NSPLIT = 36
W4_VPU = 256
W4_AT = 896
B_SEGS = (9, 12, 15, 18)
B_SEGL = 8
DA0 = 17
DW0 = 32
DB0 = 44
DA1 = 57
DB1 = 68
DQ = (26, 29, 33)
NQV = 3
B0_SEG = 20
A1_SEG = 39
B1_SEG = 12
A2_SEG = 38
A_SEG0 = 40
A_SEG3 = 40
B_SEGS3 = (9, 11, 15, 19)
XA_AT = 8
AD_SEG = 32
BD_SEG = 12
NALT = 2
W4_CHUNKS = (1024, 256, 160, 64, 32)
W4_MXU = 1280


def _mean(x):
    return jnp.mean(x, axis=-1, keepdims=True)


def _ln(x):
    c = x - _mean(x)
    return c * lax.rsqrt(_mean(c * c) + EPS)


def _wtile(wu, rows, nt):
    blk = wu[rows, nt]
    return pltpu.bitcast(blk.reshape(blk.shape[0] * 8, 128), bf16)


def _wcols(wu, rows, nts):
    return jnp.concatenate([_wtile(wu, rows, n) for n in nts], axis=1)


def _rows16(a, b):
    return jnp.concatenate([a, b], axis=0).astype(bf16)


def _slot(G, t):
    j = 4 * (t >> 3) + ((((t >> 1) & 3) + G + 2 * (t & 1) + (t >> 3)) & 3)
    return 2 * G + (t & 1), 8 * j


def _xslot(G, t):
    return G // 2, 8 * (4 * (t >> 3) + ((((t >> 1) & 3) + G + (t >> 3)) & 3))


def _vr(n):
    return slice(8 * n, 8 * n + 8)


def _kernel(*refs, t0, wt):
    pl.run_scoped(functools.partial(_body, refs, t0, wt),
                  pltpu.SemaphoreType.DMA((4 + len(W4_CHUNKS) + 2 * NP,)))


def _body(refs, t0, wt, sems):
    (x_hbm, k_hbm, v_hbm, wq_hbm, wo_hbm, w3_hbm, w4_hbm, o_ref,
     kbuf, vbuf, vx, wqu, wo, w3, w4, xbuf, lref, obuf, qa, qb, qx, scl, abuf, zs) = refs[:24]
    qt, pT = refs[24:27], refs[27:]
    ku = kbuf.bitcast(u32)
    vu = vbuf.bitcast(u32)
    wou = wo.bitcast(u32)

    x_cp = pltpu.make_async_copy(x_hbm, xbuf, sems.at[0])
    wq_cp = pltpu.make_async_copy(wq_hbm, wo, sems.at[1])
    wo_cp = pltpu.make_async_copy(wo_hbm, wo, sems.at[2])
    w3_cp = pltpu.make_async_copy(w3_hbm, w3, sems.at[3])
    w4_rows, r0 = [], 0
    for n in W4_CHUNKS:
        w4_rows.append((r0, r0 + n))
        r0 += n
    w4_cp = [pltpu.make_async_copy(w4_hbm.at[a:b], w4.at[a:b], sems.at[4 + c])
             for c, (a, b) in enumerate(w4_rows)]
    S0 = 4 + len(W4_CHUNKS)

    def k_cp(i):
        return pltpu.make_async_copy(
            k_hbm.at[pl.ds(i * GP, GP), pl.ds(t0 * 8, wt * 8), :],
            kbuf.at[pl.ds(i * GP, GP)], sems.at[S0 + i])

    def v_cp(i):
        return pltpu.make_async_copy(
            v_hbm.at[pl.ds(i * GP, GP), pl.ds(t0 * 8, wt * 8), :],
            vbuf.at[pl.ds(i * GP, GP)], sems.at[S0 + NP + i])

    for c in (wq_cp, x_cp, k_cp(0), v_cp(0)):
        c.start()

    zs[0] = 0
    for ref in (qa, qb, qx, lref):
        ref[_vr(5), :] = jnp.zeros((8, 128), u32)

    lane = lax.broadcasted_iota(jnp.int32, (8, 128), 1)
    sub = lax.broadcasted_iota(jnp.int32, (8, 128), 0)
    lane_lo = lane < 64
    sub_lo = sub < 4

    def pair_view(buf, i):
        return buf.at[pl.ds(i * GP, GP)].bitcast(u32)

    def tile(ref, g0, G, t):
        g, r = _slot(G, t)
        return ref[g0 + g, r:r + 8, :]

    def retile(ref, i, expand):
        def body(c, carry):
            g0 = 8 * c
            for G in range(4):
                for J in range(4):
                    xs = [[ref[g0 + 2 * G + e, _vr(4 * J + jj), :] for jj in range(4)]
                          for e in range(2)]
                    for jj in range(4):
                        x0, x1 = xs[0][jj], xs[1][jj]
                        ys = (jnp.where(sub_lo, x0, pltpu.roll(x1, 4, 0)),
                              jnp.where(sub_lo, pltpu.roll(x0, 4, 0), x1))
                        for e in range(2):
                            t = 8 * J + 2 * jj + e
                            g, r = _slot(G, t)
                            if expand and G % 2 and e:
                                ref[g0 + g, r:r + 8, :] = ys[e] << 16
                                g, r = _xslot(G, t)
                                vx[i * (GP // 4) + 2 * c + g, r:r + 8, :] = ys[e] & jnp.uint32(HI)
                            else:
                                ref[g0 + g, r:r + 8, :] = ys[e]
            return carry
        lax.fori_loop(0, GP // 8, body, 0)

    def merge_halves(get, nt, n):
        lo, hi = get(n // 2), get((nt + n) // 2)
        if n % 2:
            lo = pltpu.roll(lo, 4, 0)
        if (nt + n) % 2 == 0:
            hi = pltpu.roll(hi, 4, 0)
        return jnp.where(sub_lo, lo, hi)

    def retile_wq(c, carry):
        for G in range(5):
            for n in range(3 * NP):
                wqu[n // 3 * (D // 16) + 5 * c + G, n % 3] = merge_halves(
                    lambda v: wou[48 * c + (48 * G + v) // 5, (48 * G + v) % 5], 3 * NP, n)
        return carry

    def retile_wo(c, carry):
        for G in range(8):
            xs = [wou[8 * c + G, n] for n in range(5)]
            for n in range(5):
                wou[8 * c + G, n] = merge_halves(lambda v: xs[v], 5, n)
        return carry

    def lhs_at(ref, n):
        return pltpu.bitcast(ref[_vr(n), :], bf16)

    cur = [None]

    def new_block():
        cur[0] = -32 * jnp.clip(zs[0], 0, 1)

    def tick(ref, n, val):
        assert 4 <= n < ref.shape[0] // 8
        if val.dtype != ref.dtype:
            val = pltpu.bitcast(val, ref.dtype)
        ref[pl.ds(pl.multiple_of(cur[0] + 8 * n, 8), 8), :] = val

    def put_q(q, qref):
        qq = pltpu.bitcast(q.astype(bf16).astype(f32), u32)
        q0, q1, q2 = qq[:, 0:128], qq[:, 128:256], qq[:, 256:384]
        for n, v in enumerate((q0 >> 16, q0, q2 >> 16, q2, q1)):
            qref[_vr(n), :] = v
            if n < 2 and qref is qb:
                qx[_vr(n), :] = v

    def transpose_wq(i):
        for k in range(5):
            for n in range(3):
                rows = pl.ds(i * (D // 16) + 8 * k, 8)
                w = pltpu.bitcast(_wtile(wqu, rows, n).astype(f32).T, u32)
                for G in range(8):
                    wqu[i * (D // 16) + 8 * k + G, n] = (w[_vr(2 * G), :] >> 16) | w[_vr(2 * G + 1), :]

    def q_vpu(i, c, qref):
        cols = []
        for n in range(3):
            acc = []
            for G in range(8):
                ws = [wqu[i * (D // 16) + 8 * k + G, n] for k in range(5)]
                for half in (lambda w: w << 16, lambda w: w & jnp.uint32(HI)):
                    t = [pltpu.bitcast(half(ws[k]), f32) * col(c, k) for k in range(5)]
                    acc.append((t[0] + t[1]) + (t[2] + t[3]) + t[4])
            z = jnp.sum(jnp.concatenate(acc, axis=0).T.reshape(16, 8, 128), axis=0)
            cols.append(row_sum(z))
        put_q(jnp.concatenate(cols, axis=1), qref)
        return cols[0] + cols[1] + cols[2]

    def row_sum(a):
        return jnp.broadcast_to(jnp.sum(a, axis=0, keepdims=True), a.shape)

    def q_dots(i, st, qref, lhs=None, mean=None):
        def step(k):
            def run(tied=False):
                w = _wcols(wqu, pl.ds(i * (D // 16) + 8 * k, 8), range(3))
                if lhs is None:
                    r = jnp.dot(lhs_at(lref, L_Y + k), w, preferred_element_type=f32)[0:8]
                else:
                    r = jnp.dot(lhs[:, 128 * k:128 * k + 128], w, preferred_element_type=f32)
                st["q"] = r if k == 0 else st["q"] + r
                if k == 4:
                    q = st["q"] if lhs is None else st["q"][0:8] - mean * st["q"][8:16]
                    put_q(q, qref)
                return r[0:8, 256:384]
            return 3, lref, L_DUMMY, run
        return [step(k) for k in range(5)]

    def as_lhs(v, tref):
        if v.dtype == f32 and tref is None:
            return v.astype(bf16)
        if v.dtype == f32:
            v = pltpu.bitcast(_rows16(v, v), u32)
        return pltpu.bitcast(v if tref is None else v | tref[_vr(5), :], bf16)

    def o_dot(i, b, st, get_lhs, tref=None):
        def run(tied=False):
            w = _wcols(wou, pl.ds(i * (GP // 2) + 8 * b, 8), range(5))
            lhs = as_lhs(get_lhs(), tref if tied and tref is not obuf else None)
            r = jnp.dot(lhs, w, preferred_element_type=f32)[0:8]
            st["acc"] = st["acc"] + r if "acc" in st else r
            return r[:, 512:640]
        return 5, tref, (32 if tref is obuf else 6), run

    def mid_q(st, qref):
        q1 = qref[_vr(4), :]
        q1r = pltpu.roll(q1, 64, 1)
        st["u", 0, id(qref)] = jnp.where(lane_lo, q1 >> 16, q1r)
        st["u", 1, id(qref)] = jnp.where(lane_lo, q1r >> 16, q1)

    def k_dots(i, hh, st, qref, order=tuple(range(12)), nalt=0, ku=ku):
        g0 = i * GP
        gf, gh = ((0, 8), (16, 12))[hh]

        def step(r):
            src = qx if r in order[:nalt] else qref

            def run(tied=False):
                if r < 8:
                    cols = [[tile(ku, g0, gf + G, 8 * T + r) for G in range(8)] for T in range(4)]
                    base, row = src[_vr(2 * hh + r % 2), :], r // 2
                else:
                    cols = [[tile(ku, g0, gh + G % 4, 8 * T + 2 * (r - 8) + G // 4)
                             for G in range(8)] for T in range(4)]
                    if ("u", hh, id(qref)) not in st:
                        mid_q(st, qref)
                    base, row = st["u", hh, id(qref)], r - 8
                    if tied:
                        base = base | src[_vr(5), :]
                lhs = jnp.where(sub == row, base, jnp.zeros((8, 128), u32))
                w = jnp.concatenate([jnp.concatenate(c, axis=0) for c in cols], axis=1)
                res = jnp.dot(pltpu.bitcast(lhs, bf16), pltpu.bitcast(w, bf16),
                              preferred_element_type=f32)[0:8]
                st["s", hh] = res if r == order[0] else st["s", hh] + res
                return res[:, 384:512]
            return 4, src, 6, run
        return [step(r) for r in order]

    def col(s, T):
        return s[:, 128 * T:128 * T + 128]

    def row_max(s):
        m = jnp.maximum(jnp.maximum(col(s, 0), col(s, 1)), jnp.maximum(col(s, 2), col(s, 3)))
        return jnp.max(jnp.max(m, axis=1, keepdims=True), axis=0, keepdims=True)

    def prob(s, m):
        return jnp.exp2((s - m) * scl[_vr(0), :])

    def put_p(hh, T, p, ks=range(8)):
        for k in ks:
            pT[4 * hh + T][pl.ds(k, 8, stride=8), :] = p

    def part_sum(p):
        return (p[0] + p[1]) + (p[2] + p[3])

    def inv_sum(l):
        l = jnp.sum(jnp.sum(l, axis=1, keepdims=True), axis=0, keepdims=True)
        r = pl.reciprocal(l, approx=True)
        return jnp.broadcast_to(r * (2.0 - l * r), (8, 128))

    def softmax(s, hh):
        m = row_max(s)
        p = [prob(col(s, T), m) for T in range(4)]
        for T in range(4):
            put_p(hh, T, p[T])
        return p, part_sum(p)

    def get_state(i, n):
        return pltpu.bitcast(ku[i * GP + 3, _vr(n), :], f32)

    def set_state(i, n, v):
        ku[i * GP + 3, _vr(n), :] = pltpu.bitcast(v, u32)

    def stash_b(i, s):
        for T in range(4):
            set_state(i, T, col(s, T))
        m = jnp.broadcast_to(row_max(s), (8, 128))
        set_state(i, S_MAXB, m)
        return m

    def pack8(v):
        return pltpu.bitcast(v.astype(bf16), u32)

    def park_p(i, n, p):
        ku[i * GP + 3, 8 * n:8 * n + 4, :] = pack8(p)

    def parked(i, n):
        return lambda T: ku[i * GP + 3, _vr(n + T), :]

    def x_dots(i, hh, ts, get_lhs, tref=None):
        st = {}
        rows = sorted({t % 8 for t in ts})

        def step(n, rho):
            def run(tied=False):
                res = []
                for T in [t // 8 for t in ts if t % 8 == rho]:
                    w = jnp.concatenate(
                        [tile(vu, i * GP, GX[hh] + G, 8 * T + rho) for G in range(8)], axis=0)
                    lhs = as_lhs(get_lhs(T), tref if tied else None)
                    res.append(jnp.dot(lhs, pltpu.bitcast(w, bf16),
                                       preferred_element_type=f32)[0:8])
                st["x"] = jnp.where(sub == rho, sum(res[1:], res[0]), st["x"] if n else 0.0)
                if n == len(rows) - 1:
                    set_state(i, S_X + hh, st["x"])
                return res[-1]
            return sum(1 for t in ts if t % 8 == rho), tref, 6, run
        return [step(n, rho) for n, rho in enumerate(rows)]

    def transpose_x(view, xrows):
        for hh in range(2):
            for t in xrows[hh]:
                w = jnp.concatenate([tile(view, 0, GX[hh] + G, t) for G in range(8)], axis=0)
                w = pltpu.bitcast(pltpu.bitcast(w, bf16).astype(f32).T.astype(bf16), u32)
                for G in range(8):
                    g, r = _slot(GX[hh] + G, t)
                    view[g, r:r + 8, :] = w[_vr(G), :]

    def reduce_o(blocks, inva, invb, extra=(None, None, None)):
        out = []
        for b, inv in enumerate((inva, jnp.where(lane_lo, inva, invb), invb)[:len(blocks)]):
            z = jnp.sum(pltpu.bitcast(blocks[b], f32).T.reshape(16, 8, 128), axis=0)
            if extra[b] is not None:
                z = z + extra[b]
            out.append(z * inv)
        return out

    def mac(acc, n, c, G, t, pv, view=None):
        w = tile(vu, 8 * c, G, t) if view is None else tile(view[0], view[1], G, t)
        if G % 2 and t % 2:
            g, r = _xslot(G, t)
            halves = (w, vx[2 * c + g, r:r + 8, :])
        else:
            halves = (w << 16, w & jnp.uint32(HI))
        for k in range(2):
            a = pltpu.bitcast(halves[k], f32) * pv
            acc[n + k] = a if acc[n + k] is None else acc[n + k] + a

    def seg_rows(xrows, seg):
        hh, gp, T = seg // 24 % 2, seg % 24 // 4, seg % 4
        on_mxu = GX[hh] <= 12 * hh + 2 * gp < GX[hh] + 8
        return [rho for rho in range(8) if not (on_mxu and 8 * T + rho in xrows[hh])]

    def run_block(pairs, xrows, dots, hooks, plan, segs=None):
        tie, clk = plan
        clock = []

        def emit(upto):
            while len(clock) < upto:
                n = len(clock)
                for h in hooks.get(("dot", n), ()):
                    h()
                clock.append(dots[n][3](n in tie.values()))

        zero = jnp.zeros((8, 128), f32)
        used = {}
        for seg in segs or range(48 * len(pairs)):
            i, hh, gp, T = pairs[seg // 48], seg // 24 % 2, seg % 24 // 4, seg % 4
            if T == 0:
                a4 = [None] * 4
            pref = pT[4 * hh + T]
            upto = min([v for k, v in tie.items() if k >= seg]
                       + [k[1] for k, v in hooks.items() if k[0] == "after" and v >= seg]
                       + [len(dots) if tie else clk[seg] + 6])
            free = not any(k in tie for k in range(seg, seg - T + 4))
            if free or ("seg", seg) in hooks:
                upto = max(upto, clk[seg] + 1)
            emit(min(len(dots), max(upto, hooks.get(("need", seg), 0))))
            if free:
                tick(pref, 8, clock[clk[seg]])
            elif gp:
                tick(pref, 8, zero)
            for h in hooks.get(("seg", seg), ()):
                h(clock[clk[seg]])
            for rho in seg_rows(xrows, seg):
                pv = pref[_vr(rho), :]
                for e in range(2):
                    mac(a4, 2 * e, i * 6, 12 * hh + 2 * gp + e, 8 * T + rho, pv)
            if seg in tie:
                ref, slot = dots[tie[seg]][1:3]
                used[tie[seg]] = used.get(tie[seg], -1) + 1
                for k in range(4):
                    tick(ref, slot + 4 * used[tie[seg]] + k, a4[k])
            if T == 3 and ("end", 0) in hooks and seg >= 32:
                hooks["end", 0](12 * hh + 2 * gp, a4)
            elif T == 3:
                for n in range(4):
                    G = 12 * hh + 2 * gp + n // 2
                    v = a4[n] * hooks["scale", seg // 24]() if ("scale", seg // 24) in hooks else a4[n]
                    ku[i * GP + G // 8, pl.ds(16 * (G % 8) + n % 2, 8, stride=2), :] = (
                        pltpu.bitcast(v, u32))
        emit(len(dots))

    def run_all(dots):
        for d in dots:
            d[3]()

    def set_input(c, scale):
        cp = pltpu.bitcast(_rows16(c, c), u32)
        for k in range(5):
            lref[_vr(L_Y + k), :] = cp[:, 128 * k:128 * k + 128]
        scl[_vr(0), :] = jnp.broadcast_to(scale, (8, 128))

    x_cp.wait()
    x = jnp.broadcast_to(xbuf[...].astype(f32), (8, D))
    set_input(_ln(x), jnp.full((8, 1), CEXP, f32))
    wq_cp.wait()
    lax.fori_loop(0, D // 80, retile_wq, 0)
    wo_cp.start()
    for i in range(1, NP):
        k_cp(i).start()
        v_cp(i).start()
    for c in [w3_cp] + w4_cp:
        c.start()
    wo_cp.wait()
    lax.fori_loop(0, H * DH // 128, retile_wo, 0)

    def body1(i, acc):
        st = {"acc": acc}
        k_cp(i).wait()
        kv = pair_view(kbuf, i)
        retile(kv, i, False)
        run_all(q_dots(i, st, qa))
        inv = []
        for hh in range(2):
            run_all(k_dots(0, hh, st, qa, ku=kv))
            inv.append(inv_sum(softmax(st["s", hh], hh)[1]))

        @pl.when(i > 0)
        def _():
            transpose_x(pair_view(vbuf, i - 1), XROWS)

        @pl.when(jnp.logical_and(i >= 5 - NQV, i < 5))
        def _():
            transpose_wq(i)

        v_cp(i).wait()
        vv = pair_view(vbuf, i)
        retile(vv, i, True)
        for hh in range(2):
            def pv_step(c, carry, hh=hh):
                acc8 = [None] * 8
                for t in range(32):
                    pv = pT[4 * hh + t // 8][_vr(t % 8), :]
                    for G in range(4):
                        mac(acc8, 2 * G, i * 6 + c, G, t, pv, (vv, 8 * c))
                for n in range(8):
                    obuf[pl.ds(64 * c + 16 * (n // 2) + n % 2, 8, stride=2), :] = (
                        pltpu.bitcast(acc8[n], u32))
                return carry
            lax.fori_loop(3 * hh, 3 * hh + 3, pv_step, 0)
        o = reduce_o([obuf[128 * b:128 * b + 128, :] for b in range(3)], inv[0], inv[1])
        run_all([o_dot(i, b, st, lambda b=b: o[b]) for b in range(3)])
        return st["acc"]

    x = x + row_sum(lax.fori_loop(0, NP, body1, jnp.zeros((8, D), f32)))

    y = _ln(x)
    zz = _ln(y).astype(bf16)
    w3_cp.wait()
    h = jnp.dot(zz, w3[...], preferred_element_type=f32)
    h = jax.nn.gelu(h, approximate=True).astype(bf16)
    x = x + y
    transpose_x(pair_view(vbuf, NP - 1), XROWS_LAST)
    for k in range(W4_MXU, F, 128):
        hk = jnp.broadcast_to(h[0:1, k:k + 128].astype(f32), (128, 128))
        obuf[k - W4_MXU:k - W4_MXU + 128, :] = pltpu.bitcast(hk.T, u32)
    part = jnp.zeros((8, D), f32)
    for cp, (a, b) in zip(w4_cp, w4_rows):
        cp.wait()
        if a < W4_MXU:
            x = x + jnp.dot(h[:, a:b], w4[a:b, :], preferred_element_type=f32)
        else:
            for k in range(a, b, 16):
                hk = pltpu.bitcast(obuf[k - W4_MXU:k - W4_MXU + 16, :], f32)
                t = w4[k:k + 16, :].astype(f32) * jnp.concatenate([hk] * 5, axis=1)
                part = part + (t[0:8] + t[8:16])
    x = x + row_sum(part)

    ones = jnp.ones((8, D), f32)
    xl = _rows16(x, ones)
    xb = xl[0:8].astype(f32)
    mean = _mean(xb)
    c = xb - mean
    set_input(c, lax.rsqrt(_mean(c * c) + EPS) * CEXP)
    abuf[...] = jnp.where(lax.broadcasted_iota(jnp.int32, (8, D), 0) == 0, x, 0.0)

    def tail_hooks(i, st, hooks, seg0):
        def first(_):
            m = row_max(st["s", 0])
            st["pa"] = [prob(col(st["s", 0], T), m) for T in range(4)]
            set_state(i, S_INVA, inv_sum(part_sum(st["pa"])))
            for T in range(4):
                park_p(i, S_PA + T, st["pa"][T])

        def put(T, half):
            def run(clk):
                tick(pT[T], 8, clk)
                put_p(0, T, st["pa"][T], range(4 * half, 4 * half + 4))
            return run
        hooks.setdefault(("seg", seg0), []).append(first)
        for n in range(8):
            hooks.setdefault(("seg", seg0 + n), []).append(put(n // 2, n % 2))

    def head_b_hooks(i, segs, pb, final=False, park=False):
        def put_b(T):
            def run(clk):
                tick(scl, 4, clk)
                pb.append(prob(get_state(i, T), get_state(i, S_MAXB)))
                put_p(1, T, pb[T])
                if park and T < 3:
                    park_p(i, S_PB + T, pb[T])
                if T == 3:
                    set_state(i, S_LB, inv_sum(part_sum(pb)) if final else part_sum(pb))
            return run
        return {("seg", segs[T]): [put_b(T)] for T in range(4)}

    def reduce_pair(i):
        xa, xb = get_state(i, S_X), get_state(i, S_X + 1)
        invb = inv_sum(get_state(i, S_LB))
        return reduce_o([ku[i * GP + b] for b in range(3)],
                        get_state(i, S_INVA), invb, (xa, None, xb))

    st = {}
    new_block()
    late = tuple(range(8, 12)) + tuple(range(8))
    q0, q1, q2 = qt
    dots = q_dots(0, st, q0, xl, mean) + q_dots(1, st, q1, xl, mean) \
        + k_dots(0, 0, st, q0) + k_dots(0, 1, st, q0, late) + k_dots(1, 0, st, q1, late) \
        + k_dots(1, 1, st, q1, late) + k_dots(2, 0, st, q2, late) + k_dots(2, 1, st, q2)
    for n in range(4):
        dots += x_dots(n // 2, n % 2, XROWS[n % 2], parked(n // 2, (S_PA, S_PB)[n % 2]))

    def lane_softmax(h):
        i, hh = h // 2, h % 2

        def run():
            s0 = st["s", hh]
            m = jnp.maximum(jnp.maximum(col(s0, 0), col(s0, 1)),
                            jnp.maximum(col(s0, 2), col(s0, 3)))
            m = jnp.max(m, axis=0, keepdims=True)
            p = st["p", h] = [prob(col(s0, T), m) for T in range(4)]
            w = st["w", h] = prob(m, jnp.max(m, axis=1, keepdims=True))
            l = part_sum(p) * w
            set_state(i, (S_INVA, S_LB)[hh], l if hh else inv_sum(l))
            for T in range(4 - hh):
                park_p(i, (S_PA, S_PB)[hh] + T, p[T] * w)
        return run

    def put_lane(h, T):
        def run(clk):
            tick(pT[4 * (h % 2) + T], 8, clk)
            put_p(h % 2, T, st["p", h][T])
        return run

    hooks = head_b_hooks(1, range(48 + B1_SEG, 96, 3), [], park=True)
    hooks.update({("need", 0): 23, ("need", B0_SEG): 35, ("need", A1_SEG): 47,
                  ("need", 48 + B1_SEG): DB1 + 1, ("need", 48 + A2_SEG): 70,
                  ("after", 82): 48 + B1_SEG + 9})
    for n, fn in ((10, lambda: mid_q(st, q0)),
                  (DQ[0], lambda: tick(q0, 5, q_vpu(2, c, q2))),
                  (DQ[1], lambda: tick(q0, 5, q_vpu(3, c, qa))),
                  (DQ[2], lambda: tick(q0, 5, q_vpu(4, c, qb))),
                  (DA0, lambda: tick(q0, 6, scl[_vr(0), :])), (22, lane_softmax(0)),
                   (DW0, lambda: tick(q0, 7, st["w", 0])),
                  (34, lane_softmax(1)), (DB0, lambda: tick(q1, 6, st["w", 1])),
                  (46, lane_softmax(2)), (DA1, lambda: tick(q1, 6, st["w", 2])),
                  (DB1, lambda: tick(q2, 6, stash_b(1, st["s", 1]))),
                  (82, lambda: stash_b(2, st["s", 1]))):
        hooks.setdefault(("dot", n), []).append(fn)
    for h in range(3):
        hooks["scale", h] = lambda h=h: st["w", h]

    def put_first(T):
        def run(_):
            for rho in range(8):
                pT[T][_vr(rho), :] = jnp.broadcast_to(st["p", 0][T][rho:rho + 1], (8, 128))
        return run

    hooks.update({("seg", T): [put_first(T)] for T in range(4)})
    hooks.update({("seg", B0_SEG + 2 * T): [put_lane(1, T)] for T in range(4)})
    hooks.update({("seg", A1_SEG + 2 * T): [put_lane(2, T)] for T in range(4)})
    tail_hooks(2, st, hooks, 48 + A2_SEG)
    run_block([0, 1], XROWS, dots, hooks, PLANS["first"])

    qs = (qb, qa)

    def late_dots(st):
        todo = [(m, 2) for m in range(NP - 2)] + [(NP - 3, 1)] + [(NP - 2, b) for b in range(3)]
        return [o_dot(m, b, st, lambda n=m + (2 - b) * 6: obuf[_vr(n), :], obuf) for m, b in todo]

    def block(name, j, ks, reds, qn, xrows):
        last = ks == [NP - 1]
        a_seg = A_SEG3 if name == "third" else A_SEG0
        b_segs = {"third": B_SEGS3,
                  "last": range(B_SEGL, 48, 3)}.get(name, B_SEGS)
        new_block()
        st = {}
        for k in ks if not last else []:
            mid_q(st, qs[(k + 1) % 2])
        outs = [reduce_pair(j + r) for r in reds]

        def kept(n):
            return (0, 1, 2) if last else (1, 2) if reds[n] == NP - 3 else (2,)

        def keep():
            for n, r in enumerate(reds):
                for b in kept(n):
                    obuf[pl.ds(pl.multiple_of(8 * (j + r + (2 - b) * 6), 8), 4), :] = (
                        pack8(outs[n][b]))

        if not last:
            keep()
        pb = []
        hooks = head_b_hooks(j + ks[0], b_segs, pb, last)
        dots = []

        def hook(key, fn):
            hooks.setdefault(key, []).append(fn)

        def direct(i, hh, seg0, tref):
            p = []

            def run():
                m = row_max(st["s", hh])
                p.extend(prob(col(st["s", hh], T), m) for T in range(4))
                l = part_sum(p)
                set_state(i, (S_INVA, S_LB)[hh], l if hh else inv_sum(l))

            def put(T, half):
                def go(clk):
                    tick(pT[4 * hh + T], 8, clk)
                    put_p(hh, T, p[T], range(4 * half, 4 * half + 4))
                return go
            hook(("dot", len(dots)), run)
            dots.extend(x_dots(i, hh, xrows[hh], lambda T: p[T], tref))
            hooks["need", seg0] = len(dots)
            for n in range(8):
                hook(("seg", seg0 + n), put(n // 2, n % 2))

        def wo_of(n):
            return [o_dot(j + reds[n], b, st, lambda b=b: outs[n][b], lref)
                    for b in range(3) if b not in kept(n)]

        def wq_of(n):
            nq = j + qn[n]
            return q_dots(nq if isinstance(nq, int) else jnp.minimum(nq, NP - 1), st, qs[qn[n] % 2])

        if last:
            dots += late_dots(st)[:NLATE] + x_dots(NP - 1, 0, xrows[0], parked(NP - 1, S_PA), lref)

            def park_acc(G, a4):
                for n in range(4):
                    ku[(NP - 1) * GP + 2, _vr(2 * (G - 16) + n), :] = pltpu.bitcast(a4[n], u32)
            hooks["end", 0] = park_acc
        for n, k in enumerate(ks if not last else []):
            q = qs[(k + 1) % 2]
            dots += k_dots(j + (k + 1), 0, st, q, MIX if n else MIXA, NALT if n else 0)
            if n == 0:
                if xrows[1]:
                    hooks["after", len(dots)] = b_segs[3]
                dots += x_dots(j + ks[0], 1, xrows[1], lambda T: pb[T], q)
            else:
                direct(j + k, 1, 48 * n + BD_SEG, q)
            kb = k_dots(j + (k + 1), 1, st, q, MIX)
            if n < len(ks) - 1:
                dots += kb[:XA_AT]
                direct(j + (k + 1), 0, 48 * n + AD_SEG, q)
                dots += kb[XA_AT:] + wq_of(n) + wo_of(n)
            else:
                hooks["need", 48 * n + a_seg] = len(dots)
                tail_hooks(j + (k + 1), st, hooks, 48 * n + a_seg)
                dots += kb
                hook(("dot", len(dots)), lambda k=k: stash_b(j + (k + 1), st["s", 1]))
                for m in range(n, len(qn)):
                    dots += wq_of(m)
                for m in range(n, len(reds)):
                    dots += wo_of(m)
                dots += x_dots(j + ks[0], 0, xrows[0],
                               parked(j + ks[0], S_PA), lref)
        run_block([j + k for k in ks], xrows, dots, hooks,
                  PLANS[name], range(NSPLIT) if last else None)
        if last:
            keep()
        if reds:
            abuf[...] += st["acc"]

    def body2(n, carry):
        block("body", 2 * n, [2, 3], [0, 1], [5, 6], XROWS)
        return carry

    zero = zs[0]
    lax.fori_loop(0, NP // 2 - 2, body2, 0)
    pl.when(zero == 0)(lambda: block("third", 0, [NP - 2], [NP - 4, NP - 3], [], XROWS))
    pl.when(zero <= 0)(lambda: block("last", 0, [NP - 1], [NP - 2], [], XROWS_LAST))

    new_block()
    st = {"acc": abuf[...]}
    invb = get_state(NP - 1, S_LB)
    o = reduce_o([ku[(NP - 1) * GP + b] for b in range(2)], get_state(NP - 1, S_INVA), invb,
                 (get_state(NP - 1, S_X), None))
    part = [None] * 5

    def finish(G, a4):
        for k in range(4):
            tick(lref, L_DUMMY + k, a4[k])
        z = lref[_vr(5), :]
        project(G, [pltpu.bitcast(v, u32) | z for v in a4])

    def project(G, a4):
        for n in range(4):
            v = jnp.sum(pltpu.bitcast(a4[n], f32), axis=1, keepdims=True)
            for nt in range(5):
                w = wou[(NP - 1) * (GP // 2) + G + n // 2, nt]
                t = pltpu.bitcast(w & jnp.uint32(HI) if n % 2 else w << 16, f32) * v
                part[nt] = t if part[nt] is None else part[nt] + t

    for G in range(16, NSPLIT // 2, 2):
        project(G, [ku[(NP - 1) * GP + 2, _vr(2 * (G - 16) + n), :] for n in range(4)])
    dots = late_dots(st)[NLATE:] + [o_dot(NP - 1, b, st, lambda b=b: o[b], lref)
                                    for b in range(2)]
    run_block([NP - 1], XROWS_LAST, dots, {("end", 0): finish},
              PLANS["final"], range(NSPLIT, 48))
    x = row_sum(st["acc"] + jnp.concatenate([v * invb for v in part], axis=1))

    xl = _rows16(x, ones)
    d = xl[0:8].astype(f32) - mean
    md = _mean(d)
    r1 = lax.rsqrt(jnp.maximum(_mean(d * d) - md * md, 0.0) + EPS)
    mean = mean + md
    y = (d - md) * r1
    my = _mean(y)
    r2 = lax.rsqrt(jnp.maximum(_mean(y * y) - my * my, 0.0) + EPS)
    h = jnp.dot(xl, w3[...], preferred_element_type=f32)
    h = h[0:8] * (r1 * r2) - h[8:16] * ((mean * r1 + my) * r2)
    h = jax.nn.gelu(h, approximate=True).astype(bf16)
    x = x + y
    parts = []
    for k in range(0, W4_VPU, 128):
        hk = jnp.broadcast_to(h[0:1, k:k + 128].astype(f32), (128, 128)).T
        t = w4[k:k + 128, :].astype(f32) * jnp.concatenate([hk] * 5, axis=1)
        parts.append(jnp.sum(t.reshape(16, 8, D), axis=0))
    for k in range(W4_VPU, F, 128):
        if k == W4_AT:
            x = x + row_sum(sum(parts[1:], parts[0]))
        x = x + jnp.dot(h[:, k:k + 128], w4[k:k + 128, :], preferred_element_type=f32)
    o_ref[...] = x[0:1].astype(o_ref.dtype)


def _cache_view(c):
    s = c.shape[2]
    c = jnp.transpose(c, (0, 1, 3, 2)).reshape(H * DH // 8, 8, s // 128, 128)
    return jnp.transpose(c, (0, 2, 1, 3)).reshape(H * DH // 8, s // 128 * 8, 128)


def _weight_view(w):
    k, n = w.shape
    w = jnp.transpose(w.reshape(k // 16, 2, 8, n // 128, 128), (0, 1, 3, 2, 4))
    return w.reshape(k // 16, n // 128, 16, 128)


@jax.jit
def pallas_interleave_layers__sliding_block_cached__mixer_s_mlp__decode_kernel(
    A_x: jax.Array,
    A_k_cache: jax.Array,
    A_v_cache: jax.Array,
    A_wq: jax.Array,
    A_wo: jax.Array,
    B_x: jax.Array,
    B_w1: jax.Array,
    B_w2: jax.Array,
    B_w3: jax.Array,
    B_w4: jax.Array,
):
    sk = A_k_cache.shape[2]
    win = min(4096, max(256, sk // 4))
    assert win == 4096 and sk % 128 == 0
    assert A_x.shape == (1, 1, D) and A_k_cache.shape == (1, H, sk, DH)
    wt = win // 128
    t0 = sk // 128 - wt
    ng = H * DH // 8
    hbm = pl.BlockSpec(memory_space=pl.ANY)
    out = pl.pallas_call(
        functools.partial(_kernel, t0=t0, wt=wt),
        out_shape=jax.ShapeDtypeStruct((1, D), A_x.dtype),
        in_specs=[hbm] * 7,
        out_specs=pl.BlockSpec(memory_space=pltpu.VMEM),
        scratch_shapes=[
            pltpu.VMEM((ng, wt * 8, 128), bf16),
            pltpu.VMEM((ng, wt * 8, 128), bf16),
            pltpu.VMEM((ng // 4, 128, 128), u32),
            pltpu.VMEM((NP * D // 16, 3, 8, 128), u32),
            pltpu.VMEM((H * DH // 16, D // 128, 16, 128), bf16),
            pltpu.VMEM((D, F), bf16),
            pltpu.VMEM((F, D), bf16),
            pltpu.VMEM((1, D), bf16),
            pltpu.VMEM((144, 128), u32),
            pltpu.VMEM((384, 128), u32),
            pltpu.VMEM((144, 128), u32),
            pltpu.VMEM((144, 128), u32),
            pltpu.VMEM((144, 128), u32),
            pltpu.VMEM((40, 128), f32),
            pltpu.VMEM((8, D), f32),
            pltpu.SMEM((1,), jnp.int32),
        ] + [pltpu.VMEM((64, 128), u32)] * 3
        + [pltpu.VMEM((72, 128), f32)] * 8,
        compiler_params=pltpu.CompilerParams(vmem_limit_bytes=128 * 1024 * 1024),
    )(A_x.reshape(1, D), _cache_view(A_k_cache), _cache_view(A_v_cache),
      _weight_view(A_wq).reshape(H * DH // 16, D // 128, 16, 128), _weight_view(A_wo), B_w3, B_w4)
    return out.reshape(1, 1, D)
```

```python
import functools

import jax
import jax.numpy as jnp
from jax import lax
import jax.experimental.pallas as pl
import jax.experimental.pallas.tpu as pltpu

D = 640
H = 32
DH = 192
F = 1536
EPS = 1e-5
NP = H // 2
GP = 2 * DH // 8
HI = 0xFFFF0000
CEXP = DH ** -0.5 * 1.4426950408889634

f32 = jnp.float32
bf16 = jnp.bfloat16
u32 = jnp.uint32

L_Y = 0
L_DUMMY = 6
S_MAXB, S_LB, S_INVA, S_X, S_PA, S_PB = 4, 5, 6, 7, 9, 13
XROWS = ((2, 10, 18, 26), (4, 12, 20))
XROWS_LAST = ((2, 10, 18, 26, 6, 14, 22, 30, 4, 12, 20, 28), ())
GX = (0, 16)
PLANS = {
    "first": (
        {},
        (21, 22, 22, 23, 24, 23, 26, 27, 26, 27, 28, 28, 29, 29, 30, 31, 32, 31, 33, 34, 34, 35,
        36, 36, 37, 38, 38, 39, 40, 40, 41, 42, 42, 43, 44, 44, 45, 46, 46, 47, 48, 48, 49, 49,
        50, 51, 51, 53, 51, 52, 54, 55, 54, 55, 56, 56, 57, 58, 58, 59, 60, 59, 60, 62, 62, 63,
        64, 64, 65, 66, 66, 67, 68, 68, 69, 70, 70, 71, 72, 71, 73, 74, 74, 75, 76, 72, 77, 78,
        77, 79, 80, 81, 82, 82, 81, 76)),
    "body": (
        {1: 0, 3: 2, 5: 4, 7: 4, 9: 5, 11: 8, 14: 10, 15: 13, 19: 14, 21: 14, 23: 16, 25: 17,
        27: 19, 29: 22, 31: 23, 33: 23, 35: 26, 37: 26, 39: 28, 40: 33, 41: 33, 43: 34, 47: 34,
        49: 35, 51: 37, 53: 38, 55: 39, 57: 40, 59: 42, 61: 43, 63: 48, 67: 50, 70: 51, 71: 52,
        72: 53, 75: 55, 77: 56, 79: 58, 81: 59, 83: 61, 84: 62},
        (0, 0, 0, 0, 0, 0, 0, 0, 0, 0, 0, 1, 2, 2, 3, 4, 4, 5, 6, 7, 7, 8, 9, 10, 10, 12, 12,
        13, 14, 15, 15, 16, 16, 17, 17, 18, 20, 21, 21, 24, 24, 24, 21, 22, 26, 30, 24, 25, 23,
        26, 27, 29, 29, 30, 31, 31, 33, 34, 35, 36, 36, 34, 34, 37, 37, 39, 43, 42, 40, 37, 41,
        41, 43, 46, 46, 45, 46, 47, 47, 49, 50, 51, 50, 51, 52, 57, 56, 58, 57, 59, 61, 60, 62,
        62, 63, 63)),
    "third": (
        {1: 0, 3: 3, 5: 3, 6: 3, 7: 4, 9: 5, 11: 8, 15: 11, 19: 14, 21: 14, 23: 15, 25: 17,
        26: 18, 27: 19, 30: 21},
        (0, 0, 0, 0, 0, 0, 0, 0, 0, 0, 0, 0, 0, 2, 2, 4, 3, 4, 3, 10, 9, 10, 12, 13, 12, 13, 13,
        12, 14, 17, 15, 16, 17, 17, 18, 19, 20, 18, 21, 22, 22, 24, 25, 26, 24, 25, 25, 27)),
    "last": (
        {1: 0, 3: 1, 5: 1, 7: 2, 11: 3, 15: 4, 17: 6, 19: 7, 21: 9, 23: 10, 26: 12},
        (0, 0, 0, 0, 0, 1, 1, 0, 0, 0, 0, 0, 0, 0, 0, 0, 1, 1, 0, 1, 2, 8, 5, 5, 6, 7, 10, 5, 8,
        8, 9, 10, 11, 11, 12, 10)),
    "final": (
        {37: 0, 39: 1, 40: 4, 43: 4, 45: 6},
        (0, 0, 0, 0, 0, 0, 0, 0, 0, 0, 0, 0, 0, 0, 0, 0, 0, 0, 0, 0, 0, 0, 0, 0, 0, 0, 0, 0, 0,
        0, 0, 0, 0, 0, 0, 0, 0, 0, 0, 0, 0, 0, 6, 3, 1, 2, 0, 0)),
}
MIX = (0, 1, 8, 2, 3, 9, 4, 5, 10, 6, 7, 11)
MIXA = (0, 1, 2, 3, 4, 8, 5, 9, 6, 10, 7, 11)
NLATE = 12
NSPLIT = 36
W4_VPU = 256
W4_AT = 896
B_SEGS = (9, 12, 15, 18)
B_SEGL = 8
DA0 = 17
DW0 = 32
DB0 = 44
DA1 = 57
DB1 = 68
DQ = (26, 29, 33)
NQV = 3
B0_SEG = 20
A1_SEG = 39
B1_SEG = 12
A2_SEG = 38
A_SEG0 = 40
A_SEG3 = 40
B_SEGS3 = (9, 11, 15, 19)
XA_AT = 8
AD_SEG = 32
BD_SEG = 12
NALT = 2
W4_CHUNKS = (1024, 256, 160, 64, 32)
W4_MXU = 1280


def _mean(x):
    return jnp.mean(x, axis=-1, keepdims=True)


def _ln(x):
    c = x - _mean(x)
    return c * lax.rsqrt(_mean(c * c) + EPS)


def _wtile(wu, rows, nt):
    blk = wu[rows, nt]
    return pltpu.bitcast(blk.reshape(blk.shape[0] * 8, 128), bf16)


def _wcols(wu, rows, nts):
    return jnp.concatenate([_wtile(wu, rows, n) for n in nts], axis=1)


def _rows16(a, b):
    return jnp.concatenate([a, b], axis=0).astype(bf16)


def _slot(G, t):
    j = 4 * (t >> 3) + ((((t >> 1) & 3) + G + 2 * (t & 1) + (t >> 3)) & 3)
    return 2 * G + (t & 1), 8 * j


def _xslot(G, t):
    return G // 2, 8 * (4 * (t >> 3) + ((((t >> 1) & 3) + G + (t >> 3)) & 3))


def _vr(n):
    return slice(8 * n, 8 * n + 8)


def _kernel(*refs, t0, wt):
    pl.run_scoped(functools.partial(_body, refs, t0, wt),
                  pltpu.SemaphoreType.DMA((4 + len(W4_CHUNKS) + 2 * NP,)))


def _body(refs, t0, wt, sems):
    (x_hbm, k_hbm, v_hbm, wq_hbm, wo_hbm, w3_hbm, w4_hbm, o_ref,
     kbuf, vbuf, vx, wqu, wo, w3, w4, xbuf, lref, obuf, qa, qb, qx, scl, abuf, zs) = refs[:24]
    qt, pT = refs[24:27], refs[27:]
    ku = kbuf.bitcast(u32)
    vu = vbuf.bitcast(u32)
    wou = wo.bitcast(u32)

    x_cp = pltpu.make_async_copy(x_hbm, xbuf, sems.at[0])
    wq_cp = pltpu.make_async_copy(wq_hbm, wo, sems.at[1])
    wo_cp = pltpu.make_async_copy(wo_hbm, wo, sems.at[2])
    w3_cp = pltpu.make_async_copy(w3_hbm, w3, sems.at[3])
    w4_rows, r0 = [], 0
    for n in W4_CHUNKS:
        w4_rows.append((r0, r0 + n))
        r0 += n
    w4_cp = [pltpu.make_async_copy(w4_hbm.at[a:b], w4.at[a:b], sems.at[4 + c])
             for c, (a, b) in enumerate(w4_rows)]
    S0 = 4 + len(W4_CHUNKS)

    def k_cp(i):
        return pltpu.make_async_copy(
            k_hbm.at[pl.ds(i * GP, GP), pl.ds(t0 * 8, wt * 8), :],
            kbuf.at[pl.ds(i * GP, GP)], sems.at[S0 + i])

    def v_cp(i):
        return pltpu.make_async_copy(
            v_hbm.at[pl.ds(i * GP, GP), pl.ds(t0 * 8, wt * 8), :],
            vbuf.at[pl.ds(i * GP, GP)], sems.at[S0 + NP + i])

    for c in (wq_cp, x_cp, k_cp(0), v_cp(0)):
        c.start()

    zs[0] = 0
    for ref in (qa, qb, qx, lref):
        ref[_vr(5), :] = jnp.zeros((8, 128), u32)

    lane = lax.broadcasted_iota(jnp.int32, (8, 128), 1)
    sub = lax.broadcasted_iota(jnp.int32, (8, 128), 0)
    lane_lo = lane < 64
    sub_lo = sub < 4

    def pair_view(buf, i):
        return buf.at[pl.ds(i * GP, GP)].bitcast(u32)

    def tile(ref, g0, G, t):
        g, r = _slot(G, t)
        return ref[g0 + g, r:r + 8, :]

    def group_view(buf, c):
        return buf.at[pl.ds(8 * c, 8)].bitcast(u32)

    def retile(buf, i, expand):
        def body(c, carry):
            ref = group_view(buf, 6 * i + c)
            hi = vx.at[pl.ds(2 * (6 * i + c), 2)]
            for G in range(4):
                for J in range(4):
                    xs = [[ref[2 * G + e, _vr(4 * J + jj), :] for jj in range(4)]
                          for e in range(2)]
                    for jj in range(4):
                        x0, x1 = xs[0][jj], xs[1][jj]
                        ys = (jnp.where(sub_lo, x0, pltpu.roll(x1, 4, 0)),
                              jnp.where(sub_lo, pltpu.roll(x0, 4, 0), x1))
                        for e in range(2):
                            t = 8 * J + 2 * jj + e
                            g, r = _slot(G, t)
                            if expand and G % 2 and e:
                                ref[g, r:r + 8, :] = ys[e] << 16
                                g, r = _xslot(G, t)
                                hi[g, r:r + 8, :] = ys[e] & jnp.uint32(HI)
                            else:
                                ref[g, r:r + 8, :] = ys[e]
            return carry
        lax.fori_loop(0, GP // 8, body, 0)

    def merge_halves(get, nt, n):
        lo, hi = get(n // 2), get((nt + n) // 2)
        if n % 2:
            lo = pltpu.roll(lo, 4, 0)
        if (nt + n) % 2 == 0:
            hi = pltpu.roll(hi, 4, 0)
        return jnp.where(sub_lo, lo, hi)

    def retile_wq(c, carry):
        for G in range(5):
            for n in range(3 * NP):
                wqu[n // 3 * (D // 16) + 5 * c + G, n % 3] = merge_halves(
                    lambda v: wou[48 * c + (48 * G + v) // 5, (48 * G + v) % 5], 3 * NP, n)
        return carry

    def retile_wo(c, carry):
        for G in range(8):
            xs = [wou[8 * c + G, n] for n in range(5)]
            for n in range(5):
                wou[8 * c + G, n] = merge_halves(lambda v: xs[v], 5, n)
        return carry

    def lhs_at(ref, n):
        return pltpu.bitcast(ref[_vr(n), :], bf16)

    cur = [None]

    def new_block():
        cur[0] = -32 * jnp.clip(zs[0], 0, 1)

    def tick(ref, n, val):
        assert 4 <= n < ref.shape[0] // 8
        if val.dtype != ref.dtype:
            val = pltpu.bitcast(val, ref.dtype)
        ref[pl.ds(pl.multiple_of(cur[0] + 8 * n, 8), 8), :] = val

    def put_q(q, qref):
        qq = pltpu.bitcast(q.astype(bf16).astype(f32), u32)
        q0, q1, q2 = qq[:, 0:128], qq[:, 128:256], qq[:, 256:384]
        for n, v in enumerate((q0 >> 16, q0, q2 >> 16, q2, q1)):
            qref[_vr(n), :] = v
            if n < 2 and qref is qb:
                qx[_vr(n), :] = v

    def transpose_wq(i):
        for k in range(5):
            for n in range(3):
                rows = pl.ds(i * (D // 16) + 8 * k, 8)
                w = pltpu.bitcast(_wtile(wqu, rows, n).astype(f32).T, u32)
                for G in range(8):
                    wqu[i * (D // 16) + 8 * k + G, n] = (w[_vr(2 * G), :] >> 16) | w[_vr(2 * G + 1), :]

    def q_vpu(i, c, qref):
        cols = []
        for n in range(3):
            acc = []
            for G in range(8):
                ws = [wqu[i * (D // 16) + 8 * k + G, n] for k in range(5)]
                for half in (lambda w: w << 16, lambda w: w & jnp.uint32(HI)):
                    t = [pltpu.bitcast(half(ws[k]), f32) * col(c, k) for k in range(5)]
                    acc.append((t[0] + t[1]) + (t[2] + t[3]) + t[4])
            z = jnp.sum(jnp.concatenate(acc, axis=0).T.reshape(16, 8, 128), axis=0)
            cols.append(row_sum(z))
        put_q(jnp.concatenate(cols, axis=1), qref)
        return cols[0] + cols[1] + cols[2]

    def row_sum(a):
        return jnp.broadcast_to(jnp.sum(a, axis=0, keepdims=True), a.shape)

    def q_dots(i, st, qref, lhs=None, mean=None):
        def step(k):
            def run(tied=False):
                w = _wcols(wqu, pl.ds(i * (D // 16) + 8 * k, 8), range(3))
                if lhs is None:
                    r = jnp.dot(lhs_at(lref, L_Y + k), w, preferred_element_type=f32)[0:8]
                else:
                    r = jnp.dot(lhs[:, 128 * k:128 * k + 128], w, preferred_element_type=f32)
                st["q"] = r if k == 0 else st["q"] + r
                if k == 4:
                    q = st["q"] if lhs is None else st["q"][0:8] - mean * st["q"][8:16]
                    put_q(q, qref)
                return r[0:8, 256:384]
            return 3, lref, L_DUMMY, run
        return [step(k) for k in range(5)]

    def as_lhs(v, tref):
        if v.dtype == f32 and tref is None:
            return v.astype(bf16)
        if v.dtype == f32:
            v = pltpu.bitcast(_rows16(v, v), u32)
        return pltpu.bitcast(v if tref is None else v | tref[_vr(5), :], bf16)

    def o_dot(i, b, st, get_lhs, tref=None):
        def run(tied=False):
            w = _wcols(wou, pl.ds(i * (GP // 2) + 8 * b, 8), range(5))
            lhs = as_lhs(get_lhs(), tref if tied and tref is not obuf else None)
            r = jnp.dot(lhs, w, preferred_element_type=f32)[0:8]
            st["acc"] = st["acc"] + r if "acc" in st else r
            return r[:, 512:640]
        return 5, tref, (32 if tref is obuf else 6), run

    def mid_q(st, qref):
        q1 = qref[_vr(4), :]
        q1r = pltpu.roll(q1, 64, 1)
        st["u", 0, id(qref)] = jnp.where(lane_lo, q1 >> 16, q1r)
        st["u", 1, id(qref)] = jnp.where(lane_lo, q1r >> 16, q1)

    def k_dots(i, hh, st, qref, order=tuple(range(12)), nalt=0):
        kv = pair_view(kbuf, i)
        gf, gh = ((0, 8), (16, 12))[hh]

        def step(r):
            src = qx if r in order[:nalt] else qref

            def run(tied=False):
                if r < 8:
                    cols = [[tile(kv, 0, gf + G, 8 * T + r) for G in range(8)] for T in range(4)]
                    base, row = src[_vr(2 * hh + r % 2), :], r // 2
                else:
                    cols = [[tile(kv, 0, gh + G % 4, 8 * T + 2 * (r - 8) + G // 4)
                             for G in range(8)] for T in range(4)]
                    if ("u", hh, id(qref)) not in st:
                        mid_q(st, qref)
                    base, row = st["u", hh, id(qref)], r - 8
                    if tied:
                        base = base | src[_vr(5), :]
                lhs = jnp.where(sub == row, base, jnp.zeros((8, 128), u32))
                w = jnp.concatenate([jnp.concatenate(c, axis=0) for c in cols], axis=1)
                res = jnp.dot(pltpu.bitcast(lhs, bf16), pltpu.bitcast(w, bf16),
                              preferred_element_type=f32)[0:8]
                st["s", hh] = res if r == order[0] else st["s", hh] + res
                return res[:, 384:512]
            return 4, src, 6, run
        return [step(r) for r in order]

    def col(s, T):
        return s[:, 128 * T:128 * T + 128]

    def row_max(s):
        m = jnp.maximum(jnp.maximum(col(s, 0), col(s, 1)), jnp.maximum(col(s, 2), col(s, 3)))
        return jnp.max(jnp.max(m, axis=1, keepdims=True), axis=0, keepdims=True)

    def prob(s, m):
        return jnp.exp2((s - m) * scl[_vr(0), :])

    def put_p(hh, T, p, ks=range(8)):
        for k in ks:
            pT[4 * hh + T][pl.ds(k, 8, stride=8), :] = p

    def part_sum(p):
        return (p[0] + p[1]) + (p[2] + p[3])

    def inv_sum(l):
        l = jnp.sum(jnp.sum(l, axis=1, keepdims=True), axis=0, keepdims=True)
        r = pl.reciprocal(l, approx=True)
        return jnp.broadcast_to(r * (2.0 - l * r), (8, 128))

    def softmax(s, hh):
        m = row_max(s)
        p = [prob(col(s, T), m) for T in range(4)]
        for T in range(4):
            put_p(hh, T, p[T])
        return p, part_sum(p)

    def get_state(i, n):
        return pltpu.bitcast(ku[i * GP + 3, _vr(n), :], f32)

    def set_state(i, n, v):
        ku[i * GP + 3, _vr(n), :] = pltpu.bitcast(v, u32)

    def stash_b(i, s):
        for T in range(4):
            set_state(i, T, col(s, T))
        m = jnp.broadcast_to(row_max(s), (8, 128))
        set_state(i, S_MAXB, m)
        return m

    def pack8(v):
        return pltpu.bitcast(v.astype(bf16), u32)

    def park_p(i, n, p):
        ku[i * GP + 3, 8 * n:8 * n + 4, :] = pack8(p)

    def parked(i, n):
        return lambda T: ku[i * GP + 3, _vr(n + T), :]

    def x_dots(i, hh, ts, get_lhs, tref=None):
        st = {}
        rows = sorted({t % 8 for t in ts})

        def step(n, rho):
            def run(tied=False):
                res = []
                for T in [t // 8 for t in ts if t % 8 == rho]:
                    w = jnp.concatenate(
                        [tile(vu, i * GP, GX[hh] + G, 8 * T + rho) for G in range(8)], axis=0)
                    lhs = as_lhs(get_lhs(T), tref if tied else None)
                    res.append(jnp.dot(lhs, pltpu.bitcast(w, bf16),
                                       preferred_element_type=f32)[0:8])
                st["x"] = jnp.where(sub == rho, sum(res[1:], res[0]), st["x"] if n else 0.0)
                if n == len(rows) - 1:
                    set_state(i, S_X + hh, st["x"])
                return res[-1]
            return sum(1 for t in ts if t % 8 == rho), tref, 6, run
        return [step(n, rho) for n, rho in enumerate(rows)]

    def transpose_x(view, xrows):
        for hh in range(2):
            for t in xrows[hh]:
                w = jnp.concatenate([tile(view, 0, GX[hh] + G, t) for G in range(8)], axis=0)
                w = pltpu.bitcast(pltpu.bitcast(w, bf16).astype(f32).T.astype(bf16), u32)
                for G in range(8):
                    g, r = _slot(GX[hh] + G, t)
                    view[g, r:r + 8, :] = w[_vr(G), :]

    def reduce_o(blocks, inva, invb, extra=(None, None, None)):
        out = []
        for b, inv in enumerate((inva, jnp.where(lane_lo, inva, invb), invb)[:len(blocks)]):
            z = jnp.sum(pltpu.bitcast(blocks[b], f32).T.reshape(16, 8, 128), axis=0)
            if extra[b] is not None:
                z = z + extra[b]
            out.append(z * inv)
        return out

    def mac(acc, n, views, G, t, pv):
        w = tile(views[0], 0, G, t)
        if G % 2 and t % 2:
            g, r = _xslot(G, t)
            halves = (w, views[1][g, r:r + 8, :])
        else:
            halves = (w << 16, w & jnp.uint32(HI))
        for k in range(2):
            a = pltpu.bitcast(halves[k], f32) * pv
            acc[n + k] = a if acc[n + k] is None else acc[n + k] + a

    def seg_rows(xrows, seg):
        hh, gp, T = seg // 24 % 2, seg % 24 // 4, seg % 4
        on_mxu = GX[hh] <= 12 * hh + 2 * gp < GX[hh] + 8
        return [rho for rho in range(8) if not (on_mxu and 8 * T + rho in xrows[hh])]

    def run_block(pairs, xrows, dots, hooks, plan, segs=None):
        tie, clk = plan
        clock = []

        def emit(upto):
            while len(clock) < upto:
                n = len(clock)
                for h in hooks.get(("dot", n), ()):
                    h()
                clock.append(dots[n][3](n in tie.values()))

        zero = jnp.zeros((8, 128), f32)
        views = [(pair_view(vbuf, i), vx.at[pl.ds(i * (GP // 4), GP // 4)]) for i in pairs]
        used = {}
        for seg in segs or range(48 * len(pairs)):
            i, hh, gp, T = pairs[seg // 48], seg // 24 % 2, seg % 24 // 4, seg % 4
            if T == 0:
                a4 = [None] * 4
            pref = pT[4 * hh + T]
            upto = min([v for k, v in tie.items() if k >= seg]
                       + [k[1] for k, v in hooks.items() if k[0] == "after" and v >= seg]
                       + [len(dots) if tie else clk[seg] + 6])
            free = not any(k in tie for k in range(seg, seg - T + 4))
            if free or ("seg", seg) in hooks:
                upto = max(upto, clk[seg] + 1)
            emit(min(len(dots), max(upto, hooks.get(("need", seg), 0))))
            if free:
                tick(pref, 8, clock[clk[seg]])
            elif gp:
                tick(pref, 8, zero)
            for h in hooks.get(("seg", seg), ()):
                h(clock[clk[seg]])
            for rho in seg_rows(xrows, seg):
                pv = pref[_vr(rho), :]
                for e in range(2):
                    mac(a4, 2 * e, views[seg // 48], 12 * hh + 2 * gp + e, 8 * T + rho, pv)
            if seg in tie:
                ref, slot = dots[tie[seg]][1:3]
                used[tie[seg]] = used.get(tie[seg], -1) + 1
                for k in range(4):
                    tick(ref, slot + 4 * used[tie[seg]] + k, a4[k])
            if T == 3 and ("end", 0) in hooks and seg >= 32:
                hooks["end", 0](12 * hh + 2 * gp, a4)
            elif T == 3:
                for n in range(4):
                    G = 12 * hh + 2 * gp + n // 2
                    v = a4[n] * hooks["scale", seg // 24]() if ("scale", seg // 24) in hooks else a4[n]
                    ku[i * GP + G // 8, pl.ds(16 * (G % 8) + n % 2, 8, stride=2), :] = (
                        pltpu.bitcast(v, u32))
        emit(len(dots))

    def run_all(dots):
        for d in dots:
            d[3]()

    def set_input(c, scale):
        cp = pltpu.bitcast(_rows16(c, c), u32)
        for k in range(5):
            lref[_vr(L_Y + k), :] = cp[:, 128 * k:128 * k + 128]
        scl[_vr(0), :] = jnp.broadcast_to(scale, (8, 128))

    x_cp.wait()
    x = jnp.broadcast_to(xbuf[...].astype(f32), (8, D))
    set_input(_ln(x), jnp.full((8, 1), CEXP, f32))
    wq_cp.wait()
    lax.fori_loop(0, D // 80, retile_wq, 0)
    wo_cp.start()
    for i in range(1, NP):
        k_cp(i).start()
        v_cp(i).start()
    for c in [w3_cp] + w4_cp:
        c.start()
    wo_cp.wait()
    lax.fori_loop(0, H * DH // 128, retile_wo, 0)

    def body1(i, acc):
        st = {"acc": acc}
        k_cp(i).wait()
        retile(kbuf, i, False)
        run_all(q_dots(i, st, qa))
        inv = []
        for hh in range(2):
            run_all(k_dots(i, hh, st, qa))
            inv.append(inv_sum(softmax(st["s", hh], hh)[1]))

        @pl.when(i > 0)
        def _():
            transpose_x(pair_view(vbuf, i - 1), XROWS)

        @pl.when(jnp.logical_and(i >= 5 - NQV, i < 5))
        def _():
            transpose_wq(i)

        v_cp(i).wait()
        retile(vbuf, i, True)
        for hh in range(2):
            def pv_step(c, carry, hh=hh):
                acc8 = [None] * 8
                views = (group_view(vbuf, 6 * i + c), vx.at[pl.ds(2 * (6 * i + c), 2)])
                for t in range(32):
                    pv = pT[4 * hh + t // 8][_vr(t % 8), :]
                    for G in range(4):
                        mac(acc8, 2 * G, views, G, t, pv)
                for n in range(8):
                    obuf[pl.ds(64 * c + 16 * (n // 2) + n % 2, 8, stride=2), :] = (
                        pltpu.bitcast(acc8[n], u32))
                return carry
            lax.fori_loop(3 * hh, 3 * hh + 3, pv_step, 0)
        o = reduce_o([obuf[128 * b:128 * b + 128, :] for b in range(3)], inv[0], inv[1])
        run_all([o_dot(i, b, st, lambda b=b: o[b]) for b in range(3)])
        return st["acc"]

    x = x + row_sum(lax.fori_loop(0, NP, body1, jnp.zeros((8, D), f32)))

    y = _ln(x)
    zz = _ln(y).astype(bf16)
    w3_cp.wait()
    h = jnp.dot(zz, w3[...], preferred_element_type=f32)
    h = jax.nn.gelu(h, approximate=True).astype(bf16)
    x = x + y
    transpose_x(pair_view(vbuf, NP - 1), XROWS_LAST)
    for k in range(W4_MXU, F, 128):
        hk = jnp.broadcast_to(h[0:1, k:k + 128].astype(f32), (128, 128))
        obuf[k - W4_MXU:k - W4_MXU + 128, :] = pltpu.bitcast(hk.T, u32)
    part = jnp.zeros((8, D), f32)
    for cp, (a, b) in zip(w4_cp, w4_rows):
        cp.wait()
        if a < W4_MXU:
            x = x + jnp.dot(h[:, a:b], w4[a:b, :], preferred_element_type=f32)
        else:
            for k in range(a, b, 16):
                hk = pltpu.bitcast(obuf[k - W4_MXU:k - W4_MXU + 16, :], f32)
                t = w4[k:k + 16, :].astype(f32) * jnp.concatenate([hk] * 5, axis=1)
                part = part + (t[0:8] + t[8:16])
    x = x + row_sum(part)

    ones = jnp.ones((8, D), f32)
    xl = _rows16(x, ones)
    xb = xl[0:8].astype(f32)
    mean = _mean(xb)
    c = xb - mean
    set_input(c, lax.rsqrt(_mean(c * c) + EPS) * CEXP)
    abuf[...] = jnp.where(lax.broadcasted_iota(jnp.int32, (8, D), 0) == 0, x, 0.0)

    def tail_hooks(i, st, hooks, seg0):
        def first(_):
            m = row_max(st["s", 0])
            st["pa"] = [prob(col(st["s", 0], T), m) for T in range(4)]
            set_state(i, S_INVA, inv_sum(part_sum(st["pa"])))
            for T in range(4):
                park_p(i, S_PA + T, st["pa"][T])

        def put(T, half):
            def run(clk):
                tick(pT[T], 8, clk)
                put_p(0, T, st["pa"][T], range(4 * half, 4 * half + 4))
            return run
        hooks.setdefault(("seg", seg0), []).append(first)
        for n in range(8):
            hooks.setdefault(("seg", seg0 + n), []).append(put(n // 2, n % 2))

    def head_b_hooks(i, segs, pb, final=False, park=False):
        def put_b(T):
            def run(clk):
                tick(scl, 4, clk)
                pb.append(prob(get_state(i, T), get_state(i, S_MAXB)))
                put_p(1, T, pb[T])
                if park and T < 3:
                    park_p(i, S_PB + T, pb[T])
                if T == 3:
                    set_state(i, S_LB, inv_sum(part_sum(pb)) if final else part_sum(pb))
            return run
        return {("seg", segs[T]): [put_b(T)] for T in range(4)}

    def reduce_pair(i):
        xa, xb = get_state(i, S_X), get_state(i, S_X + 1)
        invb = inv_sum(get_state(i, S_LB))
        return reduce_o([ku[i * GP + b] for b in range(3)],
                        get_state(i, S_INVA), invb, (xa, None, xb))

    st = {}
    new_block()
    late = tuple(range(8, 12)) + tuple(range(8))
    q0, q1, q2 = qt
    dots = q_dots(0, st, q0, xl, mean) + q_dots(1, st, q1, xl, mean) \
        + k_dots(0, 0, st, q0) + k_dots(0, 1, st, q0, late) + k_dots(1, 0, st, q1, late) \
        + k_dots(1, 1, st, q1, late) + k_dots(2, 0, st, q2, late) + k_dots(2, 1, st, q2)
    for n in range(4):
        dots += x_dots(n // 2, n % 2, XROWS[n % 2], parked(n // 2, (S_PA, S_PB)[n % 2]))

    def lane_softmax(h):
        i, hh = h // 2, h % 2

        def run():
            s0 = st["s", hh]
            m = jnp.maximum(jnp.maximum(col(s0, 0), col(s0, 1)),
                            jnp.maximum(col(s0, 2), col(s0, 3)))
            m = jnp.max(m, axis=0, keepdims=True)
            p = st["p", h] = [prob(col(s0, T), m) for T in range(4)]
            w = st["w", h] = prob(m, jnp.max(m, axis=1, keepdims=True))
            l = part_sum(p) * w
            set_state(i, (S_INVA, S_LB)[hh], l if hh else inv_sum(l))
            for T in range(4 - hh):
                park_p(i, (S_PA, S_PB)[hh] + T, p[T] * w)
        return run

    def put_lane(h, T):
        def run(clk):
            tick(pT[4 * (h % 2) + T], 8, clk)
            put_p(h % 2, T, st["p", h][T])
        return run

    hooks = head_b_hooks(1, range(48 + B1_SEG, 96, 3), [], park=True)
    hooks.update({("need", 0): 23, ("need", B0_SEG): 35, ("need", A1_SEG): 47,
                  ("need", 48 + B1_SEG): DB1 + 1, ("need", 48 + A2_SEG): 70,
                  ("after", 82): 48 + B1_SEG + 9})
    for n, fn in ((10, lambda: mid_q(st, q0)),
                  (DQ[0], lambda: tick(q0, 5, q_vpu(2, c, q2))),
                  (DQ[1], lambda: tick(q0, 5, q_vpu(3, c, qa))),
                  (DQ[2], lambda: tick(q0, 5, q_vpu(4, c, qb))),
                  (DA0, lambda: tick(q0, 6, scl[_vr(0), :])), (22, lane_softmax(0)),
                   (DW0, lambda: tick(q0, 7, st["w", 0])),
                  (34, lane_softmax(1)), (DB0, lambda: tick(q1, 6, st["w", 1])),
                  (46, lane_softmax(2)), (DA1, lambda: tick(q1, 6, st["w", 2])),
                  (DB1, lambda: tick(q2, 6, stash_b(1, st["s", 1]))),
                  (82, lambda: stash_b(2, st["s", 1]))):
        hooks.setdefault(("dot", n), []).append(fn)
    for h in range(3):
        hooks["scale", h] = lambda h=h: st["w", h]

    def put_first(T):
        def run(_):
            for rho in range(8):
                pT[T][_vr(rho), :] = jnp.broadcast_to(st["p", 0][T][rho:rho + 1], (8, 128))
        return run

    hooks.update({("seg", T): [put_first(T)] for T in range(4)})
    hooks.update({("seg", B0_SEG + 2 * T): [put_lane(1, T)] for T in range(4)})
    hooks.update({("seg", A1_SEG + 2 * T): [put_lane(2, T)] for T in range(4)})
    tail_hooks(2, st, hooks, 48 + A2_SEG)
    run_block([0, 1], XROWS, dots, hooks, PLANS["first"])

    qs = (qb, qa)

    def late_dots(st):
        todo = [(m, 2) for m in range(NP - 2)] + [(NP - 3, 1)] + [(NP - 2, b) for b in range(3)]
        return [o_dot(m, b, st, lambda n=m + (2 - b) * 6: obuf[_vr(n), :], obuf) for m, b in todo]

    def block(name, j, ks, reds, qn, xrows):
        last = ks == [NP - 1]
        a_seg = A_SEG3 if name == "third" else A_SEG0
        b_segs = {"third": B_SEGS3,
                  "last": range(B_SEGL, 48, 3)}.get(name, B_SEGS)
        new_block()
        st = {}
        for k in ks if not last else []:
            mid_q(st, qs[(k + 1) % 2])
        outs = [reduce_pair(j + r) for r in reds]

        def kept(n):
            return (0, 1, 2) if last else (1, 2) if reds[n] == NP - 3 else (2,)

        def keep():
            for n, r in enumerate(reds):
                for b in kept(n):
                    obuf[pl.ds(pl.multiple_of(8 * (j + r + (2 - b) * 6), 8), 4), :] = (
                        pack8(outs[n][b]))

        if not last:
            keep()
        pb = []
        hooks = head_b_hooks(j + ks[0], b_segs, pb, last)
        dots = []

        def hook(key, fn):
            hooks.setdefault(key, []).append(fn)

        def direct(i, hh, seg0, tref):
            p = []

            def run():
                m = row_max(st["s", hh])
                p.extend(prob(col(st["s", hh], T), m) for T in range(4))
                l = part_sum(p)
                set_state(i, (S_INVA, S_LB)[hh], l if hh else inv_sum(l))

            def put(T, half):
                def go(clk):
                    tick(pT[4 * hh + T], 8, clk)
                    put_p(hh, T, p[T], range(4 * half, 4 * half + 4))
                return go
            hook(("dot", len(dots)), run)
            dots.extend(x_dots(i, hh, xrows[hh], lambda T: p[T], tref))
            hooks["need", seg0] = len(dots)
            for n in range(8):
                hook(("seg", seg0 + n), put(n // 2, n % 2))

        def wo_of(n):
            return [o_dot(j + reds[n], b, st, lambda b=b: outs[n][b], lref)
                    for b in range(3) if b not in kept(n)]

        def wq_of(n):
            nq = j + qn[n]
            return q_dots(nq if isinstance(nq, int) else jnp.minimum(nq, NP - 1), st, qs[qn[n] % 2])

        if last:
            dots += late_dots(st)[:NLATE] + x_dots(NP - 1, 0, xrows[0], parked(NP - 1, S_PA), lref)

            def park_acc(G, a4):
                for n in range(4):
                    ku[(NP - 1) * GP + 2, _vr(2 * (G - 16) + n), :] = pltpu.bitcast(a4[n], u32)
            hooks["end", 0] = park_acc
        for n, k in enumerate(ks if not last else []):
            q = qs[(k + 1) % 2]
            dots += k_dots(j + (k + 1), 0, st, q, MIX if n else MIXA, NALT if n else 0)
            if n == 0:
                if xrows[1]:
                    hooks["after", len(dots)] = b_segs[3]
                dots += x_dots(j + ks[0], 1, xrows[1], lambda T: pb[T], q)
            else:
                direct(j + k, 1, 48 * n + BD_SEG, q)
            kb = k_dots(j + (k + 1), 1, st, q, MIX)
            if n < len(ks) - 1:
                dots += kb[:XA_AT]
                direct(j + (k + 1), 0, 48 * n + AD_SEG, q)
                dots += kb[XA_AT:] + wq_of(n) + wo_of(n)
            else:
                hooks["need", 48 * n + a_seg] = len(dots)
                tail_hooks(j + (k + 1), st, hooks, 48 * n + a_seg)
                dots += kb
                hook(("dot", len(dots)), lambda k=k: stash_b(j + (k + 1), st["s", 1]))
                for m in range(n, len(qn)):
                    dots += wq_of(m)
                for m in range(n, len(reds)):
                    dots += wo_of(m)
                dots += x_dots(j + ks[0], 0, xrows[0],
                               parked(j + ks[0], S_PA), lref)
        run_block([j + k for k in ks], xrows, dots, hooks,
                  PLANS[name], range(NSPLIT) if last else None)
        if last:
            keep()
        if reds:
            abuf[...] += st["acc"]

    def body2(n, carry):
        block("body", 2 * n, [2, 3], [0, 1], [5, 6], XROWS)
        return carry

    zero = zs[0]
    lax.fori_loop(0, NP // 2 - 2, body2, 0)
    pl.when(zero == 0)(lambda: block("third", 0, [NP - 2], [NP - 4, NP - 3], [], XROWS))
    pl.when(zero <= 0)(lambda: block("last", 0, [NP - 1], [NP - 2], [], XROWS_LAST))

    new_block()
    st = {"acc": abuf[...]}
    invb = get_state(NP - 1, S_LB)
    o = reduce_o([ku[(NP - 1) * GP + b] for b in range(2)], get_state(NP - 1, S_INVA), invb,
                 (get_state(NP - 1, S_X), None))
    part = [None] * 5

    def finish(G, a4):
        for k in range(4):
            tick(lref, L_DUMMY + k, a4[k])
        z = lref[_vr(5), :]
        project(G, [pltpu.bitcast(v, u32) | z for v in a4])

    def project(G, a4):
        for n in range(4):
            v = jnp.sum(pltpu.bitcast(a4[n], f32), axis=1, keepdims=True)
            for nt in range(5):
                w = wou[(NP - 1) * (GP // 2) + G + n // 2, nt]
                t = pltpu.bitcast(w & jnp.uint32(HI) if n % 2 else w << 16, f32) * v
                part[nt] = t if part[nt] is None else part[nt] + t

    for G in range(16, NSPLIT // 2, 2):
        project(G, [ku[(NP - 1) * GP + 2, _vr(2 * (G - 16) + n), :] for n in range(4)])
    dots = late_dots(st)[NLATE:] + [o_dot(NP - 1, b, st, lambda b=b: o[b], lref)
                                    for b in range(2)]
    run_block([NP - 1], XROWS_LAST, dots, {("end", 0): finish},
              PLANS["final"], range(NSPLIT, 48))
    x = row_sum(st["acc"] + jnp.concatenate([v * invb for v in part], axis=1))

    xl = _rows16(x, ones)
    d = xl[0:8].astype(f32) - mean
    md = _mean(d)
    r1 = lax.rsqrt(jnp.maximum(_mean(d * d) - md * md, 0.0) + EPS)
    mean = mean + md
    y = (d - md) * r1
    my = _mean(y)
    r2 = lax.rsqrt(jnp.maximum(_mean(y * y) - my * my, 0.0) + EPS)
    h = jnp.dot(xl, w3[...], preferred_element_type=f32)
    h = h[0:8] * (r1 * r2) - h[8:16] * ((mean * r1 + my) * r2)
    h = jax.nn.gelu(h, approximate=True).astype(bf16)
    x = x + y
    parts = []
    for k in range(0, W4_VPU, 128):
        hk = jnp.broadcast_to(h[0:1, k:k + 128].astype(f32), (128, 128)).T
        t = w4[k:k + 128, :].astype(f32) * jnp.concatenate([hk] * 5, axis=1)
        parts.append(jnp.sum(t.reshape(16, 8, D), axis=0))
    for k in range(W4_VPU, F, 128):
        if k == W4_AT:
            x = x + row_sum(sum(parts[1:], parts[0]))
        x = x + jnp.dot(h[:, k:k + 128], w4[k:k + 128, :], preferred_element_type=f32)
    o_ref[...] = x[0:1].astype(o_ref.dtype)


def _cache_view(c):
    s = c.shape[2]
    c = jnp.transpose(c, (0, 1, 3, 2)).reshape(H * DH // 8, 8, s // 128, 128)
    return jnp.transpose(c, (0, 2, 1, 3)).reshape(H * DH // 8, s // 128 * 8, 128)


def _weight_view(w):
    k, n = w.shape
    w = jnp.transpose(w.reshape(k // 16, 2, 8, n // 128, 128), (0, 1, 3, 2, 4))
    return w.reshape(k // 16, n // 128, 16, 128)


@jax.jit
def pallas_interleave_layers__sliding_block_cached__mixer_s_mlp__decode_kernel(
    A_x: jax.Array,
    A_k_cache: jax.Array,
    A_v_cache: jax.Array,
    A_wq: jax.Array,
    A_wo: jax.Array,
    B_x: jax.Array,
    B_w1: jax.Array,
    B_w2: jax.Array,
    B_w3: jax.Array,
    B_w4: jax.Array,
):
    sk = A_k_cache.shape[2]
    win = min(4096, max(256, sk // 4))
    assert win == 4096 and sk % 128 == 0
    assert A_x.shape == (1, 1, D) and A_k_cache.shape == (1, H, sk, DH)
    wt = win // 128
    t0 = sk // 128 - wt
    ng = H * DH // 8
    hbm = pl.BlockSpec(memory_space=pl.ANY)
    out = pl.pallas_call(
        functools.partial(_kernel, t0=t0, wt=wt),
        out_shape=jax.ShapeDtypeStruct((1, D), A_x.dtype),
        in_specs=[hbm] * 7,
        out_specs=pl.BlockSpec(memory_space=pltpu.VMEM),
        scratch_shapes=[
            pltpu.VMEM((ng, wt * 8, 128), bf16),
            pltpu.VMEM((ng, wt * 8, 128), bf16),
            pltpu.VMEM((ng // 4, 128, 128), u32),
            pltpu.VMEM((NP * D // 16, 3, 8, 128), u32),
            pltpu.VMEM((H * DH // 16, D // 128, 16, 128), bf16),
            pltpu.VMEM((D, F), bf16),
            pltpu.VMEM((F, D), bf16),
            pltpu.VMEM((1, D), bf16),
            pltpu.VMEM((144, 128), u32),
            pltpu.VMEM((384, 128), u32),
            pltpu.VMEM((144, 128), u32),
            pltpu.VMEM((144, 128), u32),
            pltpu.VMEM((144, 128), u32),
            pltpu.VMEM((40, 128), f32),
            pltpu.VMEM((8, D), f32),
            pltpu.SMEM((1,), jnp.int32),
        ] + [pltpu.VMEM((64, 128), u32)] * 3
        + [pltpu.VMEM((72, 128), f32)] * 8,
        compiler_params=pltpu.CompilerParams(vmem_limit_bytes=128 * 1024 * 1024),
    )(A_x.reshape(1, D), _cache_view(A_k_cache), _cache_view(A_v_cache),
      _weight_view(A_wq).reshape(H * DH // 16, D // 128, 16, 128), _weight_view(A_wo), B_w3, B_w4)
    return out.reshape(1, 1, D)
```
